```python
import jax
import jax.numpy as jnp

def _softmax(x, axis=-1):
    return jax.nn.softmax(x, axis=axis)
def _gelu(x):
    return jax.nn.gelu(x, approximate=True)
def _silu(x):
    return jax.nn.silu(x)
def _sigmoid(x):
    return jax.nn.sigmoid(x)
def _layernorm(x, axis=-1, eps=1e-5):
    m = jnp.mean(x, axis=axis, keepdims=True)
    v = jnp.var(x, axis=axis, keepdims=True)
    return (x - m) / jnp.sqrt(v + eps)
def _scatter_add(tgt, idx, src, axis=0):
    return tgt.at[idx].add(src)
def _segment_sum(src, seg, n):
    return jax.ops.segment_sum(src, seg, n)
class _Rng:
    def __init__(self, key):
        self._k = key
    def _next(self):
        self._k, sub = jax.random.split(self._k)
        return sub
    def normal(self, shape):
        return jax.random.normal(self._next(), shape, dtype=jnp.bfloat16)
    def randint(self, lo, hi, shape):
        return jax.random.randint(self._next(), shape, lo, hi, dtype=jnp.int32)
    def uniform(self, shape, lo=0.0, hi=1.0):
        return jax.random.uniform(self._next(), shape, jnp.bfloat16, lo, hi)
    def permutation(self, n):
        return jax.random.permutation(self._next(), n)


kernel_name = 'interleave_layers__sliding_block__sliding_local_dilated__prompt'

def setup_inputs():
    _rng = _Rng(jax.random.key(int.from_bytes(__import__("os").urandom(4), "little")))
    _w = (lambda a: (lambda t: t.astype(jnp.bfloat16) if jnp.issubdtype(t.dtype, jnp.floating) else t)(jnp.asarray(a)))
    def _A_setup():
        B, S, D = 1, 2048, 1024
        return {
            "x": _w((lambda *s: _rng.normal(s) * 0.05)(B, S, D)),
            "wqkv": _w((lambda *s: _rng.normal(s) * 0.05)(D, 3 * D)),
            "wo": _w((lambda *s: _rng.normal(s) * 0.05)(D, D)),
        }
    _A_in = _A_setup()

    def _B_setup():
        B, S, D = 1, 2048, 1024
        return {
            "x": _w((lambda *s: _rng.normal(s) * 0.05)(B, S, D)),
            "wqkv": _w((lambda *s: _rng.normal(s) * 0.05)(D, 3 * D)),
            "wo": _w((lambda *s: _rng.normal(s) * 0.05)(D, D)),
        }
    _B_in = _B_setup()

    return {
        "A_x": _A_in["x"],
        "A_wqkv": _A_in["wqkv"],
        "A_wo": _A_in["wo"],
        "B_x": _B_in["x"],
        "B_wqkv": _B_in["wqkv"],
        "B_wo": _B_in["wo"],
    }

def reference(A_x, A_wqkv, A_wo, B_x, B_wqkv, B_wo):
    def _A_ref(x, wqkv, wo):
        B, S, D = x.shape
        H = 32; Dh = D // H; W = 256
        qkv = (lambda x, *d: x.transpose(*d))((x @ wqkv).reshape(B, S, 3, H, Dh), 2, 0, 3, 1, 4)
        q, k, v = qkv[0], qkv[1], qkv[2]
        scores = jnp.einsum("bhqd,bhkd->bhqk", q, k) * (Dh ** -0.5)
        idx = jnp.arange(S)
        mask = (idx[:, None] - idx[None, :] >= 0) & (idx[:, None] - idx[None, :] < W)
        scores = jnp.where(mask[None, None], scores, -1e9)
        p = _softmax(scores, axis=-1)
        o = jnp.einsum("bhqk,bhkd->bhqd", p, v)
        return (lambda x, *d: x.transpose(*d))(o, 0, 2, 1, 3).reshape(B, S, D) @ wo

    def _B_ref(x, wqkv, wo):
        B, S, D = x.shape
        H = 32; Dh = D // H
        W, dil = 8, 2
        qkv = (lambda x, *d: x.transpose(*d))((x @ wqkv).reshape(B, S, 3, H, Dh), 2, 0, 3, 1, 4)
        q, k, v = qkv[0], qkv[1], qkv[2]
        scale = Dh ** -0.5
        pos = jnp.arange(S)
        off = jnp.arange(W) * dil
        idx = pos[:, None] - off[None, :]
        mask = idx >= 0
        idx_c = jnp.where(mask, idx, 0).reshape(-1)
        kg = k[:, :, idx_c, :].reshape(B, H, S, W, Dh)
        vg = v[:, :, idx_c, :].reshape(B, H, S, W, Dh)
        logits = jnp.einsum("bhsd,bhswd->bhsw", q, kg) * scale
        logits = jnp.where(mask[None, None, :, :], logits, -1e9)
        attn = _softmax(logits, axis=-1)
        o = jnp.einsum("bhsw,bhswd->bhsd", attn, vg)
        return (lambda x, *d: x.transpose(*d))(o, 0, 2, 1, 3).reshape(B, S, D) @ wo

    x = A_x
    x = x + _A_ref(_layernorm(x, axis=-1), A_wqkv, A_wo)
    x = x + _B_ref(_layernorm(x, axis=-1), B_wqkv, B_wo)
    x = x + _A_ref(_layernorm(x, axis=-1), A_wqkv, A_wo)
    x = x + _B_ref(_layernorm(x, axis=-1), B_wqkv, B_wo)
    return x
```

```python
import math

import jax
import jax.numpy as jnp
from jax import lax
import jax.experimental.pallas as pl
import jax.experimental.pallas.tpu as pltpu

BF = jnp.bfloat16
F32 = jnp.float32
U32 = jnp.uint32

S = 2048
D = 1024
H = 32
DH = 32
TA = 256
NA = S // TA
TB = 512
NB = S // TB
HALO = 16
WB = 8
NEG = -1e30
EPS = 1e-5
QSCALE = (DH ** -0.5) * math.log2(math.e)
NCH = 6
CW = 3 * D // NCH
LOOK = 2


def _dot(a, b):
    return jnp.dot(a, b, preferred_element_type=F32)


def _dot_nt(a, b):
    return lax.dot_general(a, b, (((1,), (1,)), ((), ())), preferred_element_type=F32)


def _pack(x_bf16):
    return pltpu.bitcast(x_bf16, U32)


def _unpack(x_u32):
    return pltpu.bitcast(x_u32, BF)


def _layernorm(x_bf16):
    x = x_bf16.astype(F32)
    m = jnp.sum(x, axis=1, keepdims=True) * (1.0 / D)
    xc = x - m
    v = jnp.sum(xc * xc, axis=1, keepdims=True) * (1.0 / D)
    return (xc * lax.rsqrt(v + EPS)).astype(BF)


def _kernel(x_hbm, wa_hbm, woa_hbm, wb_hbm, wob_hbm, out_hbm,
            x_v, wa_v, woa_v, wb_v, wob_v, wbt, wobp, tmp, xn_v,
            k_v, qt_v, vt_v, oa_v, qkv_v, ob_v,
            sem_x, sem_wa, sem_woa, sem_wb, sem_wob, sem_out):
    def cp_x(i):
        return pltpu.make_async_copy(x_hbm.at[pl.ds(i * TA, TA), :],
                                     x_v.at[pl.ds(i * TA, TA), :], sem_x.at[i])

    ch_col = [D, D + CW, 0, CW, 2 * D, 2 * D + CW]

    def cp_wa(c):
        return pltpu.make_async_copy(wa_hbm.at[:, pl.ds(ch_col[c], CW)],
                                     wa_v.at[:, pl.ds(ch_col[c], CW)], sem_wa.at[c])

    cp_woa = pltpu.make_async_copy(woa_hbm, woa_v, sem_woa.at[0])

    def cp_wb(j):
        return pltpu.make_async_copy(wb_hbm.at[pl.ds(j * 128, 128), :],
                                     wb_v.at[j], sem_wb.at[j])

    def cp_wob(j):
        return pltpu.make_async_copy(wob_hbm.at[:, pl.ds(j * 128, 128)],
                                     wob_v.at[j], sem_wob.at[j])

    def cp_out(i):
        return pltpu.make_async_copy(x_v.at[pl.ds(i * TB, TB), :],
                                     out_hbm.at[pl.ds(i * TB, TB), :], sem_out.at[i])

    cp_x(0).start()
    for c in range(NCH):
        cp_wa(c).start()
    cp_x(1).start()
    cp_wb(0).start()
    cp_wob(0).start()
    cp_woa.start()
    for i in range(1, NA):
        if i + 1 < NA:
            cp_x(i + 1).start()
        cp_wb(i).start()
        cp_wob(i).start()

    def tri_mask():
        row = lax.broadcasted_iota(jnp.int32, (128, 128), 0)
        col = lax.broadcasted_iota(jnp.int32, (128, 128), 1)
        return col >= row

    def ln_next(blk):
        r = pl.multiple_of(blk * TA, TA)
        xn_v[...] = _layernorm(x_v[pl.ds(r, TA), :])

    def prep_b(j):
        wt = wb_v[j].T
        tmp[0:3 * D, :] = wt.astype(F32)
        tmp[3 * D:4 * D, :] = wob_v[j].astype(F32)
        for part in range(4):
            rows = [tmp[pl.ds(part * D + d, H, stride=DH), :] for d in range(DH)]
            val = _pack(jnp.concatenate(rows, axis=0).astype(BF))
            if part < 3:
                wbt[j, part * (D // 2):(part + 1) * (D // 2), :] = val
            else:
                wobp[j] = val

    def proj_a(blk, col0, ncols):
        y = _dot(xn_v[...], wa_v[:, col0:col0 + ncols])
        part, c0 = col0 // D, col0 % D
        if part == 1:
            r = pl.multiple_of(blk * (TA // 2), TA // 2)
            for t in range(ncols // 128):
                k_v[c0 // 128 + t, pl.ds(r, TA // 2), :] = _pack(
                    y[:, t * 128:(t + 1) * 128].astype(BF))
        else:
            if part == 0:
                y = y * QSCALE
            yt = _pack(y.astype(BF).T)
            for b in range(TA // 128):
                piece = yt[:, b * 128:(b + 1) * 128]
                if part == 0:
                    qt_v[b, c0 // 2:(c0 + ncols) // 2, :] = piece
                else:
                    vt_v[blk * (TA // 128) + b, c0 // 2:(c0 + ncols) // 2, :] = piece

    def scores_a(m, qb, h, ntile):
        t = h // 4
        z = jnp.zeros((16, 128), U32)
        qh = qt_v[qb, h * 16:(h + 1) * 16, :]
        wq = _unpack(jnp.concatenate([qh if jj == h % 4 else z for jj in range(4)], axis=0))
        tri = tri_mask()
        base = m * 64
        if not isinstance(m, int):
            base = pl.multiple_of(base, 64)
        back = {1: (0,), 2: (0, 1), 3: (2, 0, 1)}[ntile]
        sm, mid = [], []
        nsplit = 4 if ntile > 1 else 1
        gper = 8 // nsplit
        for c in range(nsplit):
            parts = []
            for g in range(c * gper, (c + 1) * gper):
                for bk in back:
                    parts.append(k_v[t, pl.ds(base - bk * 64 + g * 8, 8), :])
            s = _dot(_unpack(jnp.concatenate(parts, axis=0)), wq)
            for gi in range(gper):
                g = c * gper + gi
                o = gi * 16 * ntile
                tr = tri[g * 16:(g + 1) * 16]
                if ntile == 3:
                    sm.append(jnp.where(tr, s[o + 16:o + 32], s[o:o + 16]))
                    mid.append(s[o + 32:o + 48])
                else:
                    sm.append(jnp.where(tr, s[o:o + 16], NEG))
                    if ntile == 2:
                        mid.append(s[o + 16:o + 32])
        return (jnp.concatenate(sm, axis=0),
                jnp.concatenate(mid, axis=0) if mid else None)

    def finish_a(sm, mid, m, h, ntile):
        tri = tri_mask()
        if mid is None:
            mx = jnp.max(sm, axis=0, keepdims=True)
            pm = jnp.exp2(sm - mx)
            l = jnp.sum(pm, axis=0, keepdims=True)
            p = pm
        else:
            mx = jnp.max(jnp.maximum(sm, mid), axis=0, keepdims=True)
            pm = jnp.exp2(sm - mx)
            pd = jnp.exp2(mid - mx)
            l = jnp.sum(pm + pd, axis=0, keepdims=True)
            if ntile == 3:
                p = jnp.concatenate(
                    [jnp.where(tri, 0.0, pm), pd, jnp.where(tri, pm, 0.0)], axis=0)
            else:
                p = jnp.concatenate([pd, pm], axis=0)
        vv = _unpack(jnp.concatenate(
            [vt_v[m - bk, h * 16:(h + 1) * 16, :] for bk in range(ntile - 1, -1, -1)], axis=1))
        o = _dot(vv, p.astype(BF))
        return o * pl.reciprocal(l, approx=False)

    def attn_a(blk, ntiles):
        items = [(qb, h) for qb in range(TA // 128) for h in range(H)]

        def sc(it):
            qb, h = it
            return scores_a(blk * (TA // 128) + qb, qb, h, ntiles[qb])
        queue = [sc(it) for it in items[:LOOK]]
        outs = []
        for n, (qb, h) in enumerate(items):
            if n + LOOK < len(items):
                queue.append(sc(items[n + LOOK]))
            sm, mid = queue.pop(0)
            outs.append(finish_a(sm, mid, blk * (TA // 128) + qb, h, ntiles[qb]))
            if h % 4 == 3:
                ot = jnp.concatenate(outs, axis=0).astype(BF)
                oa_v[h // 4, qb * 64:(qb + 1) * 64, :] = _pack(ot.T)
                outs = []

    def out_a(blk):
        for qb in range(TA // 128):
            o = _unpack(jnp.concatenate(
                [oa_v[t, qb * 64:(qb + 1) * 64, :] for t in range(8)], axis=1))
            r = blk * TA + qb * 128
            if not isinstance(r, int):
                r = pl.multiple_of(r, 128)
            x_v[pl.ds(r, 128), :] = (
                x_v[pl.ds(r, 128), :].astype(F32) + _dot(o, woa_v[...])).astype(BF)

    def proj_b(xn, r0, nrows):
        for part in range(3):
            w = _unpack(jnp.concatenate(
                [wbt[j, part * (D // 2):(part + 1) * (D // 2), :] for j in range(8)], axis=1))
            y = _dot_nt(xn, w)
            if part == 0:
                y = y * QSCALE
            for t in range(8):
                qkv_v[part * 8 + t, HALO + r0:HALO + r0 + nrows, :] = y[:, t * 128:(t + 1) * 128]

    def attn_b(i, r0, R):
        def ld(T, r):
            return qkv_v[T, HALO + r:HALO + r + R, :]
        accs = [None] * WB
        for t in range(8):
            q = ld(t, r0)
            for w in range(WB):
                p = q * ld(8 + t, r0 - 2 * w)
                accs[w] = p if accs[w] is None else accs[w] + p
        ls = []
        for w in range(WB):
            a = accs[w]
            a = a + pltpu.roll(a, 64, 1)
            a = a + pltpu.roll(a, 32, 1)
            if r0 - 2 * w < 0:
                pos = lax.broadcasted_iota(jnp.int32, (R, 128), 0) + (i * TB + r0 - 2 * w)
                a = jnp.where(pos >= 0, a, NEG)
            ls.append(a)
        mx = ls[0]
        for w in range(1, WB):
            mx = jnp.maximum(mx, ls[w])
        es = [jnp.exp2(l - mx) for l in ls]
        s = es[0]
        for w in range(1, WB):
            s = s + es[w]
        inv = pl.reciprocal(s, approx=False)
        es = [e * inv for e in es]
        os_ = []
        for t in range(8):
            o = None
            for w in range(WB):
                pv = es[w] * ld(16 + t, r0 - 2 * w)
                o = pv if o is None else o + pv
            os_.append(o)
        ob_v[r0:r0 + R, :] = jnp.concatenate(os_, axis=1).astype(BF)

    def out_b(i, r0, nrows):
        w = _unpack(jnp.concatenate([wobp[j] for j in range(8)], axis=1))
        r = pl.multiple_of(i * TB + r0, 128)
        x_v[pl.ds(r, nrows), :] = (
            x_v[pl.ds(r, nrows), :].astype(F32) + _dot(ob_v[r0:r0 + nrows, :], w)).astype(BF)

    cp_x(0).wait()
    ln_next(0)

    def one_pass(p, carry):
        first = p == 0

        for c in range(NCH):
            @pl.when(first)
            def _():
                cp_wa(c).wait()
            proj_a(0, ch_col[c], CW)

        @pl.when(first)
        def _():
            cp_x(1).wait()
            cp_wb(0).wait()
            cp_wob(0).wait()
            cp_woa.wait()
        ln_next(1)
        prep_b(0)
        attn_a(0, (1, 2))
        out_a(0)

        def a_body(i, c_):
            @pl.when(first)
            def _():
                @pl.when(i + 1 < NA)
                def _():
                    cp_x(i + 1).wait()
                cp_wb(i).wait()
                cp_wob(i).wait()
            proj_a(i, D, D)
            proj_a(i, 0, D)
            proj_a(i, 2 * D, D)
            prep_b(i)
            ln_next((i + 1) % NA)
            attn_a(i, (3, 3))
            out_a(i)
            return c_
        lax.fori_loop(1, NA, a_body, 0)

        for T in range(8, 24):
            qkv_v[T, 0:HALO, :] = jnp.zeros((HALO, 128), F32)

        def b_body(i, c_):
            R = 8
            r1 = pl.multiple_of(i * TB + 256, 128)
            r2 = pl.multiple_of(i * TB + 384, 128)
            proj_b(xn_v[...], 0, 256)
            proj_b(_layernorm(x_v[pl.ds(r1, 128), :]), 256, 128)
            proj_b(_layernorm(x_v[pl.ds(r2, 128), :]), 384, 128)
            for g in range(384 // R):
                attn_b(i, g * R, R)
            out_b(i, 0, 384)
            for g in range(384 // R, TB // R):
                attn_b(i, g * R, R)
            out_b(i, 384, 128)
            ln_next(((i + 1) % NB) * (TB // TA))
            for T in range(8, 24):
                qkv_v[T, 0:HALO, :] = qkv_v[T, TB:TB + HALO, :]

            @pl.when(p == 1)
            def _():
                cp_out(i).start()
            return c_
        lax.fori_loop(0, NB, b_body, 0)
        return carry

    lax.fori_loop(0, 2, one_pass, 0)
    for i in range(NB):
        cp_out(i).wait()


@jax.jit
def pallas_interleave_layers__sliding_block__sliding_local_dilated__prompt_kernel(
    A_x: jax.Array,
    A_wqkv: jax.Array,
    A_wo: jax.Array,
    B_x: jax.Array,
    B_wqkv: jax.Array,
    B_wo: jax.Array,
):
    del B_x
    x = A_x.reshape(S, D)
    any_spec = pl.BlockSpec(memory_space=pl.ANY)
    out = pl.pallas_call(
        _kernel,
        out_shape=jax.ShapeDtypeStruct((S, D), BF),
        in_specs=[any_spec] * 5,
        out_specs=any_spec,
        scratch_shapes=[
            pltpu.VMEM((S, D), BF),
            pltpu.VMEM((D, 3 * D), BF),
            pltpu.VMEM((D, D), BF),
            pltpu.VMEM((8, 128, 3 * D), BF),
            pltpu.VMEM((8, D, 128), BF),
            pltpu.VMEM((8, 3 * D // 2, 128), U32),
            pltpu.VMEM((8, D // 2, 128), U32),
            pltpu.VMEM((4 * D, 128), F32),
            pltpu.VMEM((TA, D), BF),
            pltpu.VMEM((8, S // 2, 128), U32),
            pltpu.VMEM((TA // 128, D // 2, 128), U32),
            pltpu.VMEM((S // 128, D // 2, 128), U32),
            pltpu.VMEM((8, TA // 2, 128), U32),
            pltpu.VMEM((24, HALO + TB, 128), F32),
            pltpu.VMEM((TB, D), BF),
            pltpu.SemaphoreType.DMA((NA,)),
            pltpu.SemaphoreType.DMA((NCH,)),
            pltpu.SemaphoreType.DMA((1,)),
            pltpu.SemaphoreType.DMA((8,)),
            pltpu.SemaphoreType.DMA((8,)),
            pltpu.SemaphoreType.DMA((NB,)),
        ],
        compiler_params=pltpu.CompilerParams(vmem_limit_bytes=100 * 1024 * 1024),
        name="interleave_attn",
    )(x, A_wqkv, A_wo, B_wqkv, B_wo)
    return out.reshape(1, S, D)
```

```python
import math

import jax
import jax.numpy as jnp
from jax import lax
import jax.experimental.pallas as pl
import jax.experimental.pallas.tpu as pltpu

BF = jnp.bfloat16
F32 = jnp.float32
U32 = jnp.uint32

S = 2048
D = 1024
H = 32
DH = 32
TA = 256
NA = S // TA
TB = 512
NB = S // TB
HALO = 16
WB = 8
NEG = -1e30
EPS = 1e-5
QSCALE = (DH ** -0.5) * math.log2(math.e)
NCH = 6
CW = 3 * D // NCH
LOOK = 2
PITCH = 36


def _dot(a, b):
    return jnp.dot(a, b, preferred_element_type=F32)


def _dot_nt(a, b):
    return lax.dot_general(a, b, (((1,), (1,)), ((), ())), preferred_element_type=F32)


def _pack(x_bf16):
    return pltpu.bitcast(x_bf16, U32)


def _unpack(x_u32):
    return pltpu.bitcast(x_u32, BF)


def _layernorm(x_bf16):
    x = x_bf16.astype(F32)
    m = jnp.sum(x, axis=1, keepdims=True) * (1.0 / D)
    xc = x - m
    v = jnp.sum(xc * xc, axis=1, keepdims=True) * (1.0 / D)
    return (xc * lax.rsqrt(v + EPS)).astype(BF)


def _kernel(x_hbm, wa_hbm, woa_hbm, wb_hbm, wob_hbm, out_hbm,
            x_v, wa_v, woa_v, wb_v, wob_v, wbt, wobp, tmp, xn_v, xn2_v,
            k_v, qt_v, vt_v, oa_v, qk_v, v_v, ob_v,
            sem_x, sem_wa, sem_woa, sem_wb, sem_wob, sem_out):
    def cp_x(i):
        return pltpu.make_async_copy(x_hbm.at[pl.ds(i * TA, TA), :],
                                     x_v.at[pl.ds(i * TA, TA), :], sem_x.at[i])

    ch_col = [D, D + CW, 0, CW, 2 * D, 2 * D + CW]

    def cp_wa(c):
        return pltpu.make_async_copy(wa_hbm.at[:, pl.ds(ch_col[c], CW)],
                                     wa_v.at[:, pl.ds(ch_col[c], CW)], sem_wa.at[c])

    cp_woa = pltpu.make_async_copy(woa_hbm, woa_v, sem_woa.at[0])

    def cp_wb(j):
        return pltpu.make_async_copy(wb_hbm.at[pl.ds(j * 128, 128), :],
                                     wb_v.at[j], sem_wb.at[j])

    def cp_wob(j):
        return pltpu.make_async_copy(wob_hbm.at[:, pl.ds(j * 128, 128)],
                                     wob_v.at[j], sem_wob.at[j])

    def cp_out(i):
        return pltpu.make_async_copy(x_v.at[pl.ds(i * TB, TB), :],
                                     out_hbm.at[pl.ds(i * TB, TB), :], sem_out.at[i])

    def tri_mask():
        row = lax.broadcasted_iota(jnp.int32, (128, 128), 0)
        col = lax.broadcasted_iota(jnp.int32, (128, 128), 1)
        return col >= row

    def ln_chunks(row0, dst, nrows, step=16):
        def mk(c):
            def run(tok):
                if tok is not None:
                    x_v[S:S + 16, 0:128] = tok.astype(BF)
                r = pl.multiple_of(row0 + c * step, step)
                dst[c * step:(c + 1) * step, :] = _layernorm(x_v[pl.ds(r, step), :])
            return run
        return [mk(c) for c in range(nrows // step)]

    def prep_chunks(j):
        def permute(part):
            rows = [tmp[pl.ds(part * H * PITCH + d, H, stride=PITCH), :] for d in range(DH)]
            val = _pack(jnp.concatenate(rows, axis=0).astype(BF))
            if part < 3:
                wbt[j, part * (D // 2):(part + 1) * (D // 2), :] = val
            else:
                wobp[j] = val

        def mk_t(c):
            def run(tok):
                wb_v[8, 0:16, 0:128] = tok.astype(BF)
                wt = wb_v[j, :, c * 256:(c + 1) * 256].T.astype(F32)
                for hh in range(8):
                    o = (c * 8 + hh) * PITCH
                    tmp[o:o + DH, :] = wt[hh * DH:(hh + 1) * DH]
                if c % 4 == 3:
                    permute(c // 4)
            return run

        def mk_o(c):
            def run(tok):
                wob_v[8, 0:16, :] = tok.astype(BF)
                w = wob_v[j, c * 256:(c + 1) * 256, :].astype(F32)
                for hh in range(8):
                    o = (96 + c * 8 + hh) * PITCH
                    tmp[o:o + DH, :] = w[hh * DH:(hh + 1) * DH]
                if c == 3:
                    permute(3)
            return run
        return [mk_t(c) for c in range(12)] + [mk_o(c) for c in range(4)]

    def release(y, chunks):
        n = len(chunks)
        nt = y.shape[1] // 128
        for u, run in enumerate(chunks):
            pos = (u * y.shape[0] * nt // n) // 16 * 16
            t, rr = pos // y.shape[0], pos % y.shape[0]
            run(y[rr:rr + 16, t * 128:(t + 1) * 128])

    def proj_a(xn, blk, col0, ncols, side=()):
        y = _dot(xn, wa_v[:, col0:col0 + ncols])
        release(y, side)
        part, c0 = col0 // D, col0 % D
        if part == 1:
            r = blk * (TA // 2)
            if not isinstance(r, int):
                r = pl.multiple_of(r, TA // 2)
            for t in range(ncols // 128):
                k_v[c0 // 128 + t, pl.ds(r, TA // 2), :] = _pack(
                    y[:, t * 128:(t + 1) * 128].astype(BF))
        else:
            if part == 0:
                y = y * QSCALE
            yt = _pack(y.astype(BF).T)
            for b in range(TA // 128):
                piece = yt[:, b * 128:(b + 1) * 128]
                if part == 0:
                    qt_v[b, c0 // 2:(c0 + ncols) // 2, :] = piece
                else:
                    vt_v[blk * (TA // 128) + b, c0 // 2:(c0 + ncols) // 2, :] = piece

    def scores_a(m, qb, h, ntile):
        t = h // 4
        z = jnp.zeros((16, 128), U32)
        qh = qt_v[qb, h * 16:(h + 1) * 16, :]
        wq = _unpack(jnp.concatenate([qh if jj == h % 4 else z for jj in range(4)], axis=0))
        tri = tri_mask()
        base = m * 64
        if not isinstance(m, int):
            base = pl.multiple_of(base, 64)
        back = {1: (0,), 2: (0, 1), 3: (2, 0, 1)}[ntile]
        sm, mid = [], []
        nsplit = 4
        gper = 8 // nsplit
        for c in range(nsplit):
            parts = []
            for g in range(c * gper, (c + 1) * gper):
                for bk in back:
                    parts.append(k_v[t, pl.ds(base - bk * 64 + g * 8, 8), :])
            s = _dot(_unpack(jnp.concatenate(parts, axis=0)), wq)
            for gi in range(gper):
                g = c * gper + gi
                o = gi * 16 * ntile
                tr = tri[g * 16:(g + 1) * 16]
                if ntile == 3:
                    sm.append(jnp.where(tr, s[o + 16:o + 32], s[o:o + 16]))
                    mid.append(s[o + 32:o + 48])
                else:
                    sm.append(jnp.where(tr, s[o:o + 16], NEG))
                    if ntile == 2:
                        mid.append(s[o + 16:o + 32])
        return (jnp.concatenate(sm, axis=0),
                jnp.concatenate(mid, axis=0) if mid else None)

    def finish_a(sm, mid, m, h, ntile):
        tri = tri_mask()
        if mid is None:
            mx = jnp.max(sm, axis=0, keepdims=True)
            pm = jnp.exp2(sm - mx)
            l = jnp.sum(pm, axis=0, keepdims=True)
            p = pm
        else:
            mx = jnp.max(jnp.maximum(sm, mid), axis=0, keepdims=True)
            pm = jnp.exp2(sm - mx)
            pd = jnp.exp2(mid - mx)
            l = jnp.sum(pm + pd, axis=0, keepdims=True)
            if ntile == 3:
                p = jnp.concatenate(
                    [jnp.where(tri, 0.0, pm), pd, jnp.where(tri, pm, 0.0)], axis=0)
            else:
                p = jnp.concatenate([pd, pm], axis=0)
        vv = _unpack(jnp.concatenate(
            [vt_v[m - bk, h * 16:(h + 1) * 16, :] for bk in range(ntile - 1, -1, -1)], axis=1))
        o = _dot(vv, p.astype(BF))
        return o * pl.reciprocal(l, approx=False)

    def attn_a(blk, ntiles, looks, head_fill=None, tail_fill=None):
        items = [(qb, h) for qb in range(TA // 128) for h in range(H)]
        queue = []
        issued = [0]

        def issue_upto(n):
            while issued[0] < min(n, len(items)):
                qb, h = items[issued[0]]
                queue.append(scores_a(blk * (TA // 128) + qb, qb, h, ntiles[qb]))
                issued[0] += 1
        issue_upto(looks[0])
        if head_fill is not None:
            head_fill()
        outs = []
        for n, (qb, h) in enumerate(items):
            issue_upto(n + 1 + looks[qb])
            if tail_fill is not None and n + looks[qb] == len(items):
                tail_fill()
            sm, mid = queue.pop(0)
            outs.append(finish_a(sm, mid, blk * (TA // 128) + qb, h, ntiles[qb]))
            if h % 4 == 3:
                ot = jnp.concatenate(outs, axis=0).astype(BF)
                oa_v[h // 4, qb * 64:(qb + 1) * 64, :] = _pack(ot.T)
                outs = []

    def out_a(blk, qb, c0, c1, side=()):
        o = _unpack(jnp.concatenate(
            [oa_v[t, qb * 64:(qb + 1) * 64, :] for t in range(8)], axis=1))
        r = blk * TA + qb * 128
        if not isinstance(r, int):
            r = pl.multiple_of(r, 128)
        y = _dot(o, woa_v[:, c0:c1])
        release(y, side)
        x_v[pl.ds(r, 128), c0:c1] = (x_v[pl.ds(r, 128), c0:c1].astype(F32) + y).astype(BF)

    def proj_b(xn, r0, nrows, side):
        for T in range(24):
            w = _unpack(jnp.concatenate(
                [wbt[j, T * 64:(T + 1) * 64, :] for j in range(8)], axis=1))
            y = _dot_nt(xn, w)
            if T < 8:
                qk_v[T, HALO + r0:HALO + r0 + nrows, :] = y * QSCALE
            elif T < 16:
                qk_v[T, HALO + r0:HALO + r0 + nrows, :] = y
            else:
                v_v[T - 16, HALO + r0:HALO + r0 + nrows, :] = y
            release(y, side[T])

    def attn_b(i, zero, r0):
        R = 8

        def run(tok):
            qk_v[0, pl.ds(pl.multiple_of(HALO + TB + zero * 8, 8), 8), :] = tok[0:8]
            accs = [None] * WB
            for t in range(8):
                q = qk_v[t, HALO + r0:HALO + r0 + R, :]
                for w in range(WB):
                    o = HALO + r0 - 2 * w
                    p = q * qk_v[8 + t, o:o + R, :]
                    accs[w] = p if accs[w] is None else accs[w] + p
            ls = []
            for w in range(WB):
                a = accs[w]
                a = a + pltpu.roll(a, 64, 1)
                a = a + pltpu.roll(a, 32, 1)
                if r0 - 2 * w < 0:
                    pos = lax.broadcasted_iota(jnp.int32, (R, 128), 0) + (i * TB + r0 - 2 * w)
                    a = jnp.where(pos >= 0, a, NEG)
                ls.append(a)
            mx = ls[0]
            for w in range(1, WB):
                mx = jnp.maximum(mx, ls[w])
            es = [jnp.exp2(l - mx) for l in ls]
            s = es[0]
            for w in range(1, WB):
                s = s + es[w]
            inv = pl.reciprocal(s, approx=False)
            es = [e * inv for e in es]
            os_ = []
            for t in range(8):
                acc = None
                for w in range(WB):
                    o = HALO + r0 - 2 * w
                    pv = es[w] * v_v[t, o:o + R, :]
                    acc = pv if acc is None else acc + pv
                os_.append(acc)
            ob_v[r0:r0 + R, :] = jnp.concatenate(os_, axis=1).astype(BF)
        return run

    def out_b(i, r0, nrows, side):
        o = ob_v[r0:r0 + nrows, :]
        r = pl.multiple_of(i * TB + r0, 128)
        for c in range(4):
            w = _unpack(jnp.concatenate([wobp[2 * c], wobp[2 * c + 1]], axis=1))
            y = _dot(o, w)
            release(y, side[c])
            cs = slice(c * 256, (c + 1) * 256)
            x_v[pl.ds(r, nrows), cs] = (x_v[pl.ds(r, nrows), cs].astype(F32) + y).astype(BF)

    def spread(chunks, nslots, lo=0, hi=None):
        hi = nslots if hi is None else hi
        out = [[] for _ in range(nslots)]
        for u, c in enumerate(chunks):
            out[lo + u * (hi - lo) // len(chunks)].append(c)
        return out

    cp_x(0).start()
    cp_wa(0).start()
    cp_wa(1).start()
    cp_x(0).wait()
    for run in ln_chunks(0, xn_v, TA, step=TA):
        run(None)

    def one_pass(p, carry):
        first = p == 0
        zero = p // 4

        for c in range(NCH):
            @pl.when(first)
            def _():
                cp_wa(c).wait()
                if c + 2 < NCH:
                    cp_wa(c + 2).start()
                elif c + 2 == NCH:
                    cp_woa.start()
                else:
                    cp_x(1).start()
                    cp_wb(0).start()
                    cp_wob(0).start()
            if c + 1 < NCH:
                proj_a(xn_v[...], 0, ch_col[c], CW)
        xn = xn_v[...]
        proj_a(xn, 0, ch_col[-1], CW - 256)
        attn_a(0, (1, 2), (6, 3),
               head_fill=lambda: proj_a(xn, 0, 3 * D - 256, 256))

        @pl.when(first)
        def _():
            cp_woa.wait()
            cp_x(1).wait()
            cp_wb(0).wait()
            cp_wob(0).wait()
            cp_x(2).start()
            cp_wb(1).start()
            cp_wob(1).start()
        side = spread(prep_chunks(zero), 8, 0, 6)
        side2 = spread(ln_chunks(TA + zero * TA, xn_v, TA), 8, 0, 7)
        for u in range(8):
            out_a(0, u // 4, (u % 4) * 256, (u % 4 + 1) * 256, side[u] + side2[u])

        def a_body(i, c_):
            @pl.when(first)
            def _():
                @pl.when(i + 1 < NA)
                def _():
                    cp_x(i + 1).wait()
                    cp_wb(i + 1).start()
                    cp_wob(i + 1).start()

                @pl.when(i + 2 < NA)
                def _():
                    cp_x(i + 2).start()
                cp_wb(i).wait()
                cp_wob(i).wait()
            xn = xn_v[...]
            lnc = ln_chunks(((i + 1) % NA) * TA, xn_v, TA)
            prc = prep_chunks(i)
            mixed = [c for pair in zip(prc, lnc) for c in pair]
            side = spread(mixed, 11)
            cols = [D + c * 256 for c in range(4)] + [c * 256 for c in range(4)] + \
                   [2 * D + c * 256 for c in range(3)]
            for u, c0 in enumerate(cols):
                proj_a(xn, i, c0, 256, side[u])
            attn_a(i, (3, 3), (LOOK, LOOK),
                   head_fill=lambda: proj_a(xn, i, 3 * D - 256, 256),
                   tail_fill=lambda: out_a(i, 0, 0, 256))
            out_a(i, 0, 256, D)
            out_a(i, 1, 0, D)
            return c_
        lax.fori_loop(1, NA, a_body, 0)

        for T in range(8):
            qk_v[8 + T, 0:HALO, :] = jnp.zeros((HALO, 128), F32)
            v_v[T, 0:HALO, :] = jnp.zeros((HALO, 128), F32)

        def b_body(i, c_):
            xn = xn_v[...]
            ln1 = ln_chunks(i * TB + 256, xn2_v, 256)
            ln2 = ln_chunks(((i + 1) % NB) * TB, xn_v, TA)
            proj_b(xn, 0, 256, spread(ln1 + ln2, 24, 0, 23))
            groups = [attn_b(i, zero, g * 8) for g in range(TB // 8)]
            proj_b(xn2_v[0:128, :], 256, 128, spread(groups[0:22], 24))
            proj_b(xn2_v[128:256, :], 384, 128, spread(groups[22:44], 24))
            out_b(i, 0, 256, spread(groups[44:60], 4))
            out_b(i, 256, 128, spread(groups[60:64], 4, 0, 2))
            out_b(i, 384, 128, [[]] * 4)
            for T in range(8):
                qk_v[8 + T, 0:HALO, :] = qk_v[8 + T, TB:TB + HALO, :]
                v_v[T, 0:HALO, :] = v_v[T, TB:TB + HALO, :]

            @pl.when(p == 1)
            def _():
                cp_out(i).start()
            return c_
        lax.fori_loop(0, NB, b_body, 0)
        return carry

    lax.fori_loop(0, 2, one_pass, 0)
    for i in range(NB):
        cp_out(i).wait()


@jax.jit
def pallas_interleave_layers__sliding_block__sliding_local_dilated__prompt_kernel(
    A_x: jax.Array,
    A_wqkv: jax.Array,
    A_wo: jax.Array,
    B_x: jax.Array,
    B_wqkv: jax.Array,
    B_wo: jax.Array,
):
    del B_x
    x = A_x.reshape(S, D)
    any_spec = pl.BlockSpec(memory_space=pl.ANY)
    out = pl.pallas_call(
        _kernel,
        out_shape=jax.ShapeDtypeStruct((S, D), BF),
        in_specs=[any_spec] * 5,
        out_specs=any_spec,
        scratch_shapes=[
            pltpu.VMEM((S + 16, D), BF),
            pltpu.VMEM((D, 3 * D), BF),
            pltpu.VMEM((D, D), BF),
            pltpu.VMEM((9, 128, 3 * D), BF),
            pltpu.VMEM((9, D, 128), BF),
            pltpu.VMEM((8, 3 * D // 2, 128), U32),
            pltpu.VMEM((8, D // 2, 128), U32),
            pltpu.VMEM((128 * PITCH, 128), F32),
            pltpu.VMEM((TA, D), BF),
            pltpu.VMEM((TA, D), BF),
            pltpu.VMEM((8, S // 2, 128), U32),
            pltpu.VMEM((TA // 128, D // 2, 128), U32),
            pltpu.VMEM((S // 128, D // 2, 128), U32),
            pltpu.VMEM((8, TA // 2, 128), U32),
            pltpu.VMEM((16, HALO + TB + 8, 128), F32),
            pltpu.VMEM((8, HALO + TB, 128), F32),
            pltpu.VMEM((TB, D), BF),
            pltpu.SemaphoreType.DMA((NA,)),
            pltpu.SemaphoreType.DMA((NCH,)),
            pltpu.SemaphoreType.DMA((1,)),
            pltpu.SemaphoreType.DMA((8,)),
            pltpu.SemaphoreType.DMA((8,)),
            pltpu.SemaphoreType.DMA((NB,)),
        ],
        compiler_params=pltpu.CompilerParams(vmem_limit_bytes=100 * 1024 * 1024),
        name="interleave_attn",
    )(x, A_wqkv, A_wo, B_wqkv, B_wo)
    return out.reshape(1, S, D)
```

```python
import math

import jax
import jax.numpy as jnp
from jax import lax
import jax.experimental.pallas as pl
import jax.experimental.pallas.tpu as pltpu

BF = jnp.bfloat16
F32 = jnp.float32
U32 = jnp.uint32

S = 2048
D = 1024
H = 32
DH = 32
TA = 256
NA = S // TA
TB = 512
NB = S // TB
HALO = 16
WB = 8
NEG = -1e30
EPS = 1e-5
QSCALE = (DH ** -0.5) * math.log2(math.e)
NCH = 6
CW = 3 * D // NCH
LOOK = 2
PITCH = 36


def _dot(a, b):
    return jnp.dot(a, b, preferred_element_type=F32)


def _dot_nt(a, b):
    return lax.dot_general(a, b, (((1,), (1,)), ((), ())), preferred_element_type=F32)


def _pack(x_bf16):
    return pltpu.bitcast(x_bf16, U32)


def _unpack(x_u32):
    return pltpu.bitcast(x_u32, BF)


def _layernorm(x_bf16):
    x = x_bf16.astype(F32)
    m = jnp.sum(x, axis=1, keepdims=True) * (1.0 / D)
    xc = x - m
    v = jnp.sum(xc * xc, axis=1, keepdims=True) * (1.0 / D)
    return (xc * lax.rsqrt(v + EPS)).astype(BF)


def _kernel(x_hbm, wa_hbm, woa_hbm, wb_hbm, wob_hbm, out_hbm,
            x_v, wa_v, woa_v, wb_v, wob_v, wbt, wobp, tmp, xn_v,
            k_v, qt_v, vt_v, oa_v, qk_v, v_v, e_v, ob_v,
            sem_x, sem_wa, sem_woa, sem_wb, sem_wob, sem_out):
    def cp_x(i):
        return pltpu.make_async_copy(x_hbm.at[pl.ds(i * TA, TA), :],
                                     x_v.at[pl.ds(i * TA, TA), :], sem_x.at[i])

    ch_col = [D, D + CW, 0, CW, 2 * D, 2 * D + CW]

    def cp_wa(c):
        return pltpu.make_async_copy(wa_hbm.at[:, pl.ds(ch_col[c], CW)],
                                     wa_v.at[:, pl.ds(ch_col[c], CW)], sem_wa.at[c])

    cp_woa = pltpu.make_async_copy(woa_hbm, woa_v, sem_woa.at[0])

    def cp_wb(j):
        return pltpu.make_async_copy(wb_hbm.at[pl.ds(j * 128, 128), :],
                                     wb_v.at[j], sem_wb.at[j])

    def cp_wob(j):
        return pltpu.make_async_copy(wob_hbm.at[:, pl.ds(j * 128, 128)],
                                     wob_v.at[j], sem_wob.at[j])

    def cp_out(i):
        return pltpu.make_async_copy(x_v.at[pl.ds(i * TB, TB), :],
                                     out_hbm.at[pl.ds(i * TB, TB), :], sem_out.at[i])

    def tri_mask():
        row = lax.broadcasted_iota(jnp.int32, (128, 128), 0)
        col = lax.broadcasted_iota(jnp.int32, (128, 128), 1)
        return col >= row

    def ln_chunks(row0, dst, nrows, step=16):
        def mk(c):
            def run(tok):
                if tok is not None:
                    x_v[S:S + 16, 0:128] = tok.astype(BF)
                r = pl.multiple_of(row0 + c * step, step)
                xn_v[dst + c * step:dst + (c + 1) * step, :] = _layernorm(x_v[pl.ds(r, step), :])
            return run
        return [mk(c) for c in range(nrows // step)]

    def prep_chunks(j):
        def permute(part):
            rows = [tmp[pl.ds(part * H * PITCH + d, H, stride=PITCH), :] for d in range(DH)]
            val = _pack(jnp.concatenate(rows, axis=0).astype(BF))
            if part < 3:
                wbt[j, part * (D // 2):(part + 1) * (D // 2), :] = val
            else:
                wobp[j] = val

        def mk_t(c):
            def run(tok):
                wb_v[8, 0:16, 0:128] = tok.astype(BF)
                wt = wb_v[j, :, c * 256:(c + 1) * 256].T.astype(F32)
                for hh in range(8):
                    o = (c * 8 + hh) * PITCH
                    tmp[o:o + DH, :] = wt[hh * DH:(hh + 1) * DH]
                if c % 4 == 3:
                    permute(c // 4)
            return run

        def mk_o(c):
            def run(tok):
                wob_v[8, 0:16, :] = tok.astype(BF)
                w = wob_v[j, c * 256:(c + 1) * 256, :].astype(F32)
                for hh in range(8):
                    o = (96 + c * 8 + hh) * PITCH
                    tmp[o:o + DH, :] = w[hh * DH:(hh + 1) * DH]
                if c == 3:
                    permute(3)
            return run
        return [mk_t(c) for c in range(12)] + [mk_o(c) for c in range(4)]

    def fence(zero):
        zx = _pack(xn_v[pl.ds(pl.multiple_of(2 * TA + zero * 32, 32), 32), 0:128])
        return zx | wbt[8, 0:16, :] | wobp[8, 0:16, :]

    def release(y, chunks):
        n = len(chunks)
        nt = y.shape[1] // 128
        for u, run in enumerate(chunks):
            pos = (u * y.shape[0] * nt // n) // 16 * 16
            t, rr = pos // y.shape[0], pos % y.shape[0]
            run(y[rr:rr + 16, t * 128:(t + 1) * 128])

    def proj_a(xn, blk, col0, ncols, side=()):
        y = _dot(xn, wa_v[:, col0:col0 + ncols])
        release(y, side)
        part, c0 = col0 // D, col0 % D
        if part == 1:
            r = blk * (TA // 2)
            if not isinstance(r, int):
                r = pl.multiple_of(r, TA // 2)
            for t in range(ncols // 128):
                k_v[c0 // 128 + t, pl.ds(r, TA // 2), :] = _pack(
                    y[:, t * 128:(t + 1) * 128].astype(BF))
        else:
            if part == 0:
                y = y * QSCALE
            yt = _pack(y.astype(BF).T)
            for b in range(TA // 128):
                piece = yt[:, b * 128:(b + 1) * 128]
                if part == 0:
                    qt_v[b, c0 // 2:(c0 + ncols) // 2, :] = piece
                else:
                    vt_v[blk * (TA // 128) + b, c0 // 2:(c0 + ncols) // 2, :] = piece

    def scores_a(m, qb, h, ntile, fen=None):
        t = h // 4
        z = jnp.zeros((16, 128), U32)
        qh = qt_v[qb, h * 16:(h + 1) * 16, :]
        if fen is not None:
            qh = qh | fen
        wq = _unpack(jnp.concatenate([qh if jj == h % 4 else z for jj in range(4)], axis=0))
        tri = tri_mask()
        base = m * 64
        if not isinstance(m, int):
            base = pl.multiple_of(base, 64)
        back = {1: (0,), 2: (0, 1), 3: (2, 0, 1)}[ntile]
        sm, mid = [], []
        nsplit = 4
        gper = 8 // nsplit
        for c in range(nsplit):
            parts = []
            for g in range(c * gper, (c + 1) * gper):
                for bk in back:
                    parts.append(k_v[t, pl.ds(base - bk * 64 + g * 8, 8), :])
            s = _dot(_unpack(jnp.concatenate(parts, axis=0)), wq)
            for gi in range(gper):
                g = c * gper + gi
                o = gi * 16 * ntile
                tr = tri[g * 16:(g + 1) * 16]
                if ntile == 3:
                    sm.append(jnp.where(tr, s[o + 16:o + 32], s[o:o + 16]))
                    mid.append(s[o + 32:o + 48])
                else:
                    sm.append(jnp.where(tr, s[o:o + 16], NEG))
                    if ntile == 2:
                        mid.append(s[o + 16:o + 32])
        return (jnp.concatenate(sm, axis=0),
                jnp.concatenate(mid, axis=0) if mid else None)

    def finish_a(sm, mid, m, h, ntile):
        tri = tri_mask()
        if mid is None:
            mx = jnp.max(sm, axis=0, keepdims=True)
            pm = jnp.exp2(sm - mx)
            l = jnp.sum(pm, axis=0, keepdims=True)
            p = pm
        else:
            mx = jnp.max(jnp.maximum(sm, mid), axis=0, keepdims=True)
            pm = jnp.exp2(sm - mx)
            pd = jnp.exp2(mid - mx)
            l = jnp.sum(pm + pd, axis=0, keepdims=True)
            if ntile == 3:
                p = jnp.concatenate(
                    [jnp.where(tri, 0.0, pm), pd, jnp.where(tri, pm, 0.0)], axis=0)
            else:
                p = jnp.concatenate([pd, pm], axis=0)
        vv = _unpack(jnp.concatenate(
            [vt_v[m - bk, h * 16:(h + 1) * 16, :] for bk in range(ntile - 1, -1, -1)], axis=1))
        o = _dot(vv, p.astype(BF))
        return o * pl.reciprocal(l, approx=False)

    def attn_a(blk, ntiles, looks, head_fill=None, tail_fill=None, fen=None):
        items = [(qb, h) for qb in range(TA // 128) for h in range(H)]
        queue = []
        issued = [0]

        def issue_upto(n):
            while issued[0] < min(n, len(items)):
                qb, h = items[issued[0]]
                f = fen() if (fen is not None and issued[0] == looks[0]) else None
                queue.append(scores_a(blk * (TA // 128) + qb, qb, h, ntiles[qb], f))
                issued[0] += 1
        issue_upto(looks[0])
        if head_fill is not None:
            head_fill()
        outs = []
        for n, (qb, h) in enumerate(items):
            issue_upto(n + 1 + looks[qb])
            if tail_fill is not None and n + looks[qb] == len(items):
                tail_fill()
            sm, mid = queue.pop(0)
            outs.append(finish_a(sm, mid, blk * (TA // 128) + qb, h, ntiles[qb]))
            if h % 4 == 3:
                ot = jnp.concatenate(outs, axis=0).astype(BF)
                oa_v[h // 4, qb * 64:(qb + 1) * 64, :] = _pack(ot.T)
                outs = []

    def out_a(blk, qb, c0, c1, side=(), fen=None):
        tiles = [oa_v[t, qb * 64:(qb + 1) * 64, :] for t in range(8)]
        if fen is not None:
            tiles[7] = jnp.concatenate([tiles[7][0:48], tiles[7][48:64] | fen], axis=0)
        o = _unpack(jnp.concatenate(tiles, axis=1))
        r = blk * TA + qb * 128
        if not isinstance(r, int):
            r = pl.multiple_of(r, 128)
        y = _dot(o, woa_v[:, c0:c1])
        release(y, side)
        x_v[pl.ds(r, 128), c0:c1] = (x_v[pl.ds(r, 128), c0:c1].astype(F32) + y).astype(BF)

    def proj_b(xn, r0, nrows, side):
        for T in range(24):
            w = _unpack(jnp.concatenate(
                [wbt[j, T * 64:(T + 1) * 64, :] for j in range(8)], axis=1))
            y = _dot_nt(xn, w)
            if T < 8:
                qk_v[T, HALO + r0:HALO + r0 + nrows, :] = y * QSCALE
            elif T < 16:
                qk_v[T, HALO + r0:HALO + r0 + nrows, :] = y
            else:
                v_v[T - 16, HALO + r0:HALO + r0 + nrows, :] = y
            release(y, side[T])

    def logit_b(i, zero, r0):
        R = 8

        def run(tok):
            qk_v[0, pl.ds(pl.multiple_of(HALO + TB + zero * 8, 8), 8), :] = tok[0:8]
            accs = [None] * WB
            for t in range(8):
                q = qk_v[t, HALO + r0:HALO + r0 + R, :]
                for w in range(WB):
                    o = HALO + r0 - 2 * w
                    p = q * qk_v[8 + t, o:o + R, :]
                    accs[w] = p if accs[w] is None else accs[w] + p
            ls = []
            for w in range(WB):
                a = accs[w]
                a = a + pltpu.roll(a, 64, 1)
                a = a + pltpu.roll(a, 32, 1)
                if r0 - 2 * w < 0:
                    pos = lax.broadcasted_iota(jnp.int32, (R, 128), 0) + (i * TB + r0 - 2 * w)
                    a = jnp.where(pos >= 0, a, NEG)
                ls.append(a)
            mx = ls[0]
            for w in range(1, WB):
                mx = jnp.maximum(mx, ls[w])
            es = [jnp.exp2(l - mx) for l in ls]
            s = es[0]
            for w in range(1, WB):
                s = s + es[w]
            inv = pl.reciprocal(s, approx=False)
            for w in range(WB):
                e_v[w, r0:r0 + R, :] = es[w] * inv
        return run

    def pv_b(zero, r0):
        R = 8

        def run(tok):
            v_v[0, pl.ds(pl.multiple_of(HALO + TB + zero * 8, 8), 8), :] = tok[0:8]
            es = [e_v[w, r0:r0 + R, :] for w in range(WB)]
            os_ = []
            for t in range(8):
                acc = None
                for w in range(WB):
                    o = HALO + r0 - 2 * w
                    pv = es[w] * v_v[t, o:o + R, :]
                    acc = pv if acc is None else acc + pv
                os_.append(acc)
            ob_v[r0:r0 + R, :] = jnp.concatenate(os_, axis=1).astype(BF)
        return run

    def out_b(i, r0, nrows, side):
        o = ob_v[r0:r0 + nrows, :]
        r = pl.multiple_of(i * TB + r0, 128)
        for c in range(4):
            w = _unpack(jnp.concatenate([wobp[2 * c], wobp[2 * c + 1]], axis=1))
            y = _dot(o, w)
            release(y, side[c])
            cs = slice(c * 256, (c + 1) * 256)
            x_v[pl.ds(r, nrows), cs] = (x_v[pl.ds(r, nrows), cs].astype(F32) + y).astype(BF)

    def spread(chunks, nslots, lo=0, hi=None):
        hi = nslots if hi is None else hi
        out = [[] for _ in range(nslots)]
        for u, c in enumerate(chunks):
            out[lo + u * (hi - lo) // len(chunks)].append(c)
        return out

    cp_x(0).start()
    cp_wa(0).start()
    cp_wa(1).start()
    xn_v[2 * TA:2 * TA + 32, :] = jnp.zeros((32, D), BF)
    wbt[8, 0:16, :] = jnp.zeros((16, 128), U32)
    wobp[8, 0:16, :] = jnp.zeros((16, 128), U32)
    cp_x(0).wait()
    for run in ln_chunks(0, 0, TA, step=TA):
        run(None)

    def one_pass(p, carry):
        first = p == 0
        zero = p // 4

        for c in range(NCH):
            @pl.when(first)
            def _():
                cp_wa(c).wait()
                if c + 2 < NCH:
                    cp_wa(c + 2).start()
                elif c + 2 == NCH:
                    cp_woa.start()
                else:
                    cp_x(1).start()
                    cp_wb(0).start()
                    cp_wob(0).start()
            if c + 1 < NCH:
                proj_a(xn_v[0:TA, :], 0, ch_col[c], CW)
        xn = xn_v[0:TA, :]
        proj_a(xn, 0, ch_col[-1], CW - 256)
        attn_a(0, (1, 2), (6, 3),
               head_fill=lambda: proj_a(xn, 0, 3 * D - 256, 256))

        @pl.when(first)
        def _():
            cp_woa.wait()
            cp_x(1).wait()
            cp_wb(0).wait()
            cp_wob(0).wait()
            cp_x(2).start()
            cp_wb(1).start()
            cp_wob(1).start()
        side = spread(prep_chunks(zero), 8, 0, 6)
        side2 = spread(ln_chunks(TA + zero * TA, 0, TA), 8, 0, 6)
        for u in range(8):
            out_a(0, u // 4, (u % 4) * 256, (u % 4 + 1) * 256, side[u] + side2[u],
                  fence(zero) if u == 7 else None)

        def a_body(i, c_):
            @pl.when(first)
            def _():
                @pl.when(i + 1 < NA)
                def _():
                    cp_x(i + 1).wait()
                    cp_wb(i + 1).start()
                    cp_wob(i + 1).start()

                @pl.when(i + 2 < NA)
                def _():
                    cp_x(i + 2).start()
                cp_wb(i).wait()
                cp_wob(i).wait()
            xn = xn_v[0:TA, :]
            lnc = ln_chunks(((i + 1) % NA) * TA, 0, TA)
            prc = prep_chunks(i)
            mixed = [c for pair in zip(prc, lnc) for c in pair]
            side = spread(mixed, 11, 0, 10)
            cols = [D + c * 256 for c in range(4)] + [c * 256 for c in range(4)] + \
                   [2 * D + c * 256 for c in range(3)]
            for u, c0 in enumerate(cols):
                proj_a(xn, i, c0, 256, side[u])
            attn_a(i, (3, 3), (LOOK, LOOK),
                   head_fill=lambda: proj_a(xn, i, 3 * D - 256, 256),
                   tail_fill=lambda: out_a(i, 0, 0, 256),
                   fen=lambda: fence(zero))
            out_a(i, 0, 256, D)
            out_a(i, 1, 0, D)
            return c_
        lax.fori_loop(1, NA, a_body, 0)

        for T in range(8):
            qk_v[8 + T, 0:HALO, :] = jnp.zeros((HALO, 128), F32)
            v_v[T, 0:HALO, :] = jnp.zeros((HALO, 128), F32)

        def b_body(i, c_):
            xn = xn_v[0:TA, :]
            ln1 = ln_chunks(i * TB + 256, TA, 256)
            ln2 = ln_chunks(((i + 1) % NB) * TB, 0, TA)
            lg = [logit_b(i, zero, g * 8) for g in range(TB // 8)]
            pv = [pv_b(zero, g * 8) for g in range(TB // 8)]

            def both(a, b):
                return [u + v for u, v in zip(a, b)]
            proj_b(xn, 0, 256, both(spread(ln1 + ln2, 24, 0, 16), spread(lg[0:20], 24, 16, 24)))
            xn1 = xn_v[pl.ds(pl.multiple_of(TA + zero * 32, 32), TA), :]
            proj_b(xn1, 256, 256, both(spread(lg[20:32] + pv[0:32], 24, 0, 16),
                                       spread(lg[32:64], 24, 16, 24)))
            out_b(i, 0, 256, spread(pv[32:58], 4))
            out_b(i, 256, 128, spread(pv[58:64], 4, 0, 2))
            out_b(i, 384, 128, [[]] * 4)
            for T in range(8):
                qk_v[8 + T, 0:HALO, :] = qk_v[8 + T, TB:TB + HALO, :]
                v_v[T, 0:HALO, :] = v_v[T, TB:TB + HALO, :]

            @pl.when(p == 1)
            def _():
                cp_out(i).start()
            return c_
        lax.fori_loop(0, NB, b_body, 0)
        return carry

    lax.fori_loop(0, 2, one_pass, 0)
    for i in range(NB):
        cp_out(i).wait()


@jax.jit
def pallas_interleave_layers__sliding_block__sliding_local_dilated__prompt_kernel(
    A_x: jax.Array,
    A_wqkv: jax.Array,
    A_wo: jax.Array,
    B_x: jax.Array,
    B_wqkv: jax.Array,
    B_wo: jax.Array,
):
    del B_x
    x = A_x.reshape(S, D)
    any_spec = pl.BlockSpec(memory_space=pl.ANY)
    out = pl.pallas_call(
        _kernel,
        out_shape=jax.ShapeDtypeStruct((S, D), BF),
        in_specs=[any_spec] * 5,
        out_specs=any_spec,
        scratch_shapes=[
            pltpu.VMEM((S + 16, D), BF),
            pltpu.VMEM((D, 3 * D), BF),
            pltpu.VMEM((D, D), BF),
            pltpu.VMEM((9, 128, 3 * D), BF),
            pltpu.VMEM((9, D, 128), BF),
            pltpu.VMEM((9, 3 * D // 2, 128), U32),
            pltpu.VMEM((9, D // 2, 128), U32),
            pltpu.VMEM((128 * PITCH, 128), F32),
            pltpu.VMEM((2 * TA + 32, D), BF),
            pltpu.VMEM((8, S // 2, 128), U32),
            pltpu.VMEM((TA // 128, D // 2, 128), U32),
            pltpu.VMEM((S // 128, D // 2, 128), U32),
            pltpu.VMEM((8, TA // 2, 128), U32),
            pltpu.VMEM((16, HALO + TB + 8, 128), F32),
            pltpu.VMEM((8, HALO + TB + 8, 128), F32),
            pltpu.VMEM((WB, TB + 8, 128), F32),
            pltpu.VMEM((TB, D), BF),
            pltpu.SemaphoreType.DMA((NA,)),
            pltpu.SemaphoreType.DMA((NCH,)),
            pltpu.SemaphoreType.DMA((1,)),
            pltpu.SemaphoreType.DMA((8,)),
            pltpu.SemaphoreType.DMA((8,)),
            pltpu.SemaphoreType.DMA((NB,)),
        ],
        compiler_params=pltpu.CompilerParams(vmem_limit_bytes=100 * 1024 * 1024),
        name="interleave_attn",
    )(x, A_wqkv, A_wo, B_wqkv, B_wo)
    return out.reshape(1, S, D)
```

```python
import math

import jax
import jax.numpy as jnp
from jax import lax
import jax.experimental.pallas as pl
import jax.experimental.pallas.tpu as pltpu

BF = jnp.bfloat16
F32 = jnp.float32
U32 = jnp.uint32

S = 2048
D = 1024
H = 32
DH = 32
TA = 256
NA = S // TA
TB = 512
NB = S // TB
HALO = 16
WB = 8
NEG = -1e30
EPS = 1e-5
QSCALE = (DH ** -0.5) * math.log2(math.e)
NCH = 6
CW = 3 * D // NCH
LOOK = 2
PITCH = 36


def _dot(a, b):
    return jnp.dot(a, b, preferred_element_type=F32)


def _dot_nt(a, b):
    return lax.dot_general(a, b, (((1,), (1,)), ((), ())), preferred_element_type=F32)


def _pack(x_bf16):
    return pltpu.bitcast(x_bf16, U32)


def _unpack(x_u32):
    return pltpu.bitcast(x_u32, BF)


def _layernorm(x_bf16):
    x = x_bf16.astype(F32)
    m = jnp.sum(x, axis=1, keepdims=True) * (1.0 / D)
    xc = x - m
    v = jnp.sum(xc * xc, axis=1, keepdims=True) * (1.0 / D)
    return (xc * lax.rsqrt(v + EPS)).astype(BF)


def _kernel(x_hbm, wa_hbm, woa_hbm, wb_hbm, wob_hbm, out_hbm,
            x_v, wa_v, woa_v, wb_v, wob_v, wbt, wobp, tmp, xn_v,
            k0_v, kt_v, qt_v, oa_v, qk_v, v_v, e_v, ob_v,
            sem_x, sem_wa, sem_woa, sem_wb, sem_wob, sem_out, *grp):
    k4_v, vt_v = grp[:8], grp[8:]
    def cp_x(i):
        return pltpu.make_async_copy(x_hbm.at[pl.ds(i * TA, TA), :],
                                     x_v.at[pl.ds(i * TA, TA), :], sem_x.at[i])

    ch_col = [D, D + CW, 0, CW, 2 * D, 2 * D + CW]

    def cp_wa(c):
        return pltpu.make_async_copy(wa_hbm.at[:, pl.ds(ch_col[c], CW)],
                                     wa_v.at[:, pl.ds(ch_col[c], CW)], sem_wa.at[c])

    cp_woa = pltpu.make_async_copy(woa_hbm, woa_v, sem_woa.at[0])

    def cp_wb(j):
        return pltpu.make_async_copy(wb_hbm.at[pl.ds(j * 128, 128), :],
                                     wb_v.at[j], sem_wb.at[j])

    def cp_wob(j):
        return pltpu.make_async_copy(wob_hbm.at[:, pl.ds(j * 128, 128)],
                                     wob_v.at[j], sem_wob.at[j])

    def cp_out(i):
        return pltpu.make_async_copy(x_v.at[pl.ds(i * TB, TB), :],
                                     out_hbm.at[pl.ds(i * TB, TB), :], sem_out.at[i])

    def tri_mask():
        row = lax.broadcasted_iota(jnp.int32, (128, 128), 0)
        col = lax.broadcasted_iota(jnp.int32, (128, 128), 1)
        return col >= row

    def ln_chunks(row0, dst, nrows, step=16):
        def mk(c):
            def run(tok):
                if tok is not None:
                    x_v[S:S + 16, 0:128] = tok.astype(BF)
                r = pl.multiple_of(row0 + c * step, step)
                xn_v[dst + c * step:dst + (c + 1) * step, :] = _layernorm(x_v[pl.ds(r, step), :])
            return run
        return [mk(c) for c in range(nrows // step)]

    def prep_chunks(j):
        def permute(part):
            rows = [tmp[pl.ds(part * H * PITCH + d, H, stride=PITCH), :] for d in range(DH)]
            val = _pack(jnp.concatenate(rows, axis=0).astype(BF))
            if part < 3:
                wbt[j, part * (D // 2):(part + 1) * (D // 2), :] = val
            else:
                wobp[j] = val

        def mk_t(c):
            def run(tok):
                wb_v[8, 0:16, 0:128] = tok.astype(BF)
                wt = wb_v[j, :, c * 256:(c + 1) * 256].T.astype(F32)
                for hh in range(8):
                    o = (c * 8 + hh) * PITCH
                    tmp[o:o + DH, :] = wt[hh * DH:(hh + 1) * DH]
                if c % 4 == 3:
                    permute(c // 4)
            return run

        def mk_o(c):
            def run(tok):
                wob_v[8, 0:16, :] = tok.astype(BF)
                w = wob_v[j, c * 256:(c + 1) * 256, :].astype(F32)
                for hh in range(8):
                    o = (96 + c * 8 + hh) * PITCH
                    tmp[o:o + DH, :] = w[hh * DH:(hh + 1) * DH]
                if c == 3:
                    permute(3)
            return run
        return [mk_t(c) for c in range(12)] + [mk_o(c) for c in range(4)]

    def fence(zero):
        zx = _pack(xn_v[pl.ds(pl.multiple_of(2 * TA + zero * 32, 32), 32), 0:128])
        return zx | wbt[8, 0:16, :] | wobp[8, 0:16, :]

    def release(y, chunks):
        n = len(chunks)
        nt = y.shape[1] // 128
        for u, run in enumerate(chunks):
            pos = (u * y.shape[0] * nt // n) // 16 * 16
            t, rr = pos // y.shape[0], pos % y.shape[0]
            run(y[rr:rr + 16, t * 128:(t + 1) * 128])

    def iota(shape, dim):
        return lax.broadcasted_iota(jnp.int32, shape, dim)

    def store_k(y, blk, t):
        kp = _pack(y.astype(BF))
        if isinstance(blk, int):
            k0_v[t] = kp
            full, row0 = kp, 48
        else:
            full = jnp.concatenate([kt_v[t], kp], axis=0)
            row0 = pl.multiple_of(blk * (TA // 2), TA // 2)
        kt_v[t] = kp[80:128]
        n = full.shape[0] - 48
        rolled = [full] + [pltpu.roll(full, 32 * r, 1) for r in range(1, 4)]
        grp_id = iota((n, 128), 1) // 32
        for a in range(4):
            val = rolled[(0 - a) % 4][0:n]
            for g in range(1, 4):
                val = jnp.where(grp_id == g, rolled[(g - a) % 4][16 * g:16 * g + n], val)
            k4_v[t][a, pl.ds(row0, n), :] = val

    def store_qv(y, blk, t, is_q):
        if is_q:
            y = y * QSCALE
        yt = _pack(y.astype(BF).T)
        for b in range(TA // 128):
            piece = yt[:, b * 128:(b + 1) * 128]
            if is_q:
                qt_v[b, t * 64:(t + 1) * 64, :] = piece
            else:
                vt_v[t][blk * (TA // 128) + b] = piece

    def proj_a(xn, blk, col0, ncols):
        y = _dot(xn, wa_v[:, col0:col0 + ncols])
        part, t0 = col0 // D, (col0 % D) // 128
        for t in range(ncols // 128):
            yt = y[:, t * 128:(t + 1) * 128]
            if part == 1:
                store_k(yt, blk, t0 + t)
            else:
                store_qv(yt, blk, t0 + t, part == 0)
        return y

    def scores_first(qb, h):
        z = jnp.zeros((16, 128), U32)
        qh = qt_v[qb, h * 16:(h + 1) * 16, :]
        wq = _unpack(jnp.concatenate([qh if jj == h % 4 else z for jj in range(4)], axis=0))
        n = (qb + 1) * 16
        s = jnp.concatenate(
            [_dot(_unpack(k0_v[h // 4, c * n:(c + 1) * n, :]), wq) for c in range(4)], axis=0)
        diag = jnp.where(tri_mask(), s[qb * 128:], NEG)
        return diag if qb == 0 else jnp.concatenate([s[0:128], diag], axis=0)

    def scores_a(m, qb, h):
        qh = qt_v[qb, h * 16:(h + 1) * 16, :]
        grp_id = iota((16, 128), 1) // 32
        z = jnp.zeros((16, 128), U32)
        wq = _unpack(jnp.concatenate(
            [jnp.where(grp_id == g, qh, z) for g in range(4)], axis=0))
        base = pl.multiple_of(m * 64 - 80, 16)
        order = [0, 16, 1, 17] + list(range(2, 16))
        cuts = [0, 5, 9, 14, 18]
        units = {}
        for c in range(4):
            idx = order[cuts[c]:cuts[c + 1]]
            lhs = jnp.concatenate(
                [k4_v[h // 4][h % 4, pl.ds(base + u * 8, 8), :] for u in idx], axis=0)
            s = _dot(_unpack(lhs), wq)
            for n, u in enumerate(idx):
                units[u] = s[n * 16:(n + 1) * 16]
        for u in range(2):
            new = (iota((16, 128), 1) % 32) >= (iota((16, 128), 0) + u * 16)
            units[u] = jnp.where(new, units[16 + u], units[u])
        return jnp.concatenate([units[u] for u in range(16)], axis=0)

    def finish_a(s, m, h):
        mx = jnp.max(s, axis=0, keepdims=True)
        p = jnp.exp2(s - mx)
        l = jnp.sum(p, axis=0, keepdims=True)
        if not isinstance(m, int):
            lane = iota((256, 128), 1)
            p = jnp.where((lane // 32) % 2 == 1,
                          jnp.concatenate([p[224:], p[:224]], axis=0), p)
            p = jnp.where(lane >= 64, jnp.concatenate([p[192:], p[:192]], axis=0), p)
            tri = tri_mask()
            pm = p[0:128]
            p = jnp.concatenate(
                [jnp.where(tri, 0.0, pm), p[128:256], jnp.where(tri, pm, 0.0)], axis=0)
        ntile = p.shape[0] // 128
        a = h % 4
        vv = _unpack(jnp.concatenate(
            [vt_v[h // 4][m - bk, a * 16:(a + 1) * 16, :]
             for bk in range(ntile - 1, -1, -1)], axis=1))
        o = _dot(vv, p.astype(BF))
        return o * pl.reciprocal(l, approx=False)

    class Attn:
        def __init__(self, blk, items):
            self.blk, self.items = blk, items
            self.issued, self.done, self.queue, self.outs = 0, 0, [], {}

        def issue(self, n=1):
            for _ in range(n):
                if self.issued < len(self.items):
                    qb, h = self.items[self.issued]
                    if isinstance(self.blk, int):
                        self.queue.append(scores_first(qb, h))
                    else:
                        self.queue.append(scores_a(self.blk * (TA // 128) + qb, qb, h))
                    self.issued += 1

        def finish(self, n=1):
            for _ in range(n):
                if self.done < self.issued:
                    qb, h = self.items[self.done]
                    o = finish_a(self.queue.pop(0), self.blk * (TA // 128) + qb, h)
                    outs = self.outs.setdefault((qb, h // 4), [])
                    outs.append(o)
                    if len(outs) == 4:
                        ot = jnp.concatenate(outs, axis=0).astype(BF)
                        oa_v[h // 4, qb * 64:(qb + 1) * 64, :] = _pack(ot.T)
                    self.done += 1

    def with_fence(xu, fen):
        r, c = xu.shape
        last = jnp.concatenate([xu[r - 16:, :c - 128], xu[r - 16:, c - 128:] | fen], axis=1)
        return jnp.concatenate([xu[:r - 16], last], axis=0)

    def out_a(r, nrows, c0, c1, y):
        x_v[pl.ds(r, nrows), c0:c1] = (x_v[pl.ds(r, nrows), c0:c1].astype(F32) + y).astype(BF)

    def proj_b(xn, r0, nrows, side):
        for T in range(24):
            w = _unpack(jnp.concatenate(
                [wbt[j, T * 64:(T + 1) * 64, :] for j in range(8)], axis=1))
            y = _dot_nt(xn, w)
            if T < 8:
                qk_v[T, HALO + r0:HALO + r0 + nrows, :] = y * QSCALE
            elif T < 16:
                qk_v[T, HALO + r0:HALO + r0 + nrows, :] = y
            else:
                v_v[T - 16, HALO + r0:HALO + r0 + nrows, :] = y
            release(y, side[T])

    def logit_b(i, zero, r0):
        R = 8

        def run(tok):
            qk_v[0, pl.ds(pl.multiple_of(HALO + TB + zero * 8, 8), 8), :] = tok[0:8]
            accs = [None] * WB
            for t in range(8):
                q = qk_v[t, HALO + r0:HALO + r0 + R, :]
                for w in range(WB):
                    o = HALO + r0 - 2 * w
                    p = q * qk_v[8 + t, o:o + R, :]
                    accs[w] = p if accs[w] is None else accs[w] + p
            ls = []
            for w in range(WB):
                a = accs[w]
                a = a + pltpu.roll(a, 64, 1)
                a = a + pltpu.roll(a, 32, 1)
                if r0 - 2 * w < 0:
                    pos = lax.broadcasted_iota(jnp.int32, (R, 128), 0) + (i * TB + r0 - 2 * w)
                    a = jnp.where(pos >= 0, a, NEG)
                ls.append(a)
            mx = ls[0]
            for w in range(1, WB):
                mx = jnp.maximum(mx, ls[w])
            es = [jnp.exp2(l - mx) for l in ls]
            s = es[0]
            for w in range(1, WB):
                s = s + es[w]
            inv = pl.reciprocal(s, approx=False)
            for w in range(WB):
                e_v[w, r0:r0 + R, :] = es[w] * inv
        return run

    def pv_b(zero, r0):
        R = 8

        def run(tok):
            v_v[0, pl.ds(pl.multiple_of(HALO + TB + zero * 8, 8), 8), :] = tok[0:8]
            es = [e_v[w, r0:r0 + R, :] for w in range(WB)]
            os_ = []
            for t in range(8):
                acc = None
                for w in range(WB):
                    o = HALO + r0 - 2 * w
                    pv = es[w] * v_v[t, o:o + R, :]
                    acc = pv if acc is None else acc + pv
                os_.append(acc)
            ob_v[r0:r0 + R, :] = jnp.concatenate(os_, axis=1).astype(BF)
        return run

    def out_b(i, r0, nrows, side):
        o = ob_v[r0:r0 + nrows, :]
        r = pl.multiple_of(i * TB + r0, 128)
        for c in range(4):
            w = _unpack(jnp.concatenate([wobp[2 * c], wobp[2 * c + 1]], axis=1))
            y = _dot(o, w)
            release(y, side[c])
            cs = slice(c * 256, (c + 1) * 256)
            x_v[pl.ds(r, nrows), cs] = (x_v[pl.ds(r, nrows), cs].astype(F32) + y).astype(BF)

    def spread(chunks, nslots, lo=0, hi=None):
        hi = nslots if hi is None else hi
        out = [[] for _ in range(nslots)]
        for u, c in enumerate(chunks):
            out[lo + u * (hi - lo) // len(chunks)].append(c)
        return out

    cp_x(0).start()
    cp_wa(0).start()
    cp_wa(1).start()
    xn_v[2 * TA:2 * TA + 32, :] = jnp.zeros((32, D), BF)
    wbt[8, 0:16, :] = jnp.zeros((16, 128), U32)
    wobp[8, 0:16, :] = jnp.zeros((16, 128), U32)
    cp_x(0).wait()
    for run in ln_chunks(0, 0, TA, step=TA):
        run(None)

    def one_pass(p, carry):
        first = p == 0
        zero = p // 4

        for c in range(NCH):
            @pl.when(first)
            def _():
                cp_wa(c).wait()
                if c + 2 < NCH:
                    cp_wa(c + 2).start()
                elif c + 2 == NCH:
                    cp_woa.start()
                else:
                    cp_x(1).start()
                    cp_wb(0).start()
                    cp_wob(0).start()
            if c + 1 < NCH:
                proj_a(xn_v[0:TA, :], 0, ch_col[c], CW)
        xn = xn_v[0:TA, :]
        proj_a(xn, 0, ch_col[-1], CW - 256)
        at = Attn(0, [(qb, h) for qb in range(2) for h in range(H)])
        at.issue(6)
        proj_a(xn, 0, 3 * D - 256, 256)
        for n in range(2 * H):
            if n < H - 3 or n >= H:
                at.issue()
            at.finish()

        @pl.when(first)
        def _():
            cp_woa.wait()
            cp_x(1).wait()
            cp_wb(0).wait()
            cp_wob(0).wait()
            cp_x(2).start()
            cp_wb(1).start()
            cp_wob(1).start()
        side = spread(prep_chunks(zero), 8, 0, 6)
        side2 = spread(ln_chunks(TA + zero * TA, 0, TA), 8, 0, 6)
        ou = jnp.concatenate([oa_v[t] for t in range(8)], axis=1)
        ys = []
        for u in range(8):
            lhs = with_fence(ou, fence(zero)) if u == 7 else ou
            ys.append(_dot(_unpack(lhs), woa_v[:, u * 128:(u + 1) * 128]))
            release(ys[-1], side[u] + side2[u])
            if u % 2 == 1:
                out_a(0, TA, (u - 1) * 128, (u + 1) * 128, jnp.concatenate(ys[-2:], axis=1))

        def a_body(i, c_):
            @pl.when(first)
            def _():
                @pl.when(i + 1 < NA)
                def _():
                    cp_x(i + 1).wait()
                    cp_wb(i + 1).start()
                    cp_wob(i + 1).start()

                @pl.when(i + 2 < NA)
                def _():
                    cp_x(i + 2).start()
                cp_wb(i).wait()
                cp_wob(i).wait()
            xu = _pack(xn_v[0:TA, :])
            lnc = ln_chunks(((i + 1) % NA) * TA, 0, TA)
            prc = prep_chunks(i)
            mixed = [c for pair in zip(prc, lnc) for c in pair]
            side = spread(mixed, 24, 0, 21)
            at = Attn(i, [(qb, 4 * t + a) for t in range(8) for a in range(4) for qb in range(2)])
            yprev = None
            for u in range(24):
                t, kind = u // 3, u % 3
                n = 0 if t == 0 else (3, 3, 2)[kind]
                at.issue(n)
                lhs = with_fence(xu, fence(zero)) if (u >= 3 and u % 2 == 1) else xu
                y = proj_a(_unpack(lhs), i, (D, 0, 2 * D)[kind] + t * 128, 128)
                if yprev is not None:
                    release(yprev, side[u - 1])
                yprev = y
                at.finish(n)
            o1 = _unpack(jnp.concatenate([oa_v[t] for t in range(4)], axis=1))
            part = []
            for u in range(8):
                n = (2, 2, 2, 2, 0, 0, 0, 0)[u]
                at.issue(n)
                part.append(_dot(o1, woa_v[0:D // 2, u * 128:(u + 1) * 128]))
                at.finish((0, 2, 2, 2, 2, 0, 0, 0)[u])
            o2 = _unpack(jnp.concatenate([oa_v[t] for t in range(4, 8)], axis=1))
            r = pl.multiple_of(i * TA, TA)
            for c in range(4):
                y = _dot(o2, woa_v[D // 2:, c * 256:(c + 1) * 256])
                out_a(r, TA, c * 256, (c + 1) * 256,
                      y + jnp.concatenate(part[2 * c:2 * c + 2], axis=1))
            return c_
        lax.fori_loop(1, NA, a_body, 0)

        for T in range(8):
            qk_v[8 + T, 0:HALO, :] = jnp.zeros((HALO, 128), F32)
            v_v[T, 0:HALO, :] = jnp.zeros((HALO, 128), F32)

        def b_body(i, c_):
            xn = xn_v[0:TA, :]
            ln1 = ln_chunks(i * TB + 256, TA, 256)
            ln2 = ln_chunks(((i + 1) % NB) * TB, 0, TA)
            lg = [logit_b(i, zero, g * 8) for g in range(TB // 8)]
            pv = [pv_b(zero, g * 8) for g in range(TB // 8)]

            def both(a, b):
                return [u + v for u, v in zip(a, b)]
            proj_b(xn, 0, 256, both(spread(ln1 + ln2, 24, 0, 16), spread(lg[0:20], 24, 16, 24)))
            xn1 = xn_v[pl.ds(pl.multiple_of(TA + zero * 32, 32), TA), :]
            proj_b(xn1, 256, 256, both(spread(lg[20:32] + pv[0:32], 24, 0, 16),
                                       spread(lg[32:64], 24, 16, 24)))
            out_b(i, 0, 256, spread(pv[32:58], 4))
            out_b(i, 256, 128, spread(pv[58:64], 4, 0, 2))
            out_b(i, 384, 128, [[]] * 4)
            for T in range(8):
                qk_v[8 + T, 0:HALO, :] = qk_v[8 + T, TB:TB + HALO, :]
                v_v[T, 0:HALO, :] = v_v[T, TB:TB + HALO, :]

            @pl.when(p == 1)
            def _():
                cp_out(i).start()
            return c_
        lax.fori_loop(0, NB, b_body, 0)
        return carry

    lax.fori_loop(0, 2, one_pass, 0)
    for i in range(NB):
        cp_out(i).wait()


@jax.jit
def pallas_interleave_layers__sliding_block__sliding_local_dilated__prompt_kernel(
    A_x: jax.Array,
    A_wqkv: jax.Array,
    A_wo: jax.Array,
    B_x: jax.Array,
    B_wqkv: jax.Array,
    B_wo: jax.Array,
):
    del B_x
    x = A_x.reshape(S, D)
    any_spec = pl.BlockSpec(memory_space=pl.ANY)
    out = pl.pallas_call(
        _kernel,
        out_shape=jax.ShapeDtypeStruct((S, D), BF),
        in_specs=[any_spec] * 5,
        out_specs=any_spec,
        scratch_shapes=[
            pltpu.VMEM((S + 16, D), BF),
            pltpu.VMEM((D, 3 * D), BF),
            pltpu.VMEM((D, D), BF),
            pltpu.VMEM((9, 128, 3 * D), BF),
            pltpu.VMEM((9, D, 128), BF),
            pltpu.VMEM((9, 3 * D // 2, 128), U32),
            pltpu.VMEM((9, D // 2, 128), U32),
            pltpu.VMEM((128 * PITCH, 128), F32),
            pltpu.VMEM((2 * TA + 32, D), BF),
            pltpu.VMEM((8, TA // 2, 128), U32),
            pltpu.VMEM((8, 48, 128), U32),
            pltpu.VMEM((TA // 128, D // 2, 128), U32),
            pltpu.VMEM((8, TA // 2, 128), U32),
            pltpu.VMEM((16, HALO + TB + 8, 128), F32),
            pltpu.VMEM((8, HALO + TB + 8, 128), F32),
            pltpu.VMEM((WB, TB + 8, 128), F32),
            pltpu.VMEM((TB, D), BF),
            pltpu.SemaphoreType.DMA((NA,)),
            pltpu.SemaphoreType.DMA((NCH,)),
            pltpu.SemaphoreType.DMA((1,)),
            pltpu.SemaphoreType.DMA((8,)),
            pltpu.SemaphoreType.DMA((8,)),
            pltpu.SemaphoreType.DMA((NB,)),
        ] + [pltpu.VMEM((4, S // 2, 128), U32)] * 8
          + [pltpu.VMEM((S // 128, 64, 128), U32)] * 8,
        compiler_params=pltpu.CompilerParams(vmem_limit_bytes=100 * 1024 * 1024),
        name="interleave_attn",
    )(x, A_wqkv, A_wo, B_wqkv, B_wo)
    return out.reshape(1, S, D)
```

```python
import math

import jax
import jax.numpy as jnp
from jax import lax
import jax.experimental.pallas as pl
import jax.experimental.pallas.tpu as pltpu

BF = jnp.bfloat16
F32 = jnp.float32
U32 = jnp.uint32

S = 2048
D = 1024
H = 32
DH = 32
TA = 256
NA = S // TA
TB = 512
NB = S // TB
HALO = 16
WB = 8
NEG = -1e30
EPS = 1e-5
QSCALE = (DH ** -0.5) * math.log2(math.e)
NCH = 6
CW = 3 * D // NCH
PITCH = 36

CFG = dict(first=1, a=1, b=1, sched=1, look=3, side=1, pat=(0, 0, 0), fence_every=3, lag=0, hpat=(2, 1, 1, 2, 1, 1), qpre=0, order=1, early=1, split=0, efence=2, shi=21)


def _dot(a, b):
    return jnp.dot(a, b, preferred_element_type=F32)


def _dot_nt(a, b):
    return lax.dot_general(a, b, (((1,), (1,)), ((), ())), preferred_element_type=F32)


def _pack(x_bf16):
    return pltpu.bitcast(x_bf16, U32)


def _unpack(x_u32):
    return pltpu.bitcast(x_u32, BF)


def _layernorm(x_bf16):
    x = x_bf16.astype(F32)
    m = jnp.sum(x, axis=1, keepdims=True) * (1.0 / D)
    xc = x - m
    v = jnp.sum(xc * xc, axis=1, keepdims=True) * (1.0 / D)
    return (xc * lax.rsqrt(v + EPS)).astype(BF)


def _kernel(x_hbm, wa_hbm, woa_hbm, wb_hbm, wob_hbm, out_hbm,
            x_v, wa_v, woa_v, wb_v, wob_v, wap, woap, wbt, wobp, tmp, xn_v,
            k0_v, kt_v, oa_v, qk_v, v_v, e_v, ob_v,
            sem_x, sem_wa, sem_woa, sem_wb, sem_wob, sem_out, *grp):
    k4_v, vt_v, qt_v = grp[:8], grp[8:16], grp[16:]
    def cp_x(i):
        n = TA if i < 3 else S - 3 * TA
        return pltpu.make_async_copy(x_hbm.at[pl.ds(i * TA, n), :],
                                     x_v.at[pl.ds(i * TA, n), :], sem_x.at[i])

    ch_col = [D, D + CW, 0, CW, 2 * D, 2 * D + CW]

    def cp_wa(c):
        return pltpu.make_async_copy(wa_hbm.at[:, pl.ds(ch_col[c], CW)],
                                     wa_v.at[:, pl.ds(ch_col[c], CW)], sem_wa.at[c])

    cp_woa = pltpu.make_async_copy(woa_hbm, woa_v, sem_woa.at[0])

    def cp_wb(j):
        n = 128 if j < 2 else D - 256
        return pltpu.make_async_copy(wb_hbm.at[pl.ds(j * 128, n), :],
                                     wb_v.at[pl.ds(j * 128, n), :], sem_wb.at[j])

    def cp_wob(j):
        return pltpu.make_async_copy(wob_hbm.at[:, pl.ds(j * 128, 128)],
                                     wob_v.at[j], sem_wob.at[j])

    def cp_out(i):
        return pltpu.make_async_copy(x_v.at[pl.ds(i * TB, TB), :],
                                     out_hbm.at[pl.ds(i * TB, TB), :], sem_out.at[i])

    def tri_mask():
        row = lax.broadcasted_iota(jnp.int32, (128, 128), 0)
        col = lax.broadcasted_iota(jnp.int32, (128, 128), 1)
        return col >= row

    def ln_chunks(row0, dst, nrows, step=16):
        def mk(c):
            def run(tok):
                if tok is not None:
                    x_v[S:S + 16, 0:128] = tok.astype(BF)
                r = pl.multiple_of(row0 + c * step, step)
                xn_v[dst + c * step:dst + (c + 1) * step, :] = _layernorm(x_v[pl.ds(r, step), :])
            return run
        return [mk(c) for c in range(nrows // step)]

    def prep_chunks(j):
        def permute(part):
            rows = [tmp[pl.ds(part * H * PITCH + d, H, stride=PITCH), :] for d in range(DH)]
            val = _pack(jnp.concatenate(rows, axis=0).astype(BF))
            if part < 3:
                wbt[j, part * (D // 2):(part + 1) * (D // 2), :] = val
            else:
                wobp[j] = val

        def mk_t(c):
            def run(tok):
                wb_v[D:D + 16, 0:128] = tok.astype(BF)
                rows = pl.ds(pl.multiple_of(j * 128, 128), 128)
                wt = wb_v[rows, c * 256:(c + 1) * 256].T.astype(F32)
                for hh in range(8):
                    o = (c * 8 + hh) * PITCH
                    tmp[o:o + DH, :] = wt[hh * DH:(hh + 1) * DH]
                if c % 4 == 3:
                    permute(c // 4)
            return run

        def mk_o(c):
            def run(tok):
                wob_v[8, 0:16, :] = tok.astype(BF)
                w = wob_v[j, c * 256:(c + 1) * 256, :].astype(F32)
                for hh in range(8):
                    o = (96 + c * 8 + hh) * PITCH
                    tmp[o:o + DH, :] = w[hh * DH:(hh + 1) * DH]
                if c == 3:
                    permute(3)
            return run
        return [mk_t(c) for c in range(12)] + [mk_o(c) for c in range(4)]

    def fence(zero):
        zx = _pack(xn_v[pl.ds(pl.multiple_of(2 * TA + zero * 32, 32), 32), 0:128])
        return zx | wbt[8, 0:16, :] | wobp[8, 0:16, :]

    def release(y, chunks):
        n = len(chunks)
        nt = y.shape[1] // 128
        for u, run in enumerate(chunks):
            pos = (u * y.shape[0] * nt // n) // 16 * 16
            t, rr = pos // y.shape[0], pos % y.shape[0]
            run(y[rr:rr + 16, t * 128:(t + 1) * 128])

    def iota(shape, dim):
        return lax.broadcasted_iota(jnp.int32, shape, dim)

    def store_k(y, blk, t):
        kp = _pack(y.astype(BF))
        if isinstance(blk, int):
            k0_v[t] = kp
            full, row0 = kp, 48
        else:
            full = jnp.concatenate([kt_v[t], kp], axis=0)
            row0 = pl.multiple_of(blk * (TA // 2), TA // 2)
        kt_v[t] = kp[80:128]
        n = full.shape[0] - 48
        rolled = [full] + [pltpu.roll(full, 32 * r, 1) for r in range(1, 4)]
        grp_id = iota((n, 128), 1) // 32
        for a in range(4):
            val = rolled[(0 - a) % 4][0:n]
            for g in range(1, 4):
                val = jnp.where(grp_id == g, rolled[(g - a) % 4][16 * g:16 * g + n], val)
            k4_v[t][a, pl.ds(row0, n), :] = val

    def store_qv(y, blk, t, is_q):
        if is_q:
            y = y * QSCALE
        yt = _pack(y.astype(BF).T)
        for b in range(TA // 128):
            piece = yt[:, b * 128:(b + 1) * 128]
            if is_q:
                qt_v[t][b] = piece
            else:
                vt_v[t][blk * (TA // 128) + b] = piece

    def proj_a(xn, blk, col0, ncols):
        T0 = col0 // 128
        if isinstance(blk, int):
            wu = _pack(wa_v[:, col0:col0 + ncols])
            for t in range(ncols // 128):
                wap[T0 + t] = wu[:, t * 128:(t + 1) * 128]
        else:
            wu = jnp.concatenate([wap[T0 + t] for t in range(ncols // 128)], axis=1)
        y = _dot(xn, _unpack(wu))
        return epi_a(y, blk, col0)

    def epi_a(y, blk, col0):
        ncols = y.shape[1]
        part, t0 = col0 // D, (col0 % D) // 128
        for t in range(ncols // 128):
            yt = y[:, t * 128:(t + 1) * 128]
            if part == 1:
                store_k(yt, blk, t0 + t)
            else:
                store_qv(yt, blk, t0 + t, part == 0)
        return y

    def scores_first(qb, h):
        z = jnp.zeros((16, 128), U32)
        qh = qt_v[h // 4][qb, (h % 4) * 16:(h % 4 + 1) * 16, :]
        wq = _unpack(jnp.concatenate([qh if jj == h % 4 else z for jj in range(4)], axis=0))
        n = (qb + 1) * 16
        s = jnp.concatenate(
            [_dot(_unpack(k0_v[h // 4, c * n:(c + 1) * n, :]), wq) for c in range(4)], axis=0)
        diag = jnp.where(tri_mask(), s[qb * 128:], NEG)
        return diag if qb == 0 else jnp.concatenate([s[0:128], diag], axis=0)

    def scores_a(m, qb, h):
        qh = qt_v[h // 4][qb, (h % 4) * 16:(h % 4 + 1) * 16, :]
        grp_id = iota((16, 128), 1) // 32
        z = jnp.zeros((16, 128), U32)
        wq = _unpack(jnp.concatenate(
            [jnp.where(grp_id == g, qh, z) for g in range(4)], axis=0))
        base = pl.multiple_of(m * 64 - 80, 16)
        order = [0, 16, 1, 17] + list(range(2, 16))
        cuts = [0, 5, 9, 14, 18]
        if CFG['split'] == 1:
            order = [16, 0, 2, 4, 6, 8, 10, 12, 14, 17, 1, 3, 5, 7, 9, 11, 13, 15]
        if CFG['split'] == 2:
            order = [16, 0, 2, 4, 6, 8, 10, 12, 14, 17, 1, 3, 5, 7, 9, 11, 13, 15]
            cuts = [0, 9, 18]
        units = {}
        for c in range(len(cuts) - 1):
            idx = order[cuts[c]:cuts[c + 1]]
            lhs = jnp.concatenate(
                [k4_v[h // 4][h % 4, pl.ds(base + u * 8, 8), :] for u in idx], axis=0)
            s = _dot(_unpack(lhs), wq)
            for n, u in enumerate(idx):
                units[u] = s[n * 16:(n + 1) * 16]
        for u in range(2):
            new = (iota((16, 128), 1) % 32) >= (iota((16, 128), 0) + u * 16)
            units[u] = jnp.where(new, units[16 + u], units[u])
        return jnp.concatenate([units[u] for u in range(16)], axis=0)

    def deskew(p):
        lane = iota((256, 128), 1)
        p = jnp.where((lane // 32) % 2 == 1,
                      jnp.concatenate([p[224:], p[:224]], axis=0), p)
        return jnp.where(lane >= 64, jnp.concatenate([p[192:], p[:192]], axis=0), p)

    def finish_a(s, m, h):
        skewed = not isinstance(m, int)
        if skewed and CFG['early'] == 2:
            s = deskew(s)
        mx = jnp.max(s, axis=0, keepdims=True)
        if skewed and CFG['early'] == 1:
            s = deskew(s)
        p = jnp.exp2(s - mx)
        l = jnp.sum(p, axis=0, keepdims=True)
        if skewed:
            if not CFG['early']:
                p = deskew(p)
            tri = tri_mask()
            pm = p[0:128]
            p = jnp.concatenate(
                [jnp.where(tri, 0.0, pm), p[128:256], jnp.where(tri, pm, 0.0)], axis=0)
        ntile = p.shape[0] // 128
        a = h % 4
        vv = _unpack(jnp.concatenate(
            [vt_v[h // 4][m - bk, a * 16:(a + 1) * 16, :]
             for bk in range(ntile - 1, -1, -1)], axis=1))
        o = _dot(vv, p.astype(BF))
        return o * pl.reciprocal(l, approx=False)

    class Attn:
        def __init__(self, blk, items):
            self.blk, self.items = blk, items
            self.issued, self.done, self.queue, self.outs = 0, 0, [], {}

        def issue(self, n=1):
            for _ in range(n):
                if self.issued < len(self.items):
                    qb, h = self.items[self.issued]
                    if isinstance(self.blk, int):
                        self.queue.append(scores_first(qb, h))
                    else:
                        self.queue.append(scores_a(self.blk * (TA // 128) + qb, qb, h))
                    self.issued += 1

        def finish(self, n=1):
            for _ in range(n):
                if self.done < self.issued:
                    qb, h = self.items[self.done]
                    o = finish_a(self.queue.pop(0), self.blk * (TA // 128) + qb, h)
                    outs = self.outs.setdefault((qb, h // 4), [])
                    outs.append(o)
                    if len(outs) == 4:
                        ot = jnp.concatenate(outs, axis=0).astype(BF)
                        oa_v[h // 4, qb * 64:(qb + 1) * 64, :] = _pack(ot.T)
                    self.done += 1

    def with_fence(xu, fen):
        r, c = xu.shape
        last = jnp.concatenate([xu[r - 16:, :c - 128], xu[r - 16:, c - 128:] | fen], axis=1)
        return jnp.concatenate([xu[:r - 16], last], axis=0)

    def out_a(r, nrows, c0, c1, y):
        x_v[pl.ds(r, nrows), c0:c1] = (x_v[pl.ds(r, nrows), c0:c1].astype(F32) + y).astype(BF)

    def proj_b(xn, r0, nrows, side):
        for T in range(24):
            w = _unpack(jnp.concatenate(
                [wbt[j, T * 64:(T + 1) * 64, :] for j in range(8)], axis=1))
            y = _dot_nt(xn, w)
            if T < 8:
                qk_v[T, HALO + r0:HALO + r0 + nrows, :] = y * QSCALE
            elif T < 16:
                qk_v[T, HALO + r0:HALO + r0 + nrows, :] = y
            else:
                v_v[T - 16, HALO + r0:HALO + r0 + nrows, :] = y
            release(y, side[T])

    def logit_b(i, zero, r0):
        R = 8

        def run(tok):
            qk_v[0, pl.ds(pl.multiple_of(HALO + TB + zero * 8, 8), 8), :] = tok[0:8]
            accs = [None] * WB
            for t in range(8):
                q = qk_v[t, HALO + r0:HALO + r0 + R, :]
                for w in range(WB):
                    o = HALO + r0 - 2 * w
                    p = q * qk_v[8 + t, o:o + R, :]
                    accs[w] = p if accs[w] is None else accs[w] + p
            ls = []
            for w in range(WB):
                a = accs[w]
                a = a + pltpu.roll(a, 64, 1)
                a = a + pltpu.roll(a, 32, 1)
                if r0 - 2 * w < 0:
                    pos = lax.broadcasted_iota(jnp.int32, (R, 128), 0) + (i * TB + r0 - 2 * w)
                    a = jnp.where(pos >= 0, a, NEG)
                ls.append(a)
            mx = ls[0]
            for w in range(1, WB):
                mx = jnp.maximum(mx, ls[w])
            es = [jnp.exp2(l - mx) for l in ls]
            s = es[0]
            for w in range(1, WB):
                s = s + es[w]
            inv = pl.reciprocal(s, approx=False)
            for w in range(WB):
                e_v[w, r0:r0 + R, :] = es[w] * inv
        return run

    def pv_b(zero, r0):
        R = 8

        def run(tok):
            v_v[0, pl.ds(pl.multiple_of(HALO + TB + zero * 8, 8), 8), :] = tok[0:8]
            es = [e_v[w, r0:r0 + R, :] for w in range(WB)]
            os_ = []
            for t in range(8):
                acc = None
                for w in range(WB):
                    o = HALO + r0 - 2 * w
                    pv = es[w] * v_v[t, o:o + R, :]
                    acc = pv if acc is None else acc + pv
                os_.append(acc)
            ob_v[r0:r0 + R, :] = jnp.concatenate(os_, axis=1).astype(BF)
        return run

    def out_b(i, r0, nrows, side):
        o = ob_v[r0:r0 + nrows, :]
        r = pl.multiple_of(i * TB + r0, 128)
        for c in range(4):
            w = _unpack(jnp.concatenate([wobp[2 * c], wobp[2 * c + 1]], axis=1))
            y = _dot(o, w)
            release(y, side[c])
            cs = slice(c * 256, (c + 1) * 256)
            x_v[pl.ds(r, nrows), cs] = (x_v[pl.ds(r, nrows), cs].astype(F32) + y).astype(BF)

    def spread(chunks, nslots, lo=0, hi=None):
        hi = nslots if hi is None else hi
        out = [[] for _ in range(nslots)]
        for u, c in enumerate(chunks):
            out[lo + u * (hi - lo) // len(chunks)].append(c)
        return out

    cp_x(0).start()
    cp_wa(0).start()
    cp_wa(1).start()
    xn_v[2 * TA:2 * TA + 32, :] = jnp.zeros((32, D), BF)
    wbt[8, 0:16, :] = jnp.zeros((16, 128), U32)
    wobp[8, 0:16, :] = jnp.zeros((16, 128), U32)
    for t in range(8):
        k4_v[t][0, 0:16, :] = jnp.zeros((16, 128), U32)
        vt_v[t][S // 128, 0:16, :] = jnp.zeros((16, 128), U32)
        qt_v[t][2, 0:16, :] = jnp.zeros((16, 128), U32)
    cp_x(0).wait()
    for run in ln_chunks(0, 0, TA, step=TA):
        run(None)

    def one_pass(p, carry):
        first = p == 0
        zero = p // 4

        def a_first():
            for c in range(NCH):
                @pl.when(first)
                def _():
                    cp_wa(c).wait()
                    if c + 2 < NCH:
                        cp_wa(c + 2).start()
                    elif c + 2 == NCH:
                        cp_woa.start()
                    else:
                        cp_x(1).start()
                        cp_wb(0).start()
                        cp_wob(0).start()
                if c + 1 < NCH:
                    proj_a(xn_v[0:TA, :], 0, ch_col[c], CW)
            xn = xn_v[0:TA, :]
            proj_a(xn, 0, ch_col[-1], CW - 256)
            at = Attn(0, [(qb, h) for qb in range(2) for h in range(H)])
            at.issue(6)
            proj_a(xn, 0, 3 * D - 256, 256)
            for n in range(2 * H):
                if n < H - 3 or n >= H:
                    at.issue()
                at.finish()

            @pl.when(first)
            def _():
                cp_woa.wait()
                cp_x(1).wait()
                cp_wb(0).wait()
                cp_wob(0).wait()
                cp_x(2).start()
                cp_wb(1).start()
                cp_wob(1).start()
            side = spread(prep_chunks(zero), 8, 0, 6)
            side2 = spread(ln_chunks(TA + zero * TA, 0, TA), 8, 0, 6)
            ou = jnp.concatenate([oa_v[t] for t in range(8)], axis=1)
            ys = []
            for u in range(8):
                lhs = with_fence(ou, fence(zero)) if u == 7 else ou
                wu = _pack(woa_v[:, u * 128:(u + 1) * 128])
                woap[u] = wu
                ys.append(_dot(_unpack(lhs), _unpack(wu)))
                release(ys[-1], side[u] + side2[u])
                if u % 2 == 1:
                    out_a(0, TA, (u - 1) * 128, (u + 1) * 128, jnp.concatenate(ys[-2:], axis=1))

        if CFG['first']:
            a_first()

        @pl.when(first)
        def _():
            cp_x(2).wait()
            cp_wb(1).wait()
            cp_wob(1).wait()
            cp_x(3).start()
            cp_wb(2).start()
            for j in range(2, 8):
                cp_wob(j).start()

        def a_body(i, c_):
            @pl.when(jnp.logical_and(first, i == 2))
            def _():
                cp_x(3).wait()
                cp_wb(2).wait()
                for j in range(2, 8):
                    cp_wob(j).wait()
            xu = _pack(xn_v[0:TA, :])
            lnc = ln_chunks(((i + 1) % NA) * TA, 0, TA)
            prc = prep_chunks(i)
            mixed = [c for pair in zip(prc, lnc) for c in pair]
            if not CFG['side']:
                mixed = mixed[:1]
            side = spread(mixed, 24, 0, CFG['shi'])
            if CFG['order'] == 0:
                at = Attn(i, [(qb, 4 * t + a) for t in range(8) for a in range(4) for qb in range(2)])
            else:
                at = Attn(i, [(qb, 4 * t + a) for t in range(8) for qb in range(2) for a in range(4)])
            fe = CFG['fence_every']
            yprev = None
            lag = CFG['lag']
            for u in range(24 if CFG['sched'] == 2 else 0):
                t, kind = u // 3, u % 3
                T = (8, 0, 16)[kind] + t
                lhs = with_fence(xu, fence(zero)) if (u >= 3 and u % fe == fe - 1) else xu
                y = None
                for hf in range(2):
                    at.issue(0 if t == 0 else CFG['hpat'][kind * 2 + hf])
                    yh = _dot(_unpack(lhs[:, hf * 512:(hf + 1) * 512]),
                              _unpack(wap[T, hf * 256:(hf + 1) * 256, :]))
                    y = yh if y is None else y + yh
                    if hf == 1:
                        epi_a(y, i, T * 128)
                        if yprev is not None:
                            release(yprev, side[u - 1])
                        yprev = y
                    at.finish(at.issued - at.done - lag)
            for u in range(24 if CFG['sched'] < 2 else 0):
                t, kind = u // 3, u % 3
                n = 0 if t == 0 else CFG['pat'][kind]
                if CFG['sched'] == 1 and u == 23:
                    at.issue(CFG['look'])
                at.issue(n)
                fen = fence(zero) if (u >= 3 and u % fe == fe - 1) else None
                ue = u - CFG['efence']
                if CFG['efence'] and ue >= 0:
                    f2 = (k4_v[ue // 3][0, 0:16, :], qt_v[ue // 3][2 + zero, 0:16, :],
                          vt_v[ue // 3][S // 128, 0:16, :])[ue % 3]
                    fen = f2 if fen is None else fen | f2
                lhs = xu if fen is None else with_fence(xu, fen)
                y = proj_a(_unpack(lhs), i, (D, 0, 2 * D)[kind] + t * 128, 128)
                if yprev is not None:
                    release(yprev, side[u - 1])
                yprev = y
                at.finish(n)
            if CFG['sched'] == 1:
                while at.issued < 2 * H - 6:
                    at.issue()
                    at.finish()
            o1 = _unpack(jnp.concatenate([oa_v[t] for t in range(4)], axis=1))
            part = []
            for u in range(8):
                if CFG['sched'] == 2:
                    at.issue(CFG['hpat'][u] if u < 6 else 0)
                else:
                    at.issue(2)
                part.append(_dot(o1, _unpack(woap[u, 0:D // 4, :])))
                if CFG['sched'] == 2:
                    at.finish(at.issued - at.done - (lag if u < 5 else 0))
                elif u > 0:
                    at.finish(2)
            assert at.done == 2 * H
            o2 = _unpack(jnp.concatenate([oa_v[t] for t in range(4, 8)], axis=1))
            r = pl.multiple_of(i * TA, TA)
            for c in range(4):
                w2 = jnp.concatenate([woap[2 * c, D // 4:, :], woap[2 * c + 1, D // 4:, :]], axis=1)
                y = _dot(o2, _unpack(w2))
                out_a(r, TA, c * 256, (c + 1) * 256,
                      y + jnp.concatenate(part[2 * c:2 * c + 2], axis=1))
            return c_
        if CFG['a']:
            lax.fori_loop(1, NA, a_body, 0)

        for T in range(8):
            qk_v[8 + T, 0:HALO, :] = jnp.zeros((HALO, 128), F32)
            v_v[T, 0:HALO, :] = jnp.zeros((HALO, 128), F32)

        def b_body(i, c_):
            xn = xn_v[0:TA, :]
            ln1 = ln_chunks(i * TB + 256, TA, 256)
            ln2 = ln_chunks(((i + 1) % NB) * TB, 0, TA)
            lg = [logit_b(i, zero, g * 8) for g in range(TB // 8)]
            pv = [pv_b(zero, g * 8) for g in range(TB // 8)]

            def both(a, b):
                return [u + v for u, v in zip(a, b)]
            proj_b(xn, 0, 256, both(spread(ln1 + ln2, 24, 0, 16), spread(lg[0:20], 24, 16, 24)))
            xn1 = xn_v[pl.ds(pl.multiple_of(TA + zero * 32, 32), TA), :]
            proj_b(xn1, 256, 256, both(spread(lg[20:32] + pv[0:32], 24, 0, 16),
                                       spread(lg[32:64], 24, 16, 24)))
            out_b(i, 0, 256, spread(pv[32:58], 4))
            out_b(i, 256, 128, spread(pv[58:64], 4, 0, 2))
            out_b(i, 384, 128, [[]] * 4)
            for T in range(8):
                qk_v[8 + T, 0:HALO, :] = qk_v[8 + T, TB:TB + HALO, :]
                v_v[T, 0:HALO, :] = v_v[T, TB:TB + HALO, :]

            @pl.when(p == 1)
            def _():
                cp_out(i).start()
            return c_
        if CFG['b']:
            lax.fori_loop(0, NB, b_body, 0)
        return carry

    lax.fori_loop(0, 2, one_pass, 0)
    for i in range(NB):
        cp_out(i).wait()


@jax.jit
def pallas_interleave_layers__sliding_block__sliding_local_dilated__prompt_kernel(
    A_x: jax.Array,
    A_wqkv: jax.Array,
    A_wo: jax.Array,
    B_x: jax.Array,
    B_wqkv: jax.Array,
    B_wo: jax.Array,
):
    del B_x
    x = A_x.reshape(S, D)
    any_spec = pl.BlockSpec(memory_space=pl.ANY)
    out = pl.pallas_call(
        _kernel,
        out_shape=jax.ShapeDtypeStruct((S, D), BF),
        in_specs=[any_spec] * 5,
        out_specs=any_spec,
        scratch_shapes=[
            pltpu.VMEM((S + 16, D), BF),
            pltpu.VMEM((D, 3 * D), BF),
            pltpu.VMEM((D, D), BF),
            pltpu.VMEM((D + 16, 3 * D), BF),
            pltpu.VMEM((9, D, 128), BF),
            pltpu.VMEM((24, D // 2, 128), U32),
            pltpu.VMEM((8, D // 2, 128), U32),
            pltpu.VMEM((9, 3 * D // 2, 128), U32),
            pltpu.VMEM((9, D // 2, 128), U32),
            pltpu.VMEM((128 * PITCH, 128), F32),
            pltpu.VMEM((2 * TA + 32, D), BF),
            pltpu.VMEM((8, TA // 2, 128), U32),
            pltpu.VMEM((8, 48, 128), U32),
            pltpu.VMEM((8, TA // 2, 128), U32),
            pltpu.VMEM((16, HALO + TB + 8, 128), F32),
            pltpu.VMEM((8, HALO + TB + 8, 128), F32),
            pltpu.VMEM((WB, TB + 8, 128), F32),
            pltpu.VMEM((TB, D), BF),
            pltpu.SemaphoreType.DMA((4,)),
            pltpu.SemaphoreType.DMA((NCH,)),
            pltpu.SemaphoreType.DMA((1,)),
            pltpu.SemaphoreType.DMA((3,)),
            pltpu.SemaphoreType.DMA((8,)),
            pltpu.SemaphoreType.DMA((NB,)),
        ] + [pltpu.VMEM((4, S // 2, 128), U32)] * 8
          + [pltpu.VMEM((S // 128 + 1, 64, 128), U32)] * 8
          + [pltpu.VMEM((3, 64, 128), U32)] * 8,
        compiler_params=pltpu.CompilerParams(vmem_limit_bytes=100 * 1024 * 1024),
        name="interleave_attn",
    )(x, A_wqkv, A_wo, B_wqkv, B_wo)
    return out.reshape(1, S, D)
```

```python
import math

import jax
import jax.numpy as jnp
from jax import lax
import jax.experimental.pallas as pl
import jax.experimental.pallas.tpu as pltpu

BF = jnp.bfloat16
F32 = jnp.float32
U32 = jnp.uint32

S = 2048
D = 1024
H = 32
DH = 32
TA = 256
NA = S // TA
TB = 512
NB = S // TB
HALO = 16
WB = 8
NEG = -1e30
EPS = 1e-5
QSCALE = (DH ** -0.5) * math.log2(math.e)
NC1 = 4
G1 = 8 // NC1
PITCH = 36
OUT_PIECES = ((0, 256), (256, 128), (384, 128))

CFG = dict(first=1, a=1, b=1, look=3, side=1, fence_every=3, efence=2, shi=21)


def _dot(a, b):
    return jnp.dot(a, b, preferred_element_type=F32)


def _dot_nt(a, b):
    return lax.dot_general(a, b, (((1,), (1,)), ((), ())), preferred_element_type=F32)


def _pack(x_bf16):
    return pltpu.bitcast(x_bf16, U32)


def _unpack(x_u32):
    return pltpu.bitcast(x_u32, BF)


def _iota(shape, dim):
    return lax.broadcasted_iota(jnp.int32, shape, dim)


def _layernorm(x_bf16):
    x = x_bf16.astype(F32)
    m = jnp.sum(x, axis=1, keepdims=True) * (1.0 / D)
    xc = x - m
    v = jnp.sum(xc * xc, axis=1, keepdims=True) * (1.0 / D)
    return (xc * lax.rsqrt(v + EPS)).astype(BF)


def _spread(chunks, nslots, lo=0, hi=None):
    hi = nslots if hi is None else hi
    out = [[] for _ in range(nslots)]
    for u, c in enumerate(chunks):
        out[lo + u * (hi - lo) // len(chunks)].append(c)
    return out


def _both(*lists):
    return [sum(parts, []) for parts in zip(*lists)]


def _kernel(x_hbm, wa_hbm, woa_hbm, wb_hbm, wob_hbm, out_hbm,
            x_v, wa_v, woa_v, wb_v, wob_v, wap, woap, wbt, wobp, tmp, xn_v,
            k0_v, kt_v, k4_v, qt_v, vt_v, oa_v, qk_v, v_v, e_v, ob_v,
            sem_x, sem_wa, sem_woa, sem_wb, sem_wob, sem_out):
    def cp_x(i):
        n = TA if i < 3 else S - 3 * TA
        return pltpu.make_async_copy(x_hbm.at[pl.ds(i * TA, n), :],
                                     x_v.at[pl.ds(i * TA, n), :], sem_x.at[i])

    def cp_wa(c):
        w = G1 * 128
        return [pltpu.make_async_copy(wa_hbm.at[:, pl.ds(part * D + c * w, w)],
                                      wa_v.at[3 * c + part], sem_wa.at[3 * c + part])
                for part in range(3)]

    cp_woa = pltpu.make_async_copy(woa_hbm, woa_v, sem_woa.at[0])

    def cp_wb(j):
        n = 128 if j < 2 else D - 256
        return pltpu.make_async_copy(wb_hbm.at[pl.ds(j * 128, n), :],
                                     wb_v.at[pl.ds(j * 128, n), :], sem_wb.at[j])

    def cp_wob(j):
        return pltpu.make_async_copy(wob_hbm.at[:, pl.ds(j * 128, 128)],
                                     wob_v.at[j], sem_wob.at[j])

    def cp_out(i, k):
        r0, n = OUT_PIECES[k]
        return pltpu.make_async_copy(x_v.at[pl.ds(i * TB + r0, n), :],
                                     out_hbm.at[pl.ds(i * TB + r0, n), :],
                                     sem_out.at[i * len(OUT_PIECES) + k])

    def release(y, chunks):
        n = len(chunks)
        nt = y.shape[1] // 128
        for u, run in enumerate(chunks):
            pos = (u * y.shape[0] * nt // n) // 16 * 16
            t, rr = pos // y.shape[0], pos % y.shape[0]
            run(y[rr:rr + 16, t * 128:(t + 1) * 128])

    def fence_side(zero):
        zx = _pack(xn_v[pl.ds(pl.multiple_of(2 * TA + zero * 32, 32), 32), 0:128])
        return zx | wbt[8, 0:16, :] | wobp[8, 0:16, :]

    def fence_k(zero):
        return k4_v[zero, 0:16, :]

    def fence_q(zero):
        return qt_v[2 + zero, 0:16, :]

    def fence_v(zero):
        return vt_v[S // 128 + zero, 0:16, :]

    def with_fence(xu, fen):
        r, c = xu.shape
        last = jnp.concatenate([xu[r - 16:, :c - 128], xu[r - 16:, c - 128:] | fen], axis=1)
        return jnp.concatenate([xu[:r - 16], last], axis=0)

    def ln_chunks(row0, dst, nrows, step=16):
        def mk(c):
            def run(tok):
                if tok is not None:
                    x_v[S:S + 16, 0:128] = tok.astype(BF)
                r = pl.multiple_of(row0 + c * step, step)
                xn_v[dst + c * step:dst + (c + 1) * step, :] = _layernorm(x_v[pl.ds(r, step), :])
            return run
        return [mk(c) for c in range(nrows // step)]

    def prep_chunks(j):
        def permute(part):
            rows = [tmp[pl.ds(part * H * PITCH + d, H, stride=PITCH), :] for d in range(DH)]
            val = _pack(jnp.concatenate(rows, axis=0).astype(BF))
            if part < 3:
                wbt[j, part * (D // 2):(part + 1) * (D // 2), :] = val
            else:
                wobp[j] = val

        def mk_t(c):
            def run(tok):
                wb_v[D:D + 16, 0:128] = tok.astype(BF)
                rows = pl.ds(pl.multiple_of(j * 128, 128), 128)
                wt = wb_v[rows, c * 256:(c + 1) * 256].T.astype(F32)
                for hh in range(8):
                    o = (c * 8 + hh) * PITCH
                    tmp[o:o + DH, :] = wt[hh * DH:(hh + 1) * DH]
                if c % 4 == 3:
                    permute(c // 4)
            return run

        def mk_o(c):
            def run(tok):
                wob_v[8, 0:16, :] = tok.astype(BF)
                w = wob_v[j, c * 256:(c + 1) * 256, :].astype(F32)
                for hh in range(8):
                    o = (96 + c * 8 + hh) * PITCH
                    tmp[o:o + DH, :] = w[hh * DH:(hh + 1) * DH]
                if c == 3:
                    permute(3)
            return run
        return [mk_t(c) for c in range(12)] + [mk_o(c) for c in range(4)]

    def tri_mask():
        return _iota((128, 128), 1) >= _iota((128, 128), 0)

    def build_k4(full, t, row0):
        n = full.shape[0] - 48
        rolled = [full] + [pltpu.roll(full, 32 * r, 1) for r in range(1, 4)]
        grp_id = _iota((n, 128), 1) // 32
        for a in range(4):
            val = rolled[(0 - a) % 4][0:n]
            for g in range(1, 4):
                val = jnp.where(grp_id == g, rolled[(g - a) % 4][16 * g:16 * g + n], val)
            k4_v[4 * t + a, pl.ds(row0, n), :] = val

    def store_t(y, dst, slot0, t):
        yt = _pack(y.astype(BF).T)
        rows = pl.ds(t * 64 if isinstance(t, int) else pl.multiple_of(t * 64, 64), 64)
        for b in range(TA // 128):
            dst[slot0 + b, rows, :] = yt[:, b * 128:(b + 1) * 128]

    def scores_first(qb, h):
        z = jnp.zeros((16, 128), U32)
        qh = qt_v[qb, h * 16:(h + 1) * 16, :]
        wq = _unpack(jnp.concatenate([qh if jj == h % 4 else z for jj in range(4)], axis=0))
        n = (qb + 1) * 16
        s = jnp.concatenate(
            [_dot(_unpack(k0_v[h // 4, c * n:(c + 1) * n, :]), wq) for c in range(4)], axis=0)
        diag = jnp.where(tri_mask(), s[qb * 128:], NEG)
        return diag if qb == 0 else jnp.concatenate([s[0:128], diag], axis=0)

    def scores_a(m, qb, h):
        qh = qt_v[qb, h * 16:(h + 1) * 16, :]
        grp_id = _iota((16, 128), 1) // 32
        z = jnp.zeros((16, 128), U32)
        wq = _unpack(jnp.concatenate(
            [jnp.where(grp_id == g, qh, z) for g in range(4)], axis=0))
        base = pl.multiple_of(m * 64 - 80, 16)
        order = [0, 16, 1, 17] + list(range(2, 16))
        cuts = [0, 5, 9, 14, 18]
        units = {}
        for c in range(4):
            idx = order[cuts[c]:cuts[c + 1]]
            lhs = jnp.concatenate([k4_v[h, pl.ds(base + u * 8, 8), :] for u in idx], axis=0)
            s = _dot(_unpack(lhs), wq)
            for n, u in enumerate(idx):
                units[u] = s[n * 16:(n + 1) * 16]
        for u in range(2):
            new = (_iota((16, 128), 1) % 32) >= (_iota((16, 128), 0) + u * 16)
            units[u] = jnp.where(new, units[16 + u], units[u])
        return jnp.concatenate([units[u] for u in range(16)], axis=0)

    def finish_a(s, m, h):
        skewed = not isinstance(m, int)
        mx = jnp.max(s, axis=0, keepdims=True)
        if skewed:
            lane = _iota((256, 128), 1)
            s = jnp.where((lane // 32) % 2 == 1,
                          jnp.concatenate([s[224:], s[:224]], axis=0), s)
            s = jnp.where(lane >= 64, jnp.concatenate([s[192:], s[:192]], axis=0), s)
        p = jnp.exp2(s - mx)
        l = jnp.sum(p, axis=0, keepdims=True)
        if skewed:
            tri = tri_mask()
            pm = p[0:128]
            p = jnp.concatenate(
                [jnp.where(tri, 0.0, pm), p[128:256], jnp.where(tri, pm, 0.0)], axis=0)
        ntile = p.shape[0] // 128
        vv = _unpack(jnp.concatenate(
            [vt_v[m - bk, h * 16:(h + 1) * 16, :] for bk in range(ntile - 1, -1, -1)], axis=1))
        o = _dot(vv, p.astype(BF))
        return o * pl.reciprocal(l, approx=False)

    class Attn:
        def __init__(self, blk):
            self.blk = blk
            self.items = [(qb, 4 * t + a) for t in range(8) for qb in range(2) for a in range(4)]
            self.issued, self.done, self.queue, self.outs = 0, 0, [], []

        def issue(self, n=1):
            for _ in range(n):
                if self.issued < len(self.items):
                    qb, h = self.items[self.issued]
                    if isinstance(self.blk, int):
                        self.queue.append(scores_first(qb, h))
                    else:
                        self.queue.append(scores_a(self.blk * (TA // 128) + qb, qb, h))
                    self.issued += 1

        def finish(self, n=1):
            for _ in range(n):
                if self.done < self.issued:
                    qb, h = self.items[self.done]
                    self.outs.append(finish_a(self.queue.pop(0), self.blk * (TA // 128) + qb, h))
                    if len(self.outs) == 4:
                        ot = jnp.concatenate(self.outs, axis=0).astype(BF)
                        oa_v[h // 4, qb * 64:(qb + 1) * 64, :] = _pack(ot.T)
                        self.outs = []
                    self.done += 1

    def add_residual(r, nrows, c0, c1, y):
        x_v[pl.ds(r, nrows), c0:c1] = (x_v[pl.ds(r, nrows), c0:c1].astype(F32) + y).astype(BF)

    def proj_b(xn, r0, nrows, side):
        for T in range(24):
            w = _unpack(jnp.concatenate(
                [wbt[j, T * 64:(T + 1) * 64, :] for j in range(8)], axis=1))
            y = _dot_nt(xn, w)
            if T < 8:
                qk_v[T, HALO + r0:HALO + r0 + nrows, :] = y * QSCALE
            elif T < 16:
                qk_v[T, HALO + r0:HALO + r0 + nrows, :] = y
            else:
                v_v[T - 16, HALO + r0:HALO + r0 + nrows, :] = y
            release(y, side[T])

    def logit_b(i, zero, r0):
        R = 8

        def run(tok):
            qk_v[0, pl.ds(pl.multiple_of(HALO + TB + zero * 8, 8), 8), :] = tok[0:8]
            accs = [None] * WB
            for t in range(8):
                q = qk_v[t, HALO + r0:HALO + r0 + R, :]
                for w in range(WB):
                    o = HALO + r0 - 2 * w
                    p = q * qk_v[8 + t, o:o + R, :]
                    accs[w] = p if accs[w] is None else accs[w] + p
            ls = []
            for w in range(WB):
                a = accs[w]
                a = a + pltpu.roll(a, 64, 1)
                a = a + pltpu.roll(a, 32, 1)
                if r0 - 2 * w < 0:
                    a = jnp.where(_iota((R, 128), 0) + (i * TB + r0 - 2 * w) >= 0, a, NEG)
                ls.append(a)
            mx = ls[0]
            for w in range(1, WB):
                mx = jnp.maximum(mx, ls[w])
            es = [jnp.exp2(l - mx) for l in ls]
            s = es[0]
            for w in range(1, WB):
                s = s + es[w]
            inv = pl.reciprocal(s, approx=False)
            for w in range(WB):
                e_v[w, r0:r0 + R, :] = es[w] * inv
        return run

    def pv_b(zero, r0):
        R = 8

        def run(tok):
            v_v[0, pl.ds(pl.multiple_of(HALO + TB + zero * 8, 8), 8), :] = tok[0:8]
            es = [e_v[w, r0:r0 + R, :] for w in range(WB)]
            os_ = []
            for t in range(8):
                acc = None
                for w in range(WB):
                    o = HALO + r0 - 2 * w
                    pv = es[w] * v_v[t, o:o + R, :]
                    acc = pv if acc is None else acc + pv
                os_.append(acc)
            ob_v[r0:r0 + R, :] = jnp.concatenate(os_, axis=1).astype(BF)
        return run

    def out_b(i, r0, nrows, side):
        o = ob_v[r0:r0 + nrows, :]
        r = pl.multiple_of(i * TB + r0, 128)
        for c in range(4):
            w = _unpack(jnp.concatenate([wobp[2 * c], wobp[2 * c + 1]], axis=1))
            y = _dot(o, w)
            release(y, side[c])
            add_residual(r, nrows, c * 256, (c + 1) * 256, y)

    cp_x(0).start()
    for cp in cp_wa(0):
        cp.start()
    z16 = jnp.zeros((16, 128), U32)
    xn_v[2 * TA:2 * TA + 32, :] = jnp.zeros((32, D), BF)
    wbt[8, 0:16, :] = z16
    wobp[8, 0:16, :] = z16
    k4_v[0, 0:16, :] = z16
    vt_v[S // 128, 0:16, :] = z16
    qt_v[2, 0:16, :] = z16
    cp_x(0).wait()
    for cp in cp_wa(1):
        cp.start()
    for run in ln_chunks(0, 0, TA, step=TA):
        run(None)

    def one_pass(p, carry):
        first = p == 0
        zero = p // 4

        def f_body(c, c_):
            for k in range(NC1):
                @pl.when(jnp.logical_and(first, c == k))
                def _():
                    for cp in cp_wa(k):
                        cp.wait()
                    if k + 2 < NC1:
                        for cp in cp_wa(k + 2):
                            cp.start()
                    elif k + 2 == NC1:
                        cp_woa.start()
                    else:
                        cp_x(1).start()
                        cp_wb(0).start()
                        cp_wob(0).start()
            xn = xn_v[0:TA, :]
            for part in (2, 0, 1):
                wu = _pack(wa_v[3 * c + part])
                y = _dot(xn, _unpack(wu))
                for g in range(G1):
                    t = c * G1 + g
                    wap[part * 8 + t] = wu[:, g * 128:(g + 1) * 128]
                    yt = y[:, g * 128:(g + 1) * 128]
                    if part == 0:
                        store_t(yt * QSCALE, qt_v, 0, t)
                    elif part == 2:
                        store_t(yt, vt_v, 0, t)
                    else:
                        k0_v[t] = _pack(yt.astype(BF))
            return c_

        def a_first():
            lax.fori_loop(0, NC1, f_body, 0)

            @pl.when(first)
            def _():
                cp_woa.wait()
                cp_x(1).wait()
                cp_wb(0).wait()
                cp_wob(0).wait()
                cp_x(2).start()
                cp_wb(1).start()
                cp_wob(1).start()

            def mk_k4(t):
                def run(tok):
                    k0_v[8, 0:8, :] = pltpu.bitcast(tok[0:8], U32)
                    kp = k0_v[t + zero]
                    kt_v[t] = kp[80:128]
                    build_k4(kp, t, 48)
                return run
            side = _both(_spread(prep_chunks(zero), 16, 0, 13),
                         _spread(ln_chunks(TA + zero * TA, 0, TA), 16, 0, 13),
                         _spread([mk_k4(t) for t in range(8)], 16, 0, 13))
            at = Attn(0)
            at.issue(5)
            while at.done < H + 2:
                at.issue()
                at.finish()
            o1 = _unpack(jnp.concatenate([oa_v[t] for t in range(4)], axis=1))
            part = []
            for u in range(8):
                wu = _pack(woa_v[0:D // 2, u * 128:(u + 1) * 128])
                woap[u, 0:D // 4, :] = wu
                part.append(_dot(o1, _unpack(wu)))
                release(part[-1], side[u])
                for _ in range(5):
                    at.issue()
                    at.finish()
            assert at.done == 2 * H
            o2 = jnp.concatenate([oa_v[t] for t in range(4, 8)], axis=1)
            for u in range(8):
                wu = _pack(woa_v[D // 2:, u * 128:(u + 1) * 128])
                woap[u, D // 4:, :] = wu
                lhs = with_fence(o2, fence_side(zero) | fence_k(zero)) if u == 7 else o2
                part[u] = part[u] + _dot(_unpack(lhs), _unpack(wu))
                release(part[u], side[8 + u])
                if u % 2 == 1:
                    add_residual(0, TA, (u - 1) * 128, (u + 1) * 128,
                                 jnp.concatenate(part[u - 1:u + 1], axis=1))

        if CFG['first']:
            a_first()

        @pl.when(first)
        def _():
            cp_x(2).wait()
            cp_wb(1).wait()
            cp_wob(1).wait()
            cp_x(3).start()
            cp_wb(2).start()
            for j in range(2, 8):
                cp_wob(j).start()

        def a_body(i, c_):
            @pl.when(jnp.logical_and(first, i == 2))
            def _():
                cp_x(3).wait()
                cp_wb(2).wait()
                for j in range(2, 8):
                    cp_wob(j).wait()
            xu = _pack(xn_v[0:TA, :])
            lnc = ln_chunks(((i + 1) % NA) * TA, 0, TA)
            mixed = [c for pair in zip(prep_chunks(i), lnc) for c in pair]
            if not CFG['side']:
                mixed = mixed[:1]
            side = _spread(mixed, 24, 0, CFG['shi'])
            at = Attn(i)
            fe = CFG['fence_every']
            yprev = None
            for u in range(24):
                t, kind = u // 3, u % 3
                if u == 23:
                    at.issue(CFG['look'])
                fen = fence_side(zero) if (u >= 3 and u % fe == fe - 1) else None
                if u >= 2:
                    f2 = (fence_k, fence_v, fence_q)[(u - 2) % 3](zero)
                    fen = f2 if fen is None else fen | f2
                lhs = xu if fen is None else with_fence(xu, fen)
                y = _dot(_unpack(lhs), _unpack(wap[(8, 16, 0)[kind] + t]))
                if kind == 0:
                    kp = _pack(y.astype(BF))
                    full = jnp.concatenate([kt_v[t], kp], axis=0)
                    kt_v[t] = kp[80:128]
                    build_k4(full, t, pl.multiple_of(i * (TA // 2), TA // 2))
                elif kind == 1:
                    store_t(y, vt_v, i * (TA // 128), t)
                else:
                    store_t(y * QSCALE, qt_v, 0, t)
                if yprev is not None:
                    release(yprev, side[u - 1])
                yprev = y
            while at.issued < 2 * H - 6:
                at.issue()
                at.finish()
            o1 = _unpack(jnp.concatenate([oa_v[t] for t in range(4)], axis=1))
            part = []
            for u in range(8):
                at.issue(2)
                part.append(_dot(o1, _unpack(woap[u, 0:D // 4, :])))
                if u > 0:
                    at.finish(2)
            assert at.done == 2 * H
            o2 = _unpack(jnp.concatenate([oa_v[t] for t in range(4, 8)], axis=1))
            r = pl.multiple_of(i * TA, TA)
            for c in range(4):
                w2 = jnp.concatenate([woap[2 * c, D // 4:, :], woap[2 * c + 1, D // 4:, :]], axis=1)
                y = _dot(o2, _unpack(w2))
                add_residual(r, TA, c * 256, (c + 1) * 256,
                             y + jnp.concatenate(part[2 * c:2 * c + 2], axis=1))
            return c_
        if CFG['a']:
            lax.fori_loop(1, NA, a_body, 0)

        for T in range(8):
            qk_v[8 + T, 0:HALO, :] = jnp.zeros((HALO, 128), F32)
            v_v[T, 0:HALO, :] = jnp.zeros((HALO, 128), F32)

        def b_body(i, c_):
            def send(k):
                for ii in range(NB):
                    @pl.when(jnp.logical_and(p == 1, i == ii))
                    def _():
                        cp_out(ii, k).start()
            xn = xn_v[0:TA, :]
            ln1 = ln_chunks(i * TB + 256, TA, 256)
            ln2 = ln_chunks(((i + 1) % NB) * TB, 0, TA)
            lg = [logit_b(i, zero, g * 8) for g in range(TB // 8)]
            pv = [pv_b(zero, g * 8) for g in range(TB // 8)]
            proj_b(xn, 0, 256, _both(_spread(ln1 + ln2, 24, 0, 16), _spread(lg[0:20], 24, 16, 24)))
            xn1 = xn_v[pl.ds(pl.multiple_of(TA + zero * 32, 32), TA), :]
            proj_b(xn1, 256, 256, _both(_spread(lg[20:32] + pv[0:32], 24, 0, 16),
                                        _spread(lg[32:64], 24, 16, 24)))
            out_b(i, 0, 256, _spread(pv[32:58], 4))
            send(0)
            out_b(i, 256, 128, _spread(pv[58:64], 4, 0, 2))
            send(1)
            for T in range(8):
                qk_v[8 + T, 0:HALO, :] = qk_v[8 + T, TB:TB + HALO, :]
                v_v[T, 0:HALO, :] = v_v[T, TB:TB + HALO, :]
            out_b(i, 384, 128, [[]] * 4)
            send(2)
            return c_
        if CFG['b']:
            lax.fori_loop(0, NB, b_body, 0)
        return carry

    lax.fori_loop(0, 2, one_pass, 0)
    for i in range(NB):
        for k in range(len(OUT_PIECES)):
            cp_out(i, k).wait()


@jax.jit
def pallas_interleave_layers__sliding_block__sliding_local_dilated__prompt_kernel(
    A_x: jax.Array,
    A_wqkv: jax.Array,
    A_wo: jax.Array,
    B_x: jax.Array,
    B_wqkv: jax.Array,
    B_wo: jax.Array,
):
    del B_x
    x = A_x.reshape(S, D)
    any_spec = pl.BlockSpec(memory_space=pl.ANY)
    out = pl.pallas_call(
        _kernel,
        out_shape=jax.ShapeDtypeStruct((S, D), BF),
        in_specs=[any_spec] * 5,
        out_specs=any_spec,
        scratch_shapes=[
            pltpu.VMEM((S + 16, D), BF),
            pltpu.VMEM((3 * NC1, D, G1 * 128), BF),
            pltpu.VMEM((D, D), BF),
            pltpu.VMEM((D + 16, 3 * D), BF),
            pltpu.VMEM((9, D, 128), BF),
            pltpu.VMEM((24, D // 2, 128), U32),
            pltpu.VMEM((8, D // 2, 128), U32),
            pltpu.VMEM((9, 3 * D // 2, 128), U32),
            pltpu.VMEM((9, D // 2, 128), U32),
            pltpu.VMEM((128 * PITCH, 128), F32),
            pltpu.VMEM((2 * TA + 32, D), BF),
            pltpu.VMEM((9, TA // 2, 128), U32),
            pltpu.VMEM((8, 48, 128), U32),
            pltpu.VMEM((H, S // 2, 128), U32),
            pltpu.VMEM((3, D // 2, 128), U32),
            pltpu.VMEM((S // 128 + 1, D // 2, 128), U32),
            pltpu.VMEM((8, TA // 2, 128), U32),
            pltpu.VMEM((16, HALO + TB + 8, 128), F32),
            pltpu.VMEM((8, HALO + TB + 8, 128), F32),
            pltpu.VMEM((WB, TB, 128), F32),
            pltpu.VMEM((TB, D), BF),
            pltpu.SemaphoreType.DMA((4,)),
            pltpu.SemaphoreType.DMA((3 * NC1,)),
            pltpu.SemaphoreType.DMA((1,)),
            pltpu.SemaphoreType.DMA((3,)),
            pltpu.SemaphoreType.DMA((8,)),
            pltpu.SemaphoreType.DMA((NB * len(OUT_PIECES),)),
        ],
        compiler_params=pltpu.CompilerParams(vmem_limit_bytes=100 * 1024 * 1024),
        name="interleave_attn",
    )(x, A_wqkv, A_wo, B_wqkv, B_wo)
    return out.reshape(1, S, D)
```

```python
import math

import jax
import jax.numpy as jnp
from jax import lax
import jax.experimental.pallas as pl
import jax.experimental.pallas.tpu as pltpu

BF = jnp.bfloat16
F32 = jnp.float32
U32 = jnp.uint32

S = 2048
D = 1024
H = 32
DH = 32
TA = 256
NA = S // TA
TB = 512
NB = S // TB
HALO = 16
WB = 8
NEG = -1e30
EPS = 1e-5
QSCALE = (DH ** -0.5) * math.log2(math.e)
NC1 = 4
G1 = 8 // NC1
PITCH = 36
OUT_PIECES = ((0, 256), (256, 128), (384, 128))

CFG = dict(first=1, a=1, b=1, look=3, side=1, fence_every=3, efence=2, shi=21, flook=5, k4early=0, fhi=13, ffence=16)


def _dot(a, b):
    return jnp.dot(a, b, preferred_element_type=F32)


def _dot_nt(a, b):
    return lax.dot_general(a, b, (((1,), (1,)), ((), ())), preferred_element_type=F32)


def _pack(x_bf16):
    return pltpu.bitcast(x_bf16, U32)


def _unpack(x_u32):
    return pltpu.bitcast(x_u32, BF)


def _iota(shape, dim):
    return lax.broadcasted_iota(jnp.int32, shape, dim)


def _layernorm(x_bf16):
    x = x_bf16.astype(F32)
    m = jnp.sum(x, axis=1, keepdims=True) * (1.0 / D)
    xc = x - m
    v = jnp.sum(xc * xc, axis=1, keepdims=True) * (1.0 / D)
    return (xc * lax.rsqrt(v + EPS)).astype(BF)


def _spread(chunks, nslots, lo=0, hi=None):
    hi = nslots if hi is None else hi
    out = [[] for _ in range(nslots)]
    for u, c in enumerate(chunks):
        out[lo + u * (hi - lo) // len(chunks)].append(c)
    return out


def _both(*lists):
    return [sum(parts, []) for parts in zip(*lists)]


def _kernel(x_hbm, wa_hbm, woa_hbm, wb_hbm, wob_hbm, out_hbm,
            x_v, wa_v, woa_v, wb_v, wob_v, wap, woap, wbt, wobp, tmp, xn_v,
            k0_v, kt_v, k4_v, qt_v, vt_v, oa_v, qk_v, v_v, e_v, ob_v,
            sem_x, sem_wa, sem_woa, sem_wb, sem_wob, sem_out):
    def cp_x(i):
        n = TA if i < 3 else S - 3 * TA
        return pltpu.make_async_copy(x_hbm.at[pl.ds(i * TA, n), :],
                                     x_v.at[pl.ds(i * TA, n), :], sem_x.at[i])

    def cp_wa(c):
        w = G1 * 128
        return [pltpu.make_async_copy(wa_hbm.at[:, pl.ds(part * D + c * w, w)],
                                      wa_v.at[3 * c + part], sem_wa.at[3 * c + part])
                for part in range(3)]

    cp_woa = pltpu.make_async_copy(woa_hbm, woa_v, sem_woa.at[0])

    def cp_wb(j):
        n = 128 if j < 2 else D - 256
        return pltpu.make_async_copy(wb_hbm.at[pl.ds(j * 128, n), :],
                                     wb_v.at[pl.ds(j * 128, n), :], sem_wb.at[j])

    def cp_wob(j):
        return pltpu.make_async_copy(wob_hbm.at[:, pl.ds(j * 128, 128)],
                                     wob_v.at[j], sem_wob.at[j])

    def cp_out(i, k):
        r0, n = OUT_PIECES[k]
        return pltpu.make_async_copy(x_v.at[pl.ds(i * TB + r0, n), :],
                                     out_hbm.at[pl.ds(i * TB + r0, n), :],
                                     sem_out.at[i * len(OUT_PIECES) + k])

    def release(y, chunks):
        n = len(chunks)
        nt = y.shape[1] // 128
        for u, run in enumerate(chunks):
            pos = (u * y.shape[0] * nt // n) // 16 * 16
            t, rr = pos // y.shape[0], pos % y.shape[0]
            run(y[rr:rr + 16, t * 128:(t + 1) * 128])

    def fence_side(zero):
        zx = _pack(xn_v[pl.ds(pl.multiple_of(2 * TA + zero * 32, 32), 32), 0:128])
        return zx | wbt[8, 0:16, :] | wobp[8, 0:16, :]

    def fence_k(zero):
        return k4_v[zero, 0:16, :]

    def fence_q(zero):
        return qt_v[2 + zero, 0:16, :]

    def fence_v(zero):
        return vt_v[S // 128 + zero, 0:16, :]

    def with_fence(xu, fen):
        r, c = xu.shape
        last = jnp.concatenate([xu[r - 16:, :c - 128], xu[r - 16:, c - 128:] | fen], axis=1)
        return jnp.concatenate([xu[:r - 16], last], axis=0)

    def ln_chunks(row0, dst, nrows, step=16):
        def mk(c):
            def run(tok):
                if tok is not None:
                    x_v[S:S + 16, 0:128] = tok.astype(BF)
                r = pl.multiple_of(row0 + c * step, step)
                xn_v[dst + c * step:dst + (c + 1) * step, :] = _layernorm(x_v[pl.ds(r, step), :])
            return run
        return [mk(c) for c in range(nrows // step)]

    def prep_chunks(j):
        def permute(part):
            rows = [tmp[pl.ds(part * H * PITCH + d, H, stride=PITCH), :] for d in range(DH)]
            val = _pack(jnp.concatenate(rows, axis=0).astype(BF))
            if part < 3:
                wbt[j, part * (D // 2):(part + 1) * (D // 2), :] = val
            else:
                wobp[j] = val

        def mk_t(c):
            def run(tok):
                wb_v[D:D + 16, 0:128] = tok.astype(BF)
                rows = pl.ds(pl.multiple_of(j * 128, 128), 128)
                wt = wb_v[rows, c * 256:(c + 1) * 256].T.astype(F32)
                for hh in range(8):
                    o = (c * 8 + hh) * PITCH
                    tmp[o:o + DH, :] = wt[hh * DH:(hh + 1) * DH]
                if c % 4 == 3:
                    permute(c // 4)
            return run

        def mk_o(c):
            def run(tok):
                wob_v[8, 0:16, :] = tok.astype(BF)
                w = wob_v[j, c * 256:(c + 1) * 256, :].astype(F32)
                for hh in range(8):
                    o = (96 + c * 8 + hh) * PITCH
                    tmp[o:o + DH, :] = w[hh * DH:(hh + 1) * DH]
                if c == 3:
                    permute(3)
            return run
        return [mk_t(c) for c in range(12)] + [mk_o(c) for c in range(4)]

    def tri_mask():
        return _iota((128, 128), 1) >= _iota((128, 128), 0)

    def build_k4(full, t, row0):
        n = full.shape[0] - 48
        rolled = [full] + [pltpu.roll(full, 32 * r, 1) for r in range(1, 4)]
        grp_id = _iota((n, 128), 1) // 32
        for a in range(4):
            val = rolled[(0 - a) % 4][0:n]
            for g in range(1, 4):
                val = jnp.where(grp_id == g, rolled[(g - a) % 4][16 * g:16 * g + n], val)
            k4_v[4 * t + a, pl.ds(row0, n), :] = val

    def store_t(y, dst, slot0, t):
        yt = _pack(y.astype(BF).T)
        rows = pl.ds(t * 64 if isinstance(t, int) else pl.multiple_of(t * 64, 64), 64)
        for b in range(TA // 128):
            dst[slot0 + b, rows, :] = yt[:, b * 128:(b + 1) * 128]

    def scores_first(qb, h):
        z = jnp.zeros((16, 128), U32)
        qh = qt_v[qb, h * 16:(h + 1) * 16, :]
        wq = _unpack(jnp.concatenate([qh if jj == h % 4 else z for jj in range(4)], axis=0))
        n = (qb + 1) * 16
        s = jnp.concatenate(
            [_dot(_unpack(k0_v[h // 4, c * n:(c + 1) * n, :]), wq) for c in range(4)], axis=0)
        diag = jnp.where(tri_mask(), s[qb * 128:], NEG)
        return diag if qb == 0 else jnp.concatenate([s[0:128], diag], axis=0)

    def scores_a(m, qb, h):
        qh = qt_v[qb, h * 16:(h + 1) * 16, :]
        grp_id = _iota((16, 128), 1) // 32
        z = jnp.zeros((16, 128), U32)
        wq = _unpack(jnp.concatenate(
            [jnp.where(grp_id == g, qh, z) for g in range(4)], axis=0))
        base = pl.multiple_of(m * 64 - 80, 16)
        order = [0, 16, 1, 17] + list(range(2, 16))
        cuts = [0, 5, 9, 14, 18]
        units = {}
        for c in range(4):
            idx = order[cuts[c]:cuts[c + 1]]
            lhs = jnp.concatenate([k4_v[h, pl.ds(base + u * 8, 8), :] for u in idx], axis=0)
            s = _dot(_unpack(lhs), wq)
            for n, u in enumerate(idx):
                units[u] = s[n * 16:(n + 1) * 16]
        for u in range(2):
            new = (_iota((16, 128), 1) % 32) >= (_iota((16, 128), 0) + u * 16)
            units[u] = jnp.where(new, units[16 + u], units[u])
        return jnp.concatenate([units[u] for u in range(16)], axis=0)

    def finish_a(s, m, h):
        skewed = not isinstance(m, int)
        mx = jnp.max(s, axis=0, keepdims=True)
        if skewed:
            lane = _iota((256, 128), 1)
            s = jnp.where((lane // 32) % 2 == 1,
                          jnp.concatenate([s[224:], s[:224]], axis=0), s)
            s = jnp.where(lane >= 64, jnp.concatenate([s[192:], s[:192]], axis=0), s)
        p = jnp.exp2(s - mx)
        l = jnp.sum(p, axis=0, keepdims=True)
        if skewed:
            tri = tri_mask()
            pm = p[0:128]
            p = jnp.concatenate(
                [jnp.where(tri, 0.0, pm), p[128:256], jnp.where(tri, pm, 0.0)], axis=0)
        ntile = p.shape[0] // 128
        vv = _unpack(jnp.concatenate(
            [vt_v[m - bk, h * 16:(h + 1) * 16, :] for bk in range(ntile - 1, -1, -1)], axis=1))
        o = _dot(vv, p.astype(BF))
        return o * pl.reciprocal(l, approx=False)

    class Attn:
        def __init__(self, blk):
            self.blk = blk
            self.items = [(qb, 4 * t + a) for t in range(8) for qb in range(2) for a in range(4)]
            self.issued, self.done, self.queue, self.outs = 0, 0, [], []

        def issue(self, n=1):
            for _ in range(n):
                if self.issued < len(self.items):
                    qb, h = self.items[self.issued]
                    if isinstance(self.blk, int):
                        self.queue.append(scores_first(qb, h))
                    else:
                        self.queue.append(scores_a(self.blk * (TA // 128) + qb, qb, h))
                    self.issued += 1

        def finish(self, n=1):
            for _ in range(n):
                if self.done < self.issued:
                    qb, h = self.items[self.done]
                    self.outs.append(finish_a(self.queue.pop(0), self.blk * (TA // 128) + qb, h))
                    if len(self.outs) == 4:
                        ot = jnp.concatenate(self.outs, axis=0).astype(BF)
                        oa_v[h // 4, qb * 64:(qb + 1) * 64, :] = _pack(ot.T)
                        self.last, self.outs = self.outs[-1], []
                    self.done += 1

    def add_residual(r, nrows, c0, c1, y):
        x_v[pl.ds(r, nrows), c0:c1] = (x_v[pl.ds(r, nrows), c0:c1].astype(F32) + y).astype(BF)

    def proj_b(xn, r0, nrows, side):
        for T in range(24):
            w = _unpack(jnp.concatenate(
                [wbt[j, T * 64:(T + 1) * 64, :] for j in range(8)], axis=1))
            y = _dot_nt(xn, w)
            if T < 8:
                qk_v[T, HALO + r0:HALO + r0 + nrows, :] = y * QSCALE
            elif T < 16:
                qk_v[T, HALO + r0:HALO + r0 + nrows, :] = y
            else:
                v_v[T - 16, HALO + r0:HALO + r0 + nrows, :] = y
            release(y, side[T])

    def logit_b(i, zero, r0):
        R = 8

        def run(tok):
            qk_v[0, pl.ds(pl.multiple_of(HALO + TB + zero * 8, 8), 8), :] = tok[0:8]
            accs = [None] * WB
            for t in range(8):
                q = qk_v[t, HALO + r0:HALO + r0 + R, :]
                for w in range(WB):
                    o = HALO + r0 - 2 * w
                    p = q * qk_v[8 + t, o:o + R, :]
                    accs[w] = p if accs[w] is None else accs[w] + p
            ls = []
            for w in range(WB):
                a = accs[w]
                a = a + pltpu.roll(a, 64, 1)
                a = a + pltpu.roll(a, 32, 1)
                if r0 - 2 * w < 0:
                    a = jnp.where(_iota((R, 128), 0) + (i * TB + r0 - 2 * w) >= 0, a, NEG)
                ls.append(a)
            mx = ls[0]
            for w in range(1, WB):
                mx = jnp.maximum(mx, ls[w])
            es = [jnp.exp2(l - mx) for l in ls]
            s = es[0]
            for w in range(1, WB):
                s = s + es[w]
            inv = pl.reciprocal(s, approx=False)
            for w in range(WB):
                e_v[w, r0:r0 + R, :] = es[w] * inv
        return run

    def pv_b(zero, r0):
        R = 8

        def run(tok):
            v_v[0, pl.ds(pl.multiple_of(HALO + TB + zero * 8, 8), 8), :] = tok[0:8]
            es = [e_v[w, r0:r0 + R, :] for w in range(WB)]
            os_ = []
            for t in range(8):
                acc = None
                for w in range(WB):
                    o = HALO + r0 - 2 * w
                    pv = es[w] * v_v[t, o:o + R, :]
                    acc = pv if acc is None else acc + pv
                os_.append(acc)
            ob_v[r0:r0 + R, :] = jnp.concatenate(os_, axis=1).astype(BF)
        return run

    def out_b(i, r0, nrows, side):
        o = ob_v[r0:r0 + nrows, :]
        r = pl.multiple_of(i * TB + r0, 128)
        for c in range(4):
            w = _unpack(jnp.concatenate([wobp[2 * c], wobp[2 * c + 1]], axis=1))
            y = _dot(o, w)
            release(y, side[c])
            add_residual(r, nrows, c * 256, (c + 1) * 256, y)

    cp_x(0).start()
    for cp in cp_wa(0):
        cp.start()
    z16 = jnp.zeros((16, 128), U32)
    xn_v[2 * TA:2 * TA + 32, :] = jnp.zeros((32, D), BF)
    wbt[8, 0:16, :] = z16
    wobp[8, 0:16, :] = z16
    k4_v[0, 0:16, :] = z16
    vt_v[S // 128, 0:16, :] = z16
    qt_v[2, 0:16, :] = z16
    cp_x(0).wait()
    for cp in cp_wa(1):
        cp.start()
    for run in ln_chunks(0, 0, TA, step=TA):
        run(None)

    def one_pass(p, carry):
        first = p == 0
        zero = p // 4

        def f_body(c, c_):
            for k in range(NC1):
                @pl.when(jnp.logical_and(first, c == k))
                def _():
                    for cp in cp_wa(k):
                        cp.wait()
                    if k + 2 < NC1:
                        for cp in cp_wa(k + 2):
                            cp.start()
                    elif k + 2 == NC1:
                        cp_woa.start()
                    else:
                        cp_x(1).start()
                        cp_wb(0).start()
                        cp_wob(0).start()
            xn = xn_v[0:TA, :]
            for part in (2, 0, 1):
                wu = _pack(wa_v[3 * c + part])
                y = _dot(xn, _unpack(wu))
                for g in range(G1):
                    t = c * G1 + g
                    wap[part * 8 + t] = wu[:, g * 128:(g + 1) * 128]
                    yt = y[:, g * 128:(g + 1) * 128]
                    if part == 0:
                        store_t(yt * QSCALE, qt_v, 0, t)
                    elif part == 2:
                        store_t(yt, vt_v, 0, t)
                    else:
                        k0_v[t] = _pack(yt.astype(BF))
            return c_

        def a_first():
            lax.fori_loop(0, NC1, f_body, 0)

            def mk_k4(t):
                def run(tok):
                    k0_v[8, 0:8, :] = pltpu.bitcast(tok[0:8], U32)
                    kp = k0_v[t + zero]
                    kt_v[t] = kp[80:128]
                    build_k4(kp, t, 48)
                return run
            k4c = [mk_k4(t) for t in range(8)]
            at = Attn(0)
            at.issue(CFG['flook'])
            while at.issued < 2 * H:
                at.issue()
                at.finish()
                if CFG['k4early'] and at.done % 7 == 1 and k4c:
                    k4c.pop(0)(at.outs[-1][0:16] if at.outs else at.last[0:16])

            @pl.when(first)
            def _():
                cp_woa.wait()
                cp_x(1).wait()
                cp_wb(0).wait()
                cp_wob(0).wait()
                cp_x(2).start()
                cp_wb(1).start()
                cp_wob(1).start()
            hi = CFG['fhi']
            side = _both(_spread(prep_chunks(zero), 16, 0, hi),
                         _spread(ln_chunks(TA + zero * TA, 0, TA), 16, 0, hi))
            if k4c:
                side = _both(side, _spread(k4c, 16, 0, hi))
            o1 = jnp.concatenate([oa_v[t] for t in range(4)], axis=1)
            part = []
            yprev = None
            for u in range(16):
                if u == 8:
                    o1 = jnp.concatenate([oa_v[t] for t in range(4, 8)], axis=1)
                rows = slice((u // 8) * (D // 2), (u // 8 + 1) * (D // 2))
                wu = _pack(woa_v[rows, (u % 8) * 128:(u % 8 + 1) * 128])
                woap[u % 8, (u // 8) * (D // 4):(u // 8 + 1) * (D // 4), :] = wu
                ff = CFG['ffence']
                lhs = with_fence(o1, fence_side(zero) | fence_k(zero)) if (u % ff == ff - 1) else o1
                y = _dot(_unpack(lhs), _unpack(wu))
                if u == 0:
                    at.finish(2 * H)
                if yprev is not None:
                    release(yprev, side[u - 1])
                yprev = y
                if u < 8:
                    part.append(y)
                else:
                    part[u - 8] = part[u - 8] + y
                    if u % 2 == 1:
                        add_residual(0, TA, (u - 9) * 128, (u - 7) * 128,
                                     jnp.concatenate(part[u - 9:u - 7], axis=1))

        if CFG['first']:
            a_first()

        @pl.when(first)
        def _():
            cp_x(2).wait()
            cp_wb(1).wait()
            cp_wob(1).wait()
            cp_x(3).start()
            cp_wb(2).start()
            for j in range(2, 8):
                cp_wob(j).start()

        def a_body(i, c_):
            @pl.when(jnp.logical_and(first, i == 2))
            def _():
                cp_x(3).wait()
                cp_wb(2).wait()
                for j in range(2, 8):
                    cp_wob(j).wait()
            xu = _pack(xn_v[0:TA, :])
            lnc = ln_chunks(((i + 1) % NA) * TA, 0, TA)
            mixed = [c for pair in zip(prep_chunks(i), lnc) for c in pair]
            if not CFG['side']:
                mixed = mixed[:1]
            side = _spread(mixed, 24, 0, CFG['shi'])
            at = Attn(i)
            fe = CFG['fence_every']
            yprev = None
            for u in range(24):
                t, kind = u // 3, u % 3
                if u == 23:
                    at.issue(CFG['look'])
                fen = fence_side(zero) if (u >= 3 and u % fe == fe - 1) else None
                if u >= 2:
                    f2 = (fence_k, fence_v, fence_q)[(u - 2) % 3](zero)
                    fen = f2 if fen is None else fen | f2
                lhs = xu if fen is None else with_fence(xu, fen)
                y = _dot(_unpack(lhs), _unpack(wap[(8, 16, 0)[kind] + t]))
                if kind == 0:
                    kp = _pack(y.astype(BF))
                    full = jnp.concatenate([kt_v[t], kp], axis=0)
                    kt_v[t] = kp[80:128]
                    build_k4(full, t, pl.multiple_of(i * (TA // 2), TA // 2))
                elif kind == 1:
                    store_t(y, vt_v, i * (TA // 128), t)
                else:
                    store_t(y * QSCALE, qt_v, 0, t)
                if yprev is not None:
                    release(yprev, side[u - 1])
                yprev = y
            while at.issued < 2 * H - 6:
                at.issue()
                at.finish()
            o1 = _unpack(jnp.concatenate([oa_v[t] for t in range(4)], axis=1))
            part = []
            for u in range(8):
                at.issue(2)
                part.append(_dot(o1, _unpack(woap[u, 0:D // 4, :])))
                if u > 0:
                    at.finish(2)
            assert at.done == 2 * H
            o2 = _unpack(jnp.concatenate([oa_v[t] for t in range(4, 8)], axis=1))
            r = pl.multiple_of(i * TA, TA)
            for c in range(4):
                w2 = jnp.concatenate([woap[2 * c, D // 4:, :], woap[2 * c + 1, D // 4:, :]], axis=1)
                y = _dot(o2, _unpack(w2))
                add_residual(r, TA, c * 256, (c + 1) * 256,
                             y + jnp.concatenate(part[2 * c:2 * c + 2], axis=1))
            return c_
        if CFG['a']:
            lax.fori_loop(1, NA, a_body, 0)

        for T in range(8):
            qk_v[8 + T, 0:HALO, :] = jnp.zeros((HALO, 128), F32)
            v_v[T, 0:HALO, :] = jnp.zeros((HALO, 128), F32)

        def b_body(i, c_):
            def send(k):
                for ii in range(NB):
                    @pl.when(jnp.logical_and(p == 1, i == ii))
                    def _():
                        cp_out(ii, k).start()
            xn = xn_v[0:TA, :]
            ln1 = ln_chunks(i * TB + 256, TA, 256)
            ln2 = ln_chunks(((i + 1) % NB) * TB, 0, TA)
            lg = [logit_b(i, zero, g * 8) for g in range(TB // 8)]
            pv = [pv_b(zero, g * 8) for g in range(TB // 8)]
            proj_b(xn, 0, 256, _both(_spread(ln1 + ln2, 24, 0, 16), _spread(lg[0:20], 24, 16, 24)))
            xn1 = xn_v[pl.ds(pl.multiple_of(TA + zero * 32, 32), TA), :]
            proj_b(xn1, 256, 256, _both(_spread(lg[20:32] + pv[0:32], 24, 0, 16),
                                        _spread(lg[32:64], 24, 16, 24)))
            out_b(i, 0, 256, _spread(pv[32:58], 4))
            send(0)
            out_b(i, 256, 128, _spread(pv[58:64], 4, 0, 2))
            send(1)
            for T in range(8):
                qk_v[8 + T, 0:HALO, :] = qk_v[8 + T, TB:TB + HALO, :]
                v_v[T, 0:HALO, :] = v_v[T, TB:TB + HALO, :]
            out_b(i, 384, 128, [[]] * 4)
            send(2)
            return c_
        if CFG['b']:
            lax.fori_loop(0, NB, b_body, 0)
        return carry

    lax.fori_loop(0, 2, one_pass, 0)
    for i in range(NB):
        for k in range(len(OUT_PIECES)):
            cp_out(i, k).wait()


@jax.jit
def pallas_interleave_layers__sliding_block__sliding_local_dilated__prompt_kernel(
    A_x: jax.Array,
    A_wqkv: jax.Array,
    A_wo: jax.Array,
    B_x: jax.Array,
    B_wqkv: jax.Array,
    B_wo: jax.Array,
):
    del B_x
    x = A_x.reshape(S, D)
    any_spec = pl.BlockSpec(memory_space=pl.ANY)
    out = pl.pallas_call(
        _kernel,
        out_shape=jax.ShapeDtypeStruct((S, D), BF),
        in_specs=[any_spec] * 5,
        out_specs=any_spec,
        scratch_shapes=[
            pltpu.VMEM((S + 16, D), BF),
            pltpu.VMEM((3 * NC1, D, G1 * 128), BF),
            pltpu.VMEM((D, D), BF),
            pltpu.VMEM((D + 16, 3 * D), BF),
            pltpu.VMEM((9, D, 128), BF),
            pltpu.VMEM((24, D // 2, 128), U32),
            pltpu.VMEM((8, D // 2, 128), U32),
            pltpu.VMEM((9, 3 * D // 2, 128), U32),
            pltpu.VMEM((9, D // 2, 128), U32),
            pltpu.VMEM((128 * PITCH, 128), F32),
            pltpu.VMEM((2 * TA + 32, D), BF),
            pltpu.VMEM((9, TA // 2, 128), U32),
            pltpu.VMEM((8, 48, 128), U32),
            pltpu.VMEM((H, S // 2, 128), U32),
            pltpu.VMEM((3, D // 2, 128), U32),
            pltpu.VMEM((S // 128 + 1, D // 2, 128), U32),
            pltpu.VMEM((8, TA // 2, 128), U32),
            pltpu.VMEM((16, HALO + TB + 8, 128), F32),
            pltpu.VMEM((8, HALO + TB + 8, 128), F32),
            pltpu.VMEM((WB, TB, 128), F32),
            pltpu.VMEM((TB, D), BF),
            pltpu.SemaphoreType.DMA((4,)),
            pltpu.SemaphoreType.DMA((3 * NC1,)),
            pltpu.SemaphoreType.DMA((1,)),
            pltpu.SemaphoreType.DMA((3,)),
            pltpu.SemaphoreType.DMA((8,)),
            pltpu.SemaphoreType.DMA((NB * len(OUT_PIECES),)),
        ],
        compiler_params=pltpu.CompilerParams(vmem_limit_bytes=100 * 1024 * 1024),
        name="interleave_attn",
    )(x, A_wqkv, A_wo, B_wqkv, B_wo)
    return out.reshape(1, S, D)
```

```python
import math

import jax
import jax.numpy as jnp
from jax import lax
import jax.experimental.pallas as pl
import jax.experimental.pallas.tpu as pltpu

BF = jnp.bfloat16
F32 = jnp.float32
U32 = jnp.uint32

S = 2048
D = 1024
H = 32
DH = 32
TA = 256
NA = S // TA
TB = 512
NB = S // TB
HALO = 16
WB = 8
NEG = -1e30
EPS = 1e-5
QSCALE = (DH ** -0.5) * math.log2(math.e)
NC1 = 4
G1 = 8 // NC1
PITCH = 36
OUT_PIECES = ((0, 256), (256, 128), (384, 128))

CFG = dict(first=1, a=1, b=1, look=3, side=1, fence_every=3, efence=2, shi=21, flook=5, k4early=0, fhi=13, ffence=16,
           bn=(16, 56, 56), bf=(), bln=32, bmix=1, bhi=10, pvtok=2, lgtok=2, newton=1, qf32=1, lsum=2, opq=0)


def _dot(a, b):
    return jnp.dot(a, b, preferred_element_type=F32)


def _dot_nt(a, b):
    return lax.dot_general(a, b, (((1,), (1,)), ((), ())), preferred_element_type=F32)


def _pack(x_bf16):
    return pltpu.bitcast(x_bf16, U32)


def _unpack(x_u32):
    return pltpu.bitcast(x_u32, BF)


def _iota(shape, dim):
    return lax.broadcasted_iota(jnp.int32, shape, dim)


def _layernorm(x_bf16):
    x = x_bf16.astype(F32)
    m = jnp.sum(x, axis=1, keepdims=True) * (1.0 / D)
    xc = x - m
    v = jnp.sum(xc * xc, axis=1, keepdims=True) * (1.0 / D)
    return (xc * lax.rsqrt(v + EPS)).astype(BF)


def _recip(l):
    if not CFG['newton']:
        return pl.reciprocal(l, approx=False)
    r = pl.reciprocal(l, approx=True)
    return r * (2.0 - l * r)


def _spread(chunks, nslots, lo=0, hi=None):
    hi = nslots if hi is None else hi
    out = [[] for _ in range(nslots)]
    for u, c in enumerate(chunks):
        out[lo + u * (hi - lo) // len(chunks)].append(c)
    return out


def _merge(a, b):
    out = []
    for u in range(max(len(a), len(b))):
        out += a[u:u + 1] + b[u:u + 1]
    return out


def _both(*lists):
    return [sum(parts, []) for parts in zip(*lists)]


def _kernel(x_hbm, wa_hbm, woa_hbm, wb_hbm, wob_hbm, out_hbm,
            x_v, wa_v, woa_v, wb_v, wob_v, wap, woap, wbt, wobp, tmp, xn_v,
            k0_v, kt_v, k4_v, qt_v, vt_v, oa0_v, oa1_v, qk_v, v_v, e_v, ob_v, tk_v,
            sem_x, sem_wa, sem_woa, sem_wb, sem_wob, sem_out):
    def cp_x(i):
        n = TA if i < 3 else S - 3 * TA
        return pltpu.make_async_copy(x_hbm.at[pl.ds(i * TA, n), :],
                                     x_v.at[pl.ds(i * TA, n), :], sem_x.at[i])

    def cp_wa(c):
        w = G1 * 128
        return [pltpu.make_async_copy(wa_hbm.at[:, pl.ds(part * D + c * w, w)],
                                      wa_v.at[3 * c + part], sem_wa.at[3 * c + part])
                for part in range(3)]

    cp_woa = pltpu.make_async_copy(woa_hbm, woa_v, sem_woa.at[0])

    def cp_wb(j):
        n = 128 if j < 2 else D - 256
        return pltpu.make_async_copy(wb_hbm.at[pl.ds(j * 128, n), :],
                                     wb_v.at[pl.ds(j * 128, n), :], sem_wb.at[j])

    def cp_wob(j):
        return pltpu.make_async_copy(wob_hbm.at[:, pl.ds(j * 128, 128)],
                                     wob_v.at[j], sem_wob.at[j])

    def cp_out(i, k):
        r0, n = OUT_PIECES[k]
        return pltpu.make_async_copy(x_v.at[pl.ds(i * TB + r0, n), :],
                                     out_hbm.at[pl.ds(i * TB + r0, n), :],
                                     sem_out.at[i * len(OUT_PIECES) + k])

    def release(y, chunks):
        n = len(chunks)
        nt = y.shape[1] // 128
        for u, run in enumerate(chunks):
            pos = (u * y.shape[0] * nt // n) // 16 * 16
            t, rr = pos // y.shape[0], pos % y.shape[0]
            run(y[rr:rr + 16, t * 128:(t + 1) * 128])

    def fence_xn(zero):
        return _pack(xn_v[pl.ds(pl.multiple_of(2 * TA + zero * 32, 32), 32), 0:128])

    def fence_side(zero):
        return fence_xn(zero) | wbt[8, 0:16, :] | wobp[8, 0:16, :]

    def fence_k(zero):
        return k4_v[zero, 0:16, :]

    def fence_q(zero):
        return qt_v[2 + zero, 0:16, :]

    def fence_v(zero):
        return vt_v[S // 128 + zero, 0:16, :]

    def gate(tok, zero):
        tk_v[1] = pltpu.bitcast(tok[0:8], U32)
        return tk_v[zero]

    def with_fence(xu, fen):
        r, c = xu.shape
        last = jnp.concatenate([xu[r - 16:, :c - 128], xu[r - 16:, c - 128:] | fen], axis=1)
        return jnp.concatenate([xu[:r - 16], last], axis=0)

    def ln_chunks(row0, dst, nrows, step=16):
        def mk(c):
            def run(tok):
                if tok is not None:
                    x_v[S:S + 16, 0:128] = tok.astype(BF)
                r = pl.multiple_of(row0 + c * step, step)
                xn_v[dst + c * step:dst + (c + 1) * step, :] = _layernorm(x_v[pl.ds(r, step), :])
            return run
        return [mk(c) for c in range(nrows // step)]

    def prep_chunks(j):
        def permute(part):
            rows = [tmp[pl.ds(part * H * PITCH + d, H, stride=PITCH), :] for d in range(DH)]
            val = _pack(jnp.concatenate(rows, axis=0).astype(BF))
            if part < 3:
                wbt[j, part * (D // 2):(part + 1) * (D // 2), :] = val
            else:
                wobp[j] = val

        def mk_t(c):
            def run(tok):
                wb_v[D:D + 16, 0:128] = tok.astype(BF)
                rows = pl.ds(pl.multiple_of(j * 128, 128), 128)
                wt = wb_v[rows, c * 256:(c + 1) * 256].T.astype(F32)
                for hh in range(8):
                    o = (c * 8 + hh) * PITCH
                    tmp[o:o + DH, :] = wt[hh * DH:(hh + 1) * DH]
                if c % 4 == 3:
                    permute(c // 4)
            return run

        def mk_o(c):
            def run(tok):
                wob_v[8, 0:16, :] = tok.astype(BF)
                w = wob_v[j, c * 256:(c + 1) * 256, :].astype(F32)
                for hh in range(8):
                    o = (96 + c * 8 + hh) * PITCH
                    tmp[o:o + DH, :] = w[hh * DH:(hh + 1) * DH]
                if c == 3:
                    permute(3)
            return run
        return [mk_t(c) for c in range(12)] + [mk_o(c) for c in range(4)]

    def tri_mask():
        return _iota((128, 128), 1) >= _iota((128, 128), 0)

    def build_k4(full, t, row0):
        n = full.shape[0] - 48
        rolled = [full] + [pltpu.roll(full, 32 * r, 1) for r in range(1, 4)]
        grp_id = _iota((n, 128), 1) // 32
        for a in range(4):
            val = rolled[(0 - a) % 4][0:n]
            for g in range(1, 4):
                val = jnp.where(grp_id == g, rolled[(g - a) % 4][16 * g:16 * g + n], val)
            k4_v[4 * t + a, pl.ds(row0, n), :] = val

    def store_t(y, dst, slot0, t):
        yt = _pack(y.astype(BF).T)
        rows = pl.ds(t * 64 if isinstance(t, int) else pl.multiple_of(t * 64, 64), 64)
        for b in range(TA // 128):
            dst[slot0 + b, rows, :] = yt[:, b * 128:(b + 1) * 128]

    def scores_first(qb, h):
        z = jnp.zeros((16, 128), U32)
        qh = qt_v[qb, h * 16:(h + 1) * 16, :]
        wq = _unpack(jnp.concatenate([qh if jj == h % 4 else z for jj in range(4)], axis=0))
        n = (qb + 1) * 16
        s = jnp.concatenate(
            [_dot(_unpack(k0_v[h // 4, c * n:(c + 1) * n, :]), wq) for c in range(4)], axis=0)
        diag = jnp.where(tri_mask(), s[qb * 128:], NEG)
        return diag if qb == 0 else jnp.concatenate([s[0:128], diag], axis=0)

    def scores_a(m, qb, h):
        qh = qt_v[qb, h * 16:(h + 1) * 16, :]
        if CFG['qf32']:
            qf = _unpack(qh).astype(F32)
            grp_id = _iota((32, 128), 1) // 32
            wq = jnp.concatenate(
                [jnp.where(grp_id == g, qf, 0.0) for g in range(4)], axis=0).astype(BF)
        else:
            grp_id = _iota((16, 128), 1) // 32
            z = jnp.zeros((16, 128), U32)
            wq = _unpack(jnp.concatenate(
                [jnp.where(grp_id == g, qh, z) for g in range(4)], axis=0))
        base = pl.multiple_of(m * 64 - 80, 16)
        order = [0, 16, 1, 17] + list(range(2, 16))
        cuts = [0, 5, 9, 14, 18]
        units = {}
        for c in range(4):
            idx = order[cuts[c]:cuts[c + 1]]
            lhs = jnp.concatenate([k4_v[h, pl.ds(base + u * 8, 8), :] for u in idx], axis=0)
            s = _dot(_unpack(lhs), wq)
            for n, u in enumerate(idx):
                units[u] = s[n * 16:(n + 1) * 16]
        for u in range(2):
            new = (_iota((16, 128), 1) % 32) >= (_iota((16, 128), 0) + u * 16)
            units[u] = jnp.where(new, units[16 + u], units[u])
        return jnp.concatenate([units[u] for u in range(16)], axis=0)

    def finish_a(s, m, h):
        skewed = not isinstance(m, int)
        mx = jnp.max(s, axis=0, keepdims=True)
        if skewed:
            lane = _iota((256, 128), 1)
            s = jnp.where((lane // 32) % 2 == 1,
                          jnp.concatenate([s[224:], s[:224]], axis=0), s)
            s = jnp.where(lane >= 64, jnp.concatenate([s[192:], s[:192]], axis=0), s)
        p = jnp.exp2(s - mx)
        nv = p.shape[0] // 8
        if CFG['lsum'] == 0:
            l = jnp.sum(p, axis=0, keepdims=True)
        else:
            pieces = [p[8 * v:8 * v + 8] for v in range(nv)]
            if CFG['lsum'] == 1:
                orders = [[v for t in range(nv // 16) for v in range(16 * t + 15, 16 * t - 1, -1)]]
            elif CFG['lsum'] == 2:
                orders = [list(range(16 * t + 15, 16 * t - 1, -1)) for t in range(nv // 16)]
            elif CFG['lsum'] == 3:
                pieces = [pieces[2 * v] + pieces[2 * v + 1] for v in range(nv // 2)]
                orders = [list(range(8 * t + 7, 8 * t - 1, -1)) for t in range(nv // 16)]
            elif CFG['lsum'] == 4:
                orders = [list(range(nv - 1, -1, -1))]
            accs = []
            for od in orders:
                acc = pieces[od[0]]
                for v in od[1:]:
                    acc = acc + pieces[v]
                accs.append(acc)
            l = jnp.sum(sum(accs[1:], accs[0]), axis=0, keepdims=True)
        if skewed:
            tri = tri_mask()
            pm = p[0:128]
            p = jnp.concatenate(
                [jnp.where(tri, 0.0, pm), p[128:256], jnp.where(tri, pm, 0.0)], axis=0)
        ntile = p.shape[0] // 128
        vv = _unpack(jnp.concatenate(
            [vt_v[m - bk, h * 16:(h + 1) * 16, :] for bk in range(ntile - 1, -1, -1)], axis=1))
        o = _dot(vv, p.astype(BF))
        return o * _recip(l)

    class Attn:
        def __init__(self, blk):
            self.blk = blk
            self.items = [(qb, 4 * t + a) for t in range(8) for qb in range(2) for a in range(4)]
            self.issued, self.done, self.queue, self.outs = 0, 0, [], []

        def issue(self, n=1):
            for _ in range(n):
                if self.issued < len(self.items):
                    qb, h = self.items[self.issued]
                    if isinstance(self.blk, int):
                        self.queue.append(scores_first(qb, h))
                    else:
                        self.queue.append(scores_a(self.blk * (TA // 128) + qb, qb, h))
                    self.issued += 1

        def finish(self, n=1):
            for _ in range(n):
                if self.done < self.issued:
                    qb, h = self.items[self.done]
                    self.outs.append(finish_a(self.queue.pop(0), self.blk * (TA // 128) + qb, h))
                    if len(self.outs) == 4:
                        ot = jnp.concatenate(self.outs, axis=0).astype(BF)
                        (oa0_v, oa1_v)[h // 16][(h // 4) % 4, qb * 64:(qb + 1) * 64, :] = _pack(ot.T)
                        self.last, self.outs = self.outs[-1], []
                    self.done += 1

    def add_residual(r, nrows, c0, c1, y):
        x_v[pl.ds(r, nrows), c0:c1] = (x_v[pl.ds(r, nrows), c0:c1].astype(F32) + y).astype(BF)

    def proj_b(xu, r0, side, fences):
        nrows = 2 * xu.shape[0]
        for T in range(24):
            y = None
            for hf in range(2):
                u = 2 * T + hf
                w = _unpack(jnp.concatenate(
                    [wbt[j, T * 64:(T + 1) * 64, :] for j in range(4 * hf, 4 * hf + 4)], axis=1))
                lhs = xu[:, hf * 512:(hf + 1) * 512]
                if u in fences:
                    lhs = with_fence(lhs, fences[u]())
                yh = _dot_nt(_unpack(lhs), w)
                y = yh if y is None else y + yh
                if hf == 1:
                    if T < 8:
                        qk_v[T, HALO + r0:HALO + r0 + nrows, :] = y * QSCALE
                    elif T < 16:
                        qk_v[T, HALO + r0:HALO + r0 + nrows, :] = y
                    else:
                        v_v[T - 16, HALO + r0:HALO + r0 + nrows, :] = y
                release(y, side[u])

    def logit_b(i, zero, r0):
        R = 8

        def run(tok):
            if CFG['lgtok'] == 0:
                qk_v[0, pl.ds(pl.multiple_of(HALO + TB + zero * 8, 8), 8), :] = tok[0:8]
            else:
                g = gate(tok, zero)
            accs = [None] * WB
            for t in range(8):
                q = qk_v[t, HALO + r0:HALO + r0 + R, :]
                if CFG['lgtok'] == 2:
                    q = pltpu.bitcast(pltpu.bitcast(q, U32) | g, F32)
                for w in range(WB):
                    o = HALO + r0 - 2 * w
                    p = q * qk_v[8 + t, o:o + R, :]
                    accs[w] = p if accs[w] is None else accs[w] + p
            ls = []
            for w in range(WB):
                a = accs[w]
                a = a + pltpu.roll(a, 64, 1)
                a = a + pltpu.roll(a, 32, 1)
                if r0 - 2 * w < 0:
                    a = jnp.where(_iota((R, 128), 0) + (i * TB + r0 - 2 * w) >= 0, a, NEG)
                ls.append(a)
            mx = ls[0]
            for w in range(1, WB):
                mx = jnp.maximum(mx, ls[w])
            es = [jnp.exp2(l - mx) for l in ls]
            s = es[0]
            for w in range(1, WB):
                s = s + es[w]
            inv = _recip(s)
            for w in range(WB):
                e_v[w, r0:r0 + R, :] = es[w] * inv
        return run

    def pv_b(zero, r0):
        R = 8

        def run(tok):
            if CFG['pvtok'] == 0:
                v_v[0, pl.ds(pl.multiple_of(HALO + TB + zero * 8, 8), 8), :] = tok[0:8]
            elif CFG['pvtok'] == 1:
                e_v[0, pl.ds(pl.multiple_of(TB + zero * 8, 8), 8), :] = tok[0:8]
            es = [e_v[w, r0:r0 + R, :] for w in range(WB)]
            if CFG['pvtok'] == 2:
                g = gate(tok, zero)
                es = [pltpu.bitcast(pltpu.bitcast(e, U32) | g, F32) for e in es]
            os_ = []
            for t in range(8):
                acc = None
                for w in range(WB):
                    o = HALO + r0 - 2 * w
                    pv = es[w] * v_v[t, o:o + R, :]
                    acc = pv if acc is None else acc + pv
                os_.append(acc)
            ob_v[r0:r0 + R, :] = jnp.concatenate(os_, axis=1).astype(BF)
        return run

    def out_b(i, r0, nrows, side):
        o = ob_v[r0:r0 + nrows, :]
        r = pl.multiple_of(i * TB + r0, 128)
        ys = []
        for T in range(8):
            y = None
            for hf in range(2):
                yh = _dot(o[:, hf * 512:(hf + 1) * 512],
                          _unpack(wobp[T, hf * 256:(hf + 1) * 256, :]))
                y = yh if y is None else y + yh
                release(y, side[2 * T + hf])
            ys.append(y)
            if T % 2 == 1:
                add_residual(r, nrows, (T - 1) * 128, (T + 1) * 128,
                             jnp.concatenate(ys[-2:], axis=1))

    cp_x(0).start()
    for cp in cp_wa(0):
        cp.start()
    z16 = jnp.zeros((16, 128), U32)
    xn_v[2 * TA:2 * TA + 32, :] = jnp.zeros((32, D), BF)
    wbt[8, 0:16, :] = z16
    wobp[8, 0:16, :] = z16
    k4_v[0, 0:16, :] = z16
    vt_v[S // 128, 0:16, :] = z16
    qt_v[2, 0:16, :] = z16
    tk_v[0] = z16[0:8]
    cp_x(0).wait()
    for cp in cp_wa(1):
        cp.start()
    for run in ln_chunks(0, 0, TA, step=TA):
        run(None)

    def one_pass(p, carry):
        first = p == 0
        zero = p // 4

        def f_body(c, c_):
            for k in range(NC1):
                @pl.when(jnp.logical_and(first, c == k))
                def _():
                    for cp in cp_wa(k):
                        cp.wait()
                    if k + 2 < NC1:
                        for cp in cp_wa(k + 2):
                            cp.start()
                    elif k + 2 == NC1:
                        cp_woa.start()
                    else:
                        cp_x(1).start()
                        cp_wb(0).start()
                        cp_wob(0).start()
            xn = xn_v[0:TA, :]
            for part in (2, 0, 1):
                wu = _pack(wa_v[3 * c + part])
                y = _dot(xn, _unpack(wu))
                for g in range(G1):
                    t = c * G1 + g
                    wap[part * 8 + t] = wu[:, g * 128:(g + 1) * 128]
                    yt = y[:, g * 128:(g + 1) * 128]
                    if part == 0:
                        store_t(yt * QSCALE, qt_v, 0, t)
                    elif part == 2:
                        store_t(yt, vt_v, 0, t)
                    else:
                        k0_v[t] = _pack(yt.astype(BF))
            return c_

        def a_first():
            lax.fori_loop(0, NC1, f_body, 0)

            def mk_k4(t):
                def run(tok):
                    k0_v[8, 0:8, :] = pltpu.bitcast(tok[0:8], U32)
                    kp = k0_v[t + zero]
                    kt_v[t] = kp[80:128]
                    build_k4(kp, t, 48)
                return run
            k4c = [mk_k4(t) for t in range(8)]
            at = Attn(0)
            at.issue(CFG['flook'])
            while at.issued < 2 * H:
                at.issue()
                at.finish()
                if CFG['k4early'] and at.done % 7 == 1 and k4c:
                    k4c.pop(0)(at.outs[-1][0:16] if at.outs else at.last[0:16])

            @pl.when(first)
            def _():
                cp_woa.wait()
                cp_x(1).wait()
                cp_wb(0).wait()
                cp_wob(0).wait()
                cp_x(2).start()
                cp_wb(1).start()
                cp_wob(1).start()
            hi = CFG['fhi']
            side = _both(_spread(prep_chunks(zero), 16, 0, hi),
                         _spread(ln_chunks(TA + zero * TA, 0, TA), 16, 0, hi))
            if k4c:
                side = _both(side, _spread(k4c, 16, 0, hi))
            o1 = jnp.concatenate([oa0_v[t + zero * CFG['opq']] if CFG['opq'] else oa0_v[t] for t in range(4)], axis=1)
            part = []
            yprev = None
            for u in range(16):
                if u == 8:
                    o1 = jnp.concatenate([oa1_v[t + zero * CFG['opq']] if CFG['opq'] else oa1_v[t] for t in range(4)], axis=1)
                rows = slice((u // 8) * (D // 2), (u // 8 + 1) * (D // 2))
                wu = _pack(woa_v[rows, (u % 8) * 128:(u % 8 + 1) * 128])
                woap[u % 8, (u // 8) * (D // 4):(u // 8 + 1) * (D // 4), :] = wu
                ff = CFG['ffence']
                lhs = with_fence(o1, fence_side(zero) | fence_k(zero)) if (u % ff == ff - 1) else o1
                y = _dot(_unpack(lhs), _unpack(wu))
                if u == 0:
                    at.finish(2 * H)
                if yprev is not None:
                    release(yprev, side[u - 1])
                yprev = y
                if u < 8:
                    part.append(y)
                else:
                    part[u - 8] = part[u - 8] + y
                    if u % 2 == 1:
                        add_residual(0, TA, (u - 9) * 128, (u - 7) * 128,
                                     jnp.concatenate(part[u - 9:u - 7], axis=1))

        if CFG['first']:
            a_first()

        @pl.when(first)
        def _():
            cp_x(2).wait()
            cp_wb(1).wait()
            cp_wob(1).wait()
            cp_x(3).start()
            cp_wb(2).start()
            for j in range(2, 8):
                cp_wob(j).start()

        def a_body(i, c_):
            @pl.when(jnp.logical_and(first, i == 2))
            def _():
                cp_x(3).wait()
                cp_wb(2).wait()
                for j in range(2, 8):
                    cp_wob(j).wait()
            xu = _pack(xn_v[0:TA, :])
            lnc = ln_chunks(((i + 1) % NA) * TA, 0, TA)
            mixed = [c for pair in zip(prep_chunks(i), lnc) for c in pair]
            if not CFG['side']:
                mixed = mixed[:1]
            side = _spread(mixed, 24, 0, CFG['shi'])
            at = Attn(i)
            fe = CFG['fence_every']
            yprev = None
            for u in range(24):
                t, kind = u // 3, u % 3
                if u == 23:
                    at.issue(CFG['look'])
                fen = fence_side(zero) if (u >= 3 and u % fe == fe - 1) else None
                if u >= 2:
                    f2 = (fence_k, fence_v, fence_q)[(u - 2) % 3](zero)
                    fen = f2 if fen is None else fen | f2
                lhs = xu if fen is None else with_fence(xu, fen)
                y = _dot(_unpack(lhs), _unpack(wap[(8, 16, 0)[kind] + t]))
                if kind == 0:
                    kp = _pack(y.astype(BF))
                    full = jnp.concatenate([kt_v[t], kp], axis=0)
                    kt_v[t] = kp[80:128]
                    build_k4(full, t, pl.multiple_of(i * (TA // 2), TA // 2))
                elif kind == 1:
                    store_t(y, vt_v, i * (TA // 128), t)
                else:
                    store_t(y * QSCALE, qt_v, 0, t)
                if yprev is not None:
                    release(yprev, side[u - 1])
                yprev = y
            while at.issued < 2 * H - 6:
                at.issue()
                at.finish()
            o1 = _unpack(jnp.concatenate([oa0_v[t + zero * CFG['opq']] if CFG['opq'] else oa0_v[t] for t in range(4)], axis=1))
            part = []
            for u in range(8):
                at.issue(2)
                part.append(_dot(o1, _unpack(woap[u, 0:D // 4, :])))
                if u > 0:
                    at.finish(2)
            assert at.done == 2 * H
            o2 = _unpack(jnp.concatenate([oa1_v[t + zero * CFG['opq']] if CFG['opq'] else oa1_v[t] for t in range(4)], axis=1))
            r = pl.multiple_of(i * TA, TA)
            for c in range(4):
                w2 = jnp.concatenate([woap[2 * c, D // 4:, :], woap[2 * c + 1, D // 4:, :]], axis=1)
                y = _dot(o2, _unpack(w2))
                add_residual(r, TA, c * 256, (c + 1) * 256,
                             y + jnp.concatenate(part[2 * c:2 * c + 2], axis=1))
            return c_
        if CFG['a']:
            lax.fori_loop(1, NA, a_body, 0)

        for T in range(8):
            qk_v[8 + T, 0:HALO, :] = jnp.zeros((HALO, 128), F32)
            v_v[T, 0:HALO, :] = jnp.zeros((HALO, 128), F32)

        def b_body(i, c_):
            def send(k):
                for ii in range(NB):
                    @pl.when(jnp.logical_and(p == 1, i == ii))
                    def _():
                        cp_out(ii, k).start()
            xu = _pack(xn_v[0:TA, :])
            ln1 = ln_chunks(i * TB + 256, TA, 256)
            ln2 = ln_chunks(((i + 1) % NB) * TB, 0, TA)
            lg = [logit_b(i, zero, g * 8) for g in range(TB // 8)]
            pv = [pv_b(zero, g * 8) for g in range(TB // 8)]
            n0, n1, n2 = CFG['bn']
            fx = {u: (lambda: fence_xn(zero)) for u in CFG['bf']}
            proj_b(xu, 0, _both(_spread(ln1 + ln2, 48, 0, CFG['bln']),
                                _spread(lg[0:n0], 48, 32, 48)), fx)
            xu1 = _pack(xn_v[pl.ds(pl.multiple_of(TA + zero * 32, 32), TA), :])
            mix0 = _merge(lg[n0:32], pv[0:32]) if CFG['bmix'] else lg[n0:32] + pv[0:32]
            proj_b(xu1, 256, _both(_spread(mix0, 48, 0, 32),
                                   _spread(lg[32:n1], 48, 32, 48)), {})
            mix1 = _merge(lg[n1:64], pv[32:n2])
            out_b(i, 0, 256, _spread(mix1, 16))
            send(0)
            out_b(i, 256, 128, _spread(pv[n2:64], 16, 0, CFG['bhi']))
            send(1)
            for T in range(8):
                qk_v[8 + T, 0:HALO, :] = qk_v[8 + T, TB:TB + HALO, :]
                v_v[T, 0:HALO, :] = v_v[T, TB:TB + HALO, :]
            out_b(i, 384, 128, [[]] * 16)
            send(2)
            return c_
        if CFG['b']:
            lax.fori_loop(0, NB, b_body, 0)
        return carry

    lax.fori_loop(0, 2, one_pass, 0)
    for i in range(NB):
        for k in range(len(OUT_PIECES)):
            cp_out(i, k).wait()


@jax.jit
def pallas_interleave_layers__sliding_block__sliding_local_dilated__prompt_kernel(
    A_x: jax.Array,
    A_wqkv: jax.Array,
    A_wo: jax.Array,
    B_x: jax.Array,
    B_wqkv: jax.Array,
    B_wo: jax.Array,
):
    del B_x
    x = A_x.reshape(S, D)
    any_spec = pl.BlockSpec(memory_space=pl.ANY)
    out = pl.pallas_call(
        _kernel,
        out_shape=jax.ShapeDtypeStruct((S, D), BF),
        in_specs=[any_spec] * 5,
        out_specs=any_spec,
        scratch_shapes=[
            pltpu.VMEM((S + 16, D), BF),
            pltpu.VMEM((3 * NC1, D, G1 * 128), BF),
            pltpu.VMEM((D, D), BF),
            pltpu.VMEM((D + 16, 3 * D), BF),
            pltpu.VMEM((9, D, 128), BF),
            pltpu.VMEM((24, D // 2, 128), U32),
            pltpu.VMEM((8, D // 2, 128), U32),
            pltpu.VMEM((9, 3 * D // 2, 128), U32),
            pltpu.VMEM((9, D // 2, 128), U32),
            pltpu.VMEM((128 * PITCH, 128), F32),
            pltpu.VMEM((2 * TA + 32, D), BF),
            pltpu.VMEM((9, TA // 2, 128), U32),
            pltpu.VMEM((8, 48, 128), U32),
            pltpu.VMEM((H, S // 2, 128), U32),
            pltpu.VMEM((3, D // 2, 128), U32),
            pltpu.VMEM((S // 128 + 1, D // 2, 128), U32),
            pltpu.VMEM((4, TA // 2, 128), U32),
            pltpu.VMEM((4, TA // 2, 128), U32),
            pltpu.VMEM((16, HALO + TB + 8, 128), F32),
            pltpu.VMEM((8, HALO + TB + 8, 128), F32),
            pltpu.VMEM((WB, TB + 8, 128), F32),
            pltpu.VMEM((TB, D), BF),
            pltpu.VMEM((2, 8, 128), U32),
            pltpu.SemaphoreType.DMA((4,)),
            pltpu.SemaphoreType.DMA((3 * NC1,)),
            pltpu.SemaphoreType.DMA((1,)),
            pltpu.SemaphoreType.DMA((3,)),
            pltpu.SemaphoreType.DMA((8,)),
            pltpu.SemaphoreType.DMA((NB * len(OUT_PIECES),)),
        ],
        compiler_params=pltpu.CompilerParams(vmem_limit_bytes=100 * 1024 * 1024),
        name="interleave_attn",
    )(x, A_wqkv, A_wo, B_wqkv, B_wo)
    return out.reshape(1, S, D)
```

```python
import math

import jax
import jax.numpy as jnp
from jax import lax
import jax.experimental.pallas as pl
import jax.experimental.pallas.tpu as pltpu

BF = jnp.bfloat16
F32 = jnp.float32
U32 = jnp.uint32

S = 2048
D = 1024
H = 32
DH = 32
TA = 256
NA = S // TA
TB = 512
NB = S // TB
HALO = 16
WB = 8
NEG = -1e30
EPS = 1e-5
QSCALE = (DH ** -0.5) * math.log2(math.e)
NC1 = 4
G1 = 8 // NC1
PITCH = 36
OUT_PIECES = ((0, 256), (256, 128), (384, 128))

CFG = dict(first=1, a=1, b=1, look=3, side=1, fence_every=3, efence=2, shi=21, flook=5, k4early=0, fhi=13, ffence=16,
           bn=(16, 60, 54), bf=(), bln=28, bmix=1, bhi=11, lns=2, pns=2, newton=1, qf32=1, lsum=2, opq=0, k4t=0)


def _dot(a, b):
    return jnp.dot(a, b, preferred_element_type=F32)


def _dot_nt(a, b):
    return lax.dot_general(a, b, (((1,), (1,)), ((), ())), preferred_element_type=F32)


def _pack(x_bf16):
    return pltpu.bitcast(x_bf16, U32)


def _unpack(x_u32):
    return pltpu.bitcast(x_u32, BF)


def _iota(shape, dim):
    return lax.broadcasted_iota(jnp.int32, shape, dim)


def _layernorm(x_bf16):
    x = x_bf16.astype(F32)
    m = jnp.sum(x, axis=1, keepdims=True) * (1.0 / D)
    xc = x - m
    v = jnp.sum(xc * xc, axis=1, keepdims=True) * (1.0 / D)
    return (xc * lax.rsqrt(v + EPS)).astype(BF)


def _recip(l):
    if not CFG['newton']:
        return pl.reciprocal(l, approx=False)
    r = pl.reciprocal(l, approx=True)
    return r * (2.0 - l * r)


def _spread(chunks, nslots, lo=0, hi=None):
    hi = nslots if hi is None else hi
    out = [[] for _ in range(nslots)]
    for u, c in enumerate(chunks):
        out[lo + u * (hi - lo) // len(chunks)].append(c)
    return out


def _merge(a, b):
    out = []
    for u in range(max(len(a), len(b))):
        out += a[u:u + 1] + b[u:u + 1]
    return out


def _flat(lists):
    return sum(lists, [])


def _both(*lists):
    return [sum(parts, []) for parts in zip(*lists)]


def _kernel(x_hbm, wa_hbm, woa_hbm, wb_hbm, wob_hbm, out_hbm,
            x_v, wa_v, woa_v, wb_v, wob_v, wap, woap, wbt, wobp, tmp, xn_v,
            k0_v, kt_v, k4_v, qt_v, vt_v, oa0_v, oa1_v, qk_v, v_v, e_v, ob_v, tk_v,
            sem_x, sem_wa, sem_woa, sem_wb, sem_wob, sem_out):
    def cp_x(i):
        n = TA if i < 3 else S - 3 * TA
        return pltpu.make_async_copy(x_hbm.at[pl.ds(i * TA, n), :],
                                     x_v.at[pl.ds(i * TA, n), :], sem_x.at[i])

    def cp_wa(c):
        w = G1 * 128
        return [pltpu.make_async_copy(wa_hbm.at[:, pl.ds(part * D + c * w, w)],
                                      wa_v.at[3 * c + part], sem_wa.at[3 * c + part])
                for part in range(3)]

    cp_woa = pltpu.make_async_copy(woa_hbm, woa_v, sem_woa.at[0])

    def cp_wb(j):
        n = 128 if j < 2 else D - 256
        return pltpu.make_async_copy(wb_hbm.at[pl.ds(j * 128, n), :],
                                     wb_v.at[pl.ds(j * 128, n), :], sem_wb.at[j])

    def cp_wob(j):
        return pltpu.make_async_copy(wob_hbm.at[:, pl.ds(j * 128, 128)],
                                     wob_v.at[j], sem_wob.at[j])

    def cp_out(i, k):
        r0, n = OUT_PIECES[k]
        return pltpu.make_async_copy(x_v.at[pl.ds(i * TB + r0, n), :],
                                     out_hbm.at[pl.ds(i * TB + r0, n), :],
                                     sem_out.at[i * len(OUT_PIECES) + k])

    def release(y, chunks):
        n = len(chunks)
        nt = y.shape[1] // 128
        for u, run in enumerate(chunks):
            pos = (u * y.shape[0] * nt // n) // 16 * 16
            t, rr = pos // y.shape[0], pos % y.shape[0]
            run(y[rr:rr + 16, t * 128:(t + 1) * 128])

    def fence_xn(zero):
        return _pack(xn_v[pl.ds(pl.multiple_of(2 * TA + zero * 32, 32), 32), 0:128])

    def fence_side(zero):
        return fence_xn(zero) | wbt[8, 0:16, :] | wobp[8, 0:16, :]

    def fence_k(zero):
        return k4_v[zero, 0:16, :]

    def fence_q(zero):
        return qt_v[2 + zero, 0:16, :]

    def fence_v(zero):
        return vt_v[S // 128 + zero, 0:16, :]

    def gate(tok, zero):
        tk_v[1] = pltpu.bitcast(tok[0:8], U32)
        return tk_v[zero]

    def with_fence(xu, fen):
        r, c = xu.shape
        last = jnp.concatenate([xu[r - 16:, :c - 128], xu[r - 16:, c - 128:] | fen], axis=1)
        return jnp.concatenate([xu[:r - 16], last], axis=0)

    def ln_chunks(row0, dst, nrows, step=16):
        def mk(c):
            def run(tok):
                if tok is not None:
                    x_v[S:S + 16, 0:128] = tok.astype(BF)
                r = pl.multiple_of(row0 + c * step, step)
                xn_v[dst + c * step:dst + (c + 1) * step, :] = _layernorm(x_v[pl.ds(r, step), :])
            return run
        return [mk(c) for c in range(nrows // step)]

    def prep_chunks(j):
        def permute(part):
            rows = [tmp[pl.ds(part * H * PITCH + d, H, stride=PITCH), :] for d in range(DH)]
            val = _pack(jnp.concatenate(rows, axis=0).astype(BF))
            if part < 3:
                wbt[j, part * (D // 2):(part + 1) * (D // 2), :] = val
            else:
                wobp[j] = val

        def mk_t(c):
            def run(tok):
                wb_v[D:D + 16, 0:128] = tok.astype(BF)
                rows = pl.ds(pl.multiple_of(j * 128, 128), 128)
                wt = wb_v[rows, c * 256:(c + 1) * 256].T.astype(F32)
                for hh in range(8):
                    o = (c * 8 + hh) * PITCH
                    tmp[o:o + DH, :] = wt[hh * DH:(hh + 1) * DH]
                if c % 4 == 3:
                    permute(c // 4)
            return run

        def mk_o(c):
            def run(tok):
                wob_v[8, 0:16, :] = tok.astype(BF)
                w = wob_v[j, c * 256:(c + 1) * 256, :].astype(F32)
                for hh in range(8):
                    o = (96 + c * 8 + hh) * PITCH
                    tmp[o:o + DH, :] = w[hh * DH:(hh + 1) * DH]
                if c == 3:
                    permute(3)
            return run
        return [mk_t(c) for c in range(12)] + [mk_o(c) for c in range(4)]

    def tri_mask():
        return _iota((128, 128), 1) >= _iota((128, 128), 0)

    def build_k4(full, t, row0):
        n = full.shape[0] - 48
        if CFG['k4t'] and n == 128:
            xt = [_pack(_unpack(full[16 * g:16 * g + n]).T) for g in range(4)]
            for a in range(4):
                za = jnp.concatenate([xt[g][16 * a:16 * a + 16] for g in range(4)], axis=0)
                k4_v[4 * t + a, pl.ds(row0, n), :] = _pack(_unpack(za).T)
            return
        rolled = [full] + [pltpu.roll(full, 32 * r, 1) for r in range(1, 4)]
        grp_id = _iota((n, 128), 1) // 32
        for a in range(4):
            val = rolled[(0 - a) % 4][0:n]
            for g in range(1, 4):
                val = jnp.where(grp_id == g, rolled[(g - a) % 4][16 * g:16 * g + n], val)
            k4_v[4 * t + a, pl.ds(row0, n), :] = val

    def store_t(y, dst, slot0, t):
        yt = _pack(y.astype(BF).T)
        rows = pl.ds(t * 64 if isinstance(t, int) else pl.multiple_of(t * 64, 64), 64)
        for b in range(TA // 128):
            dst[slot0 + b, rows, :] = yt[:, b * 128:(b + 1) * 128]

    def scores_first(qb, h):
        z = jnp.zeros((16, 128), U32)
        qh = qt_v[qb, h * 16:(h + 1) * 16, :]
        wq = _unpack(jnp.concatenate([qh if jj == h % 4 else z for jj in range(4)], axis=0))
        n = (qb + 1) * 16
        s = jnp.concatenate(
            [_dot(_unpack(k0_v[h // 4, c * n:(c + 1) * n, :]), wq) for c in range(4)], axis=0)
        diag = jnp.where(tri_mask(), s[qb * 128:], NEG)
        return diag if qb == 0 else jnp.concatenate([s[0:128], diag], axis=0)

    def scores_a(m, qb, h):
        qh = qt_v[qb, h * 16:(h + 1) * 16, :]
        if CFG['qf32']:
            qf = _unpack(qh).astype(F32)
            grp_id = _iota((32, 128), 1) // 32
            wq = jnp.concatenate(
                [jnp.where(grp_id == g, qf, 0.0) for g in range(4)], axis=0).astype(BF)
        else:
            grp_id = _iota((16, 128), 1) // 32
            z = jnp.zeros((16, 128), U32)
            wq = _unpack(jnp.concatenate(
                [jnp.where(grp_id == g, qh, z) for g in range(4)], axis=0))
        base = pl.multiple_of(m * 64 - 80, 16)
        order = [0, 16, 1, 17] + list(range(2, 16))
        cuts = [0, 5, 9, 14, 18]
        units = {}
        for c in range(4):
            idx = order[cuts[c]:cuts[c + 1]]
            lhs = jnp.concatenate([k4_v[h, pl.ds(base + u * 8, 8), :] for u in idx], axis=0)
            s = _dot(_unpack(lhs), wq)
            for n, u in enumerate(idx):
                units[u] = s[n * 16:(n + 1) * 16]
        for u in range(2):
            new = (_iota((16, 128), 1) % 32) >= (_iota((16, 128), 0) + u * 16)
            units[u] = jnp.where(new, units[16 + u], units[u])
        return jnp.concatenate([units[u] for u in range(16)], axis=0)

    def finish_a(s, m, h):
        skewed = not isinstance(m, int)
        mx = jnp.max(s, axis=0, keepdims=True)
        if skewed:
            lane = _iota((256, 128), 1)
            s = jnp.where((lane // 32) % 2 == 1,
                          jnp.concatenate([s[224:], s[:224]], axis=0), s)
            s = jnp.where(lane >= 64, jnp.concatenate([s[192:], s[:192]], axis=0), s)
        p = jnp.exp2(s - mx)
        nv = p.shape[0] // 8
        if CFG['lsum'] == 0:
            l = jnp.sum(p, axis=0, keepdims=True)
        else:
            pieces = [p[8 * v:8 * v + 8] for v in range(nv)]
            if CFG['lsum'] == 1:
                orders = [[v for t in range(nv // 16) for v in range(16 * t + 15, 16 * t - 1, -1)]]
            elif CFG['lsum'] == 2:
                orders = [list(range(16 * t + 15, 16 * t - 1, -1)) for t in range(nv // 16)]
            elif CFG['lsum'] == 3:
                pieces = [pieces[2 * v] + pieces[2 * v + 1] for v in range(nv // 2)]
                orders = [list(range(8 * t + 7, 8 * t - 1, -1)) for t in range(nv // 16)]
            elif CFG['lsum'] == 4:
                orders = [list(range(nv - 1, -1, -1))]
            accs = []
            for od in orders:
                acc = pieces[od[0]]
                for v in od[1:]:
                    acc = acc + pieces[v]
                accs.append(acc)
            l = jnp.sum(sum(accs[1:], accs[0]), axis=0, keepdims=True)
        if skewed:
            tri = tri_mask()
            pm = p[0:128]
            p = jnp.concatenate(
                [jnp.where(tri, 0.0, pm), p[128:256], jnp.where(tri, pm, 0.0)], axis=0)
        ntile = p.shape[0] // 128
        vv = _unpack(jnp.concatenate(
            [vt_v[m - bk, h * 16:(h + 1) * 16, :] for bk in range(ntile - 1, -1, -1)], axis=1))
        o = _dot(vv, p.astype(BF))
        return o * _recip(l)

    class Attn:
        def __init__(self, blk):
            self.blk = blk
            self.items = [(qb, 4 * t + a) for t in range(8) for qb in range(2) for a in range(4)]
            self.issued, self.done, self.queue, self.outs = 0, 0, [], []

        def issue(self, n=1):
            for _ in range(n):
                if self.issued < len(self.items):
                    qb, h = self.items[self.issued]
                    if isinstance(self.blk, int):
                        self.queue.append(scores_first(qb, h))
                    else:
                        self.queue.append(scores_a(self.blk * (TA // 128) + qb, qb, h))
                    self.issued += 1

        def finish(self, n=1):
            for _ in range(n):
                if self.done < self.issued:
                    qb, h = self.items[self.done]
                    self.outs.append(finish_a(self.queue.pop(0), self.blk * (TA // 128) + qb, h))
                    if len(self.outs) == 4:
                        ot = jnp.concatenate(self.outs, axis=0).astype(BF)
                        (oa0_v, oa1_v)[h // 16][(h // 4) % 4, qb * 64:(qb + 1) * 64, :] = _pack(ot.T)
                        self.last, self.outs = self.outs[-1], []
                    self.done += 1

    def add_residual(r, nrows, c0, c1, y):
        x_v[pl.ds(r, nrows), c0:c1] = (x_v[pl.ds(r, nrows), c0:c1].astype(F32) + y).astype(BF)

    def proj_b(xu, r0, side, fences):
        nrows = 2 * xu.shape[0]
        for T in range(24):
            y = None
            for hf in range(2):
                u = 2 * T + hf
                w = _unpack(jnp.concatenate(
                    [wbt[j, T * 64:(T + 1) * 64, :] for j in range(4 * hf, 4 * hf + 4)], axis=1))
                lhs = xu[:, hf * 512:(hf + 1) * 512]
                if u in fences:
                    lhs = with_fence(lhs, fences[u]())
                yh = _dot_nt(_unpack(lhs), w)
                y = yh if y is None else y + yh
                if hf == 1:
                    if T < 8:
                        qk_v[T, HALO + r0:HALO + r0 + nrows, :] = y * QSCALE
                    elif T < 16:
                        qk_v[T, HALO + r0:HALO + r0 + nrows, :] = y
                    else:
                        v_v[T - 16, HALO + r0:HALO + r0 + nrows, :] = y
                release(y, side[u])

    def gated(x, g):
        return pltpu.bitcast(pltpu.bitcast(x, U32) | g, F32)

    def logit_b(i, zero, r0):
        R = 8
        ns = CFG['lns']
        accs = [None] * WB

        def mk(st):
            def run(tok):
                g = gate(tok, zero)
                for t in range(st * 8 // ns, (st + 1) * 8 // ns):
                    q = gated(qk_v[t, HALO + r0:HALO + r0 + R, :], g)
                    for w in range(WB):
                        o = HALO + r0 - 2 * w
                        p = q * qk_v[8 + t, o:o + R, :]
                        accs[w] = p if accs[w] is None else accs[w] + p
                if st + 1 < ns:
                    return
                ls = []
                for w in range(WB):
                    a = accs[w]
                    a = a + pltpu.roll(a, 64, 1)
                    a = a + pltpu.roll(a, 32, 1)
                    if r0 - 2 * w < 0:
                        a = jnp.where(_iota((R, 128), 0) + (i * TB + r0 - 2 * w) >= 0, a, NEG)
                    ls.append(a)
                mx = ls[0]
                for w in range(1, WB):
                    mx = jnp.maximum(mx, ls[w])
                es = [jnp.exp2(l - mx) for l in ls]
                s = es[0]
                for w in range(1, WB):
                    s = s + es[w]
                inv = _recip(s)
                for w in range(WB):
                    e_v[w, r0:r0 + R, :] = es[w] * inv
            return run
        return [mk(st) for st in range(ns)]

    def pv_b(zero, r0):
        R = 8
        ns = CFG['pns']

        def mk(st):
            def run(tok):
                g = gate(tok, zero)
                es = [gated(e_v[w, r0:r0 + R, :], g) for w in range(WB)]
                os_ = []
                t0, t1 = st * 8 // ns, (st + 1) * 8 // ns
                for t in range(t0, t1):
                    acc = None
                    for w in range(WB):
                        o = HALO + r0 - 2 * w
                        pv = es[w] * v_v[t, o:o + R, :]
                        acc = pv if acc is None else acc + pv
                    os_.append(acc)
                ob_v[r0:r0 + R, t0 * 128:t1 * 128] = jnp.concatenate(os_, axis=1).astype(BF)
            return run
        return [mk(st) for st in range(ns)]

    def out_b(i, r0, nrows, side):
        o = ob_v[r0:r0 + nrows, :]
        r = pl.multiple_of(i * TB + r0, 128)
        ys = []
        for T in range(8):
            y = None
            for hf in range(2):
                yh = _dot(o[:, hf * 512:(hf + 1) * 512],
                          _unpack(wobp[T, hf * 256:(hf + 1) * 256, :]))
                y = yh if y is None else y + yh
                release(y, side[2 * T + hf])
            ys.append(y)
            if T % 2 == 1:
                add_residual(r, nrows, (T - 1) * 128, (T + 1) * 128,
                             jnp.concatenate(ys[-2:], axis=1))

    cp_x(0).start()
    for cp in cp_wa(0):
        cp.start()
    z16 = jnp.zeros((16, 128), U32)
    xn_v[2 * TA:2 * TA + 32, :] = jnp.zeros((32, D), BF)
    wbt[8, 0:16, :] = z16
    wobp[8, 0:16, :] = z16
    k4_v[0, 0:16, :] = z16
    vt_v[S // 128, 0:16, :] = z16
    qt_v[2, 0:16, :] = z16
    tk_v[0] = z16[0:8]
    cp_x(0).wait()
    for cp in cp_wa(1):
        cp.start()
    for run in ln_chunks(0, 0, TA, step=TA):
        run(None)

    def one_pass(p, carry):
        first = p == 0
        zero = p // 4

        def f_body(c, c_):
            for k in range(NC1):
                @pl.when(jnp.logical_and(first, c == k))
                def _():
                    for cp in cp_wa(k):
                        cp.wait()
                    if k + 2 < NC1:
                        for cp in cp_wa(k + 2):
                            cp.start()
                    elif k + 2 == NC1:
                        cp_woa.start()
                    else:
                        cp_x(1).start()
                        cp_wb(0).start()
                        cp_wob(0).start()
            xn = xn_v[0:TA, :]
            for part in (2, 0, 1):
                wu = _pack(wa_v[3 * c + part])
                y = _dot(xn, _unpack(wu))
                for g in range(G1):
                    t = c * G1 + g
                    wap[part * 8 + t] = wu[:, g * 128:(g + 1) * 128]
                    yt = y[:, g * 128:(g + 1) * 128]
                    if part == 0:
                        store_t(yt * QSCALE, qt_v, 0, t)
                    elif part == 2:
                        store_t(yt, vt_v, 0, t)
                    else:
                        k0_v[t] = _pack(yt.astype(BF))
            return c_

        def a_first():
            lax.fori_loop(0, NC1, f_body, 0)

            def mk_k4(t):
                def run(tok):
                    k0_v[8, 0:8, :] = pltpu.bitcast(tok[0:8], U32)
                    kp = k0_v[t + zero]
                    kt_v[t] = kp[80:128]
                    build_k4(kp, t, 48)
                return run
            k4c = [mk_k4(t) for t in range(8)]
            at = Attn(0)
            at.issue(CFG['flook'])
            while at.issued < 2 * H:
                at.issue()
                at.finish()
                if CFG['k4early'] and at.done % 7 == 1 and k4c:
                    k4c.pop(0)(at.outs[-1][0:16] if at.outs else at.last[0:16])

            @pl.when(first)
            def _():
                cp_woa.wait()
                cp_x(1).wait()
                cp_wb(0).wait()
                cp_wob(0).wait()
                cp_x(2).start()
                cp_wb(1).start()
                cp_wob(1).start()
            hi = CFG['fhi']
            side = _both(_spread(prep_chunks(zero), 16, 0, hi),
                         _spread(ln_chunks(TA + zero * TA, 0, TA), 16, 0, hi))
            if k4c:
                side = _both(side, _spread(k4c, 16, 0, hi))
            o1 = jnp.concatenate([oa0_v[t + zero * CFG['opq']] if CFG['opq'] else oa0_v[t] for t in range(4)], axis=1)
            part = []
            yprev = None
            for u in range(16):
                if u == 8:
                    o1 = jnp.concatenate([oa1_v[t + zero * CFG['opq']] if CFG['opq'] else oa1_v[t] for t in range(4)], axis=1)
                rows = slice((u // 8) * (D // 2), (u // 8 + 1) * (D // 2))
                wu = _pack(woa_v[rows, (u % 8) * 128:(u % 8 + 1) * 128])
                woap[u % 8, (u // 8) * (D // 4):(u // 8 + 1) * (D // 4), :] = wu
                ff = CFG['ffence']
                lhs = with_fence(o1, fence_side(zero) | fence_k(zero)) if (u % ff == ff - 1) else o1
                y = _dot(_unpack(lhs), _unpack(wu))
                if u == 0:
                    at.finish(2 * H)
                if yprev is not None:
                    release(yprev, side[u - 1])
                yprev = y
                if u < 8:
                    part.append(y)
                else:
                    part[u - 8] = part[u - 8] + y
                    if u % 2 == 1:
                        add_residual(0, TA, (u - 9) * 128, (u - 7) * 128,
                                     jnp.concatenate(part[u - 9:u - 7], axis=1))

        if CFG['first']:
            a_first()

        @pl.when(first)
        def _():
            cp_x(2).wait()
            cp_wb(1).wait()
            cp_wob(1).wait()
            cp_x(3).start()
            cp_wb(2).start()
            for j in range(2, 8):
                cp_wob(j).start()

        def a_body(i, c_):
            @pl.when(jnp.logical_and(first, i == 2))
            def _():
                cp_x(3).wait()
                cp_wb(2).wait()
                for j in range(2, 8):
                    cp_wob(j).wait()
            xu = _pack(xn_v[0:TA, :])
            lnc = ln_chunks(((i + 1) % NA) * TA, 0, TA)
            mixed = [c for pair in zip(prep_chunks(i), lnc) for c in pair]
            if not CFG['side']:
                mixed = mixed[:1]
            side = _spread(mixed, 24, 0, CFG['shi'])
            at = Attn(i)
            fe = CFG['fence_every']
            yprev = None
            for u in range(24):
                t, kind = u // 3, u % 3
                if u == 23:
                    at.issue(CFG['look'])
                fen = fence_side(zero) if (u >= 3 and u % fe == fe - 1) else None
                if u >= 2 and CFG['efence']:
                    f2 = (fence_k, fence_v, fence_q)[(u - 2) % 3](zero)
                    fen = f2 if fen is None else fen | f2
                lhs = xu if fen is None else with_fence(xu, fen)
                y = _dot(_unpack(lhs), _unpack(wap[(8, 16, 0)[kind] + t]))
                if kind == 0:
                    kp = _pack(y.astype(BF))
                    full = jnp.concatenate([kt_v[t], kp], axis=0)
                    kt_v[t] = kp[80:128]
                    build_k4(full, t, pl.multiple_of(i * (TA // 2), TA // 2))
                elif kind == 1:
                    store_t(y, vt_v, i * (TA // 128), t)
                else:
                    store_t(y * QSCALE, qt_v, 0, t)
                if yprev is not None:
                    release(yprev, side[u - 1])
                yprev = y
            while at.issued < 2 * H - 6:
                at.issue()
                at.finish()
            o1 = _unpack(jnp.concatenate([oa0_v[t + zero * CFG['opq']] if CFG['opq'] else oa0_v[t] for t in range(4)], axis=1))
            part = []
            for u in range(8):
                at.issue(2)
                part.append(_dot(o1, _unpack(woap[u, 0:D // 4, :])))
                if u > 0:
                    at.finish(2)
            assert at.done == 2 * H
            o2 = _unpack(jnp.concatenate([oa1_v[t + zero * CFG['opq']] if CFG['opq'] else oa1_v[t] for t in range(4)], axis=1))
            r = pl.multiple_of(i * TA, TA)
            for c in range(4):
                w2 = jnp.concatenate([woap[2 * c, D // 4:, :], woap[2 * c + 1, D // 4:, :]], axis=1)
                y = _dot(o2, _unpack(w2))
                add_residual(r, TA, c * 256, (c + 1) * 256,
                             y + jnp.concatenate(part[2 * c:2 * c + 2], axis=1))
            return c_
        if CFG['a']:
            lax.fori_loop(1, NA, a_body, 0)

        for T in range(8):
            qk_v[8 + T, 0:HALO, :] = jnp.zeros((HALO, 128), F32)
            v_v[T, 0:HALO, :] = jnp.zeros((HALO, 128), F32)

        def b_body(i, c_):
            def send(k):
                for ii in range(NB):
                    @pl.when(jnp.logical_and(p == 1, i == ii))
                    def _():
                        cp_out(ii, k).start()
            xu = _pack(xn_v[0:TA, :])
            ln1 = ln_chunks(i * TB + 256, TA, 256)
            ln2 = ln_chunks(((i + 1) % NB) * TB, 0, TA)
            lg = [logit_b(i, zero, g * 8) for g in range(TB // 8)]
            pv = [pv_b(zero, g * 8) for g in range(TB // 8)]
            n0, n1, n2 = CFG['bn']
            fx = {u: (lambda: fence_xn(zero)) for u in CFG['bf']}
            proj_b(xu, 0, _both(_spread(ln1 + ln2, 48, 0, CFG['bln']),
                                _spread(_flat(lg[0:n0]), 48, 32, 48)), fx)
            xu1 = _pack(xn_v[pl.ds(pl.multiple_of(TA + zero * 32, 32), TA), :])
            mix0 = _merge(lg[n0:32], pv[0:32]) if CFG['bmix'] else lg[n0:32] + pv[0:32]
            proj_b(xu1, 256, _both(_spread(_flat(mix0), 48, 0, 32),
                                   _spread(_flat(lg[32:n1]), 48, 32, 48)), {})
            mix1 = _merge(lg[n1:64], pv[32:n2])
            out_b(i, 0, 256, _spread(_flat(mix1), 16))
            send(0)
            out_b(i, 256, 128, _spread(_flat(pv[n2:64]), 16, 0, CFG['bhi']))
            send(1)
            for T in range(8):
                qk_v[8 + T, 0:HALO, :] = qk_v[8 + T, TB:TB + HALO, :]
                v_v[T, 0:HALO, :] = v_v[T, TB:TB + HALO, :]
            out_b(i, 384, 128, [[]] * 16)
            send(2)
            return c_
        if CFG['b']:
            lax.fori_loop(0, NB, b_body, 0)
        return carry

    lax.fori_loop(0, 2, one_pass, 0)
    for i in range(NB):
        for k in range(len(OUT_PIECES)):
            cp_out(i, k).wait()


@jax.jit
def pallas_interleave_layers__sliding_block__sliding_local_dilated__prompt_kernel(
    A_x: jax.Array,
    A_wqkv: jax.Array,
    A_wo: jax.Array,
    B_x: jax.Array,
    B_wqkv: jax.Array,
    B_wo: jax.Array,
):
    del B_x
    x = A_x.reshape(S, D)
    any_spec = pl.BlockSpec(memory_space=pl.ANY)
    out = pl.pallas_call(
        _kernel,
        out_shape=jax.ShapeDtypeStruct((S, D), BF),
        in_specs=[any_spec] * 5,
        out_specs=any_spec,
        scratch_shapes=[
            pltpu.VMEM((S + 16, D), BF),
            pltpu.VMEM((3 * NC1, D, G1 * 128), BF),
            pltpu.VMEM((D, D), BF),
            pltpu.VMEM((D + 16, 3 * D), BF),
            pltpu.VMEM((9, D, 128), BF),
            pltpu.VMEM((24, D // 2, 128), U32),
            pltpu.VMEM((8, D // 2, 128), U32),
            pltpu.VMEM((9, 3 * D // 2, 128), U32),
            pltpu.VMEM((9, D // 2, 128), U32),
            pltpu.VMEM((128 * PITCH, 128), F32),
            pltpu.VMEM((2 * TA + 32, D), BF),
            pltpu.VMEM((9, TA // 2, 128), U32),
            pltpu.VMEM((8, 48, 128), U32),
            pltpu.VMEM((H, S // 2, 128), U32),
            pltpu.VMEM((3, D // 2, 128), U32),
            pltpu.VMEM((S // 128 + 1, D // 2, 128), U32),
            pltpu.VMEM((4, TA // 2, 128), U32),
            pltpu.VMEM((4, TA // 2, 128), U32),
            pltpu.VMEM((16, HALO + TB, 128), F32),
            pltpu.VMEM((8, HALO + TB, 128), F32),
            pltpu.VMEM((WB, TB, 128), F32),
            pltpu.VMEM((TB, D), BF),
            pltpu.VMEM((2, 8, 128), U32),
            pltpu.SemaphoreType.DMA((4,)),
            pltpu.SemaphoreType.DMA((3 * NC1,)),
            pltpu.SemaphoreType.DMA((1,)),
            pltpu.SemaphoreType.DMA((3,)),
            pltpu.SemaphoreType.DMA((8,)),
            pltpu.SemaphoreType.DMA((NB * len(OUT_PIECES),)),
        ],
        compiler_params=pltpu.CompilerParams(vmem_limit_bytes=100 * 1024 * 1024),
        name="interleave_attn",
    )(x, A_wqkv, A_wo, B_wqkv, B_wo)
    return out.reshape(1, S, D)
```

```python
import math

import jax
import jax.numpy as jnp
from jax import lax
import jax.experimental.pallas as pl
import jax.experimental.pallas.tpu as pltpu

BF = jnp.bfloat16
F32 = jnp.float32
U32 = jnp.uint32

S = 2048
D = 1024
H = 32
DH = 32
TA = 256
NA = S // TA
TB = 512
NB = S // TB
HALO = 16
WB = 8
NEG = -1e30
EPS = 1e-5
QSCALE = (DH ** -0.5) * math.log2(math.e)
NC1 = 4
G1 = 8 // NC1
PITCH = 36
OUT_PIECES = ((0, 256), (256, 128), (384, 128))

CFG = dict(first=1, a=1, b=1, look=3, side=1, fence_every=3, efence=2, shi=21, flook=5, k4early=0, fhi=13, ffence=16,
           bn=(16, 60, 54), bf=(), bln=28, bmix=1, bhi=11, lns=2, pns=2, newton=1, qf32=1, lsum=2, opq=1, k4t=0, tail=6)


def _dot(a, b):
    return jnp.dot(a, b, preferred_element_type=F32)


def _dot_nt(a, b):
    return lax.dot_general(a, b, (((1,), (1,)), ((), ())), preferred_element_type=F32)


def _pack(x_bf16):
    return pltpu.bitcast(x_bf16, U32)


def _unpack(x_u32):
    return pltpu.bitcast(x_u32, BF)


def _iota(shape, dim):
    return lax.broadcasted_iota(jnp.int32, shape, dim)


def _layernorm(x_bf16):
    x = x_bf16.astype(F32)
    m = jnp.sum(x, axis=1, keepdims=True) * (1.0 / D)
    xc = x - m
    v = jnp.sum(xc * xc, axis=1, keepdims=True) * (1.0 / D)
    return (xc * lax.rsqrt(v + EPS)).astype(BF)


def _recip(l):
    if not CFG['newton']:
        return pl.reciprocal(l, approx=False)
    r = pl.reciprocal(l, approx=True)
    return r * (2.0 - l * r)


def _spread(chunks, nslots, lo=0, hi=None):
    hi = nslots if hi is None else hi
    out = [[] for _ in range(nslots)]
    for u, c in enumerate(chunks):
        out[lo + u * (hi - lo) // len(chunks)].append(c)
    return out


def _merge(a, b):
    out = []
    for u in range(max(len(a), len(b))):
        out += a[u:u + 1] + b[u:u + 1]
    return out


def _flat(lists):
    return sum(lists, [])


def _both(*lists):
    return [sum(parts, []) for parts in zip(*lists)]


def _kernel(x_hbm, wa_hbm, woa_hbm, wb_hbm, wob_hbm, out_hbm,
            x_v, wa_v, woa_v, wb_v, wob_v, wap, woap, wbt, wobp, tmp, xn_v,
            k0_v, kt_v, k4_v, qt_v, vt_v, oa0_v, oa1_v, qk_v, v_v, e_v, ob_v, tk_v,
            sem_x, sem_wa, sem_woa, sem_wb, sem_wob, sem_out):
    def cp_x(i):
        n = TA if i < 3 else S - 3 * TA
        return pltpu.make_async_copy(x_hbm.at[pl.ds(i * TA, n), :],
                                     x_v.at[pl.ds(i * TA, n), :], sem_x.at[i])

    def cp_wa(c):
        w = G1 * 128
        return [pltpu.make_async_copy(wa_hbm.at[:, pl.ds(part * D + c * w, w)],
                                      wa_v.at[3 * c + part], sem_wa.at[3 * c + part])
                for part in range(3)]

    cp_woa = pltpu.make_async_copy(woa_hbm, woa_v, sem_woa.at[0])

    def cp_wb(j):
        n = 128 if j < 2 else D - 256
        return pltpu.make_async_copy(wb_hbm.at[pl.ds(j * 128, n), :],
                                     wb_v.at[pl.ds(j * 128, n), :], sem_wb.at[j])

    def cp_wob(j):
        return pltpu.make_async_copy(wob_hbm.at[:, pl.ds(j * 128, 128)],
                                     wob_v.at[j], sem_wob.at[j])

    def cp_out(i, k):
        r0, n = OUT_PIECES[k]
        return pltpu.make_async_copy(x_v.at[pl.ds(i * TB + r0, n), :],
                                     out_hbm.at[pl.ds(i * TB + r0, n), :],
                                     sem_out.at[i * len(OUT_PIECES) + k])

    def release(y, chunks):
        n = len(chunks)
        nt = y.shape[1] // 128
        for u, run in enumerate(chunks):
            pos = (u * y.shape[0] * nt // n) // 16 * 16
            t, rr = pos // y.shape[0], pos % y.shape[0]
            run(y[rr:rr + 16, t * 128:(t + 1) * 128])

    def fence_xn(zero):
        return _pack(xn_v[pl.ds(pl.multiple_of(2 * TA + zero * 32, 32), 32), 0:128])

    def fence_side(zero):
        return fence_xn(zero) | wbt[8, 0:16, :] | wobp[8, 0:16, :]

    def fence_k(zero):
        return k4_v[zero, 0:16, :]

    def fence_q(zero):
        return qt_v[2 + zero, 0:16, :]

    def fence_v(zero):
        return vt_v[S // 128 + zero, 0:16, :]

    def gate(tok, zero):
        tk_v[1] = pltpu.bitcast(tok[0:8], U32)
        return tk_v[zero]

    def with_fence(xu, fen):
        r, c = xu.shape
        last = jnp.concatenate([xu[r - 16:, :c - 128], xu[r - 16:, c - 128:] | fen], axis=1)
        return jnp.concatenate([xu[:r - 16], last], axis=0)

    def ln_chunks(row0, dst, nrows, step=16):
        def mk(c):
            def run(tok):
                if tok is not None:
                    x_v[S:S + 16, 0:128] = tok.astype(BF)
                r = pl.multiple_of(row0 + c * step, step)
                xn_v[dst + c * step:dst + (c + 1) * step, :] = _layernorm(x_v[pl.ds(r, step), :])
            return run
        return [mk(c) for c in range(nrows // step)]

    def prep_chunks(j):
        def permute(part):
            rows = [tmp[pl.ds(part * H * PITCH + d, H, stride=PITCH), :] for d in range(DH)]
            val = _pack(jnp.concatenate(rows, axis=0).astype(BF))
            if part < 3:
                wbt[j, part * (D // 2):(part + 1) * (D // 2), :] = val
            else:
                wobp[j] = val

        def mk_t(c):
            def run(tok):
                wb_v[D:D + 16, 0:128] = tok.astype(BF)
                rows = pl.ds(pl.multiple_of(j * 128, 128), 128)
                wt = wb_v[rows, c * 256:(c + 1) * 256].T.astype(F32)
                for hh in range(8):
                    o = (c * 8 + hh) * PITCH
                    tmp[o:o + DH, :] = wt[hh * DH:(hh + 1) * DH]
                if c % 4 == 3:
                    permute(c // 4)
            return run

        def mk_o(c):
            def run(tok):
                wob_v[8, 0:16, :] = tok.astype(BF)
                w = wob_v[j, c * 256:(c + 1) * 256, :].astype(F32)
                for hh in range(8):
                    o = (96 + c * 8 + hh) * PITCH
                    tmp[o:o + DH, :] = w[hh * DH:(hh + 1) * DH]
                if c == 3:
                    permute(3)
            return run
        return [mk_t(c) for c in range(12)] + [mk_o(c) for c in range(4)]

    def tri_mask():
        return _iota((128, 128), 1) >= _iota((128, 128), 0)

    def build_k4(full, t, row0):
        n = full.shape[0] - 48
        if CFG['k4t'] and n == 128:
            xt = [_pack(_unpack(full[16 * g:16 * g + n]).T) for g in range(4)]
            for a in range(4):
                za = jnp.concatenate([xt[g][16 * a:16 * a + 16] for g in range(4)], axis=0)
                k4_v[4 * t + a, pl.ds(row0, n), :] = _pack(_unpack(za).T)
            return
        rolled = [full] + [pltpu.roll(full, 32 * r, 1) for r in range(1, 4)]
        grp_id = _iota((n, 128), 1) // 32
        for a in range(4):
            val = rolled[(0 - a) % 4][0:n]
            for g in range(1, 4):
                val = jnp.where(grp_id == g, rolled[(g - a) % 4][16 * g:16 * g + n], val)
            k4_v[4 * t + a, pl.ds(row0, n), :] = val

    def store_t(y, dst, slot0, t):
        yt = _pack(y.astype(BF).T)
        rows = pl.ds(t * 64 if isinstance(t, int) else pl.multiple_of(t * 64, 64), 64)
        for b in range(TA // 128):
            dst[slot0 + b, rows, :] = yt[:, b * 128:(b + 1) * 128]

    def scores_first(qb, h):
        z = jnp.zeros((16, 128), U32)
        qh = qt_v[qb, h * 16:(h + 1) * 16, :]
        wq = _unpack(jnp.concatenate([qh if jj == h % 4 else z for jj in range(4)], axis=0))
        n = (qb + 1) * 16
        s = jnp.concatenate(
            [_dot(_unpack(k0_v[h // 4, c * n:(c + 1) * n, :]), wq) for c in range(4)], axis=0)
        diag = jnp.where(tri_mask(), s[qb * 128:], NEG)
        return diag if qb == 0 else jnp.concatenate([s[0:128], diag], axis=0)

    def scores_a(m, qb, h):
        qh = qt_v[qb, h * 16:(h + 1) * 16, :]
        if CFG['qf32']:
            qf = _unpack(qh).astype(F32)
            grp_id = _iota((32, 128), 1) // 32
            wq = jnp.concatenate(
                [jnp.where(grp_id == g, qf, 0.0) for g in range(4)], axis=0).astype(BF)
        else:
            grp_id = _iota((16, 128), 1) // 32
            z = jnp.zeros((16, 128), U32)
            wq = _unpack(jnp.concatenate(
                [jnp.where(grp_id == g, qh, z) for g in range(4)], axis=0))
        base = pl.multiple_of(m * 64 - 80, 16)
        order = [0, 16, 1, 17] + list(range(2, 16))
        cuts = [0, 5, 9, 14, 18]
        units = {}
        for c in range(4):
            idx = order[cuts[c]:cuts[c + 1]]
            lhs = jnp.concatenate([k4_v[h, pl.ds(base + u * 8, 8), :] for u in idx], axis=0)
            s = _dot(_unpack(lhs), wq)
            for n, u in enumerate(idx):
                units[u] = s[n * 16:(n + 1) * 16]
        for u in range(2):
            new = (_iota((16, 128), 1) % 32) >= (_iota((16, 128), 0) + u * 16)
            units[u] = jnp.where(new, units[16 + u], units[u])
        return jnp.concatenate([units[u] for u in range(16)], axis=0)

    def finish_a(s, m, h):
        skewed = not isinstance(m, int)
        mx = jnp.max(s, axis=0, keepdims=True)
        if skewed:
            lane = _iota((256, 128), 1)
            s = jnp.where((lane // 32) % 2 == 1,
                          jnp.concatenate([s[224:], s[:224]], axis=0), s)
            s = jnp.where(lane >= 64, jnp.concatenate([s[192:], s[:192]], axis=0), s)
        p = jnp.exp2(s - mx)
        nv = p.shape[0] // 8
        if CFG['lsum'] == 0:
            l = jnp.sum(p, axis=0, keepdims=True)
        else:
            pieces = [p[8 * v:8 * v + 8] for v in range(nv)]
            if CFG['lsum'] == 1:
                orders = [[v for t in range(nv // 16) for v in range(16 * t + 15, 16 * t - 1, -1)]]
            elif CFG['lsum'] == 2:
                orders = [list(range(16 * t + 15, 16 * t - 1, -1)) for t in range(nv // 16)]
            elif CFG['lsum'] == 3:
                pieces = [pieces[2 * v] + pieces[2 * v + 1] for v in range(nv // 2)]
                orders = [list(range(8 * t + 7, 8 * t - 1, -1)) for t in range(nv // 16)]
            elif CFG['lsum'] == 4:
                orders = [list(range(nv - 1, -1, -1))]
            accs = []
            for od in orders:
                acc = pieces[od[0]]
                for v in od[1:]:
                    acc = acc + pieces[v]
                accs.append(acc)
            l = jnp.sum(sum(accs[1:], accs[0]), axis=0, keepdims=True)
        if skewed:
            tri = tri_mask()
            pm = p[0:128]
            p = jnp.concatenate(
                [jnp.where(tri, 0.0, pm), p[128:256], jnp.where(tri, pm, 0.0)], axis=0)
        ntile = p.shape[0] // 128
        vv = _unpack(jnp.concatenate(
            [vt_v[m - bk, h * 16:(h + 1) * 16, :] for bk in range(ntile - 1, -1, -1)], axis=1))
        o = _dot(vv, p.astype(BF))
        return o * _recip(l)

    class Attn:
        def __init__(self, blk):
            self.blk = blk
            self.items = [(qb, 4 * t + a) for t in range(8) for qb in range(2) for a in range(4)]
            self.issued, self.done, self.queue, self.outs = 0, 0, [], []

        def issue(self, n=1):
            for _ in range(n):
                if self.issued < len(self.items):
                    qb, h = self.items[self.issued]
                    if isinstance(self.blk, int):
                        self.queue.append(scores_first(qb, h))
                    else:
                        self.queue.append(scores_a(self.blk * (TA // 128) + qb, qb, h))
                    self.issued += 1

        def finish(self, n=1):
            for _ in range(n):
                if self.done < self.issued:
                    qb, h = self.items[self.done]
                    self.outs.append(finish_a(self.queue.pop(0), self.blk * (TA // 128) + qb, h))
                    if len(self.outs) == 4:
                        ot = jnp.concatenate(self.outs, axis=0).astype(BF)
                        (oa0_v, oa1_v)[h // 16][(h // 4) % 4, qb * 64:(qb + 1) * 64, :] = _pack(ot.T)
                        self.last, self.outs = self.outs[-1], []
                    self.done += 1

    def add_residual(r, nrows, c0, c1, y):
        x_v[pl.ds(r, nrows), c0:c1] = (x_v[pl.ds(r, nrows), c0:c1].astype(F32) + y).astype(BF)

    def proj_b(xu, r0, side, fences):
        nrows = 2 * xu.shape[0]
        for T in range(24):
            y = None
            for hf in range(2):
                u = 2 * T + hf
                w = _unpack(jnp.concatenate(
                    [wbt[j, T * 64:(T + 1) * 64, :] for j in range(4 * hf, 4 * hf + 4)], axis=1))
                lhs = xu[:, hf * 512:(hf + 1) * 512]
                if u in fences:
                    lhs = with_fence(lhs, fences[u]())
                yh = _dot_nt(_unpack(lhs), w)
                y = yh if y is None else y + yh
                if hf == 1:
                    if T < 8:
                        qk_v[T, HALO + r0:HALO + r0 + nrows, :] = y * QSCALE
                    elif T < 16:
                        qk_v[T, HALO + r0:HALO + r0 + nrows, :] = y
                    else:
                        v_v[T - 16, HALO + r0:HALO + r0 + nrows, :] = y
                release(y, side[u])

    def gated(x, g):
        return pltpu.bitcast(pltpu.bitcast(x, U32) | g, F32)

    def logit_b(i, zero, r0):
        R = 8
        ns = CFG['lns']
        accs = [None] * WB

        def mk(st):
            def run(tok):
                g = gate(tok, zero)
                for t in range(st * 8 // ns, (st + 1) * 8 // ns):
                    q = gated(qk_v[t, HALO + r0:HALO + r0 + R, :], g)
                    for w in range(WB):
                        o = HALO + r0 - 2 * w
                        p = q * qk_v[8 + t, o:o + R, :]
                        accs[w] = p if accs[w] is None else accs[w] + p
                if st + 1 < ns:
                    return
                ls = []
                for w in range(WB):
                    a = accs[w]
                    a = a + pltpu.roll(a, 64, 1)
                    a = a + pltpu.roll(a, 32, 1)
                    if r0 - 2 * w < 0:
                        a = jnp.where(_iota((R, 128), 0) + (i * TB + r0 - 2 * w) >= 0, a, NEG)
                    ls.append(a)
                mx = ls[0]
                for w in range(1, WB):
                    mx = jnp.maximum(mx, ls[w])
                es = [jnp.exp2(l - mx) for l in ls]
                s = es[0]
                for w in range(1, WB):
                    s = s + es[w]
                inv = _recip(s)
                for w in range(WB):
                    e_v[w, r0:r0 + R, :] = es[w] * inv
            return run
        return [mk(st) for st in range(ns)]

    def pv_b(zero, r0):
        R = 8
        ns = CFG['pns']

        def mk(st):
            def run(tok):
                g = gate(tok, zero)
                es = [gated(e_v[w, r0:r0 + R, :], g) for w in range(WB)]
                os_ = []
                t0, t1 = st * 8 // ns, (st + 1) * 8 // ns
                for t in range(t0, t1):
                    acc = None
                    for w in range(WB):
                        o = HALO + r0 - 2 * w
                        pv = es[w] * v_v[t, o:o + R, :]
                        acc = pv if acc is None else acc + pv
                    os_.append(acc)
                ob_v[r0:r0 + R, t0 * 128:t1 * 128] = jnp.concatenate(os_, axis=1).astype(BF)
            return run
        return [mk(st) for st in range(ns)]

    def out_b(i, r0, nrows, side):
        o = ob_v[r0:r0 + nrows, :]
        r = pl.multiple_of(i * TB + r0, 128)
        ys = []
        for T in range(8):
            y = None
            for hf in range(2):
                yh = _dot(o[:, hf * 512:(hf + 1) * 512],
                          _unpack(wobp[T, hf * 256:(hf + 1) * 256, :]))
                y = yh if y is None else y + yh
                release(y, side[2 * T + hf])
            ys.append(y)
            if T % 2 == 1:
                add_residual(r, nrows, (T - 1) * 128, (T + 1) * 128,
                             jnp.concatenate(ys[-2:], axis=1))

    cp_x(0).start()
    for cp in cp_wa(0):
        cp.start()
    z16 = jnp.zeros((16, 128), U32)
    xn_v[2 * TA:2 * TA + 32, :] = jnp.zeros((32, D), BF)
    wbt[8, 0:16, :] = z16
    wobp[8, 0:16, :] = z16
    k4_v[0, 0:16, :] = z16
    vt_v[S // 128, 0:16, :] = z16
    qt_v[2, 0:16, :] = z16
    tk_v[0] = z16[0:8]
    cp_x(0).wait()
    for cp in cp_wa(1):
        cp.start()
    for run in ln_chunks(0, 0, TA, step=TA):
        run(None)

    def one_pass(p, carry):
        first = p == 0
        zero = p // 4

        def f_body(c, c_):
            for k in range(NC1):
                @pl.when(jnp.logical_and(first, c == k))
                def _():
                    for cp in cp_wa(k):
                        cp.wait()
                    if k + 2 < NC1:
                        for cp in cp_wa(k + 2):
                            cp.start()
                    elif k + 2 == NC1:
                        cp_woa.start()
                    else:
                        cp_x(1).start()
                        cp_wb(0).start()
                        cp_wob(0).start()
            xn = xn_v[0:TA, :]
            for part in (2, 0, 1):
                wu = _pack(wa_v[3 * c + part])
                y = _dot(xn, _unpack(wu))
                for g in range(G1):
                    t = c * G1 + g
                    wap[part * 8 + t] = wu[:, g * 128:(g + 1) * 128]
                    yt = y[:, g * 128:(g + 1) * 128]
                    if part == 0:
                        store_t(yt * QSCALE, qt_v, 0, t)
                    elif part == 2:
                        store_t(yt, vt_v, 0, t)
                    else:
                        k0_v[t] = _pack(yt.astype(BF))
            return c_

        def a_first():
            lax.fori_loop(0, NC1, f_body, 0)

            def mk_k4(t):
                def run(tok):
                    k0_v[8, 0:8, :] = pltpu.bitcast(tok[0:8], U32)
                    kp = k0_v[t + zero]
                    kt_v[t] = kp[80:128]
                    build_k4(kp, t, 48)
                return run
            k4c = [mk_k4(t) for t in range(8)]
            at = Attn(0)
            at.issue(CFG['flook'])
            while at.issued < 2 * H:
                at.issue()
                at.finish()
                if CFG['k4early'] and at.done % 7 == 1 and k4c:
                    k4c.pop(0)(at.outs[-1][0:16] if at.outs else at.last[0:16])

            @pl.when(first)
            def _():
                cp_woa.wait()
                cp_x(1).wait()
                cp_wb(0).wait()
                cp_wob(0).wait()
                cp_x(2).start()
                cp_wb(1).start()
                cp_wob(1).start()
            hi = CFG['fhi']
            side = _both(_spread(prep_chunks(zero), 16, 0, hi),
                         _spread(ln_chunks(TA + zero * TA, 0, TA), 16, 0, hi))
            if k4c:
                side = _both(side, _spread(k4c, 16, 0, hi))
            o1 = jnp.concatenate([oa0_v[t + zero] if CFG['opq'] & 1 else oa0_v[t] for t in range(4)], axis=1)
            part = []
            yprev = None
            for u in range(16):
                if u == 8:
                    o1 = jnp.concatenate([oa1_v[t + zero] if CFG['opq'] & 2 else oa1_v[t] for t in range(4)], axis=1)
                rows = slice((u // 8) * (D // 2), (u // 8 + 1) * (D // 2))
                wu = _pack(woa_v[rows, (u % 8) * 128:(u % 8 + 1) * 128])
                woap[u % 8, (u // 8) * (D // 4):(u // 8 + 1) * (D // 4), :] = wu
                ff = CFG['ffence']
                lhs = with_fence(o1, fence_side(zero) | fence_k(zero)) if (u % ff == ff - 1) else o1
                y = _dot(_unpack(lhs), _unpack(wu))
                if u == 0:
                    at.finish(2 * H)
                if yprev is not None:
                    release(yprev, side[u - 1])
                yprev = y
                if u < 8:
                    part.append(y)
                else:
                    part[u - 8] = part[u - 8] + y
                    if u % 2 == 1:
                        add_residual(0, TA, (u - 9) * 128, (u - 7) * 128,
                                     jnp.concatenate(part[u - 9:u - 7], axis=1))

        if CFG['first']:
            a_first()

        @pl.when(first)
        def _():
            cp_x(2).wait()
            cp_wb(1).wait()
            cp_wob(1).wait()
            cp_x(3).start()
            cp_wb(2).start()
            for j in range(2, 8):
                cp_wob(j).start()

        def a_body(i, c_):
            @pl.when(jnp.logical_and(first, i == 2))
            def _():
                cp_x(3).wait()
                cp_wb(2).wait()
                for j in range(2, 8):
                    cp_wob(j).wait()
            xu = _pack(xn_v[0:TA, :])
            lnc = ln_chunks(((i + 1) % NA) * TA, 0, TA)
            mixed = [c for pair in zip(prep_chunks(i), lnc) for c in pair]
            if not CFG['side']:
                mixed = mixed[:1]
            side = _spread(mixed, 24, 0, CFG['shi'])
            at = Attn(i)
            fe = CFG['fence_every']
            yprev = None
            for u in range(24):
                t, kind = u // 3, u % 3
                if u == 23:
                    at.issue(CFG['look'])
                fen = fence_side(zero) if (u >= 3 and u % fe == fe - 1) else None
                if u >= 2 and CFG['efence']:
                    f2 = (fence_k, fence_v, fence_q)[(u - 2) % 3](zero)
                    fen = f2 if fen is None else fen | f2
                lhs = xu if fen is None else with_fence(xu, fen)
                y = _dot(_unpack(lhs), _unpack(wap[(8, 16, 0)[kind] + t]))
                if kind == 0:
                    kp = _pack(y.astype(BF))
                    full = jnp.concatenate([kt_v[t], kp], axis=0)
                    kt_v[t] = kp[80:128]
                    build_k4(full, t, pl.multiple_of(i * (TA // 2), TA // 2))
                elif kind == 1:
                    store_t(y, vt_v, i * (TA // 128), t)
                else:
                    store_t(y * QSCALE, qt_v, 0, t)
                if yprev is not None:
                    release(yprev, side[u - 1])
                yprev = y
            while at.issued < 2 * H - CFG['tail']:
                at.issue()
                at.finish()
            o1 = _unpack(jnp.concatenate([oa0_v[t + zero] if CFG['opq'] & 1 else oa0_v[t] for t in range(4)], axis=1))
            part = []
            for u in range(8):
                at.issue(2)
                part.append(_dot(o1, _unpack(woap[u, 0:D // 4, :])))
                if u > 0:
                    at.finish(2)
            assert at.done == 2 * H
            o2 = _unpack(jnp.concatenate([oa1_v[t + zero] if CFG['opq'] & 2 else oa1_v[t] for t in range(4)], axis=1))
            r = pl.multiple_of(i * TA, TA)
            for c in range(4):
                w2 = jnp.concatenate([woap[2 * c, D // 4:, :], woap[2 * c + 1, D // 4:, :]], axis=1)
                y = _dot(o2, _unpack(w2))
                add_residual(r, TA, c * 256, (c + 1) * 256,
                             y + jnp.concatenate(part[2 * c:2 * c + 2], axis=1))
            return c_
        if CFG['a']:
            lax.fori_loop(1, NA, a_body, 0)

        for T in range(8):
            qk_v[8 + T, 0:HALO, :] = jnp.zeros((HALO, 128), F32)
            v_v[T, 0:HALO, :] = jnp.zeros((HALO, 128), F32)

        def b_body(i, c_):
            def send(k):
                for ii in range(NB):
                    @pl.when(jnp.logical_and(p == 1, i == ii))
                    def _():
                        cp_out(ii, k).start()
            xu = _pack(xn_v[0:TA, :])
            ln1 = ln_chunks(i * TB + 256, TA, 256)
            ln2 = ln_chunks(((i + 1) % NB) * TB, 0, TA)
            lg = [logit_b(i, zero, g * 8) for g in range(TB // 8)]
            pv = [pv_b(zero, g * 8) for g in range(TB // 8)]
            n0, n1, n2 = CFG['bn']
            fx = {u: (lambda: fence_xn(zero)) for u in CFG['bf']}
            proj_b(xu, 0, _both(_spread(ln1 + ln2, 48, 0, CFG['bln']),
                                _spread(_flat(lg[0:n0]), 48, 32, 48)), fx)
            xu1 = _pack(xn_v[pl.ds(pl.multiple_of(TA + zero * 32, 32), TA), :])
            mix0 = _merge(lg[n0:32], pv[0:32]) if CFG['bmix'] else lg[n0:32] + pv[0:32]
            proj_b(xu1, 256, _both(_spread(_flat(mix0), 48, 0, 32),
                                   _spread(_flat(lg[32:n1]), 48, 32, 48)), {})
            mix1 = _merge(lg[n1:64], pv[32:n2])
            out_b(i, 0, 256, _spread(_flat(mix1), 16))
            send(0)
            out_b(i, 256, 128, _spread(_flat(pv[n2:64]), 16, 0, CFG['bhi']))
            send(1)
            for T in range(8):
                qk_v[8 + T, 0:HALO, :] = qk_v[8 + T, TB:TB + HALO, :]
                v_v[T, 0:HALO, :] = v_v[T, TB:TB + HALO, :]
            out_b(i, 384, 128, [[]] * 16)
            send(2)
            return c_
        if CFG['b']:
            lax.fori_loop(0, NB, b_body, 0)
        return carry

    lax.fori_loop(0, 2, one_pass, 0)
    for i in range(NB):
        for k in range(len(OUT_PIECES)):
            cp_out(i, k).wait()


@jax.jit
def pallas_interleave_layers__sliding_block__sliding_local_dilated__prompt_kernel(
    A_x: jax.Array,
    A_wqkv: jax.Array,
    A_wo: jax.Array,
    B_x: jax.Array,
    B_wqkv: jax.Array,
    B_wo: jax.Array,
):
    del B_x
    x = A_x.reshape(S, D)
    any_spec = pl.BlockSpec(memory_space=pl.ANY)
    out = pl.pallas_call(
        _kernel,
        out_shape=jax.ShapeDtypeStruct((S, D), BF),
        in_specs=[any_spec] * 5,
        out_specs=any_spec,
        scratch_shapes=[
            pltpu.VMEM((S + 16, D), BF),
            pltpu.VMEM((3 * NC1, D, G1 * 128), BF),
            pltpu.VMEM((D, D), BF),
            pltpu.VMEM((D + 16, 3 * D), BF),
            pltpu.VMEM((9, D, 128), BF),
            pltpu.VMEM((24, D // 2, 128), U32),
            pltpu.VMEM((8, D // 2, 128), U32),
            pltpu.VMEM((9, 3 * D // 2, 128), U32),
            pltpu.VMEM((9, D // 2, 128), U32),
            pltpu.VMEM((128 * PITCH, 128), F32),
            pltpu.VMEM((2 * TA + 32, D), BF),
            pltpu.VMEM((9, TA // 2, 128), U32),
            pltpu.VMEM((8, 48, 128), U32),
            pltpu.VMEM((H, S // 2, 128), U32),
            pltpu.VMEM((3, D // 2, 128), U32),
            pltpu.VMEM((S // 128 + 1, D // 2, 128), U32),
            pltpu.VMEM((4, TA // 2, 128), U32),
            pltpu.VMEM((4, TA // 2, 128), U32),
            pltpu.VMEM((16, HALO + TB, 128), F32),
            pltpu.VMEM((8, HALO + TB, 128), F32),
            pltpu.VMEM((WB, TB, 128), F32),
            pltpu.VMEM((TB, D), BF),
            pltpu.VMEM((2, 8, 128), U32),
            pltpu.SemaphoreType.DMA((4,)),
            pltpu.SemaphoreType.DMA((3 * NC1,)),
            pltpu.SemaphoreType.DMA((1,)),
            pltpu.SemaphoreType.DMA((3,)),
            pltpu.SemaphoreType.DMA((8,)),
            pltpu.SemaphoreType.DMA((NB * len(OUT_PIECES),)),
        ],
        compiler_params=pltpu.CompilerParams(vmem_limit_bytes=100 * 1024 * 1024),
        name="interleave_attn",
    )(x, A_wqkv, A_wo, B_wqkv, B_wo)
    return out.reshape(1, S, D)
```

```python
import math

import jax
import jax.numpy as jnp
from jax import lax
import jax.experimental.pallas as pl
import jax.experimental.pallas.tpu as pltpu

BF = jnp.bfloat16
F32 = jnp.float32
U32 = jnp.uint32

S = 2048
D = 1024
H = 32
DH = 32
TA = 256
NA = S // TA
TB = 512
NB = S // TB
HALO = 16
WB = 8
NEG = -1e30
EPS = 1e-5
QSCALE = (DH ** -0.5) * math.log2(math.e)
NC1 = 4
G1 = 8 // NC1
PITCH = 36
OUT_PIECES = ((0, 256), (256, 128), (384, 128))

CFG = dict(first=1, a=1, b=1, look=3, side=1, fence_every=3, efence=2, shi=21, flook=5, k4early=0, fhi=13, ffence=16,
           bn=(16, 60, 54), bf=(), bln=28, bmix=1, bhi=11, lns=2, pns=2, newton=1, qf32=1, lsum=2, opq=1, k4t=0, tail=8, ord=0, cuts=(0, 5, 10, 14, 18))


def _dot(a, b):
    return jnp.dot(a, b, preferred_element_type=F32)


def _dot_nt(a, b):
    return lax.dot_general(a, b, (((1,), (1,)), ((), ())), preferred_element_type=F32)


def _pack(x_bf16):
    return pltpu.bitcast(x_bf16, U32)


def _unpack(x_u32):
    return pltpu.bitcast(x_u32, BF)


def _iota(shape, dim):
    return lax.broadcasted_iota(jnp.int32, shape, dim)


def _layernorm(x_bf16):
    x = x_bf16.astype(F32)
    m = jnp.sum(x, axis=1, keepdims=True) * (1.0 / D)
    xc = x - m
    v = jnp.sum(xc * xc, axis=1, keepdims=True) * (1.0 / D)
    return (xc * lax.rsqrt(v + EPS)).astype(BF)


def _recip(l):
    if not CFG['newton']:
        return pl.reciprocal(l, approx=False)
    r = pl.reciprocal(l, approx=True)
    return r * (2.0 - l * r)


def _spread(chunks, nslots, lo=0, hi=None):
    hi = nslots if hi is None else hi
    out = [[] for _ in range(nslots)]
    for u, c in enumerate(chunks):
        out[lo + u * (hi - lo) // len(chunks)].append(c)
    return out


def _merge(a, b):
    out = []
    for u in range(max(len(a), len(b))):
        out += a[u:u + 1] + b[u:u + 1]
    return out


def _flat(lists):
    return sum(lists, [])


def _both(*lists):
    return [sum(parts, []) for parts in zip(*lists)]


def _kernel(x_hbm, wa_hbm, woa_hbm, wb_hbm, wob_hbm, out_hbm,
            x_v, wa_v, woa_v, wb_v, wob_v, wap, woap, wbt, wobp, tmp, xn_v,
            k0_v, kt_v, k4_v, qt_v, vt_v, oa0_v, oa1_v, qk_v, v_v, e_v, ob_v, tk_v,
            sems):
    def cp_x(i):
        n = TA if i < 3 else S - 3 * TA
        return pltpu.make_async_copy(x_hbm.at[pl.ds(i * TA, n), :],
                                     x_v.at[pl.ds(i * TA, n), :], sems.at[i])

    def cp_wa(c):
        w = G1 * 128
        return [pltpu.make_async_copy(wa_hbm.at[:, pl.ds(part * D + c * w, w)],
                                      wa_v.at[3 * c + part], sems.at[5 + c])
                for part in range(3)]

    cp_woa = pltpu.make_async_copy(woa_hbm, woa_v, sems.at[1])

    def cp_wb(j):
        n = 128 if j < 2 else D - 256
        return pltpu.make_async_copy(wb_hbm.at[pl.ds(j * 128, n), :],
                                     wb_v.at[pl.ds(j * 128, n), :], sems.at[j + 1])

    def cp_wob(j):
        return pltpu.make_async_copy(wob_hbm.at[:, pl.ds(j * 128, 128)],
                                     wob_v.at[j], sems.at[min(j, 2) + 1])

    def cp_out(i, k):
        r0, n = OUT_PIECES[k]
        return pltpu.make_async_copy(x_v.at[pl.ds(i * TB + r0, n), :],
                                     out_hbm.at[pl.ds(i * TB + r0, n), :], sems.at[4])

    def release(y, chunks):
        n = len(chunks)
        nt = y.shape[1] // 128
        for u, run in enumerate(chunks):
            pos = (u * y.shape[0] * nt // n) // 16 * 16
            t, rr = pos // y.shape[0], pos % y.shape[0]
            run(y[rr:rr + 16, t * 128:(t + 1) * 128])

    def fence_xn(zero):
        return _pack(xn_v[pl.ds(pl.multiple_of(2 * TA + zero * 32, 32), 32), 0:128])

    def fence_side(zero):
        return fence_xn(zero) | wbt[8, 0:16, :] | wobp[8, 0:16, :]

    def fence_k(zero):
        return k4_v[zero, 0:16, :]

    def fence_q(zero):
        return qt_v[2 + zero, 0:16, :]

    def fence_v(zero):
        return vt_v[S // 128 + zero, 0:16, :]

    def gate(tok, zero):
        tk_v[1] = pltpu.bitcast(tok[0:8], U32)
        return tk_v[zero]

    def with_fence(xu, fen):
        r, c = xu.shape
        last = jnp.concatenate([xu[r - 16:, :c - 128], xu[r - 16:, c - 128:] | fen], axis=1)
        return jnp.concatenate([xu[:r - 16], last], axis=0)

    def ln_chunks(row0, dst, nrows, step=16):
        def mk(c):
            def run(tok):
                if tok is not None:
                    x_v[S:S + 16, 0:128] = tok.astype(BF)
                r = pl.multiple_of(row0 + c * step, step)
                xn_v[dst + c * step:dst + (c + 1) * step, :] = _layernorm(x_v[pl.ds(r, step), :])
            return run
        return [mk(c) for c in range(nrows // step)]

    def prep_chunks(j):
        def permute(part):
            rows = [tmp[pl.ds(part * H * PITCH + d, H, stride=PITCH), :] for d in range(DH)]
            val = _pack(jnp.concatenate(rows, axis=0).astype(BF))
            if part < 3:
                wbt[j, part * (D // 2):(part + 1) * (D // 2), :] = val
            else:
                wobp[j] = val

        def mk_t(c):
            def run(tok):
                wb_v[D:D + 16, 0:128] = tok.astype(BF)
                rows = pl.ds(pl.multiple_of(j * 128, 128), 128)
                wt = wb_v[rows, c * 256:(c + 1) * 256].T.astype(F32)
                for hh in range(8):
                    o = (c * 8 + hh) * PITCH
                    tmp[o:o + DH, :] = wt[hh * DH:(hh + 1) * DH]
                if c % 4 == 3:
                    permute(c // 4)
            return run

        def mk_o(c):
            def run(tok):
                wob_v[8, 0:16, :] = tok.astype(BF)
                w = wob_v[j, c * 256:(c + 1) * 256, :].astype(F32)
                for hh in range(8):
                    o = (96 + c * 8 + hh) * PITCH
                    tmp[o:o + DH, :] = w[hh * DH:(hh + 1) * DH]
                if c == 3:
                    permute(3)
            return run
        return [mk_t(c) for c in range(12)] + [mk_o(c) for c in range(4)]

    def tri_mask():
        return _iota((128, 128), 1) >= _iota((128, 128), 0)

    def build_k4(full, t, row0):
        n = full.shape[0] - 48
        if CFG['k4t'] and n == 128:
            xt = [_pack(_unpack(full[16 * g:16 * g + n]).T) for g in range(4)]
            for a in range(4):
                za = jnp.concatenate([xt[g][16 * a:16 * a + 16] for g in range(4)], axis=0)
                k4_v[4 * t + a, pl.ds(row0, n), :] = _pack(_unpack(za).T)
            return
        rolled = [full] + [pltpu.roll(full, 32 * r, 1) for r in range(1, 4)]
        grp_id = _iota((n, 128), 1) // 32
        for a in range(4):
            val = rolled[(0 - a) % 4][0:n]
            for g in range(1, 4):
                val = jnp.where(grp_id == g, rolled[(g - a) % 4][16 * g:16 * g + n], val)
            k4_v[4 * t + a, pl.ds(row0, n), :] = val

    def store_t(y, dst, slot0, t):
        yt = _pack(y.astype(BF).T)
        rows = pl.ds(t * 64 if isinstance(t, int) else pl.multiple_of(t * 64, 64), 64)
        for b in range(TA // 128):
            dst[slot0 + b, rows, :] = yt[:, b * 128:(b + 1) * 128]

    def scores_first(qb, h):
        z = jnp.zeros((16, 128), U32)
        qh = qt_v[qb, h * 16:(h + 1) * 16, :]
        wq = _unpack(jnp.concatenate([qh if jj == h % 4 else z for jj in range(4)], axis=0))
        n = (qb + 1) * 16
        s = jnp.concatenate(
            [_dot(_unpack(k0_v[h // 4, c * n:(c + 1) * n, :]), wq) for c in range(4)], axis=0)
        diag = jnp.where(tri_mask(), s[qb * 128:], NEG)
        return diag if qb == 0 else jnp.concatenate([s[0:128], diag], axis=0)

    def scores_a(m, qb, h):
        qh = qt_v[qb, h * 16:(h + 1) * 16, :]
        if CFG['qf32']:
            qf = _unpack(qh).astype(F32)
            grp_id = _iota((32, 128), 1) // 32
            wq = jnp.concatenate(
                [jnp.where(grp_id == g, qf, 0.0) for g in range(4)], axis=0).astype(BF)
        else:
            grp_id = _iota((16, 128), 1) // 32
            z = jnp.zeros((16, 128), U32)
            wq = _unpack(jnp.concatenate(
                [jnp.where(grp_id == g, qh, z) for g in range(4)], axis=0))
        base = pl.multiple_of(m * 64 - 80, 16)
        order = {0: [0, 16, 1, 17] + list(range(2, 16)),
                 1: [16, 0, 2, 4, 6, 8, 10, 12, 14, 17, 1, 3, 5, 7, 9, 11, 13, 15],
                 2: list(range(15, 1, -1)) + [17, 1, 16, 0],
                 3: [16, 0, 4, 8, 12, 2, 6, 10, 14, 17, 1, 5, 9, 13, 3, 7, 11, 15]}[CFG['ord']]
        cuts = CFG['cuts']
        units = {}
        for c in range(len(cuts) - 1):
            idx = order[cuts[c]:cuts[c + 1]]
            lhs = jnp.concatenate([k4_v[h, pl.ds(base + u * 8, 8), :] for u in idx], axis=0)
            s = _dot(_unpack(lhs), wq)
            for n, u in enumerate(idx):
                units[u] = s[n * 16:(n + 1) * 16]
        for u in range(2):
            new = (_iota((16, 128), 1) % 32) >= (_iota((16, 128), 0) + u * 16)
            units[u] = jnp.where(new, units[16 + u], units[u])
        return jnp.concatenate([units[u] for u in range(16)], axis=0)

    def finish_a(s, m, h):
        skewed = not isinstance(m, int)
        mx = jnp.max(s, axis=0, keepdims=True)
        if skewed:
            lane = _iota((256, 128), 1)
            s = jnp.where((lane // 32) % 2 == 1,
                          jnp.concatenate([s[224:], s[:224]], axis=0), s)
            s = jnp.where(lane >= 64, jnp.concatenate([s[192:], s[:192]], axis=0), s)
        p = jnp.exp2(s - mx)
        nv = p.shape[0] // 8
        if CFG['lsum'] == 0 or not skewed:
            l = jnp.sum(p, axis=0, keepdims=True)
        else:
            pieces = [p[8 * v:8 * v + 8] for v in range(nv)]
            if CFG['lsum'] == 1:
                orders = [[v for t in range(nv // 16) for v in range(16 * t + 15, 16 * t - 1, -1)]]
            elif CFG['lsum'] == 2:
                orders = [list(range(16 * t + 15, 16 * t - 1, -1)) for t in range(nv // 16)]
            elif CFG['lsum'] == 3:
                pieces = [pieces[2 * v] + pieces[2 * v + 1] for v in range(nv // 2)]
                orders = [list(range(8 * t + 7, 8 * t - 1, -1)) for t in range(nv // 16)]
            elif CFG['lsum'] == 4:
                orders = [list(range(nv - 1, -1, -1))]
            accs = []
            for od in orders:
                acc = pieces[od[0]]
                for v in od[1:]:
                    acc = acc + pieces[v]
                accs.append(acc)
            l = jnp.sum(sum(accs[1:], accs[0]), axis=0, keepdims=True)
        if skewed:
            tri = tri_mask()
            pm = p[0:128]
            p = jnp.concatenate(
                [jnp.where(tri, 0.0, pm), p[128:256], jnp.where(tri, pm, 0.0)], axis=0)
        ntile = p.shape[0] // 128
        vv = _unpack(jnp.concatenate(
            [vt_v[m - bk, h * 16:(h + 1) * 16, :] for bk in range(ntile - 1, -1, -1)], axis=1))
        o = _dot(vv, p.astype(BF))
        return o * _recip(l)

    class Attn:
        def __init__(self, blk):
            self.blk = blk
            self.items = [(qb, 4 * t + a) for t in range(8) for qb in range(2) for a in range(4)]
            self.issued, self.done, self.queue, self.outs = 0, 0, [], []

        def issue(self, n=1):
            for _ in range(n):
                if self.issued < len(self.items):
                    qb, h = self.items[self.issued]
                    if isinstance(self.blk, int):
                        self.queue.append(scores_first(qb, h))
                    else:
                        self.queue.append(scores_a(self.blk * (TA // 128) + qb, qb, h))
                    self.issued += 1

        def finish(self, n=1):
            for _ in range(n):
                if self.done < self.issued:
                    qb, h = self.items[self.done]
                    self.outs.append(finish_a(self.queue.pop(0), self.blk * (TA // 128) + qb, h))
                    if len(self.outs) == 4:
                        ot = jnp.concatenate(self.outs, axis=0).astype(BF)
                        (oa0_v, oa1_v)[h // 16][(h // 4) % 4, qb * 64:(qb + 1) * 64, :] = _pack(ot.T)
                        self.last, self.outs = self.outs[-1], []
                    self.done += 1

    def add_residual(r, nrows, c0, c1, y):
        x_v[pl.ds(r, nrows), c0:c1] = (x_v[pl.ds(r, nrows), c0:c1].astype(F32) + y).astype(BF)

    def proj_b(xu, r0, side, fences):
        nrows = 2 * xu.shape[0]
        for T in range(24):
            y = None
            for hf in range(2):
                u = 2 * T + hf
                w = _unpack(jnp.concatenate(
                    [wbt[j, T * 64:(T + 1) * 64, :] for j in range(4 * hf, 4 * hf + 4)], axis=1))
                lhs = xu[:, hf * 512:(hf + 1) * 512]
                if u in fences:
                    lhs = with_fence(lhs, fences[u]())
                yh = _dot_nt(_unpack(lhs), w)
                y = yh if y is None else y + yh
                if hf == 1:
                    if T < 8:
                        qk_v[T, HALO + r0:HALO + r0 + nrows, :] = y * QSCALE
                    elif T < 16:
                        qk_v[T, HALO + r0:HALO + r0 + nrows, :] = y
                    else:
                        v_v[T - 16, HALO + r0:HALO + r0 + nrows, :] = y
                release(y, side[u])

    def gated(x, g):
        return pltpu.bitcast(pltpu.bitcast(x, U32) | g, F32)

    def logit_b(i, zero, r0):
        R = 8
        ns = CFG['lns']
        accs = [None] * WB

        def mk(st):
            def run(tok):
                g = gate(tok, zero)
                for t in range(st * 8 // ns, (st + 1) * 8 // ns):
                    q = gated(qk_v[t, HALO + r0:HALO + r0 + R, :], g)
                    for w in range(WB):
                        o = HALO + r0 - 2 * w
                        p = q * qk_v[8 + t, o:o + R, :]
                        accs[w] = p if accs[w] is None else accs[w] + p
                if st + 1 < ns:
                    return
                ls = []
                for w in range(WB):
                    a = accs[w]
                    a = a + pltpu.roll(a, 64, 1)
                    a = a + pltpu.roll(a, 32, 1)
                    if r0 - 2 * w < 0:
                        a = jnp.where(_iota((R, 128), 0) + (i * TB + r0 - 2 * w) >= 0, a, NEG)
                    ls.append(a)
                mx = ls[0]
                for w in range(1, WB):
                    mx = jnp.maximum(mx, ls[w])
                es = [jnp.exp2(l - mx) for l in ls]
                s = es[0]
                for w in range(1, WB):
                    s = s + es[w]
                inv = _recip(s)
                for w in range(WB):
                    e_v[w, r0:r0 + R, :] = es[w] * inv
            return run
        return [mk(st) for st in range(ns)]

    def pv_b(zero, r0):
        R = 8
        ns = CFG['pns']

        def mk(st):
            def run(tok):
                g = gate(tok, zero)
                es = [gated(e_v[w, r0:r0 + R, :], g) for w in range(WB)]
                os_ = []
                t0, t1 = st * 8 // ns, (st + 1) * 8 // ns
                for t in range(t0, t1):
                    acc = None
                    for w in range(WB):
                        o = HALO + r0 - 2 * w
                        pv = es[w] * v_v[t, o:o + R, :]
                        acc = pv if acc is None else acc + pv
                    os_.append(acc)
                ob_v[r0:r0 + R, t0 * 128:t1 * 128] = jnp.concatenate(os_, axis=1).astype(BF)
            return run
        return [mk(st) for st in range(ns)]

    def out_b(i, r0, nrows, side):
        o = ob_v[r0:r0 + nrows, :]
        r = pl.multiple_of(i * TB + r0, 128)
        ys = []
        for T in range(8):
            y = None
            for hf in range(2):
                yh = _dot(o[:, hf * 512:(hf + 1) * 512],
                          _unpack(wobp[T, hf * 256:(hf + 1) * 256, :]))
                y = yh if y is None else y + yh
                release(y, side[2 * T + hf])
            ys.append(y)
            if T % 2 == 1:
                add_residual(r, nrows, (T - 1) * 128, (T + 1) * 128,
                             jnp.concatenate(ys[-2:], axis=1))

    cp_x(0).start()
    for cp in cp_wa(0):
        cp.start()
    z16 = jnp.zeros((16, 128), U32)
    xn_v[2 * TA:2 * TA + 32, :] = jnp.zeros((32, D), BF)
    wbt[8, 0:16, :] = z16
    wobp[8, 0:16, :] = z16
    k4_v[0, 0:16, :] = z16
    vt_v[S // 128, 0:16, :] = z16
    qt_v[2, 0:16, :] = z16
    tk_v[0] = z16[0:8]
    cp_x(0).wait()
    for cp in cp_wa(1):
        cp.start()
    for run in ln_chunks(0, 0, TA, step=TA):
        run(None)

    def one_pass(p, carry):
        first = p == 0
        zero = p // 4

        def f_body(c, c_):
            for k in range(NC1):
                @pl.when(jnp.logical_and(first, c == k))
                def _():
                    for cp in cp_wa(k):
                        cp.wait()
                    if k + 2 < NC1:
                        for cp in cp_wa(k + 2):
                            cp.start()
                    elif k + 2 == NC1:
                        cp_woa.start()
                    else:
                        cp_x(1).start()
                        cp_wb(0).start()
                        cp_wob(0).start()
            xn = xn_v[0:TA, :]
            for part in (2, 0, 1):
                wu = _pack(wa_v[3 * c + part])
                y = _dot(xn, _unpack(wu))
                for g in range(G1):
                    t = c * G1 + g
                    wap[part * 8 + t] = wu[:, g * 128:(g + 1) * 128]
                    yt = y[:, g * 128:(g + 1) * 128]
                    if part == 0:
                        store_t(yt * QSCALE, qt_v, 0, t)
                    elif part == 2:
                        store_t(yt, vt_v, 0, t)
                    else:
                        k0_v[t] = _pack(yt.astype(BF))
            return c_

        def a_first():
            lax.fori_loop(0, NC1, f_body, 0)

            def mk_k4(t):
                def run(tok):
                    k0_v[8, 0:8, :] = pltpu.bitcast(tok[0:8], U32)
                    kp = k0_v[t + zero]
                    kt_v[t] = kp[80:128]
                    build_k4(kp, t, 48)
                return run
            k4c = [mk_k4(t) for t in range(8)]
            at = Attn(0)
            at.issue(CFG['flook'])
            while at.issued < 2 * H:
                at.issue()
                at.finish()
                if CFG['k4early'] and at.done % 7 == 1 and k4c:
                    k4c.pop(0)(at.outs[-1][0:16] if at.outs else at.last[0:16])

            @pl.when(first)
            def _():
                cp_woa.wait()
                cp_x(1).wait()
                cp_wb(0).wait()
                cp_wob(0).wait()
                cp_x(2).start()
                cp_wb(1).start()
                cp_wob(1).start()
            hi = CFG['fhi']
            side = _both(_spread(prep_chunks(zero), 16, 0, hi),
                         _spread(ln_chunks(TA + zero * TA, 0, TA), 16, 0, hi))
            if k4c:
                side = _both(side, _spread(k4c, 16, 0, hi))
            o1 = jnp.concatenate([oa0_v[t + zero] if CFG['opq'] & 1 else oa0_v[t] for t in range(4)], axis=1)
            part = []
            yprev = None
            for u in range(16):
                if u == 8:
                    o1 = jnp.concatenate([oa1_v[t + zero] if CFG['opq'] & 2 else oa1_v[t] for t in range(4)], axis=1)
                rows = slice((u // 8) * (D // 2), (u // 8 + 1) * (D // 2))
                wu = _pack(woa_v[rows, (u % 8) * 128:(u % 8 + 1) * 128])
                woap[u % 8, (u // 8) * (D // 4):(u // 8 + 1) * (D // 4), :] = wu
                ff = CFG['ffence']
                lhs = with_fence(o1, fence_side(zero) | fence_k(zero)) if (u % ff == ff - 1) else o1
                y = _dot(_unpack(lhs), _unpack(wu))
                if u == 0:
                    at.finish(2 * H)
                if yprev is not None:
                    release(yprev, side[u - 1])
                yprev = y
                if u < 8:
                    part.append(y)
                else:
                    part[u - 8] = part[u - 8] + y
                    if u % 2 == 1:
                        add_residual(0, TA, (u - 9) * 128, (u - 7) * 128,
                                     jnp.concatenate(part[u - 9:u - 7], axis=1))

        if CFG['first']:
            a_first()

        @pl.when(first)
        def _():
            cp_x(2).wait()
            cp_wb(1).wait()
            cp_wob(1).wait()
            cp_x(3).start()
            cp_wb(2).start()
            for j in range(2, 8):
                cp_wob(j).start()

        def a_body(i, c_):
            @pl.when(jnp.logical_and(first, i == 2))
            def _():
                cp_x(3).wait()
                cp_wb(2).wait()
                for j in range(2, 8):
                    cp_wob(j).wait()
            xu = _pack(xn_v[0:TA, :])
            lnc = ln_chunks(((i + 1) % NA) * TA, 0, TA)
            mixed = [c for pair in zip(prep_chunks(i), lnc) for c in pair]
            if not CFG['side']:
                mixed = mixed[:1]
            side = _spread(mixed, 24, 0, CFG['shi'])
            at = Attn(i)
            fe = CFG['fence_every']
            yprev = None
            for u in range(24):
                t, kind = u // 3, u % 3
                if u == 23:
                    at.issue(CFG['look'])
                fen = fence_side(zero) if (u >= 3 and u % fe == fe - 1) else None
                if u >= 2 and CFG['efence']:
                    f2 = (fence_k, fence_v, fence_q)[(u - 2) % 3](zero)
                    fen = f2 if fen is None else fen | f2
                lhs = xu if fen is None else with_fence(xu, fen)
                y = _dot(_unpack(lhs), _unpack(wap[(8, 16, 0)[kind] + t]))
                if kind == 0:
                    kp = _pack(y.astype(BF))
                    full = jnp.concatenate([kt_v[t], kp], axis=0)
                    kt_v[t] = kp[80:128]
                    build_k4(full, t, pl.multiple_of(i * (TA // 2), TA // 2))
                elif kind == 1:
                    store_t(y, vt_v, i * (TA // 128), t)
                else:
                    store_t(y * QSCALE, qt_v, 0, t)
                if yprev is not None:
                    release(yprev, side[u - 1])
                yprev = y
            while at.issued < 2 * H - CFG['tail']:
                at.issue()
                at.finish()
            o1 = _unpack(jnp.concatenate([oa0_v[t + zero] if CFG['opq'] & 1 else oa0_v[t] for t in range(4)], axis=1))
            part = []
            for u in range(8):
                at.issue(2)
                part.append(_dot(o1, _unpack(woap[u, 0:D // 4, :])))
                if u > 0:
                    at.finish(2)
            assert at.done == 2 * H
            o2 = _unpack(jnp.concatenate([oa1_v[t + zero] if CFG['opq'] & 2 else oa1_v[t] for t in range(4)], axis=1))
            r = pl.multiple_of(i * TA, TA)
            for c in range(4):
                w2 = jnp.concatenate([woap[2 * c, D // 4:, :], woap[2 * c + 1, D // 4:, :]], axis=1)
                y = _dot(o2, _unpack(w2))
                add_residual(r, TA, c * 256, (c + 1) * 256,
                             y + jnp.concatenate(part[2 * c:2 * c + 2], axis=1))
            return c_
        if CFG['a']:
            lax.fori_loop(1, NA, a_body, 0)

        for T in range(8):
            qk_v[8 + T, 0:HALO, :] = jnp.zeros((HALO, 128), F32)
            v_v[T, 0:HALO, :] = jnp.zeros((HALO, 128), F32)

        def b_body(i, c_):
            def send(k):
                for ii in range(NB):
                    @pl.when(jnp.logical_and(p == 1, i == ii))
                    def _():
                        cp_out(ii, k).start()
            xu = _pack(xn_v[0:TA, :])
            ln1 = ln_chunks(i * TB + 256, TA, 256)
            ln2 = ln_chunks(((i + 1) % NB) * TB, 0, TA)
            lg = [logit_b(i, zero, g * 8) for g in range(TB // 8)]
            pv = [pv_b(zero, g * 8) for g in range(TB // 8)]
            n0, n1, n2 = CFG['bn']
            fx = {u: (lambda: fence_xn(zero)) for u in CFG['bf']}
            proj_b(xu, 0, _both(_spread(ln1 + ln2, 48, 0, CFG['bln']),
                                _spread(_flat(lg[0:n0]), 48, 32, 48)), fx)
            xu1 = _pack(xn_v[pl.ds(pl.multiple_of(TA + zero * 32, 32), TA), :])
            mix0 = _merge(lg[n0:32], pv[0:32]) if CFG['bmix'] else lg[n0:32] + pv[0:32]
            proj_b(xu1, 256, _both(_spread(_flat(mix0), 48, 0, 32),
                                   _spread(_flat(lg[32:n1]), 48, 32, 48)), {})
            mix1 = _merge(lg[n1:64], pv[32:n2])
            out_b(i, 0, 256, _spread(_flat(mix1), 16))
            send(0)
            out_b(i, 256, 128, _spread(_flat(pv[n2:64]), 16, 0, CFG['bhi']))
            send(1)
            for T in range(8):
                qk_v[8 + T, 0:HALO, :] = qk_v[8 + T, TB:TB + HALO, :]
                v_v[T, 0:HALO, :] = v_v[T, TB:TB + HALO, :]
            out_b(i, 384, 128, [[]] * 16)
            send(2)
            return c_
        if CFG['b']:
            lax.fori_loop(0, NB, b_body, 0)
        return carry

    lax.fori_loop(0, 2, one_pass, 0)
    for i in range(NB):
        for k in range(len(OUT_PIECES)):
            cp_out(i, k).wait()


@jax.jit
def pallas_interleave_layers__sliding_block__sliding_local_dilated__prompt_kernel(
    A_x: jax.Array,
    A_wqkv: jax.Array,
    A_wo: jax.Array,
    B_x: jax.Array,
    B_wqkv: jax.Array,
    B_wo: jax.Array,
):
    del B_x
    x = A_x.reshape(S, D)
    any_spec = pl.BlockSpec(memory_space=pl.ANY)
    out = pl.pallas_call(
        _kernel,
        out_shape=jax.ShapeDtypeStruct((S, D), BF),
        in_specs=[any_spec] * 5,
        out_specs=any_spec,
        scratch_shapes=[
            pltpu.VMEM((S + 16, D), BF),
            pltpu.VMEM((3 * NC1, D, G1 * 128), BF),
            pltpu.VMEM((D, D), BF),
            pltpu.VMEM((D + 16, 3 * D), BF),
            pltpu.VMEM((9, D, 128), BF),
            pltpu.VMEM((24, D // 2, 128), U32),
            pltpu.VMEM((8, D // 2, 128), U32),
            pltpu.VMEM((9, 3 * D // 2, 128), U32),
            pltpu.VMEM((9, D // 2, 128), U32),
            pltpu.VMEM((128 * PITCH + 64, 128), F32),
            pltpu.VMEM((2 * TA + 32, D), BF),
            pltpu.VMEM((9, TA // 2, 128), U32),
            pltpu.VMEM((8, 48, 128), U32),
            pltpu.VMEM((H, S // 2, 128), U32),
            pltpu.VMEM((3, D // 2, 128), U32),
            pltpu.VMEM((S // 128 + 1, D // 2, 128), U32),
            pltpu.VMEM((4, TA // 2, 128), U32),
            pltpu.VMEM((4, TA // 2, 128), U32),
            pltpu.VMEM((16, HALO + TB, 128), F32),
            pltpu.VMEM((8, HALO + TB, 128), F32),
            pltpu.VMEM((WB, TB, 128), F32),
            pltpu.VMEM((TB, D), BF),
            pltpu.VMEM((4, 8, 128), U32),
            pltpu.SemaphoreType.DMA((5 + NC1,)),
        ],
        compiler_params=pltpu.CompilerParams(vmem_limit_bytes=100 * 1024 * 1024),
        name="interleave_attn",
    )(x, A_wqkv, A_wo, B_wqkv, B_wo)
    return out.reshape(1, S, D)
```

```python
import math

import jax
import jax.numpy as jnp
from jax import lax
import jax.experimental.pallas as pl
import jax.experimental.pallas.tpu as pltpu

BF = jnp.bfloat16
F32 = jnp.float32
U32 = jnp.uint32

S = 2048
D = 1024
H = 32
DH = 32
TA = 256
NA = S // TA
TB = 512
NB = S // TB
HALO = 16
WB = 8
NEG = -1e30
EPS = 1e-5
QSCALE = (DH ** -0.5) * math.log2(math.e)
NC1 = 4
G1 = 8 // NC1
OUT_PIECES = ((0, 256), (256, 128), (384, 128))

CFG = dict(first=1, a=1, b=1, look=3, efence=2,
           ppos=(1, 3, 6, 8, 11, 14, 30, 32), lpos=(1, 2, 4, 5, 7, 8, 10, 11, 13, 14, 16, 17, 19, 20, 20, 21),
           fpos=(5, 8, 11, 14, 17, 20, 23, 35),
           flook=5, k4early=0, fhi=13, ffence=16,
           bn=(16, 60, 54), bf=(), bln=28, bmix=1, bhi=11, lns=2, pns=2, newton=1, qf32=1, lsum=2, opq=1, k4t=0, tail=8, ord=0, cuts=(0, 5, 10, 14, 18))


def _dot(a, b):
    return jnp.dot(a, b, preferred_element_type=F32)


def _dot_nt(a, b):
    return lax.dot_general(a, b, (((1,), (1,)), ((), ())), preferred_element_type=F32)


def _pack(x_bf16):
    return pltpu.bitcast(x_bf16, U32)


def _unpack(x_u32):
    return pltpu.bitcast(x_u32, BF)


def _iota(shape, dim):
    return lax.broadcasted_iota(jnp.int32, shape, dim)


def _layernorm(x_bf16):
    x = x_bf16.astype(F32)
    m = jnp.sum(x, axis=1, keepdims=True) * (1.0 / D)
    xc = x - m
    v = jnp.sum(xc * xc, axis=1, keepdims=True) * (1.0 / D)
    return (xc * lax.rsqrt(v + EPS)).astype(BF)


def _recip(l):
    if not CFG['newton']:
        return pl.reciprocal(l, approx=False)
    r = pl.reciprocal(l, approx=True)
    return r * (2.0 - l * r)


def _swap16(vs):
    vs = list(vs)
    for a in range(0, 16, 2):
        x, y = vs[a], vs[a + 1]
        vs[a] = (x & U32(0xFFFF)) | (y << 16)
        vs[a + 1] = (x >> 16) | (y & U32(0xFFFF0000))
    sub = _iota((8, 128), 0)
    for dist in (1, 2, 4):
        lo = (sub & dist) == 0
        for a in range(16):
            if not a & (2 * dist):
                x, y = vs[a], vs[a + 2 * dist]
                vs[a] = jnp.where(lo, x, pltpu.roll(y, dist, 0))
                vs[a + 2 * dist] = jnp.where(lo, pltpu.roll(x, 8 - dist, 0), y)
    return vs


def _spread(chunks, nslots, lo=0, hi=None):
    hi = nslots if hi is None else hi
    out = [[] for _ in range(nslots)]
    for u, c in enumerate(chunks):
        out[lo + u * (hi - lo) // len(chunks)].append(c)
    return out


def _merge(a, b):
    out = []
    for u in range(max(len(a), len(b))):
        out += a[u:u + 1] + b[u:u + 1]
    return out


def _flat(lists):
    return sum(lists, [])


def _both(*lists):
    return [sum(parts, []) for parts in zip(*lists)]


def _kernel(x_hbm, wa_hbm, woa_hbm, wb_hbm, wob_hbm, out_hbm,
            x_v, wa_v, woa_v, wb_v, wob_v, wap, woap, wbt, wobp, xn_v,
            k0_v, kt_v, k4_v, qt_v, vt_v, oa0_v, oa1_v, qk_v, v_v, e_v, ob_v, tk_v,
            sems):
    def cp_x(i):
        n = TA if i < 3 else S - 3 * TA
        return pltpu.make_async_copy(x_hbm.at[pl.ds(i * TA, n), :],
                                     x_v.at[pl.ds(i * TA, n), :], sems.at[i])

    def cp_wa(c):
        w = G1 * 128
        return [pltpu.make_async_copy(wa_hbm.at[:, pl.ds(part * D + c * w, w)],
                                      wa_v.at[3 * c + part], sems.at[5 + c])
                for part in range(3)]

    cp_woa = pltpu.make_async_copy(woa_hbm, woa_v, sems.at[1])

    def cp_wb(j):
        n = 128 if j < 2 else D - 256
        return pltpu.make_async_copy(wb_hbm.at[pl.ds(j * 128, n), :],
                                     wb_v.at[pl.ds(j * 128, n), :], sems.at[j + 1])

    def cp_wob(j):
        return pltpu.make_async_copy(wob_hbm.at[:, pl.ds(j * 128, 128)],
                                     wob_v.at[j], sems.at[min(j, 2) + 1])

    def cp_out(i, k):
        r0, n = OUT_PIECES[k]
        return pltpu.make_async_copy(x_v.at[pl.ds(i * TB + r0, n), :],
                                     out_hbm.at[pl.ds(i * TB + r0, n), :], sems.at[4])

    def release(y, chunks):
        n = len(chunks)
        nt = y.shape[1] // 128
        for u, run in enumerate(chunks):
            pos = (u * y.shape[0] * nt // n) // 16 * 16
            t, rr = pos // y.shape[0], pos % y.shape[0]
            run(y[rr:rr + 16, t * 128:(t + 1) * 128])

    def fence_xn(zero):
        return _pack(xn_v[pl.ds(pl.multiple_of(2 * TA + zero * 32, 32), 32), 0:128])

    def fence_side(zero):
        return fence_xn(zero) | wbt[8, 0:16, :] | wobp[8, 0:16, :]

    def fence_k(zero):
        return k4_v[zero, 0:16, :]

    def fence_q(zero):
        return qt_v[2 + zero, 0:16, :]

    def fence_v(zero):
        return vt_v[S // 128 + zero, 0:16, :]

    def gate(tok, zero):
        tk_v[1] = pltpu.bitcast(tok[0:8], U32)
        return tk_v[zero]

    def with_fence(xu, fen):
        r, c = xu.shape
        last = jnp.concatenate([xu[r - 16:, :c - 128], xu[r - 16:, c - 128:] | fen], axis=1)
        return jnp.concatenate([xu[:r - 16], last], axis=0)

    def ln_chunks(row0, dst, nrows, step=16):
        def mk(c):
            def run(tok):
                if tok is not None:
                    x_v[S:S + 16, 0:128] = tok.astype(BF)
                r = pl.multiple_of(row0 + c * step, step)
                xn_v[dst + c * step:dst + (c + 1) * step, :] = _layernorm(x_v[pl.ds(r, step), :])
            return run
        return [mk(c) for c in range(nrows // step)]

    def prep_chunks(j):
        def put(xu, dst, base, hh):
            for dh in range(2):
                grp = _swap16([xu[(2 * h + dh) * 8:(2 * h + dh + 1) * 8] for h in range(16)])
                for d in range(16):
                    o = base + ((dh * 16 + d) * 2 + hh) * 8
                    dst[j, o:o + 8, :] = grp[d]

        def mk_t(c):
            def run(tok):
                wb_v[D:D + 16, 0:128] = tok.astype(BF)
                rows = pl.ds(pl.multiple_of(j * 128, 128), 128)
                put(_pack(wb_v[rows, c * 512:(c + 1) * 512].T), wbt, (c // 2) * (D // 2), c % 2)
            return run

        def mk_o(c):
            def run(tok):
                wob_v[8, 0:16, :] = tok.astype(BF)
                put(_pack(wob_v[j, c * 512:(c + 1) * 512, :]), wobp, 0, c)
            return run
        return [mk_t(c) for c in range(6)] + [mk_o(c) for c in range(2)]

    def tri_mask():
        return _iota((128, 128), 1) >= _iota((128, 128), 0)

    def build_k4(full, t, row0):
        n = full.shape[0] - 48
        if CFG['k4t'] and n == 128:
            xt = [_pack(_unpack(full[16 * g:16 * g + n]).T) for g in range(4)]
            for a in range(4):
                za = jnp.concatenate([xt[g][16 * a:16 * a + 16] for g in range(4)], axis=0)
                k4_v[4 * t + a, pl.ds(row0, n), :] = _pack(_unpack(za).T)
            return
        rolled = [full] + [pltpu.roll(full, 32 * r, 1) for r in range(1, 4)]
        grp_id = _iota((n, 128), 1) // 32
        for a in range(4):
            val = rolled[(0 - a) % 4][0:n]
            for g in range(1, 4):
                val = jnp.where(grp_id == g, rolled[(g - a) % 4][16 * g:16 * g + n], val)
            k4_v[4 * t + a, pl.ds(row0, n), :] = val

    def store_t(y, dst, slot0, t):
        yt = _pack(y.astype(BF).T)
        rows = pl.ds(t * 64 if isinstance(t, int) else pl.multiple_of(t * 64, 64), 64)
        for b in range(TA // 128):
            dst[slot0 + b, rows, :] = yt[:, b * 128:(b + 1) * 128]

    def scores_first(qb, h):
        z = jnp.zeros((16, 128), U32)
        qh = qt_v[qb, h * 16:(h + 1) * 16, :]
        wq = _unpack(jnp.concatenate([qh if jj == h % 4 else z for jj in range(4)], axis=0))
        n = (qb + 1) * 16
        s = jnp.concatenate(
            [_dot(_unpack(k0_v[h // 4, c * n:(c + 1) * n, :]), wq) for c in range(4)], axis=0)
        diag = jnp.where(tri_mask(), s[qb * 128:], NEG)
        return diag if qb == 0 else jnp.concatenate([s[0:128], diag], axis=0)

    def scores_a(m, qb, h):
        qh = qt_v[qb, h * 16:(h + 1) * 16, :]
        if CFG['qf32']:
            qf = _unpack(qh).astype(F32)
            grp_id = _iota((32, 128), 1) // 32
            wq = jnp.concatenate(
                [jnp.where(grp_id == g, qf, 0.0) for g in range(4)], axis=0).astype(BF)
        else:
            grp_id = _iota((16, 128), 1) // 32
            z = jnp.zeros((16, 128), U32)
            wq = _unpack(jnp.concatenate(
                [jnp.where(grp_id == g, qh, z) for g in range(4)], axis=0))
        base = pl.multiple_of(m * 64 - 80, 16)
        order = {0: [0, 16, 1, 17] + list(range(2, 16)),
                 1: [16, 0, 2, 4, 6, 8, 10, 12, 14, 17, 1, 3, 5, 7, 9, 11, 13, 15],
                 2: list(range(15, 1, -1)) + [17, 1, 16, 0],
                 3: [16, 0, 4, 8, 12, 2, 6, 10, 14, 17, 1, 5, 9, 13, 3, 7, 11, 15]}[CFG['ord']]
        cuts = CFG['cuts']
        units = {}
        for c in range(len(cuts) - 1):
            idx = order[cuts[c]:cuts[c + 1]]
            lhs = jnp.concatenate([k4_v[h, pl.ds(base + u * 8, 8), :] for u in idx], axis=0)
            s = _dot(_unpack(lhs), wq)
            for n, u in enumerate(idx):
                units[u] = s[n * 16:(n + 1) * 16]
        for u in range(2):
            new = (_iota((16, 128), 1) % 32) >= (_iota((16, 128), 0) + u * 16)
            units[u] = jnp.where(new, units[16 + u], units[u])
        return jnp.concatenate([units[u] for u in range(16)], axis=0)

    def finish_a(s, m, h):
        skewed = not isinstance(m, int)
        mx = jnp.max(s, axis=0, keepdims=True)
        if skewed:
            lane = _iota((256, 128), 1)
            s = jnp.where((lane // 32) % 2 == 1,
                          jnp.concatenate([s[224:], s[:224]], axis=0), s)
            s = jnp.where(lane >= 64, jnp.concatenate([s[192:], s[:192]], axis=0), s)
        p = jnp.exp2(s - mx)
        nv = p.shape[0] // 8
        if CFG['lsum'] == 0 or not skewed:
            l = jnp.sum(p, axis=0, keepdims=True)
        else:
            pieces = [p[8 * v:8 * v + 8] for v in range(nv)]
            if CFG['lsum'] == 1:
                orders = [[v for t in range(nv // 16) for v in range(16 * t + 15, 16 * t - 1, -1)]]
            elif CFG['lsum'] == 2:
                orders = [list(range(16 * t + 15, 16 * t - 1, -1)) for t in range(nv // 16)]
            elif CFG['lsum'] == 3:
                pieces = [pieces[2 * v] + pieces[2 * v + 1] for v in range(nv // 2)]
                orders = [list(range(8 * t + 7, 8 * t - 1, -1)) for t in range(nv // 16)]
            elif CFG['lsum'] == 4:
                orders = [list(range(nv - 1, -1, -1))]
            accs = []
            for od in orders:
                acc = pieces[od[0]]
                for v in od[1:]:
                    acc = acc + pieces[v]
                accs.append(acc)
            l = jnp.sum(sum(accs[1:], accs[0]), axis=0, keepdims=True)
        if skewed:
            tri = tri_mask()
            pm = p[0:128]
            p = jnp.concatenate(
                [jnp.where(tri, 0.0, pm), p[128:256], jnp.where(tri, pm, 0.0)], axis=0)
        ntile = p.shape[0] // 128
        vv = _unpack(jnp.concatenate(
            [vt_v[m - bk, h * 16:(h + 1) * 16, :] for bk in range(ntile - 1, -1, -1)], axis=1))
        o = _dot(vv, p.astype(BF))
        return o * _recip(l)

    class Attn:
        def __init__(self, blk):
            self.blk = blk
            self.items = [(qb, 4 * t + a) for t in range(8) for qb in range(2) for a in range(4)]
            self.issued, self.done, self.queue, self.outs = 0, 0, [], []

        def issue(self, n=1):
            for _ in range(n):
                if self.issued < len(self.items):
                    qb, h = self.items[self.issued]
                    if isinstance(self.blk, int):
                        self.queue.append(scores_first(qb, h))
                    else:
                        self.queue.append(scores_a(self.blk * (TA // 128) + qb, qb, h))
                    self.issued += 1

        def finish(self, n=1):
            for _ in range(n):
                if self.done < self.issued:
                    qb, h = self.items[self.done]
                    self.outs.append(finish_a(self.queue.pop(0), self.blk * (TA // 128) + qb, h))
                    if len(self.outs) == 4:
                        ot = jnp.concatenate(self.outs, axis=0).astype(BF)
                        (oa0_v, oa1_v)[h // 16][(h // 4) % 4, qb * 64:(qb + 1) * 64, :] = _pack(ot.T)
                        self.last, self.outs = self.outs[-1], []
                    self.done += 1

    def add_residual(r, nrows, c0, c1, y):
        x_v[pl.ds(r, nrows), c0:c1] = (x_v[pl.ds(r, nrows), c0:c1].astype(F32) + y).astype(BF)

    def proj_b(xu, r0, side, fences):
        nrows = 2 * xu.shape[0]
        for T in range(24):
            y = None
            for hf in range(2):
                u = 2 * T + hf
                w = _unpack(jnp.concatenate(
                    [wbt[j, T * 64:(T + 1) * 64, :] for j in range(4 * hf, 4 * hf + 4)], axis=1))
                lhs = xu[:, hf * 512:(hf + 1) * 512]
                if u in fences:
                    lhs = with_fence(lhs, fences[u]())
                yh = _dot_nt(_unpack(lhs), w)
                y = yh if y is None else y + yh
                if hf == 1:
                    if T < 8:
                        qk_v[T, HALO + r0:HALO + r0 + nrows, :] = y * QSCALE
                    elif T < 16:
                        qk_v[T, HALO + r0:HALO + r0 + nrows, :] = y
                    else:
                        v_v[T - 16, HALO + r0:HALO + r0 + nrows, :] = y
                release(y, side[u])

    def gated(x, g):
        return pltpu.bitcast(pltpu.bitcast(x, U32) | g, F32)

    def logit_b(i, zero, r0):
        R = 8
        ns = CFG['lns']
        accs = [None] * WB

        def mk(st):
            def run(tok):
                g = gate(tok, zero)
                for t in range(st * 8 // ns, (st + 1) * 8 // ns):
                    q = gated(qk_v[t, HALO + r0:HALO + r0 + R, :], g)
                    for w in range(WB):
                        o = HALO + r0 - 2 * w
                        p = q * qk_v[8 + t, o:o + R, :]
                        accs[w] = p if accs[w] is None else accs[w] + p
                if st + 1 < ns:
                    return
                ls = []
                for w in range(WB):
                    a = accs[w]
                    a = a + pltpu.roll(a, 64, 1)
                    a = a + pltpu.roll(a, 32, 1)
                    if r0 - 2 * w < 0:
                        a = jnp.where(_iota((R, 128), 0) + (i * TB + r0 - 2 * w) >= 0, a, NEG)
                    ls.append(a)
                mx = ls[0]
                for w in range(1, WB):
                    mx = jnp.maximum(mx, ls[w])
                es = [jnp.exp2(l - mx) for l in ls]
                s = es[0]
                for w in range(1, WB):
                    s = s + es[w]
                inv = _recip(s)
                for w in range(WB):
                    e_v[w, r0:r0 + R, :] = es[w] * inv
            return run
        return [mk(st) for st in range(ns)]

    def pv_b(zero, r0):
        R = 8
        ns = CFG['pns']

        def mk(st):
            def run(tok):
                g = gate(tok, zero)
                es = [gated(e_v[w, r0:r0 + R, :], g) for w in range(WB)]
                os_ = []
                t0, t1 = st * 8 // ns, (st + 1) * 8 // ns
                for t in range(t0, t1):
                    acc = None
                    for w in range(WB):
                        o = HALO + r0 - 2 * w
                        pv = es[w] * v_v[t, o:o + R, :]
                        acc = pv if acc is None else acc + pv
                    os_.append(acc)
                ob_v[r0:r0 + R, t0 * 128:t1 * 128] = jnp.concatenate(os_, axis=1).astype(BF)
            return run
        return [mk(st) for st in range(ns)]

    def out_b(i, r0, nrows, side):
        o = ob_v[r0:r0 + nrows, :]
        r = pl.multiple_of(i * TB + r0, 128)
        ys = []
        for T in range(8):
            y = None
            for hf in range(2):
                yh = _dot(o[:, hf * 512:(hf + 1) * 512],
                          _unpack(wobp[T, hf * 256:(hf + 1) * 256, :]))
                y = yh if y is None else y + yh
                release(y, side[2 * T + hf])
            ys.append(y)
            if T % 2 == 1:
                add_residual(r, nrows, (T - 1) * 128, (T + 1) * 128,
                             jnp.concatenate(ys[-2:], axis=1))

    cp_x(0).start()
    for cp in cp_wa(0):
        cp.start()
    z16 = jnp.zeros((16, 128), U32)
    xn_v[2 * TA:2 * TA + 32, :] = jnp.zeros((32, D), BF)
    wbt[8, 0:16, :] = z16
    wobp[8, 0:16, :] = z16
    k4_v[0, 0:16, :] = z16
    vt_v[S // 128, 0:16, :] = z16
    qt_v[2, 0:16, :] = z16
    tk_v[0] = z16[0:8]
    cp_x(0).wait()
    for cp in cp_wa(1):
        cp.start()
    for run in ln_chunks(0, 0, TA, step=TA):
        run(None)

    def one_pass(p, carry):
        first = p == 0
        zero = p // 4

        def f_body(c, c_):
            for k in range(NC1):
                @pl.when(jnp.logical_and(first, c == k))
                def _():
                    for cp in cp_wa(k):
                        cp.wait()
                    if k + 2 < NC1:
                        for cp in cp_wa(k + 2):
                            cp.start()
                    elif k + 2 == NC1:
                        cp_woa.start()
                    else:
                        cp_x(1).start()
                        cp_wb(0).start()
                        cp_wob(0).start()
            xn = xn_v[0:TA, :]
            for part in (2, 0, 1):
                wu = _pack(wa_v[3 * c + part])
                y = _dot(xn, _unpack(wu))
                for g in range(G1):
                    t = c * G1 + g
                    wap[part * 8 + t] = wu[:, g * 128:(g + 1) * 128]
                    yt = y[:, g * 128:(g + 1) * 128]
                    if part == 0:
                        store_t(yt * QSCALE, qt_v, 0, t)
                    elif part == 2:
                        store_t(yt, vt_v, 0, t)
                    else:
                        k0_v[t] = _pack(yt.astype(BF))
            return c_

        def a_first():
            lax.fori_loop(0, NC1, f_body, 0)

            def mk_k4(t):
                def run(tok):
                    k0_v[8, 0:8, :] = pltpu.bitcast(tok[0:8], U32)
                    kp = k0_v[t + zero]
                    kt_v[t] = kp[80:128]
                    build_k4(kp, t, 48)
                return run
            k4c = [mk_k4(t) for t in range(8)]
            at = Attn(0)
            at.issue(CFG['flook'])
            while at.issued < 2 * H:
                at.issue()
                at.finish()
                if CFG['k4early'] and at.done % 7 == 1 and k4c:
                    k4c.pop(0)(at.outs[-1][0:16] if at.outs else at.last[0:16])

            @pl.when(first)
            def _():
                cp_woa.wait()
                cp_x(1).wait()
                cp_wb(0).wait()
                cp_wob(0).wait()
                cp_x(2).start()
                cp_wb(1).start()
                cp_wob(1).start()
            hi = CFG['fhi']
            side = _both(_spread(prep_chunks(zero), 16, 0, hi),
                         _spread(ln_chunks(TA + zero * TA, 0, TA), 16, 0, hi))
            if k4c:
                side = _both(side, _spread(k4c, 16, 0, hi))
            o1 = jnp.concatenate([oa0_v[t + zero] if CFG['opq'] & 1 else oa0_v[t] for t in range(4)], axis=1)
            part = []
            yprev = None
            for u in range(16):
                if u == 8:
                    o1 = jnp.concatenate([oa1_v[t + zero] if CFG['opq'] & 2 else oa1_v[t] for t in range(4)], axis=1)
                rows = slice((u // 8) * (D // 2), (u // 8 + 1) * (D // 2))
                wu = _pack(woa_v[rows, (u % 8) * 128:(u % 8 + 1) * 128])
                woap[u % 8, (u // 8) * (D // 4):(u // 8 + 1) * (D // 4), :] = wu
                ff = CFG['ffence']
                lhs = with_fence(o1, fence_side(zero) | fence_k(zero)) if (u % ff == ff - 1) else o1
                y = _dot(_unpack(lhs), _unpack(wu))
                if u == 0:
                    at.finish(2 * H)
                if yprev is not None:
                    release(yprev, side[u - 1])
                yprev = y
                if u < 8:
                    part.append(y)
                else:
                    part[u - 8] = part[u - 8] + y
                    if u % 2 == 1:
                        add_residual(0, TA, (u - 9) * 128, (u - 7) * 128,
                                     jnp.concatenate(part[u - 9:u - 7], axis=1))

        if CFG['first']:
            a_first()

        @pl.when(first)
        def _():
            cp_x(2).wait()
            cp_wb(1).wait()
            cp_wob(1).wait()
            cp_x(3).start()
            cp_wb(2).start()
            for j in range(2, 8):
                cp_wob(j).start()

        def a_body(i, c_):
            @pl.when(jnp.logical_and(first, i == 2))
            def _():
                cp_x(3).wait()
                cp_wb(2).wait()
                for j in range(2, 8):
                    cp_wob(j).wait()
            xu = _pack(xn_v[0:TA, :])
            lnc = ln_chunks(((i + 1) % NA) * TA, 0, TA)
            side = [[] for _ in range(40)]
            for u, c in zip(CFG['ppos'], prep_chunks(i)):
                side[u].append(c)
            for u, c in zip(CFG['lpos'], lnc):
                side[u].append(c)
            at = Attn(i)
            yprev = None
            for u in range(24):
                t, kind = u // 3, u % 3
                if u == 23:
                    at.issue(CFG['look'])
                fen = fence_side(zero) if u in CFG['fpos'] else None
                if u >= 2 and CFG['efence']:
                    f2 = (fence_k, fence_v, fence_q)[(u - 2) % 3](zero)
                    fen = f2 if fen is None else fen | f2
                lhs = xu if fen is None else with_fence(xu, fen)
                y = _dot(_unpack(lhs), _unpack(wap[(8, 16, 0)[kind] + t]))
                if kind == 0:
                    kp = _pack(y.astype(BF))
                    full = jnp.concatenate([kt_v[t], kp], axis=0)
                    kt_v[t] = kp[80:128]
                    build_k4(full, t, pl.multiple_of(i * (TA // 2), TA // 2))
                elif kind == 1:
                    store_t(y, vt_v, i * (TA // 128), t)
                else:
                    store_t(y * QSCALE, qt_v, 0, t)
                if yprev is not None:
                    release(yprev, side[u - 1])
                yprev = y
            while at.issued < 2 * H - CFG['tail']:
                at.issue()
                at.finish()
            o1 = _unpack(jnp.concatenate([oa0_v[t + zero] for t in range(4)], axis=1))
            part = []
            for u in range(8):
                at.issue(2)
                part.append(_dot(o1, _unpack(woap[u, 0:D // 4, :])))
                if u > 0:
                    at.finish(2)
                release(part[-1], side[24 + u])
            assert at.done == 2 * H
            o2 = jnp.concatenate([oa1_v[t] for t in range(4)], axis=1)
            r = pl.multiple_of(i * TA, TA)
            for c in range(4):
                w2 = jnp.concatenate([woap[2 * c, D // 4:, :], woap[2 * c + 1, D // 4:, :]], axis=1)
                lhs = with_fence(o2, fence_side(zero)) if 32 + c in CFG['fpos'] else o2
                y = _dot(_unpack(lhs), _unpack(w2))
                release(y, side[32 + c])
                add_residual(r, TA, c * 256, (c + 1) * 256,
                             y + jnp.concatenate(part[2 * c:2 * c + 2], axis=1))
            return c_
        if CFG['a']:
            lax.fori_loop(1, NA, a_body, 0)

        for T in range(8):
            qk_v[8 + T, 0:HALO, :] = jnp.zeros((HALO, 128), F32)
            v_v[T, 0:HALO, :] = jnp.zeros((HALO, 128), F32)

        def b_body(i, c_):
            def send(k):
                for ii in range(NB):
                    @pl.when(jnp.logical_and(p == 1, i == ii))
                    def _():
                        cp_out(ii, k).start()
            xu = _pack(xn_v[0:TA, :])
            ln1 = ln_chunks(i * TB + 256, TA, 256)
            ln2 = ln_chunks(((i + 1) % NB) * TB, 0, TA)
            lg = [logit_b(i, zero, g * 8) for g in range(TB // 8)]
            pv = [pv_b(zero, g * 8) for g in range(TB // 8)]
            n0, n1, n2 = CFG['bn']
            fx = {u: (lambda: fence_xn(zero)) for u in CFG['bf']}
            proj_b(xu, 0, _both(_spread(ln1 + ln2, 48, 0, CFG['bln']),
                                _spread(_flat(lg[0:n0]), 48, 32, 48)), fx)
            xu1 = _pack(xn_v[pl.ds(pl.multiple_of(TA + zero * 32, 32), TA), :])
            mix0 = _merge(lg[n0:32], pv[0:32]) if CFG['bmix'] else lg[n0:32] + pv[0:32]
            proj_b(xu1, 256, _both(_spread(_flat(mix0), 48, 0, 32),
                                   _spread(_flat(lg[32:n1]), 48, 32, 48)), {})
            mix1 = _merge(lg[n1:64], pv[32:n2])
            out_b(i, 0, 256, _spread(_flat(mix1), 16))
            send(0)
            out_b(i, 256, 128, _spread(_flat(pv[n2:64]), 16, 0, CFG['bhi']))
            send(1)
            for T in range(8):
                qk_v[8 + T, 0:HALO, :] = qk_v[8 + T, TB:TB + HALO, :]
                v_v[T, 0:HALO, :] = v_v[T, TB:TB + HALO, :]
            out_b(i, 384, 128, [[]] * 16)
            send(2)
            return c_
        if CFG['b']:
            lax.fori_loop(0, NB, b_body, 0)
        return carry

    lax.fori_loop(0, 2, one_pass, 0)
    for i in range(NB):
        for k in range(len(OUT_PIECES)):
            cp_out(i, k).wait()


@jax.jit
def pallas_interleave_layers__sliding_block__sliding_local_dilated__prompt_kernel(
    A_x: jax.Array,
    A_wqkv: jax.Array,
    A_wo: jax.Array,
    B_x: jax.Array,
    B_wqkv: jax.Array,
    B_wo: jax.Array,
):
    del B_x
    x = A_x.reshape(S, D)
    any_spec = pl.BlockSpec(memory_space=pl.ANY)
    out = pl.pallas_call(
        _kernel,
        out_shape=jax.ShapeDtypeStruct((S, D), BF),
        in_specs=[any_spec] * 5,
        out_specs=any_spec,
        scratch_shapes=[
            pltpu.VMEM((S + 16, D), BF),
            pltpu.VMEM((3 * NC1, D, G1 * 128), BF),
            pltpu.VMEM((D, D), BF),
            pltpu.VMEM((D + 16, 3 * D), BF),
            pltpu.VMEM((9, D, 128), BF),
            pltpu.VMEM((24, D // 2, 128), U32),
            pltpu.VMEM((8, D // 2, 128), U32),
            pltpu.VMEM((9, 3 * D // 2, 128), U32),
            pltpu.VMEM((9, D // 2, 128), U32),
            pltpu.VMEM((2 * TA + 32, D), BF),
            pltpu.VMEM((9, TA // 2, 128), U32),
            pltpu.VMEM((8, 48, 128), U32),
            pltpu.VMEM((H, S // 2, 128), U32),
            pltpu.VMEM((3, D // 2, 128), U32),
            pltpu.VMEM((S // 128 + 1, D // 2, 128), U32),
            pltpu.VMEM((4, TA // 2, 128), U32),
            pltpu.VMEM((4, TA // 2, 128), U32),
            pltpu.VMEM((16, HALO + TB, 128), F32),
            pltpu.VMEM((8, HALO + TB, 128), F32),
            pltpu.VMEM((WB, TB, 128), F32),
            pltpu.VMEM((TB, D), BF),
            pltpu.VMEM((4, 8, 128), U32),
            pltpu.SemaphoreType.DMA((5 + NC1,)),
        ],
        compiler_params=pltpu.CompilerParams(vmem_limit_bytes=100 * 1024 * 1024),
        name="interleave_attn",
    )(x, A_wqkv, A_wo, B_wqkv, B_wo)
    return out.reshape(1, S, D)
```

```python
import math

import jax
import jax.numpy as jnp
from jax import lax
import jax.experimental.pallas as pl
import jax.experimental.pallas.tpu as pltpu

BF = jnp.bfloat16
F32 = jnp.float32
U32 = jnp.uint32

S = 2048
D = 1024
H = 32
DH = 32
TA = 256
NA = S // TA
TB = 512
NB = S // TB
HALO = 16
WB = 8
NEG = -1e30
EPS = 1e-5
QSCALE = (DH ** -0.5) * math.log2(math.e)
NC1 = 4
G1 = 8 // NC1
OUT_PIECES = ((0, 256), (256, 128), (384, 128))

CFG = dict(first=1, a=1, b=1, look=3, efence=2,
           ppos=(1, 3, 6, 8, 11, 14, 30, 32), lpos=(1, 2, 4, 5, 7, 8, 10, 11, 13, 14, 16, 17, 19, 20, 20, 21),
           fpos=(5, 8, 11, 14, 17, 20, 23, 35),
           flook=5, k4early=0, fhi=13, ffence=16,
           bn=(16, 60, 54), bf=(), bln=28, bmix=1, bhi=11, lns=2, pns=2, newton=1, qf32=1, lsum=2, opq=1, k4t=0, tail=8, ord=0, cuts=(0, 5, 10, 14, 18))


def _dot(a, b):
    return jnp.dot(a, b, preferred_element_type=F32)


def _dot_nt(a, b):
    return lax.dot_general(a, b, (((1,), (1,)), ((), ())), preferred_element_type=F32)


def _pack(x_bf16):
    return pltpu.bitcast(x_bf16, U32)


def _unpack(x_u32):
    return pltpu.bitcast(x_u32, BF)


def _iota(shape, dim):
    return lax.broadcasted_iota(jnp.int32, shape, dim)


def _layernorm(x_bf16):
    x = x_bf16.astype(F32)
    m = jnp.sum(x, axis=1, keepdims=True) * (1.0 / D)
    xc = x - m
    v = jnp.sum(xc * xc, axis=1, keepdims=True) * (1.0 / D)
    return (xc * lax.rsqrt(v + EPS)).astype(BF)


def _recip(l):
    if not CFG['newton']:
        return pl.reciprocal(l, approx=False)
    r = pl.reciprocal(l, approx=True)
    return r * (2.0 - l * r)


def _swap16(vs):
    vs = list(vs)
    for a in range(0, 16, 2):
        x, y = vs[a], vs[a + 1]
        vs[a] = (x & U32(0xFFFF)) | (y << 16)
        vs[a + 1] = (x >> 16) | (y & U32(0xFFFF0000))
    sub = _iota((8, 128), 0)
    for dist in (1, 2, 4):
        lo = (sub & dist) == 0
        for a in range(16):
            if not a & (2 * dist):
                x, y = vs[a], vs[a + 2 * dist]
                vs[a] = jnp.where(lo, x, pltpu.roll(y, dist, 0))
                vs[a + 2 * dist] = jnp.where(lo, pltpu.roll(x, 8 - dist, 0), y)
    return vs


def _spread(chunks, nslots, lo=0, hi=None):
    hi = nslots if hi is None else hi
    out = [[] for _ in range(nslots)]
    for u, c in enumerate(chunks):
        out[lo + u * (hi - lo) // len(chunks)].append(c)
    return out


def _merge(a, b):
    out = []
    for u in range(max(len(a), len(b))):
        out += a[u:u + 1] + b[u:u + 1]
    return out


def _flat(lists):
    return sum(lists, [])


def _both(*lists):
    return [sum(parts, []) for parts in zip(*lists)]


def _kernel(x_hbm, wa_hbm, woa_hbm, wb_hbm, wob_hbm, out_hbm,
            x_v, wa_v, woa_v, wb_v, wob_v, wap, woap, wbt, wobp, xn_v,
            k0_v, kt_v, k4_v, qt_v, vt_v, oa0_v, oa1_v, qk_v, v_v, e_v, ob_v, tk_v,
            sems):
    def cp_x(i):
        n = TA if i < 3 else S - 3 * TA
        return pltpu.make_async_copy(x_hbm.at[pl.ds(i * TA, n), :],
                                     x_v.at[pl.ds(i * TA, n), :], sems.at[i])

    def cp_wa(c):
        w = G1 * 128
        return [pltpu.make_async_copy(wa_hbm.at[:, pl.ds(part * D + c * w, w)],
                                      wa_v.at[3 * c + part], sems.at[5 + c])
                for part in range(3)]

    cp_woa = pltpu.make_async_copy(woa_hbm, woa_v, sems.at[1])

    def cp_wb(j):
        n = 128 if j < 2 else D - 256
        return pltpu.make_async_copy(wb_hbm.at[pl.ds(j * 128, n), :],
                                     wb_v.at[pl.ds(j * 128, n), :], sems.at[j + 1])

    def cp_wob(j):
        return pltpu.make_async_copy(wob_hbm.at[:, pl.ds(j * 128, 128)],
                                     wob_v.at[j], sems.at[min(j, 2) + 1])

    def cp_out(i, k):
        r0, n = OUT_PIECES[k]
        return pltpu.make_async_copy(x_v.at[pl.ds(i * TB + r0, n), :],
                                     out_hbm.at[pl.ds(i * TB + r0, n), :], sems.at[4])

    def release(y, chunks):
        n = len(chunks)
        nt = y.shape[1] // 128
        for u, run in enumerate(chunks):
            pos = (u * y.shape[0] * nt // n) // 16 * 16
            t, rr = pos // y.shape[0], pos % y.shape[0]
            run(y[rr:rr + 16, t * 128:(t + 1) * 128])

    def fence_xn(zero):
        return _pack(xn_v[pl.ds(pl.multiple_of(2 * TA + zero * 32, 32), 32), 0:128])

    def fence_side(zero):
        return fence_xn(zero) | wbt[8, 0:16, :] | wobp[8, 0:16, :]

    def fence_k(zero):
        return k4_v[zero, 0:16, :]

    def fence_q(zero):
        return qt_v[2 + zero, 0:16, :]

    def fence_v(zero):
        return vt_v[S // 128 + zero, 0:16, :]

    def gate(tok, zero):
        tk_v[1] = pltpu.bitcast(tok[0:8], U32)
        return tk_v[zero]

    def with_fence(xu, fen):
        r, c = xu.shape
        last = jnp.concatenate([xu[r - 16:, :c - 128], xu[r - 16:, c - 128:] | fen], axis=1)
        return jnp.concatenate([xu[:r - 16], last], axis=0)

    def ln_chunks(row0, dst, nrows, step=16):
        def mk(c):
            def run(tok):
                if tok is not None:
                    x_v[S:S + 16, 0:128] = tok.astype(BF)
                r = pl.multiple_of(row0 + c * step, step)
                xn_v[dst + c * step:dst + (c + 1) * step, :] = _layernorm(x_v[pl.ds(r, step), :])
            return run
        return [mk(c) for c in range(nrows // step)]

    def prep_chunks(j):
        def put(xu, dst, base, hh):
            for dh in range(2):
                grp = _swap16([xu[(2 * h + dh) * 8:(2 * h + dh + 1) * 8] for h in range(16)])
                for d in range(16):
                    o = base + ((dh * 16 + d) * 2 + hh) * 8
                    dst[j, o:o + 8, :] = grp[d]

        def mk_t(c):
            def run(tok):
                wb_v[D:D + 16, 0:128] = tok.astype(BF)
                rows = pl.ds(pl.multiple_of(j * 128, 128), 128)
                put(_pack(wb_v[rows, c * 512:(c + 1) * 512].T), wbt, (c // 2) * (D // 2), c % 2)
            return run

        def mk_o(c):
            def run(tok):
                wob_v[8, 0:16, :] = tok.astype(BF)
                put(_pack(wob_v[j, c * 512:(c + 1) * 512, :]), wobp, 0, c)
            return run
        return [mk_t(c) for c in range(6)] + [mk_o(c) for c in range(2)]

    def tri_mask():
        return _iota((128, 128), 1) >= _iota((128, 128), 0)

    def build_k4(full, t, row0):
        n = full.shape[0] - 48
        if CFG['k4t'] and n == 128:
            xt = [_pack(_unpack(full[16 * g:16 * g + n]).T) for g in range(4)]
            for a in range(4):
                za = jnp.concatenate([xt[g][16 * a:16 * a + 16] for g in range(4)], axis=0)
                k4_v[4 * t + a, pl.ds(row0, n), :] = _pack(_unpack(za).T)
            return
        rolled = [full] + [pltpu.roll(full, 32 * r, 1) for r in range(1, 4)]
        grp_id = _iota((n, 128), 1) // 32
        for a in range(4):
            val = rolled[(0 - a) % 4][0:n]
            for g in range(1, 4):
                val = jnp.where(grp_id == g, rolled[(g - a) % 4][16 * g:16 * g + n], val)
            k4_v[4 * t + a, pl.ds(row0, n), :] = val

    def store_t(y, dst, slot0, t):
        yt = _pack(y.astype(BF).T)
        rows = pl.ds(t * 64 if isinstance(t, int) else pl.multiple_of(t * 64, 64), 64)
        for b in range(TA // 128):
            dst[slot0 + b, rows, :] = yt[:, b * 128:(b + 1) * 128]

    def scores_first(qb, h):
        z = jnp.zeros((16, 128), U32)
        qh = qt_v[qb, h * 16:(h + 1) * 16, :]
        wq = _unpack(jnp.concatenate([qh if jj == h % 4 else z for jj in range(4)], axis=0))
        n = (qb + 1) * 16
        s = jnp.concatenate(
            [_dot(_unpack(k0_v[h // 4, c * n:(c + 1) * n, :]), wq) for c in range(4)], axis=0)
        diag = jnp.where(tri_mask(), s[qb * 128:], NEG)
        return diag if qb == 0 else jnp.concatenate([s[0:128], diag], axis=0)

    def scores_a(m, qb, h):
        qh = qt_v[qb, h * 16:(h + 1) * 16, :]
        if CFG['qf32']:
            qf = _unpack(qh).astype(F32)
            grp_id = _iota((32, 128), 1) // 32
            wq = jnp.concatenate(
                [jnp.where(grp_id == g, qf, 0.0) for g in range(4)], axis=0).astype(BF)
        else:
            grp_id = _iota((16, 128), 1) // 32
            z = jnp.zeros((16, 128), U32)
            wq = _unpack(jnp.concatenate(
                [jnp.where(grp_id == g, qh, z) for g in range(4)], axis=0))
        base = pl.multiple_of(m * 64 - 80, 16)
        order = {0: [0, 16, 1, 17] + list(range(2, 16)),
                 1: [16, 0, 2, 4, 6, 8, 10, 12, 14, 17, 1, 3, 5, 7, 9, 11, 13, 15],
                 2: list(range(15, 1, -1)) + [17, 1, 16, 0],
                 3: [16, 0, 4, 8, 12, 2, 6, 10, 14, 17, 1, 5, 9, 13, 3, 7, 11, 15]}[CFG['ord']]
        cuts = CFG['cuts']
        units = {}
        for c in range(len(cuts) - 1):
            idx = order[cuts[c]:cuts[c + 1]]
            lhs = jnp.concatenate([k4_v[h, pl.ds(base + u * 8, 8), :] for u in idx], axis=0)
            s = _dot(_unpack(lhs), wq)
            for n, u in enumerate(idx):
                units[u] = s[n * 16:(n + 1) * 16]
        for u in range(2):
            new = (_iota((16, 128), 1) % 32) >= (_iota((16, 128), 0) + u * 16)
            units[u] = jnp.where(new, units[16 + u], units[u])
        return jnp.concatenate([units[u] for u in range(16)], axis=0)

    def finish_a(s, m, h):
        skewed = not isinstance(m, int)
        mx = jnp.max(s, axis=0, keepdims=True)
        if skewed:
            lane = _iota((256, 128), 1)
            s = jnp.where((lane // 32) % 2 == 1,
                          jnp.concatenate([s[224:], s[:224]], axis=0), s)
            s = jnp.where(lane >= 64, jnp.concatenate([s[192:], s[:192]], axis=0), s)
        p = jnp.exp2(s - mx)
        nv = p.shape[0] // 8
        if CFG['lsum'] == 0 or not skewed:
            l = jnp.sum(p, axis=0, keepdims=True)
        else:
            pieces = [p[8 * v:8 * v + 8] for v in range(nv)]
            if CFG['lsum'] == 1:
                orders = [[v for t in range(nv // 16) for v in range(16 * t + 15, 16 * t - 1, -1)]]
            elif CFG['lsum'] == 2:
                orders = [list(range(16 * t + 15, 16 * t - 1, -1)) for t in range(nv // 16)]
            elif CFG['lsum'] == 3:
                pieces = [pieces[2 * v] + pieces[2 * v + 1] for v in range(nv // 2)]
                orders = [list(range(8 * t + 7, 8 * t - 1, -1)) for t in range(nv // 16)]
            elif CFG['lsum'] == 4:
                orders = [list(range(nv - 1, -1, -1))]
            accs = []
            for od in orders:
                acc = pieces[od[0]]
                for v in od[1:]:
                    acc = acc + pieces[v]
                accs.append(acc)
            l = jnp.sum(sum(accs[1:], accs[0]), axis=0, keepdims=True)
        if skewed:
            tri = tri_mask()
            pm = p[0:128]
            p = jnp.concatenate(
                [jnp.where(tri, 0.0, pm), p[128:256], jnp.where(tri, pm, 0.0)], axis=0)
        ntile = p.shape[0] // 128
        vv = _unpack(jnp.concatenate(
            [vt_v[m - bk, h * 16:(h + 1) * 16, :] for bk in range(ntile - 1, -1, -1)], axis=1))
        o = _dot(vv, p.astype(BF))
        return o * _recip(l)

    class Attn:
        def __init__(self, blk):
            self.blk = blk
            self.items = [(qb, 4 * t + a) for t in range(8) for qb in range(2) for a in range(4)]
            self.issued, self.done, self.queue, self.outs = 0, 0, [], []

        def issue(self, n=1):
            for _ in range(n):
                if self.issued < len(self.items):
                    qb, h = self.items[self.issued]
                    if isinstance(self.blk, int):
                        self.queue.append(scores_first(qb, h))
                    else:
                        self.queue.append(scores_a(self.blk * (TA // 128) + qb, qb, h))
                    self.issued += 1

        def finish(self, n=1):
            for _ in range(n):
                if self.done < self.issued:
                    qb, h = self.items[self.done]
                    self.outs.append(finish_a(self.queue.pop(0), self.blk * (TA // 128) + qb, h))
                    if len(self.outs) == 4:
                        ot = jnp.concatenate(self.outs, axis=0).astype(BF)
                        (oa0_v, oa1_v)[h // 16][(h // 4) % 4, qb * 64:(qb + 1) * 64, :] = _pack(ot.T)
                        self.last, self.outs = self.outs[-1], []
                    self.done += 1

    def add_residual(r, nrows, c0, c1, y):
        x_v[pl.ds(r, nrows), c0:c1] = (x_v[pl.ds(r, nrows), c0:c1].astype(F32) + y).astype(BF)

    def proj_b(xu, r0, side, fences):
        nrows = 2 * xu.shape[0]
        for T in range(24):
            y = None
            for hf in range(2):
                u = 2 * T + hf
                w = _unpack(jnp.concatenate(
                    [wbt[j, T * 64:(T + 1) * 64, :] for j in range(4 * hf, 4 * hf + 4)], axis=1))
                lhs = xu[:, hf * 512:(hf + 1) * 512]
                if u in fences:
                    lhs = with_fence(lhs, fences[u]())
                yh = _dot_nt(_unpack(lhs), w)
                y = yh if y is None else y + yh
                if hf == 1:
                    if T < 8:
                        qk_v[T, HALO + r0:HALO + r0 + nrows, :] = y * QSCALE
                    elif T < 16:
                        qk_v[T, HALO + r0:HALO + r0 + nrows, :] = y
                    else:
                        v_v[T - 16, HALO + r0:HALO + r0 + nrows, :] = y
                release(y, side[u])

    def gated(x, g):
        return pltpu.bitcast(pltpu.bitcast(x, U32) | g, F32)

    def logit_b(i, zero, r0):
        R = 8
        ns = CFG['lns']
        accs = [None] * WB

        def mk(st):
            def run(tok):
                g = gate(tok, zero)
                for t in range(st * 8 // ns, (st + 1) * 8 // ns):
                    q = gated(qk_v[t, HALO + r0:HALO + r0 + R, :], g)
                    for w in range(WB):
                        o = HALO + r0 - 2 * w
                        p = q * qk_v[8 + t, o:o + R, :]
                        accs[w] = p if accs[w] is None else accs[w] + p
                if st + 1 < ns:
                    return
                ls = []
                for w in range(WB):
                    a = accs[w]
                    a = a + pltpu.roll(a, 64, 1)
                    a = a + pltpu.roll(a, 32, 1)
                    if r0 - 2 * w < 0:
                        a = jnp.where(_iota((R, 128), 0) + (i * TB + r0 - 2 * w) >= 0, a, NEG)
                    ls.append(a)
                mx = ls[0]
                for w in range(1, WB):
                    mx = jnp.maximum(mx, ls[w])
                es = [jnp.exp2(l - mx) for l in ls]
                s = es[0]
                for w in range(1, WB):
                    s = s + es[w]
                inv = _recip(s)
                for w in range(WB):
                    e_v[w, r0:r0 + R, :] = es[w] * inv
            return run
        return [mk(st) for st in range(ns)]

    def pv_b(zero, r0):
        R = 8
        ns = CFG['pns']

        def mk(st):
            def run(tok):
                g = gate(tok, zero)
                es = [gated(e_v[w, r0:r0 + R, :], g) for w in range(WB)]
                os_ = []
                t0, t1 = st * 8 // ns, (st + 1) * 8 // ns
                for t in range(t0, t1):
                    acc = None
                    for w in range(WB):
                        o = HALO + r0 - 2 * w
                        pv = es[w] * v_v[t, o:o + R, :]
                        acc = pv if acc is None else acc + pv
                    os_.append(acc)
                ob_v[r0:r0 + R, t0 * 128:t1 * 128] = jnp.concatenate(os_, axis=1).astype(BF)
            return run
        return [mk(st) for st in range(ns)]

    def out_b(i, r0, nrows, side):
        o = ob_v[r0:r0 + nrows, :]
        r = pl.multiple_of(i * TB + r0, 128)
        ys = []
        for T in range(8):
            y = None
            for hf in range(2):
                yh = _dot(o[:, hf * 512:(hf + 1) * 512],
                          _unpack(wobp[T, hf * 256:(hf + 1) * 256, :]))
                y = yh if y is None else y + yh
                release(y, side[2 * T + hf])
            ys.append(y)
            if T % 2 == 1:
                add_residual(r, nrows, (T - 1) * 128, (T + 1) * 128,
                             jnp.concatenate(ys[-2:], axis=1))

    cp_x(0).start()
    for cp in cp_wa(0):
        cp.start()
    z16 = jnp.zeros((16, 128), U32)
    xn_v[2 * TA:2 * TA + 32, :] = jnp.zeros((32, D), BF)
    wbt[8, 0:16, :] = z16
    wobp[8, 0:16, :] = z16
    k4_v[0, 0:16, :] = z16
    vt_v[S // 128, 0:16, :] = z16
    qt_v[2, 0:16, :] = z16
    tk_v[0] = z16[0:8]
    cp_x(0).wait()
    for cp in cp_wa(1):
        cp.start()
    for run in ln_chunks(0, 0, TA, step=TA):
        run(None)

    def one_pass(p, carry):
        first = p == 0
        zero = p // 4

        def f_body(c, c_):
            @pl.when(first)
            def _():
                buf = wa_v.at[pl.ds(3 * c, 3)]
                pltpu.make_async_copy(buf, buf, sems.at[5 + c]).wait()
            xn = xn_v[0:TA, :]

            def tile(part, g):
                t = c * G1 + g
                wu = _pack(wa_v[3 * c + part, :, g * 128:(g + 1) * 128])
                wap[part * 8 + t] = wu
                y = _dot(xn, _unpack(wu))
                if part == 0:
                    store_t(y * QSCALE, qt_v, 0, t)
                elif part == 2:
                    store_t(y, vt_v, 0, t)
                else:
                    kp = _pack(y.astype(BF))
                    k0_v[t] = kp
                    if g + 1 < G1:
                        kt_v[t] = kp[80:128]
                        build_k4(kp, t, 48)
            order = [(1, g) for g in range(G1 - 1)] + \
                    [(part, g) for part in (2, 0) for g in range(G1)] + [(1, G1 - 1)]
            for n, (part, g) in enumerate(order):
                tile(part, g)
                if n == 0:
                    for k in range(NC1 - 2):
                        @pl.when(jnp.logical_and(first, c == k))
                        def _():
                            for cp in cp_wa(k + 2):
                                cp.start()

            @pl.when(jnp.logical_and(first, c == NC1 - 3))
            def _():
                cp_woa.start()

            @pl.when(jnp.logical_and(first, c == NC1 - 2))
            def _():
                cp_x(1).start()
                cp_wb(0).start()
                cp_wob(0).start()
            return c_

        def a_first():
            lax.fori_loop(0, NC1, f_body, 0)

            def mk_k4(t):
                def run(tok):
                    k0_v[8, 0:8, :] = pltpu.bitcast(tok[0:8], U32)
                    kp = k0_v[t + zero]
                    kt_v[t] = kp[80:128]
                    build_k4(kp, t, 48)
                return run
            k4c = [mk_k4(t) for t in range(G1 - 1, 8, G1)]
            at = Attn(0)
            at.issue(CFG['flook'])
            while at.issued < 2 * H:
                at.issue()
                at.finish()
                if CFG['k4early'] and at.done % 7 == 1 and k4c:
                    k4c.pop(0)(at.outs[-1][0:16] if at.outs else at.last[0:16])

            @pl.when(first)
            def _():
                cp_woa.wait()
                cp_x(1).wait()
                cp_wb(0).wait()
                cp_wob(0).wait()
                cp_x(2).start()
                cp_wb(1).start()
                cp_wob(1).start()
            hi = CFG['fhi']
            side = _both(_spread(prep_chunks(zero), 16, 0, hi),
                         _spread(ln_chunks(TA + zero * TA, 0, TA), 16, 0, hi))
            if k4c:
                side = _both(side, _spread(k4c, 16, 0, hi))
            o1 = jnp.concatenate([oa0_v[t + zero] if CFG['opq'] & 1 else oa0_v[t] for t in range(4)], axis=1)
            part = []
            yprev = None
            for u in range(16):
                if u == 8:
                    o1 = jnp.concatenate([oa1_v[t + zero] if CFG['opq'] & 2 else oa1_v[t] for t in range(4)], axis=1)
                rows = slice((u // 8) * (D // 2), (u // 8 + 1) * (D // 2))
                wu = _pack(woa_v[rows, (u % 8) * 128:(u % 8 + 1) * 128])
                woap[u % 8, (u // 8) * (D // 4):(u // 8 + 1) * (D // 4), :] = wu
                ff = CFG['ffence']
                lhs = with_fence(o1, fence_side(zero) | fence_k(zero)) if (u % ff == ff - 1) else o1
                y = _dot(_unpack(lhs), _unpack(wu))
                if u == 0:
                    at.finish(2 * H)
                if yprev is not None:
                    release(yprev, side[u - 1])
                yprev = y
                if u < 8:
                    part.append(y)
                else:
                    part[u - 8] = part[u - 8] + y
                    if u % 2 == 1:
                        add_residual(0, TA, (u - 9) * 128, (u - 7) * 128,
                                     jnp.concatenate(part[u - 9:u - 7], axis=1))

        if CFG['first']:
            a_first()

        @pl.when(first)
        def _():
            cp_x(2).wait()
            cp_wb(1).wait()
            cp_wob(1).wait()
            cp_x(3).start()
            cp_wb(2).start()
            for j in range(2, 8):
                cp_wob(j).start()

        def a_body(i, c_):
            @pl.when(jnp.logical_and(first, i == 2))
            def _():
                cp_x(3).wait()
                cp_wb(2).wait()
                for j in range(2, 8):
                    cp_wob(j).wait()
            xu = _pack(xn_v[0:TA, :])
            lnc = ln_chunks(((i + 1) % NA) * TA, 0, TA)
            side = [[] for _ in range(40)]
            for u, c in zip(CFG['ppos'], prep_chunks(i)):
                side[u].append(c)
            for u, c in zip(CFG['lpos'], lnc):
                side[u].append(c)
            at = Attn(i)
            yprev = None
            for u in range(24):
                t, kind = u // 3, u % 3
                if u == 23:
                    at.issue(CFG['look'])
                fen = fence_side(zero) if u in CFG['fpos'] else None
                if u >= 2 and CFG['efence']:
                    f2 = (fence_k, fence_v, fence_q)[(u - 2) % 3](zero)
                    fen = f2 if fen is None else fen | f2
                lhs = xu if fen is None else with_fence(xu, fen)
                y = _dot(_unpack(lhs), _unpack(wap[(8, 16, 0)[kind] + t]))
                if kind == 0:
                    kp = _pack(y.astype(BF))
                    full = jnp.concatenate([kt_v[t], kp], axis=0)
                    kt_v[t] = kp[80:128]
                    build_k4(full, t, pl.multiple_of(i * (TA // 2), TA // 2))
                elif kind == 1:
                    store_t(y, vt_v, i * (TA // 128), t)
                else:
                    store_t(y * QSCALE, qt_v, 0, t)
                if yprev is not None:
                    release(yprev, side[u - 1])
                yprev = y
            while at.issued < 2 * H - CFG['tail']:
                at.issue()
                at.finish()
            o1 = _unpack(jnp.concatenate([oa0_v[t + zero] for t in range(4)], axis=1))
            part = []
            for u in range(8):
                at.issue(2)
                part.append(_dot(o1, _unpack(woap[u, 0:D // 4, :])))
                if u > 0:
                    at.finish(2)
                release(part[-1], side[24 + u])
            assert at.done == 2 * H
            o2 = jnp.concatenate([oa1_v[t] for t in range(4)], axis=1)
            r = pl.multiple_of(i * TA, TA)
            for c in range(4):
                w2 = jnp.concatenate([woap[2 * c, D // 4:, :], woap[2 * c + 1, D // 4:, :]], axis=1)
                lhs = with_fence(o2, fence_side(zero)) if 32 + c in CFG['fpos'] else o2
                y = _dot(_unpack(lhs), _unpack(w2))
                release(y, side[32 + c])
                add_residual(r, TA, c * 256, (c + 1) * 256,
                             y + jnp.concatenate(part[2 * c:2 * c + 2], axis=1))
            return c_
        if CFG['a']:
            lax.fori_loop(1, NA, a_body, 0)

        for T in range(8):
            qk_v[8 + T, 0:HALO, :] = jnp.zeros((HALO, 128), F32)
            v_v[T, 0:HALO, :] = jnp.zeros((HALO, 128), F32)

        def b_body(i, c_):
            def send(k):
                for ii in range(NB):
                    @pl.when(jnp.logical_and(p == 1, i == ii))
                    def _():
                        cp_out(ii, k).start()
            xu = _pack(xn_v[0:TA, :])
            ln1 = ln_chunks(i * TB + 256, TA, 256)
            ln2 = ln_chunks(((i + 1) % NB) * TB, 0, TA)
            lg = [logit_b(i, zero, g * 8) for g in range(TB // 8)]
            pv = [pv_b(zero, g * 8) for g in range(TB // 8)]
            n0, n1, n2 = CFG['bn']
            fx = {u: (lambda: fence_xn(zero)) for u in CFG['bf']}
            proj_b(xu, 0, _both(_spread(ln1 + ln2, 48, 0, CFG['bln']),
                                _spread(_flat(lg[0:n0]), 48, 32, 48)), fx)
            xu1 = _pack(xn_v[pl.ds(pl.multiple_of(TA + zero * 32, 32), TA), :])
            mix0 = _merge(lg[n0:32], pv[0:32]) if CFG['bmix'] else lg[n0:32] + pv[0:32]
            proj_b(xu1, 256, _both(_spread(_flat(mix0), 48, 0, 32),
                                   _spread(_flat(lg[32:n1]), 48, 32, 48)), {})
            mix1 = _merge(lg[n1:64], pv[32:n2])
            out_b(i, 0, 256, _spread(_flat(mix1), 16))
            send(0)
            out_b(i, 256, 128, _spread(_flat(pv[n2:64]), 16, 0, CFG['bhi']))
            send(1)
            for T in range(8):
                qk_v[8 + T, 0:HALO, :] = qk_v[8 + T, TB:TB + HALO, :]
                v_v[T, 0:HALO, :] = v_v[T, TB:TB + HALO, :]
            out_b(i, 384, 128, [[]] * 16)
            send(2)
            return c_
        if CFG['b']:
            lax.fori_loop(0, NB, b_body, 0)
        return carry

    lax.fori_loop(0, 2, one_pass, 0)
    for i in range(NB):
        for k in range(len(OUT_PIECES)):
            cp_out(i, k).wait()


@jax.jit
def pallas_interleave_layers__sliding_block__sliding_local_dilated__prompt_kernel(
    A_x: jax.Array,
    A_wqkv: jax.Array,
    A_wo: jax.Array,
    B_x: jax.Array,
    B_wqkv: jax.Array,
    B_wo: jax.Array,
):
    del B_x
    x = A_x.reshape(S, D)
    any_spec = pl.BlockSpec(memory_space=pl.ANY)
    out = pl.pallas_call(
        _kernel,
        out_shape=jax.ShapeDtypeStruct((S, D), BF),
        in_specs=[any_spec] * 5,
        out_specs=any_spec,
        scratch_shapes=[
            pltpu.VMEM((S + 16, D), BF),
            pltpu.VMEM((3 * NC1, D, G1 * 128), BF),
            pltpu.VMEM((D, D), BF),
            pltpu.VMEM((D + 16, 3 * D), BF),
            pltpu.VMEM((9, D, 128), BF),
            pltpu.VMEM((24, D // 2, 128), U32),
            pltpu.VMEM((8, D // 2, 128), U32),
            pltpu.VMEM((9, 3 * D // 2, 128), U32),
            pltpu.VMEM((9, D // 2, 128), U32),
            pltpu.VMEM((2 * TA + 32, D), BF),
            pltpu.VMEM((9, TA // 2, 128), U32),
            pltpu.VMEM((8, 48, 128), U32),
            pltpu.VMEM((H, S // 2, 128), U32),
            pltpu.VMEM((3, D // 2, 128), U32),
            pltpu.VMEM((S // 128 + 1, D // 2, 128), U32),
            pltpu.VMEM((4, TA // 2, 128), U32),
            pltpu.VMEM((4, TA // 2, 128), U32),
            pltpu.VMEM((16, HALO + TB, 128), F32),
            pltpu.VMEM((8, HALO + TB, 128), F32),
            pltpu.VMEM((WB, TB, 128), F32),
            pltpu.VMEM((TB, D), BF),
            pltpu.VMEM((4, 8, 128), U32),
            pltpu.SemaphoreType.DMA((5 + NC1,)),
        ],
        compiler_params=pltpu.CompilerParams(vmem_limit_bytes=100 * 1024 * 1024),
        name="interleave_attn",
    )(x, A_wqkv, A_wo, B_wqkv, B_wo)
    return out.reshape(1, S, D)
```

```python
import math

import jax
import jax.numpy as jnp
from jax import lax
import jax.experimental.pallas as pl
import jax.experimental.pallas.tpu as pltpu

BF = jnp.bfloat16
F32 = jnp.float32
U32 = jnp.uint32

S = 2048
D = 1024
H = 32
DH = 32
TA = 256
NA = S // TA
TB = 512
NB = S // TB
HALO = 16
WB = 8
NEG = -1e30
EPS = 1e-5
QSCALE = (DH ** -0.5) * math.log2(math.e)
NC1 = 4
G1 = 8 // NC1
OUT_PIECES = ((0, 256), (256, 128), (384, 128))

CFG = dict(first=1, a=1, b=1, look=3, tail=8, cuts=(5, 10, 14), lsum=2,
           ppos=(1, 3, 6, 8, 11, 14, 30, 32),
           lpos=(1, 2, 4, 5, 7, 8, 10, 11, 13, 14, 16, 17, 19, 20, 20, 21),
           fpos=(5, 8, 11, 14, 17, 20, 23, 35),
           flook=5, fhi=13,
           bn=(16, 60, 54), bln=28, bhi=11, lns=2, pns=2, lchain=1, lnz=1)


def _dot(a, b):
    return lax.dot_general(a, b, (((1,), (0,)), ((), ())), preferred_element_type=F32)


def _dot_nt(a, b):
    return lax.dot_general(a, b, (((1,), (1,)), ((), ())), preferred_element_type=F32)


def _pack(x_bf16):
    return pltpu.bitcast(x_bf16, U32)


def _unpack(x_u32):
    return pltpu.bitcast(x_u32, BF)


def _iota(shape, dim):
    return lax.broadcasted_iota(jnp.int32, shape, dim)


def _rows(xs):
    return lax.concatenate(xs, 0)


def _lanes(x3):
    n, r, _ = x3.shape
    x2 = x3.reshape(n * r, 128)
    return lax.concatenate([x2[t * r:(t + 1) * r] for t in range(n)], 1)


def _layernorm(x_bf16):
    x = x_bf16.astype(F32)
    m = jnp.sum(x, axis=1, keepdims=True) * (1.0 / D)
    xc = x - m
    v = jnp.sum(xc * xc, axis=1, keepdims=True) * (1.0 / D)
    return (xc * lax.rsqrt(v + EPS)).astype(BF)


def _recip(l):
    r = pl.reciprocal(l, approx=True)
    return r * (2.0 - l * r)


def _swap16(xu):
    for bit in range(4):
        x5 = xu.reshape(8 >> bit, 2, 2 << bit, 8, 128)
        x, y = x5[:, 0:1], x5[:, 1:2]
        if bit == 0:
            x, y = ((x & U32(0xFFFF)) | (y << 16), (x >> 16) | (y & U32(0xFFFF0000)))
        else:
            dist = 1 << (bit - 1)
            lo = (_iota(x.shape, 3) & dist) == 0
            x, y = (lax.select(lo, x, pltpu.roll(y, dist, 3)),
                    lax.select(lo, pltpu.roll(x, 8 - dist, 3), y))
        xu = lax.concatenate([x, y], 1)
    return xu.reshape(16, 2, 8, 128)


def _spread(chunks, nslots, lo=0, hi=None):
    hi = nslots if hi is None else hi
    out = [[] for _ in range(nslots)]
    for u, c in enumerate(chunks):
        out[lo + u * (hi - lo) // len(chunks)].append(c)
    return out


def _merge(a, b):
    out = []
    for u in range(max(len(a), len(b))):
        out += a[u:u + 1] + b[u:u + 1]
    return out


def _flat(lists):
    return sum(lists, [])


def _both(*lists):
    return [sum(parts, []) for parts in zip(*lists)]


def _kernel(x_hbm, wa_hbm, woa_hbm, wb_hbm, wob_hbm, out_hbm,
            x_v, wa_v, woa_v, wb_v, wob_v, wap, woap, wbt, wobp, xn_v,
            k0_v, kt_v, k4_v, qt_v, vt_v, oa0_v, oa1_v, qk_v, v_v, e_v, ob_v, tk_v,
            sems):
    def cp_x(i):
        n = TA if i < 3 else S - 3 * TA
        return pltpu.make_async_copy(x_hbm.at[pl.ds(i * TA, n), :],
                                     x_v.at[pl.ds(i * TA, n), :], sems.at[i])

    def cp_wa(c):
        w = G1 * 128
        return [pltpu.make_async_copy(wa_hbm.at[:, pl.ds(part * D + c * w, w)],
                                      wa_v.at[3 * c + part], sems.at[5 + c])
                for part in range(3)]

    cp_woa = pltpu.make_async_copy(woa_hbm, woa_v, sems.at[1])

    def cp_wb(j):
        n = 128 if j < 2 else D - 256
        return pltpu.make_async_copy(wb_hbm.at[pl.ds(j * 128, n), :],
                                     wb_v.at[pl.ds(j * 128, n), :], sems.at[j + 1])

    def cp_wob(j):
        return pltpu.make_async_copy(wob_hbm.at[:, pl.ds(j * 128, 128)],
                                     wob_v.at[j], sems.at[min(j, 2) + 1])

    def cp_out(i, k):
        r0, n = OUT_PIECES[k]
        return pltpu.make_async_copy(x_v.at[pl.ds(i * TB + r0, n), :],
                                     out_hbm.at[pl.ds(i * TB + r0, n), :], sems.at[4])

    def release(y, chunks):
        n = len(chunks)
        nt = y.shape[1] // 128
        for u, run in enumerate(chunks):
            pos = (u * y.shape[0] * nt // n) // 16 * 16
            t, rr = pos // y.shape[0], pos % y.shape[0]
            run(y[rr:rr + 16, t * 128:(t + 1) * 128])

    def gated(x, tok, zero):
        tk_v[1] = pltpu.bitcast(tok[0:8], U32)
        return pltpu.bitcast(pltpu.bitcast(x, U32) | tk_v[pl.ds(zero, 1)], F32)

    def fence_side(zero):
        zx = _pack(xn_v[pl.ds(pl.multiple_of(2 * TA + zero * 32, 32), 32), 0:128])
        return zx | (wbt[8, 0] | wobp[8, 0]).reshape(16, 128)

    def fence_k(zero):
        return k4_v[zero, 0:16, :]

    def fence_q(zero):
        return qt_v[2 + zero, 0:16, :]

    def fence_v(zero):
        return vt_v[S // 128 + zero, 0:16, :]

    def with_fence(xu, fen):
        r, c = xu.shape
        last = lax.concatenate([xu[r - 16:, :c - 128], xu[r - 16:, c - 128:] | fen], 1)
        return _rows([xu[:r - 16], last])

    def ln_chunks(row0, dst, nrows, step=16):
        def mk(c):
            def run(tok):
                if tok is not None:
                    x_v[S:S + 16, 0:128] = tok.astype(BF)
                r = pl.multiple_of(row0 + c * step, step)
                xn_v[dst + c * step:dst + (c + 1) * step, :] = _layernorm(x_v[pl.ds(r, step), :])
            return run
        return [mk(c) for c in range(nrows // step)]

    def prep_chunks(j):
        def put(xu, dst, d0, hh):
            val = _swap16(xu)
            for dh in range(2):
                dst[j, d0 + dh * 16:d0 + (dh + 1) * 16, hh] = val[:, dh]

        def mk_t(c):
            def run(tok):
                wb_v[D:D + 16, 0:128] = tok.astype(BF)
                rows = pl.ds(pl.multiple_of(j * 128, 128), 128)
                put(_pack(wb_v[rows, c * 512:(c + 1) * 512].T), wbt, (c // 2) * DH, c % 2)
            return run

        def mk_o(c):
            def run(tok):
                wob_v[8, 0:16, :] = tok.astype(BF)
                put(_pack(wob_v[j, c * 512:(c + 1) * 512, :]), wobp, 0, c)
            return run
        return [mk_t(c) for c in range(6)] + [mk_o(c) for c in range(2)]

    def build_k4(full, t, row0):
        n = full.shape[0] - 48
        rolled = [full] + [pltpu.roll(full, 32 * r, 1) for r in range(1, 4)]
        grp_id = _iota((n, 128), 1) >> 5
        is_g = [grp_id == g for g in range(4)]
        for a in range(4):
            val = rolled[(0 - a) % 4][0:n]
            for g in range(1, 4):
                val = lax.select(is_g[g], rolled[(g - a) % 4][16 * g:16 * g + n], val)
            k4_v[4 * t + a, pl.ds(row0, n), :] = val

    def store_t(y, dst, slot0, t):
        yt = _pack(y.astype(BF).T)
        rows = pl.ds(t * 64 if isinstance(t, int) else pl.multiple_of(t * 64, 64), 64)
        for b in range(TA // 128):
            dst[slot0 + b, rows, :] = yt[:, b * 128:(b + 1) * 128]

    class Attn:
        def __init__(self, blk):
            self.blk = blk
            self.first = isinstance(blk, int)
            self.items = [(qb, 4 * t + a) for t in range(8) for qb in range(2) for a in range(4)]
            self.issued, self.done, self.queue, self.outs = 0, 0, [], []
            row, lane = _iota((128, 128), 0), _iota((128, 128), 1)
            self.tri = lane >= row
            if self.first:
                self.neg = jnp.full((128, 128), NEG, F32)
                self.zq = jnp.zeros((16, 128), U32)
            else:
                self.zero = jnp.zeros((128, 128), F32)
                self.slot = (lane >> 5) == (row >> 5)
                new = (_iota((32, 128), 1) & 31) >= _iota((32, 128), 0)
                self.new = (new[0:16], new[16:32])
                lane2 = _iota((256, 128), 1)
                self.odd, self.hi = (lane2 & 32) != 0, lane2 >= 64
                self.base = [pl.multiple_of((blk * 2 + qb) * 64 - 80, 16) for qb in range(2)]

        def scores_first(self, qb, h):
            qh = qt_v[qb, h * 16:(h + 1) * 16, :]
            wq = _unpack(_rows([qh if jj == h % 4 else self.zq for jj in range(4)]))
            n = (qb + 1) * 32
            kk = _unpack(k0_v[h // 4, 0:2 * n, :])
            s = _rows([_dot(kk[c * n:(c + 1) * n], wq) for c in range(4)])
            diag = lax.select(self.tri, s[qb * 128:], self.neg)
            return diag if qb == 0 else _rows([s[0:128], diag])

        def scores(self, qb, h):
            qf = _unpack(qt_v[qb, h * 16:(h + 1) * 16, :]).astype(F32)
            wq = lax.select(self.slot, _rows([qf] * 4), self.zero).astype(BF)
            w = k4_v[h, pl.ds(self.base[qb], 144), :]
            kk = _unpack(_rows([w[0:8], w[128:136], w[8:16], w[136:144], w[16:128]]))
            cuts = (0,) + CFG['cuts'] + (18,)
            s = _rows([_dot(kk[16 * a:16 * b], wq) for a, b in zip(cuts[:-1], cuts[1:])])
            return _rows([lax.select(self.new[0], s[16:32], s[0:16]),
                          lax.select(self.new[1], s[48:64], s[32:48]), s[64:]])

        def softmax_pv(self, s, qb, h):
            mx = jnp.max(s, axis=0, keepdims=True)
            if self.first:
                p = jnp.exp2(s - mx)
                l = jnp.sum(p, axis=0, keepdims=True)
                v3 = vt_v[0:qb + 1, h * 16:(h + 1) * 16, :]
            else:
                s = lax.select(self.odd, _rows([s[224:], s[:224]]), s)
                s = lax.select(self.hi, _rows([s[192:], s[:192]]), s)
                p = jnp.exp2(s - mx)
                if CFG['lsum'] == 0:
                    l = jnp.sum(p, axis=0, keepdims=True)
                else:
                    p3 = p.reshape(2, 128, 128)
                    if CFG['lsum'] == 1:
                        acc = jnp.sum(p.reshape(2, 16, 8, 128), axis=1)
                    else:
                        acc = p3[:, 120:128]
                        for v in range(14, -1, -1):
                            acc = acc + p3[:, 8 * v:8 * v + 8]
                    l = jnp.sum(acc.reshape(16, 128), axis=0, keepdims=True)
                pm = p[0:128]
                p = _rows([lax.select(self.tri, self.zero, pm), p[128:256],
                           lax.select(self.tri, pm, self.zero)])
                v3 = vt_v[pl.ds(self.blk * 2 + qb - 2, 3), h * 16:(h + 1) * 16, :]
            return _dot(_unpack(_lanes(v3)), p.astype(BF)) * _recip(l)

        def issue(self, n=1):
            for _ in range(n):
                if self.issued < len(self.items):
                    fn = self.scores_first if self.first else self.scores
                    self.queue.append(fn(*self.items[self.issued]))
                    self.issued += 1

        def finish(self, n=1):
            for _ in range(n):
                if self.done < self.issued:
                    qb, h = self.items[self.done]
                    self.outs.append(self.softmax_pv(self.queue.pop(0), qb, h))
                    if len(self.outs) == 4:
                        ot = _rows(self.outs).astype(BF)
                        dst = (oa0_v, oa1_v)[h // 16]
                        dst[(h // 4) % 4, qb * 64:(qb + 1) * 64, :] = _pack(ot.T)
                        self.outs = []
                    self.done += 1

    def add_residual(r, nrows, c0, c1, y):
        x_v[pl.ds(r, nrows), c0:c1] = (x_v[pl.ds(r, nrows), c0:c1].astype(F32) + y).astype(BF)

    def proj_b(xn, r0, side):
        rows = slice(HALO + r0, HALO + r0 + xn.shape[0])
        halves = (xn[:, 0:512], xn[:, 512:1024])
        for T in range(24):
            y = None
            for hf in range(2):
                w = wbt[4 * hf:4 * hf + 4, 4 * T:4 * T + 4].reshape(4, 64, 128)
                yh = _dot_nt(halves[hf], _unpack(_lanes(w)))
                y = yh if y is None else y + yh
                if hf == 1:
                    if T < 8:
                        qk_v[T, rows, :] = y * QSCALE
                    elif T < 16:
                        qk_v[T, rows, :] = y
                    else:
                        v_v[T - 16, rows, :] = y
                release(y, side[2 * T + hf])

    def taps(ref, t0, t1, r0):
        wins = [ref[t0:t1, HALO + r0 - 2 * w:HALO + r0 - 2 * w + 8, :] for w in range(WB)]
        return _rows(wins).reshape(WB, t1 - t0, 8, 128)

    def logit_b(i, zero, r0):
        ns = CFG['lns']
        acc = []

        def mk(st):
            def run(tok):
                t0, t1 = st * 8 // ns, (st + 1) * 8 // ns
                q = gated(qk_v[t0:t1, HALO + r0:HALO + r0 + 8, :], tok, zero)
                p = q[None] * taps(qk_v, 8 + t0, 8 + t1, r0)
                if acc and CFG['lchain']:
                    a = jnp.sum(lax.concatenate([acc.pop()[:, None], p], 1), axis=1)
                else:
                    a = jnp.sum(p, axis=1)
                    a = acc.pop() + a if acc else a
                if st + 1 < ns:
                    acc.append(a)
                    return
                a = a + pltpu.roll(a, 64, 2)
                a = a + pltpu.roll(a, 32, 2)
                if r0 < 2 * (WB - 1):
                    pos = _iota(a.shape, 1) - 2 * _iota(a.shape, 0) + (i * TB + r0)
                    a = lax.select(pos >= 0, a, jnp.full(a.shape, NEG, F32))
                e = jnp.exp2(a - jnp.max(a, axis=0, keepdims=True))
                e_v[:, r0:r0 + 8, :] = e * _recip(jnp.sum(e, axis=0, keepdims=True))
            return run
        return [mk(st) for st in range(ns)]

    def pv_b(zero, r0):
        ns = CFG['pns']

        def mk(st):
            def run(tok):
                t0, t1 = st * 8 // ns, (st + 1) * 8 // ns
                e = gated(e_v[:, r0:r0 + 8, :], tok, zero)
                o = jnp.sum(e[:, None] * taps(v_v, t0, t1, r0), axis=0)
                ob_v[r0:r0 + 8, t0 * 128:t1 * 128] = _lanes(o).astype(BF)
            return run
        return [mk(st) for st in range(ns)]

    def out_b(i, r0, nrows, side):
        o = ob_v[r0:r0 + nrows, :]
        halves = (o[:, 0:512], o[:, 512:1024])
        r = pl.multiple_of(i * TB + r0, 128)
        ys = []
        for T in range(8):
            y = None
            for hf in range(2):
                w = wobp[T, hf * 16:(hf + 1) * 16].reshape(256, 128)
                yh = _dot(halves[hf], _unpack(w))
                y = yh if y is None else y + yh
                release(y, side[2 * T + hf])
            ys.append(y)
            if T % 2 == 1:
                add_residual(r, nrows, (T - 1) * 128, (T + 1) * 128, lax.concatenate(ys[-2:], 1))

    cp_x(0).start()
    for cp in cp_wa(0):
        cp.start()
    z16 = jnp.zeros((16, 128), U32)
    xn_v[2 * TA:2 * TA + 32, :] = jnp.zeros((32, D), BF)
    wbt[8, 0] = z16.reshape(2, 8, 128)
    wobp[8, 0] = z16.reshape(2, 8, 128)
    k4_v[0, 0:16, :] = z16
    vt_v[S // 128, 0:16, :] = z16
    qt_v[2, 0:16, :] = z16
    tk_v[0] = z16[0:8]
    cp_x(0).wait()
    for cp in cp_wa(1):
        cp.start()
    for run in ln_chunks(0, 0, TA, step=TA):
        run(None)

    def one_pass(p, carry):
        first = p == 0
        zero = p >> 2

        def f_body(c, c_):
            @pl.when(first)
            def _():
                buf = wa_v.at[pl.ds(3 * c, 3)]
                pltpu.make_async_copy(buf, buf, sems.at[5 + c]).wait()
            xn = xn_v[0:TA, :]

            def tile(part, g):
                t = c * G1 + g
                wu = _pack(wa_v[3 * c + part, :, g * 128:(g + 1) * 128])
                wap[part * 8 + t] = wu
                y = _dot(xn, _unpack(wu))
                if part == 0:
                    store_t(y * QSCALE, qt_v, 0, t)
                elif part == 2:
                    store_t(y, vt_v, 0, t)
                else:
                    kp = _pack(y.astype(BF))
                    k0_v[t] = kp
                    if g + 1 < G1:
                        kt_v[t] = kp[80:128]
                        build_k4(kp, t, 48)
            order = [(1, g) for g in range(G1 - 1)] + \
                    [(part, g) for part in (2, 0) for g in range(G1)] + [(1, G1 - 1)]
            for n, (part, g) in enumerate(order):
                tile(part, g)
                if n == 0:
                    for k in range(NC1 - 2):
                        @pl.when(jnp.logical_and(first, c == k))
                        def _():
                            for cp in cp_wa(k + 2):
                                cp.start()

            @pl.when(jnp.logical_and(first, c == NC1 - 3))
            def _():
                cp_woa.start()

            @pl.when(jnp.logical_and(first, c == NC1 - 2))
            def _():
                cp_x(1).start()
                cp_wb(0).start()
                cp_wob(0).start()
            return c_

        def a_first():
            lax.fori_loop(0, NC1, f_body, 0)
            at = Attn(0)
            at.issue(CFG['flook'])
            while at.issued < 2 * H:
                at.issue()
                at.finish()

            @pl.when(first)
            def _():
                cp_woa.wait()
                cp_x(1).wait()
                cp_wb(0).wait()
                cp_wob(0).wait()
                cp_x(2).start()
                cp_wb(1).start()
                cp_wob(1).start()

            def mk_k4(t):
                def run(tok):
                    k0_v[8, 0:8, :] = pltpu.bitcast(tok[0:8], U32)
                    kp = k0_v[t + zero]
                    kt_v[t] = kp[80:128]
                    build_k4(kp, t, 48)
                return run
            hi = CFG['fhi']
            side = _both(_spread(prep_chunks(zero), 16, 0, hi),
                         _spread(ln_chunks(TA + zero * TA, 0, TA), 16, 0, hi),
                         _spread([mk_k4(t) for t in range(G1 - 1, 8, G1)], 16, 0, hi))
            ou = _lanes(oa0_v[pl.ds(zero, 4)])
            part = []
            yprev = None
            for u in range(16):
                if u == 8:
                    ou = _lanes(oa1_v[...])
                rows = slice((u // 8) * (D // 2), (u // 8 + 1) * (D // 2))
                wu = _pack(woa_v[rows, (u % 8) * 128:(u % 8 + 1) * 128])
                woap[u % 8, (u // 8) * (D // 4):(u // 8 + 1) * (D // 4), :] = wu
                lhs = with_fence(ou, fence_side(zero) | fence_k(zero)) if u == 15 else ou
                y = _dot(_unpack(lhs), _unpack(wu))
                if u == 0:
                    at.finish(2 * H)
                if yprev is not None:
                    release(yprev, side[u - 1])
                yprev = y
                if u < 8:
                    part.append(y)
                else:
                    part[u - 8] = part[u - 8] + y
                    if u % 2 == 1:
                        add_residual(0, TA, (u - 9) * 128, (u - 7) * 128,
                                     lax.concatenate(part[u - 9:u - 7], 1))

        if CFG['first']:
            a_first()

        @pl.when(first)
        def _():
            cp_x(2).wait()
            cp_wb(1).wait()
            cp_wob(1).wait()
            cp_x(3).start()
            cp_wb(2).start()
            for j in range(2, 8):
                cp_wob(j).start()

        def a_body(i, c_):
            @pl.when(jnp.logical_and(first, i == 2))
            def _():
                cp_x(3).wait()
                cp_wb(2).wait()
                for j in range(2, 8):
                    cp_wob(j).wait()
            xu = _pack(xn_v[0:TA, :])
            side = [[] for _ in range(36)]
            for u, c in zip(CFG['ppos'], prep_chunks(i)):
                side[u].append(c)
            for u, c in zip(CFG['lpos'], ln_chunks((((i + 1) & (NA - 1)) + (zero if CFG['lnz'] else 0)) * TA, 0, TA)):
                side[u].append(c)
            at = Attn(i)
            yprev = None
            for u in range(24):
                t, kind = u // 3, u % 3
                if u == 23:
                    at.issue(CFG['look'])
                lhs = xu
                if u >= 2:
                    fen = (fence_k, fence_v, fence_q)[(u - 2) % 3](zero)
                    if u in CFG['fpos']:
                        fen = fence_side(zero) | fen
                    lhs = with_fence(xu, fen)
                y = _dot(_unpack(lhs), _unpack(wap[(8, 16, 0)[kind] + t]))
                if kind == 0:
                    kp = _pack(y.astype(BF))
                    full = _rows([kt_v[t], kp])
                    kt_v[t] = kp[80:128]
                    build_k4(full, t, pl.multiple_of(i * (TA // 2), TA // 2))
                elif kind == 1:
                    store_t(y, vt_v, i * (TA // 128), t)
                else:
                    store_t(y * QSCALE, qt_v, 0, t)
                if yprev is not None:
                    release(yprev, side[u - 1])
                yprev = y
            while at.issued < 2 * H - CFG['tail']:
                at.issue()
                at.finish()
            o1 = _unpack(_lanes(oa0_v[pl.ds(zero, 4)]))
            part = []
            for u in range(8):
                at.issue(2)
                part.append(_dot(o1, _unpack(woap[u, 0:D // 4, :])))
                if u > 0:
                    at.finish(2)
                release(part[-1], side[24 + u])
            assert at.done == 2 * H
            o2 = _lanes(oa1_v[...])
            r = pl.multiple_of(i * TA, TA)
            for c in range(4):
                lhs = with_fence(o2, fence_side(zero)) if 32 + c in CFG['fpos'] else o2
                y = _dot(_unpack(lhs), _unpack(_lanes(woap[2 * c:2 * c + 2, D // 4:, :])))
                release(y, side[32 + c])
                add_residual(r, TA, c * 256, (c + 1) * 256,
                             y + lax.concatenate(part[2 * c:2 * c + 2], 1))
            return c_
        if CFG['a']:
            lax.fori_loop(1, NA, a_body, 0)

        qk_v[8:16, 0:HALO, :] = jnp.zeros((8, HALO, 128), F32)
        v_v[:, 0:HALO, :] = jnp.zeros((8, HALO, 128), F32)

        def b_body(i, c_):
            def send(k):
                for ii in range(NB):
                    @pl.when(jnp.logical_and(p == 1, i == ii))
                    def _():
                        cp_out(ii, k).start()
            ln1 = ln_chunks(i * TB + 256, TA, 256)
            ln2 = ln_chunks((((i + 1) & (NB - 1)) + zero) * TB, 0, TA)
            lg = [logit_b(i, zero, g * 8) for g in range(TB // 8)]
            pv = [pv_b(zero, g * 8) for g in range(TB // 8)]
            n0, n1, n2 = CFG['bn']
            proj_b(xn_v[0:TA, :], 0, _both(_spread(ln1 + ln2, 48, 0, CFG['bln']),
                                           _spread(_flat(lg[0:n0]), 48, 32, 48)))
            xn1 = xn_v[pl.ds(pl.multiple_of(TA + zero * 32, 32), TA), :]
            proj_b(xn1, 256, _both(_spread(_flat(_merge(lg[n0:32], pv[0:32])), 48, 0, 32),
                                   _spread(_flat(lg[32:n1]), 48, 32, 48)))
            out_b(i, 0, 256, _spread(_flat(_merge(lg[n1:64], pv[32:n2])), 16))
            send(0)
            out_b(i, 256, 128, _spread(_flat(pv[n2:64]), 16, 0, CFG['bhi']))
            send(1)
            qk_v[8:16, 0:HALO, :] = qk_v[8:16, TB:TB + HALO, :]
            v_v[:, 0:HALO, :] = v_v[:, TB:TB + HALO, :]
            out_b(i, 384, 128, [[]] * 16)
            send(2)
            return c_
        if CFG['b']:
            lax.fori_loop(0, NB, b_body, 0)
        return carry

    lax.fori_loop(0, 2, one_pass, 0)
    for i in range(NB):
        for k in range(len(OUT_PIECES)):
            cp_out(i, k).wait()


@jax.jit
def pallas_interleave_layers__sliding_block__sliding_local_dilated__prompt_kernel(
    A_x: jax.Array,
    A_wqkv: jax.Array,
    A_wo: jax.Array,
    B_x: jax.Array,
    B_wqkv: jax.Array,
    B_wo: jax.Array,
):
    del B_x
    x = A_x.reshape(S, D)
    any_spec = pl.BlockSpec(memory_space=pl.ANY)
    out = pl.pallas_call(
        _kernel,
        out_shape=jax.ShapeDtypeStruct((S, D), BF),
        in_specs=[any_spec] * 5,
        out_specs=any_spec,
        scratch_shapes=[
            pltpu.VMEM((S + 16, D), BF),
            pltpu.VMEM((3 * NC1, D, G1 * 128), BF),
            pltpu.VMEM((D, D), BF),
            pltpu.VMEM((D + 16, 3 * D), BF),
            pltpu.VMEM((9, D, 128), BF),
            pltpu.VMEM((24, D // 2, 128), U32),
            pltpu.VMEM((8, D // 2, 128), U32),
            pltpu.VMEM((9, 3 * DH, 2, 8, 128), U32),
            pltpu.VMEM((9, DH, 2, 8, 128), U32),
            pltpu.VMEM((2 * TA + 32, D), BF),
            pltpu.VMEM((9, TA // 2, 128), U32),
            pltpu.VMEM((8, 48, 128), U32),
            pltpu.VMEM((H, S // 2, 128), U32),
            pltpu.VMEM((3, D // 2, 128), U32),
            pltpu.VMEM((S // 128 + 1, D // 2, 128), U32),
            pltpu.VMEM((4, TA // 2, 128), U32),
            pltpu.VMEM((4, TA // 2, 128), U32),
            pltpu.VMEM((16, HALO + TB, 128), F32),
            pltpu.VMEM((8, HALO + TB, 128), F32),
            pltpu.VMEM((WB, TB, 128), F32),
            pltpu.VMEM((TB, D), BF),
            pltpu.VMEM((4, 8, 128), U32),
            pltpu.SemaphoreType.DMA((5 + NC1,)),
        ],
        compiler_params=pltpu.CompilerParams(vmem_limit_bytes=100 * 1024 * 1024),
        name="interleave_attn",
    )(x, A_wqkv, A_wo, B_wqkv, B_wo)
    return out.reshape(1, S, D)
```

```python
import math

import jax
import jax.numpy as jnp
from jax import lax
import jax.experimental.pallas as pl
import jax.experimental.pallas.tpu as pltpu

BF = jnp.bfloat16
F32 = jnp.float32
U32 = jnp.uint32

S = 2048
D = 1024
H = 32
DH = 32
TA = 256
NA = S // TA
TB = 512
NB = S // TB
HALO = 16
WB = 8
NEG = -1e30
EPS = 1e-5
QSCALE = (DH ** -0.5) * math.log2(math.e)
NC1 = 4
G1 = 8 // NC1
OUT_PIECES = ((0, 256), (256, 128), (384, 128))

CFG = dict(first=1, a=1, b=1, look=3, tail=8, cuts=(5, 10, 14), lsum=2,
           ppos=(1, 3, 6, 8, 11, 14, 30, 32),
           lpos=(1, 2, 4, 5, 7, 8, 10, 11, 13, 14, 16, 17, 19, 20, 20, 21),
           fpos=(5, 8, 11, 14, 17, 20, 23, 35),
           flook=5, fhi=13,
           bn=(16, 60, 54), bln=28, bhi=11, lns=2, pns=2, lchain=1, lnz=1)


def _dot(a, b):
    return lax.dot_general(a, b, (((1,), (0,)), ((), ())), preferred_element_type=F32)


def _dot_nt(a, b):
    return lax.dot_general(a, b, (((1,), (1,)), ((), ())), preferred_element_type=F32)


def _pack(x_bf16):
    return pltpu.bitcast(x_bf16, U32)


def _unpack(x_u32):
    return pltpu.bitcast(x_u32, BF)


def _iota(shape, dim):
    return lax.broadcasted_iota(jnp.int32, shape, dim)


def _rows(xs):
    return lax.concatenate(xs, 0)


def _lanes(x3):
    n, r, _ = x3.shape
    x2 = x3.reshape(n * r, 128)
    return lax.concatenate([x2[t * r:(t + 1) * r] for t in range(n)], 1)


def _layernorm(x_bf16):
    x = x_bf16.astype(F32)
    m = jnp.sum(x, axis=1, keepdims=True) * (1.0 / D)
    xc = x - m
    v = jnp.sum(xc * xc, axis=1, keepdims=True) * (1.0 / D)
    return (xc * lax.rsqrt(v + EPS)).astype(BF)


def _recip(l):
    r = pl.reciprocal(l, approx=True)
    return r * (2.0 - l * r)


def _swap16(xu):
    for bit in range(4):
        x5 = xu.reshape(8 >> bit, 2, 2 << bit, 8, 128)
        x, y = x5[:, 0:1], x5[:, 1:2]
        if bit == 0:
            x, y = ((x & U32(0xFFFF)) | (y << 16), (x >> 16) | (y & U32(0xFFFF0000)))
        else:
            dist = 1 << (bit - 1)
            lo = (_iota(x.shape, 3) & dist) == 0
            x, y = (lax.select(lo, x, pltpu.roll(y, dist, 3)),
                    lax.select(lo, pltpu.roll(x, 8 - dist, 3), y))
        xu = lax.concatenate([x, y], 1)
    return xu.reshape(16, 2, 8, 128)


def _spread(chunks, nslots, lo=0, hi=None):
    hi = nslots if hi is None else hi
    out = [[] for _ in range(nslots)]
    for u, c in enumerate(chunks):
        out[lo + u * (hi - lo) // len(chunks)].append(c)
    return out


def _merge(a, b):
    out = []
    for u in range(max(len(a), len(b))):
        out += a[u:u + 1] + b[u:u + 1]
    return out


def _flat(lists):
    return sum(lists, [])


def _both(*lists):
    return [sum(parts, []) for parts in zip(*lists)]


def _kernel(x_hbm, wa_hbm, woa_hbm, wb_hbm, wob_hbm, out_hbm,
            x_v, wa_v, woa_v, wb_v, wob_v, wap, woap, wbt, wobp, xn_v,
            k0_v, kt_v, k4_v, qt_v, vt_v, oa0_v, oa1_v, qk_v, v_v, e_v, ob_v, tk_v,
            sems):
    def cp_x(i):
        n = TA if i < 3 else S - 3 * TA
        return pltpu.make_async_copy(x_hbm.at[pl.ds(i * TA, n), :],
                                     x_v.at[pl.ds(i * TA, n), :], sems.at[i])

    def cp_wa(c):
        w = G1 * 128
        return [pltpu.make_async_copy(wa_hbm.at[:, pl.ds(part * D + c * w, w)],
                                      wa_v.at[3 * c + part], sems.at[5 + c])
                for part in range(3)]

    cp_woa = pltpu.make_async_copy(woa_hbm, woa_v, sems.at[1])

    def cp_wb(j):
        n = 128 if j < 2 else D - 256
        return pltpu.make_async_copy(wb_hbm.at[pl.ds(j * 128, n), :],
                                     wb_v.at[pl.ds(j * 128, n), :], sems.at[j + 1])

    def cp_wob(j):
        return pltpu.make_async_copy(wob_hbm.at[:, pl.ds(j * 128, 128)],
                                     wob_v.at[j], sems.at[min(j, 2) + 1])

    def cp_out(i, k, c=None):
        rows = pl.ds(i * TB + OUT_PIECES[k][0], OUT_PIECES[k][1])
        cols = pl.ds(0, D) if c is None else pl.ds(c * (D // 4), D // 4)
        return pltpu.make_async_copy(x_v.at[rows, cols], out_hbm.at[rows, cols], sems.at[4])

    def release(y, chunks):
        n = len(chunks)
        nt = y.shape[1] // 128
        for u, run in enumerate(chunks):
            pos = (u * y.shape[0] * nt // n) // 16 * 16
            t, rr = pos // y.shape[0], pos % y.shape[0]
            run(y[rr:rr + 16, t * 128:(t + 1) * 128])

    def gated(x, tok, zero):
        tk_v[1] = pltpu.bitcast(tok[0:8], U32)
        return pltpu.bitcast(pltpu.bitcast(x, U32) | tk_v[pl.ds(zero, 1)], F32)

    def fence_side(zero):
        zx = _pack(xn_v[pl.ds(pl.multiple_of(2 * TA + zero * 32, 32), 32), 0:128])
        return zx | (wbt[8, 0] | wobp[8, 0]).reshape(16, 128)

    def fence_k(zero):
        return k4_v[zero, 0:16, :]

    def fence_q(zero):
        return qt_v[2 + zero, 0:16, :]

    def fence_v(zero):
        return vt_v[S // 128 + zero, 0:16, :]

    def with_fence(xu, fen):
        r, c = xu.shape
        last = lax.concatenate([xu[r - 16:, :c - 128], xu[r - 16:, c - 128:] | fen], 1)
        return _rows([xu[:r - 16], last])

    def ln_chunks(row0, dst, nrows, step=16):
        def mk(c):
            def run(tok):
                if tok is not None:
                    x_v[S:S + 16, 0:128] = tok.astype(BF)
                r = pl.multiple_of(row0 + c * step, step)
                xn_v[dst + c * step:dst + (c + 1) * step, :] = _layernorm(x_v[pl.ds(r, step), :])
            return run
        return [mk(c) for c in range(nrows // step)]

    def prep_chunks(j):
        def put(xu, dst, d0, hh):
            val = _swap16(xu)
            for dh in range(2):
                dst[j, d0 + dh * 16:d0 + (dh + 1) * 16, hh] = val[:, dh]

        def mk_t(c):
            def run(tok):
                wb_v[D:D + 16, 0:128] = tok.astype(BF)
                rows = pl.ds(pl.multiple_of(j * 128, 128), 128)
                put(_pack(wb_v[rows, c * 512:(c + 1) * 512].T), wbt, (c // 2) * DH, c % 2)
            return run

        def mk_o(c):
            def run(tok):
                wob_v[8, 0:16, :] = tok.astype(BF)
                put(_pack(wob_v[j, c * 512:(c + 1) * 512, :]), wobp, 0, c)
            return run
        return [mk_t(c) for c in range(6)] + [mk_o(c) for c in range(2)]

    def build_k4(full, t, row0):
        n = full.shape[0] - 48
        rolled = [full] + [pltpu.roll(full, 32 * r, 1) for r in range(1, 4)]
        grp_id = _iota((n, 128), 1) >> 5
        is_g = [grp_id == g for g in range(4)]
        for a in range(4):
            val = rolled[(0 - a) % 4][0:n]
            for g in range(1, 4):
                val = lax.select(is_g[g], rolled[(g - a) % 4][16 * g:16 * g + n], val)
            k4_v[4 * t + a, pl.ds(row0, n), :] = val

    def store_t(y, dst, slot0, t):
        yt = _pack(y.astype(BF).T)
        rows = pl.ds(t * 64 if isinstance(t, int) else pl.multiple_of(t * 64, 64), 64)
        for b in range(TA // 128):
            dst[slot0 + b, rows, :] = yt[:, b * 128:(b + 1) * 128]

    class Attn:
        def __init__(self, blk):
            self.blk = blk
            self.first = isinstance(blk, int)
            self.items = [(qb, 4 * t + a) for t in range(8) for qb in range(2) for a in range(4)]
            self.issued, self.done, self.queue, self.outs = 0, 0, [], []
            row, lane = _iota((128, 128), 0), _iota((128, 128), 1)
            self.tri = lane >= row
            if self.first:
                self.neg = jnp.full((128, 128), NEG, F32)
                self.zq = jnp.zeros((16, 128), U32)
            else:
                self.zero = jnp.zeros((128, 128), F32)
                self.slot = (lane >> 5) == (row >> 5)
                new = (_iota((32, 128), 1) & 31) >= _iota((32, 128), 0)
                self.new = (new[0:16], new[16:32])
                lane2 = _iota((256, 128), 1)
                self.odd, self.hi = (lane2 & 32) != 0, lane2 >= 64
                self.base = [pl.multiple_of((blk * 2 + qb) * 64 - 80, 16) for qb in range(2)]

        def scores_first(self, qb, h):
            qh = qt_v[qb, h * 16:(h + 1) * 16, :]
            wq = _unpack(_rows([qh if jj == h % 4 else self.zq for jj in range(4)]))
            n = (qb + 1) * 32
            kk = _unpack(k0_v[h // 4, 0:2 * n, :])
            s = _rows([_dot(kk[c * n:(c + 1) * n], wq) for c in range(4)])
            diag = lax.select(self.tri, s[qb * 128:], self.neg)
            return diag if qb == 0 else _rows([s[0:128], diag])

        def scores(self, qb, h):
            qf = _unpack(qt_v[qb, h * 16:(h + 1) * 16, :]).astype(F32)
            wq = lax.select(self.slot, _rows([qf] * 4), self.zero).astype(BF)
            w = k4_v[h, pl.ds(self.base[qb], 144), :]
            kk = _unpack(_rows([w[0:8], w[128:136], w[8:16], w[136:144], w[16:128]]))
            cuts = (0,) + CFG['cuts'] + (18,)
            s = _rows([_dot(kk[16 * a:16 * b], wq) for a, b in zip(cuts[:-1], cuts[1:])])
            return _rows([lax.select(self.new[0], s[16:32], s[0:16]),
                          lax.select(self.new[1], s[48:64], s[32:48]), s[64:]])

        def softmax_pv(self, s, qb, h):
            mx = jnp.max(s, axis=0, keepdims=True)
            if self.first:
                p = jnp.exp2(s - mx)
                l = jnp.sum(p, axis=0, keepdims=True)
                v3 = vt_v[0:qb + 1, h * 16:(h + 1) * 16, :]
            else:
                s = lax.select(self.odd, _rows([s[224:], s[:224]]), s)
                s = lax.select(self.hi, _rows([s[192:], s[:192]]), s)
                p = jnp.exp2(s - mx)
                if CFG['lsum'] == 0:
                    l = jnp.sum(p, axis=0, keepdims=True)
                else:
                    p3 = p.reshape(2, 128, 128)
                    if CFG['lsum'] == 1:
                        acc = jnp.sum(p.reshape(2, 16, 8, 128), axis=1)
                    else:
                        acc = p3[:, 120:128]
                        for v in range(14, -1, -1):
                            acc = acc + p3[:, 8 * v:8 * v + 8]
                    l = jnp.sum(acc.reshape(16, 128), axis=0, keepdims=True)
                pm = p[0:128]
                p = _rows([lax.select(self.tri, self.zero, pm), p[128:256],
                           lax.select(self.tri, pm, self.zero)])
                v3 = vt_v[pl.ds(self.blk * 2 + qb - 2, 3), h * 16:(h + 1) * 16, :]
            return _dot(_unpack(_lanes(v3)), p.astype(BF)) * _recip(l)

        def issue(self, n=1):
            for _ in range(n):
                if self.issued < len(self.items):
                    fn = self.scores_first if self.first else self.scores
                    self.queue.append(fn(*self.items[self.issued]))
                    self.issued += 1

        def finish(self, n=1):
            for _ in range(n):
                if self.done < self.issued:
                    qb, h = self.items[self.done]
                    self.outs.append(self.softmax_pv(self.queue.pop(0), qb, h))
                    if len(self.outs) == 4:
                        ot = _rows(self.outs).astype(BF)
                        dst = (oa0_v, oa1_v)[h // 16]
                        dst[(h // 4) % 4, qb * 64:(qb + 1) * 64, :] = _pack(ot.T)
                        self.outs = []
                    self.done += 1

    def add_residual(r, nrows, c0, c1, y):
        x_v[pl.ds(r, nrows), c0:c1] = (x_v[pl.ds(r, nrows), c0:c1].astype(F32) + y).astype(BF)

    def proj_b(xn, r0, side):
        rows = slice(HALO + r0, HALO + r0 + xn.shape[0])
        halves = (xn[:, 0:512], xn[:, 512:1024])
        for T in range(24):
            y = None
            for hf in range(2):
                w = wbt[4 * hf:4 * hf + 4, 4 * T:4 * T + 4].reshape(4, 64, 128)
                yh = _dot_nt(halves[hf], _unpack(_lanes(w)))
                y = yh if y is None else y + yh
                if hf == 1:
                    if T < 8:
                        qk_v[T, rows, :] = y * QSCALE
                    elif T < 16:
                        qk_v[T, rows, :] = y
                    else:
                        v_v[T - 16, rows, :] = y
                release(y, side[2 * T + hf])

    def taps(ref, t0, t1, r0):
        wins = [ref[t0:t1, HALO + r0 - 2 * w:HALO + r0 - 2 * w + 8, :] for w in range(WB)]
        return _rows(wins).reshape(WB, t1 - t0, 8, 128)

    def logit_b(i, zero, r0):
        ns = CFG['lns']
        acc = []

        def mk(st):
            def run(tok):
                t0, t1 = st * 8 // ns, (st + 1) * 8 // ns
                q = gated(qk_v[t0:t1, HALO + r0:HALO + r0 + 8, :], tok, zero)
                p = q[None] * taps(qk_v, 8 + t0, 8 + t1, r0)
                if acc and CFG['lchain']:
                    a = jnp.sum(lax.concatenate([acc.pop()[:, None], p], 1), axis=1)
                else:
                    a = jnp.sum(p, axis=1)
                    a = acc.pop() + a if acc else a
                if st + 1 < ns:
                    acc.append(a)
                    return
                a = a + pltpu.roll(a, 64, 2)
                a = a + pltpu.roll(a, 32, 2)
                if r0 < 2 * (WB - 1):
                    pos = _iota(a.shape, 1) - 2 * _iota(a.shape, 0) + (i * TB + r0)
                    a = lax.select(pos >= 0, a, jnp.full(a.shape, NEG, F32))
                e = jnp.exp2(a - jnp.max(a, axis=0, keepdims=True))
                e_v[:, r0:r0 + 8, :] = e * _recip(jnp.sum(e, axis=0, keepdims=True))
            return run
        return [mk(st) for st in range(ns)]

    def pv_b(zero, r0):
        ns = CFG['pns']

        def mk(st):
            def run(tok):
                t0, t1 = st * 8 // ns, (st + 1) * 8 // ns
                e = gated(e_v[:, r0:r0 + 8, :], tok, zero)
                o = jnp.sum(e[:, None] * taps(v_v, t0, t1, r0), axis=0)
                ob_v[r0:r0 + 8, t0 * 128:t1 * 128] = _lanes(o).astype(BF)
            return run
        return [mk(st) for st in range(ns)]

    def out_b(i, r0, nrows, side, done=None):
        o = ob_v[r0:r0 + nrows, :]
        halves = (o[:, 0:512], o[:, 512:1024])
        r = pl.multiple_of(i * TB + r0, 128)
        ys = []
        for T in range(8):
            y = None
            for hf in range(2):
                w = wobp[T, hf * 16:(hf + 1) * 16].reshape(256, 128)
                yh = _dot(halves[hf], _unpack(w))
                y = yh if y is None else y + yh
                release(y, side[2 * T + hf])
            ys.append(y)
            if T % 2 == 1:
                add_residual(r, nrows, (T - 1) * 128, (T + 1) * 128, lax.concatenate(ys[-2:], 1))
                if done is not None:
                    done(T // 2)

    cp_x(0).start()
    for cp in cp_wa(0):
        cp.start()
    z16 = jnp.zeros((16, 128), U32)
    xn_v[2 * TA:2 * TA + 32, :] = jnp.zeros((32, D), BF)
    wbt[8, 0] = z16.reshape(2, 8, 128)
    wobp[8, 0] = z16.reshape(2, 8, 128)
    k4_v[0, 0:16, :] = z16
    vt_v[S // 128, 0:16, :] = z16
    qt_v[2, 0:16, :] = z16
    tk_v[0] = z16[0:8]
    cp_x(0).wait()
    for cp in cp_wa(1):
        cp.start()
    for run in ln_chunks(0, 0, TA, step=TA):
        run(None)

    def one_pass(p, carry):
        first = p == 0
        zero = p >> 2

        def f_body(c, c_):
            @pl.when(first)
            def _():
                buf = wa_v.at[pl.ds(3 * c, 3)]
                pltpu.make_async_copy(buf, buf, sems.at[5 + c]).wait()
            xn = xn_v[0:TA, :]

            def tile(part, g):
                t = c * G1 + g
                wu = _pack(wa_v[3 * c + part, :, g * 128:(g + 1) * 128])
                wap[part * 8 + t] = wu
                y = _dot(xn, _unpack(wu))
                if part == 0:
                    store_t(y * QSCALE, qt_v, 0, t)
                elif part == 2:
                    store_t(y, vt_v, 0, t)
                else:
                    kp = _pack(y.astype(BF))
                    k0_v[t] = kp
                    if g + 1 < G1:
                        kt_v[t] = kp[80:128]
                        build_k4(kp, t, 48)
            order = [(1, g) for g in range(G1 - 1)] + \
                    [(part, g) for part in (2, 0) for g in range(G1)] + [(1, G1 - 1)]
            for n, (part, g) in enumerate(order):
                tile(part, g)
                if n == 0:
                    for k in range(NC1 - 2):
                        @pl.when(jnp.logical_and(first, c == k))
                        def _():
                            for cp in cp_wa(k + 2):
                                cp.start()

            @pl.when(jnp.logical_and(first, c == NC1 - 3))
            def _():
                cp_woa.start()

            @pl.when(jnp.logical_and(first, c == NC1 - 2))
            def _():
                cp_x(1).start()
                cp_wb(0).start()
                cp_wob(0).start()
            return c_

        def a_first():
            lax.fori_loop(0, NC1, f_body, 0)
            at = Attn(0)
            at.issue(CFG['flook'])
            while at.issued < 2 * H:
                at.issue()
                at.finish()

            @pl.when(first)
            def _():
                cp_woa.wait()
                cp_x(1).wait()
                cp_wb(0).wait()
                cp_wob(0).wait()
                cp_x(2).start()
                cp_wb(1).start()
                cp_wob(1).start()

            def mk_k4(t):
                def run(tok):
                    k0_v[8, 0:8, :] = pltpu.bitcast(tok[0:8], U32)
                    kp = k0_v[t + zero]
                    kt_v[t] = kp[80:128]
                    build_k4(kp, t, 48)
                return run
            hi = CFG['fhi']
            side = _both(_spread(prep_chunks(zero), 16, 0, hi),
                         _spread(ln_chunks(TA + zero * TA, 0, TA), 16, 0, hi),
                         _spread([mk_k4(t) for t in range(G1 - 1, 8, G1)], 16, 0, hi))
            ou = _lanes(oa0_v[pl.ds(zero, 4)])
            part = []
            yprev = None
            for u in range(16):
                if u == 8:
                    ou = _lanes(oa1_v[...])
                rows = slice((u // 8) * (D // 2), (u // 8 + 1) * (D // 2))
                wu = _pack(woa_v[rows, (u % 8) * 128:(u % 8 + 1) * 128])
                woap[u % 8, (u // 8) * (D // 4):(u // 8 + 1) * (D // 4), :] = wu
                lhs = with_fence(ou, fence_side(zero) | fence_k(zero)) if u == 15 else ou
                y = _dot(_unpack(lhs), _unpack(wu))
                if u == 0:
                    at.finish(2 * H)
                if yprev is not None:
                    release(yprev, side[u - 1])
                yprev = y
                if u < 8:
                    part.append(y)
                else:
                    part[u - 8] = part[u - 8] + y
                    if u % 2 == 1:
                        add_residual(0, TA, (u - 9) * 128, (u - 7) * 128,
                                     lax.concatenate(part[u - 9:u - 7], 1))

        if CFG['first']:
            a_first()

        @pl.when(first)
        def _():
            cp_x(2).wait()
            cp_wb(1).wait()
            cp_wob(1).wait()
            cp_x(3).start()
            cp_wb(2).start()
            for j in range(2, 8):
                cp_wob(j).start()

        def a_body(i, c_):
            @pl.when(jnp.logical_and(first, i == 2))
            def _():
                cp_x(3).wait()
                cp_wb(2).wait()
                for j in range(2, 8):
                    cp_wob(j).wait()
            xu = _pack(xn_v[0:TA, :])
            side = [[] for _ in range(36)]
            for u, c in zip(CFG['ppos'], prep_chunks(i)):
                side[u].append(c)
            for u, c in zip(CFG['lpos'], ln_chunks((((i + 1) & (NA - 1)) + (zero if CFG['lnz'] else 0)) * TA, 0, TA)):
                side[u].append(c)
            at = Attn(i)
            yprev = None
            for u in range(24):
                t, kind = u // 3, u % 3
                if u == 23:
                    at.issue(CFG['look'])
                lhs = xu
                if u >= 2:
                    fen = (fence_k, fence_v, fence_q)[(u - 2) % 3](zero)
                    if u in CFG['fpos']:
                        fen = fence_side(zero) | fen
                    lhs = with_fence(xu, fen)
                y = _dot(_unpack(lhs), _unpack(wap[(8, 16, 0)[kind] + t]))
                if kind == 0:
                    kp = _pack(y.astype(BF))
                    full = _rows([kt_v[t], kp])
                    kt_v[t] = kp[80:128]
                    build_k4(full, t, pl.multiple_of(i * (TA // 2), TA // 2))
                elif kind == 1:
                    store_t(y, vt_v, i * (TA // 128), t)
                else:
                    store_t(y * QSCALE, qt_v, 0, t)
                if yprev is not None:
                    release(yprev, side[u - 1])
                yprev = y
            while at.issued < 2 * H - CFG['tail']:
                at.issue()
                at.finish()
            o1 = _unpack(_lanes(oa0_v[pl.ds(zero, 4)]))
            part = []
            for u in range(8):
                at.issue(2)
                part.append(_dot(o1, _unpack(woap[u, 0:D // 4, :])))
                if u > 0:
                    at.finish(2)
                release(part[-1], side[24 + u])
            assert at.done == 2 * H
            o2 = _lanes(oa1_v[...])
            r = pl.multiple_of(i * TA, TA)
            for c in range(4):
                lhs = with_fence(o2, fence_side(zero)) if 32 + c in CFG['fpos'] else o2
                y = _dot(_unpack(lhs), _unpack(_lanes(woap[2 * c:2 * c + 2, D // 4:, :])))
                release(y, side[32 + c])
                add_residual(r, TA, c * 256, (c + 1) * 256,
                             y + lax.concatenate(part[2 * c:2 * c + 2], 1))
            return c_
        if CFG['a']:
            lax.fori_loop(1, NA, a_body, 0)

        qk_v[8:16, 0:HALO, :] = jnp.zeros((8, HALO, 128), F32)
        v_v[:, 0:HALO, :] = jnp.zeros((8, HALO, 128), F32)

        def b_body(i, c_):
            def send(k):
                for ii in range(NB if k < 2 else NB - 1):
                    @pl.when(jnp.logical_and(p == 1, i == ii))
                    def _():
                        cp_out(ii, k).start()

            def send_last(c):
                @pl.when(jnp.logical_and(p == 1, i == NB - 1))
                def _():
                    cp_out(NB - 1, 2, c).start()
            ln1 = ln_chunks(i * TB + 256, TA, 256)
            ln2 = ln_chunks((((i + 1) & (NB - 1)) + zero) * TB, 0, TA)
            lg = [logit_b(i, zero, g * 8) for g in range(TB // 8)]
            pv = [pv_b(zero, g * 8) for g in range(TB // 8)]
            n0, n1, n2 = CFG['bn']
            proj_b(xn_v[0:TA, :], 0, _both(_spread(ln1 + ln2, 48, 0, CFG['bln']),
                                           _spread(_flat(lg[0:n0]), 48, 32, 48)))
            xn1 = xn_v[pl.ds(pl.multiple_of(TA + zero * 32, 32), TA), :]
            proj_b(xn1, 256, _both(_spread(_flat(_merge(lg[n0:32], pv[0:32])), 48, 0, 32),
                                   _spread(_flat(lg[32:n1]), 48, 32, 48)))
            out_b(i, 0, 256, _spread(_flat(_merge(lg[n1:64], pv[32:n2])), 16))
            send(0)
            out_b(i, 256, 128, _spread(_flat(pv[n2:64]), 16, 0, CFG['bhi']))
            send(1)
            qk_v[8:16, 0:HALO, :] = qk_v[8:16, TB:TB + HALO, :]
            v_v[:, 0:HALO, :] = v_v[:, TB:TB + HALO, :]
            out_b(i, 384, 128, [[]] * 16, send_last)
            send(2)
            return c_
        if CFG['b']:
            lax.fori_loop(0, NB, b_body, 0)
        return carry

    lax.fori_loop(0, 2, one_pass, 0)
    for i in range(NB):
        for k in range(len(OUT_PIECES)):
            if (i, k) != (NB - 1, 2):
                cp_out(i, k).wait()
    for c in range(4):
        cp_out(NB - 1, 2, c).wait()


@jax.jit
def pallas_interleave_layers__sliding_block__sliding_local_dilated__prompt_kernel(
    A_x: jax.Array,
    A_wqkv: jax.Array,
    A_wo: jax.Array,
    B_x: jax.Array,
    B_wqkv: jax.Array,
    B_wo: jax.Array,
):
    del B_x
    x = A_x.reshape(S, D)
    any_spec = pl.BlockSpec(memory_space=pl.ANY)
    out = pl.pallas_call(
        _kernel,
        out_shape=jax.ShapeDtypeStruct((S, D), BF),
        in_specs=[any_spec] * 5,
        out_specs=any_spec,
        scratch_shapes=[
            pltpu.VMEM((S + 16, D), BF),
            pltpu.VMEM((3 * NC1, D, G1 * 128), BF),
            pltpu.VMEM((D, D), BF),
            pltpu.VMEM((D + 16, 3 * D), BF),
            pltpu.VMEM((9, D, 128), BF),
            pltpu.VMEM((24, D // 2, 128), U32),
            pltpu.VMEM((8, D // 2, 128), U32),
            pltpu.VMEM((9, 3 * DH, 2, 8, 128), U32),
            pltpu.VMEM((9, DH, 2, 8, 128), U32),
            pltpu.VMEM((2 * TA + 32, D), BF),
            pltpu.VMEM((9, TA // 2, 128), U32),
            pltpu.VMEM((8, 48, 128), U32),
            pltpu.VMEM((H, S // 2, 128), U32),
            pltpu.VMEM((3, D // 2, 128), U32),
            pltpu.VMEM((S // 128 + 1, D // 2, 128), U32),
            pltpu.VMEM((4, TA // 2, 128), U32),
            pltpu.VMEM((4, TA // 2, 128), U32),
            pltpu.VMEM((16, HALO + TB, 128), F32),
            pltpu.VMEM((8, HALO + TB, 128), F32),
            pltpu.VMEM((WB, TB, 128), F32),
            pltpu.VMEM((TB, D), BF),
            pltpu.VMEM((4, 8, 128), U32),
            pltpu.SemaphoreType.DMA((5 + NC1,)),
        ],
        compiler_params=pltpu.CompilerParams(vmem_limit_bytes=100 * 1024 * 1024),
        name="interleave_attn",
    )(x, A_wqkv, A_wo, B_wqkv, B_wo)
    return out.reshape(1, S, D)
```

```python
import math

import jax
import jax.numpy as jnp
from jax import lax
import jax.experimental.pallas as pl
import jax.experimental.pallas.tpu as pltpu

BF = jnp.bfloat16
F32 = jnp.float32
U32 = jnp.uint32

S = 2048
D = 1024
H = 32
DH = 32
TA = 256
NA = S // TA
TB = 512
NB = S // TB
HALO = 16
WB = 8
NEG = -1e30
EPS = 1e-5
HD = D // 2
QSCALE = (DH ** -0.5) * math.log2(math.e)
NC1 = 4
G1 = 8 // NC1
OUT_PIECES = ((0, 256), (256, 128), (384, 128))

CFG = dict(first=1, a=1, b=1, look=3, tail=8, cuts=(5, 10, 14), lsum=2,
           lag=4, ppos=(6, 27, 48, 98), llo=2, lhi=72,
           fpos=(20, 34, 48, 62, 76, 83, 111),
           flook=5, fhi=22, forder=(2, 0, 1),
           bn=(16, 60, 27), bln=50, bhi=18, lns=2, lchain=1)


def _dot(a, b):
    return lax.dot_general(a, b, (((1,), (0,)), ((), ())), preferred_element_type=F32)


def _dot_nt(a, b):
    return lax.dot_general(a, b, (((1,), (1,)), ((), ())), preferred_element_type=F32)


def _pack(x_bf16):
    return pltpu.bitcast(x_bf16, U32)


def _unpack(x_u32):
    return pltpu.bitcast(x_u32, BF)


def _iota(shape, dim):
    return lax.broadcasted_iota(jnp.int32, shape, dim)


def _rows(xs):
    return lax.concatenate(xs, 0)


def _lanes(x3):
    n, r, _ = x3.shape
    x2 = x3.reshape(n * r, 128)
    return lax.concatenate([x2[t * r:(t + 1) * r] for t in range(n)], 1)


def _layernorm(x_bf16):
    x = x_bf16.astype(F32)
    m = jnp.sum(x, axis=1, keepdims=True) * (1.0 / D)
    xc = x - m
    v = jnp.sum(xc * xc, axis=1, keepdims=True) * (1.0 / D)
    return xc * lax.rsqrt(v + EPS)


def _lhs7(x11, x12, x21, x22):
    return [x11 + x22, x21 + x22, x11, x22, x11 + x12, x21 - x11, x12 - x22]


def _rhs7(w11, w12, w21, w22):
    return [w11 + w22, w11, w12 - w22, w21 - w11, w22, w11 + w12, w21 + w22]


RAW = (1, 4)


def _strassen(prod, left, right=None):
    m1 = prod(1)
    m3 = prod(3)
    y21 = m1 + m3
    m0 = prod(0)
    y11, y22 = m3 + m0, m0 - m1
    y11 = y11 + prod(6)
    m4 = prod(4)
    y11 = y11 - m4
    if right is not None:
        left(y11, y21)
    m2 = prod(2)
    y12 = m2 + m4
    y22 = (y22 + m2) + prod(5)
    if right is not None:
        right(y12, y22)
    else:
        left(y11, y12, y21, y22)


def _weave(top, bot):
    n, c = top.shape
    both = lax.concatenate([top.reshape(n // 8, 1, 8, c), bot.reshape(n // 8, 1, 8, c)], 1)
    return both.reshape(2 * n, c)


def _recip(l):
    r = pl.reciprocal(l, approx=True)
    return r * (2.0 - l * r)


def _swap16(xu):
    for bit in range(4):
        x5 = xu.reshape(8 >> bit, 2, 2 << bit, 8, 128)
        x, y = x5[:, 0:1], x5[:, 1:2]
        if bit == 0:
            x, y = ((x & U32(0xFFFF)) | (y << 16), (x >> 16) | (y & U32(0xFFFF0000)))
        else:
            dist = 1 << (bit - 1)
            lo = (_iota(x.shape, 3) & dist) == 0
            x, y = (lax.select(lo, x, pltpu.roll(y, dist, 3)),
                    lax.select(lo, pltpu.roll(x, 8 - dist, 3), y))
        xu = lax.concatenate([x, y], 1)
    return xu.reshape(16, 2, 8, 128)


def _spread(chunks, nslots, lo=0, hi=None):
    hi = nslots if hi is None else hi
    out = [[] for _ in range(nslots)]
    for u, c in enumerate(chunks):
        out[lo + u * (hi - lo) // len(chunks)].append(c)
    return out


def _merge(a, b):
    out = []
    for u in range(max(len(a), len(b))):
        out += a[u:u + 1] + b[u:u + 1]
    return out


def _flat(lists):
    return sum(lists, [])


def _both(*lists):
    return [sum(parts, []) for parts in zip(*lists)]


def _kernel(x_hbm, wa_hbm, woa_hbm, wb_hbm, wob_hbm, out_hbm,
            x_v, wa_v, woa_v, wb_v, wob_v, wap, woap, wbt, wobp, xl_v,
            k0_v, kt_v, k4_v, qt_v, vt_v, oa0_v, oa1_v, qk_v, v_v, e_v, ob_v, tk_v,
            sems):
    def cp_x(i):
        n = TA if i < 3 else S - 3 * TA
        return pltpu.make_async_copy(x_hbm.at[pl.ds(i * TA, n), :],
                                     x_v.at[pl.ds(i * TA, n), :], sems.at[i])

    def cp_wa(c):
        w = G1 * 128
        return [pltpu.make_async_copy(wa_hbm.at[:, pl.ds(part * D + c * w, w)],
                                      wa_v.at[3 * c + part], sems.at[5 + c])
                for part in range(3)]

    cp_woa = pltpu.make_async_copy(woa_hbm, woa_v, sems.at[1])

    def cp_wb(st):
        if st < 2:
            qkv = [(2 * part + st, r0, 128) for part in range(3) for r0 in (0, 512)]
            out = [(0, 512 * st, 512)]
        else:
            qkv = [(c, r0, 384) for c in range(6) for r0 in (128, 640)]
            out = [(c, 0, D) for c in range(1, 4)]
        sem = sems.at[st + 1]
        return ([pltpu.make_async_copy(wb_hbm.at[pl.ds(r0, n), pl.ds(c * 512, 512)],
                                       wb_v.at[c, pl.ds(r0, n), :], sem) for c, r0, n in qkv]
                + [pltpu.make_async_copy(wob_hbm.at[pl.ds(r0, n), pl.ds(c * 256, 256)],
                                         wob_v.at[c, pl.ds(r0, n), :], sem) for c, r0, n in out])

    def cp_out(i, k, c=None):
        rows = pl.ds(i * TB + OUT_PIECES[k][0], OUT_PIECES[k][1])
        cols = pl.ds(0, D) if c is None else pl.ds(c * (D // 4), D // 4)
        return pltpu.make_async_copy(x_v.at[rows, cols], out_hbm.at[rows, cols], sems.at[4])

    def release(y, chunks):
        n = len(chunks)
        nt = y.shape[1] // 128
        for u, run in enumerate(chunks):
            pos = (u * y.shape[0] * nt // n) // 16 * 16
            t, rr = pos // y.shape[0], pos % y.shape[0]
            run(y[rr:rr + 16, t * 128:(t + 1) * 128])

    def gated(x, tok, zero):
        tk_v[1] = pltpu.bitcast(tok[0:8], U32)
        return pltpu.bitcast(pltpu.bitcast(x, U32) | tk_v[pl.ds(zero, 1)], F32)

    def fence_side(zero):
        zx = _pack(xl_v[pl.ds(pl.multiple_of(TA + zero * 32, 32), 32), 0:128])
        return zx | (wbt[4, 0, 0] | wobp[4, 0, 0]).reshape(16, 128)

    def fence_k(zero):
        return k4_v[zero, 0:16, :]

    def fence_q(zero):
        return qt_v[2 + zero, 0:16, :]

    def fence_v(zero):
        return vt_v[S // 128 + zero, 0:16, :]

    def with_fence(xu, fen):
        r, c = xu.shape
        last = lax.concatenate([xu[r - 16:, :c - 128], xu[r - 16:, c - 128:] | fen], 1)
        return _rows([xu[:r - 16], last])

    def ln_chunks(row0, dst, nrows, step=16):
        def mk(c):
            def run(tok):
                if tok is not None:
                    x_v[S:S + 16, 0:128] = tok.astype(BF)
                r = pl.multiple_of(row0 + c * step, step)
                xn = _layernorm(x_v[pl.ds(r, step), :]).reshape(step // 16, 2, 8, D)
                top, bot = xn[:, 0].reshape(step // 2, D), xn[:, 1].reshape(step // 2, D)
                ls = _lhs7(top[:, :HD], top[:, HD:], bot[:, :HD], bot[:, HD:])
                o = dst + c * (step // 2)
                xl_v[o:o + step // 2, :] = lax.concatenate(ls, 1).astype(BF)
            return run
        return [mk(c) for c in range(nrows // step)]

    def prep_chunks(j):
        blk, hh = j >> 1, j & 1

        def put(dst, d0, quads):
            wide = [_unpack(w.reshape(128, 128)).astype(F32) for w in quads]
            for k, r in enumerate(_rhs7(*wide)):
                val = quads[3 * (k == 4)] if k in RAW else _pack(r.astype(BF)).reshape(16, 8, 128)
                dst[blk, k, d0:d0 + 16, hh] = val

        def mk_t(part):
            def run(tok):
                wb_v[0, D:D + 16, 0:128] = tok.astype(BF)
                v1, v2 = [_swap16(_pack(
                    wb_v[2 * part + hh, pl.ds(pl.multiple_of(blk * 128 + r0, 128), 128), :].T))
                    for r0 in (0, HD)]
                put(wbt, part * 16, [v1[:, 0], v1[:, 1], v2[:, 0], v2[:, 1]])
            return run

        def run_o(tok):
            wob_v[4, 0:16, 0:128] = tok.astype(BF)
            w = _pack(wob_v[blk, pl.ds(pl.multiple_of(hh * HD, HD), HD), :])
            va, vb = _swap16(w[:, 0:128]), _swap16(w[:, 128:256])
            put(wobp, 0, [va[:, 0], vb[:, 0], va[:, 1], vb[:, 1]])
        return [mk_t(part) for part in range(3)] + [run_o]

    class Stream:
        def __init__(self, side, fences, lag):
            self.side, self.fences, self.lag = side, fences, lag
            self.u, self.ys = 0, []

        def dot(self, fn, lhs_u, w):
            if self.u in self.fences:
                lhs_u = with_fence(lhs_u, self.fences[self.u]())
            y = fn(_unpack(lhs_u), w)
            self.ys.append(y)
            if self.u >= self.lag:
                release(self.ys[self.u - self.lag], self.side[self.u - self.lag])
            self.u += 1
            return y

    def make_rhs(quads, store):
        rs = _rhs7(*[w.astype(F32) for w in quads])
        out = []
        for k, r in enumerate(rs):
            if k in RAW:
                wu = _pack(quads[3 * (k == 4)])
                store(k, wu)
                out.append(_unpack(wu))
            else:
                r = r.astype(BF)
                store(k, _pack(r.T))
                out.append(r)
        return out

    def build_k4(full, t, row0):
        n = full.shape[0] - 48
        rolled = [full] + [pltpu.roll(full, 32 * r, 1) for r in range(1, 4)]
        grp_id = _iota((n, 128), 1) >> 5
        is_g = [grp_id == g for g in range(4)]
        for a in range(4):
            val = rolled[(0 - a) % 4][0:n]
            for g in range(1, 4):
                val = lax.select(is_g[g], rolled[(g - a) % 4][16 * g:16 * g + n], val)
            k4_v[4 * t + a, pl.ds(row0, n), :] = val

    def store_t(y, dst, slot0, t):
        yt = _pack(y.astype(BF).T)
        rows = pl.ds(t * 64 if isinstance(t, int) else pl.multiple_of(t * 64, 64), 64)
        for b in range(TA // 128):
            dst[slot0 + b, rows, :] = yt[:, b * 128:(b + 1) * 128]

    class Attn:
        def __init__(self, blk):
            self.blk = blk
            self.first = isinstance(blk, int)
            self.items = [(qb, 4 * t + a) for t in range(8) for qb in range(2) for a in range(4)]
            self.issued, self.done, self.queue, self.outs, self.tiles = 0, 0, [], [], []
            row, lane = _iota((128, 128), 0), _iota((128, 128), 1)
            self.tri = lane >= row
            if self.first:
                self.neg = jnp.full((128, 128), NEG, F32)
                self.zq = jnp.zeros((16, 128), U32)
            else:
                self.zero = jnp.zeros((128, 128), F32)
                self.slot = (lane >> 5) == (row >> 5)
                new = (_iota((32, 128), 1) & 31) >= _iota((32, 128), 0)
                self.new = (new[0:16], new[16:32])
                lane2 = _iota((256, 128), 1)
                self.odd, self.hi = (lane2 & 32) != 0, lane2 >= 64
                self.base = [pl.multiple_of((blk * 2 + qb) * 64 - 80, 16) for qb in range(2)]

        def scores_first(self, qb, h):
            qh = qt_v[qb, h * 16:(h + 1) * 16, :]
            wq = _unpack(_rows([qh if jj == h % 4 else self.zq for jj in range(4)]))
            n = (qb + 1) * 32
            kk = _unpack(k0_v[h // 4, 0:2 * n, :])
            s = _rows([_dot(kk[c * n:(c + 1) * n], wq) for c in range(4)])
            diag = lax.select(self.tri, s[qb * 128:], self.neg)
            return diag if qb == 0 else _rows([s[0:128], diag])

        def scores(self, qb, h):
            qf = _unpack(qt_v[qb, h * 16:(h + 1) * 16, :]).astype(F32)
            wq = lax.select(self.slot, _rows([qf] * 4), self.zero).astype(BF)
            w = k4_v[h, pl.ds(self.base[qb], 144), :]
            kk = _unpack(_rows([w[0:8], w[128:136], w[8:16], w[136:144], w[16:128]]))
            cuts = (0,) + CFG['cuts'] + (18,)
            s = _rows([_dot(kk[16 * a:16 * b], wq) for a, b in zip(cuts[:-1], cuts[1:])])
            return _rows([lax.select(self.new[0], s[16:32], s[0:16]),
                          lax.select(self.new[1], s[48:64], s[32:48]), s[64:]])

        def softmax_pv(self, s, qb, h):
            mx = jnp.max(s, axis=0, keepdims=True)
            if self.first:
                p = jnp.exp2(s - mx)
                l = jnp.sum(p, axis=0, keepdims=True)
                v3 = vt_v[0:qb + 1, h * 16:(h + 1) * 16, :]
            else:
                s = lax.select(self.odd, _rows([s[224:], s[:224]]), s)
                s = lax.select(self.hi, _rows([s[192:], s[:192]]), s)
                p = jnp.exp2(s - mx)
                if CFG['lsum'] == 0:
                    l = jnp.sum(p, axis=0, keepdims=True)
                else:
                    p3 = p.reshape(2, 128, 128)
                    if CFG['lsum'] == 1:
                        acc = jnp.sum(p.reshape(2, 16, 8, 128), axis=1)
                    else:
                        acc = p3[:, 120:128]
                        for v in range(14, -1, -1):
                            acc = acc + p3[:, 8 * v:8 * v + 8]
                    l = jnp.sum(acc.reshape(16, 128), axis=0, keepdims=True)
                pm = p[0:128]
                p = _rows([lax.select(self.tri, self.zero, pm), p[128:256],
                           lax.select(self.tri, pm, self.zero)])
                v3 = vt_v[pl.ds(self.blk * 2 + qb - 2, 3), h * 16:(h + 1) * 16, :]
            return _dot(_unpack(_lanes(v3)), p.astype(BF)) * _recip(l)

        def store_o(self, gp):
            x = self.tiles
            ready = {2: (2, 5), 4: (4, 0, 1, 3, 6)}.get(len(x), ())
            if ready:
                ls = _lhs7(x[0], x[2 % len(x)], x[1], x[3 % len(x)])
                for k in ready:
                    (oa0_v, oa1_v)[gp // 2][k, gp % 2] = _pack(ls[k].astype(BF).T)
            if len(x) == 4:
                self.tiles = []

        def issue(self, n=1):
            for _ in range(n):
                if self.issued < len(self.items):
                    fn = self.scores_first if self.first else self.scores
                    self.queue.append(fn(*self.items[self.issued]))
                    self.issued += 1

        def finish(self, n=1):
            for _ in range(n):
                if self.done < self.issued:
                    qb, h = self.items[self.done]
                    self.outs.append(self.softmax_pv(self.queue.pop(0), qb, h))
                    if len(self.outs) == 4:
                        self.tiles.append(_rows(self.outs))
                        self.outs = []
                        self.store_o(h // 8)
                    self.done += 1

    def add_residual(r, nrows, c0, c1, y):
        x_v[pl.ds(r, nrows), c0:c1] = (x_v[pl.ds(r, nrows), c0:c1].astype(F32) + y).astype(BF)

    def proj_b(xl, r0, side):
        rows = slice(HALO + r0, HALO + r0 + TA)
        xu = _pack(xl)
        st = Stream(side, {}, 0)
        for P in range(12):
            def prod(k):
                w = wbt[0:4, k, 4 * P:4 * P + 4].reshape(4, 64, 128)
                return st.dot(_dot_nt, xu[:, k * HD:(k + 1) * HD], _unpack(_lanes(w)))

            def put(T):
                def run(top, bot):
                    y = _weave(top, bot)
                    if T < 8:
                        qk_v[T, rows, :] = y * QSCALE
                    elif T < 16:
                        qk_v[T, rows, :] = y
                    else:
                        v_v[T - 16, rows, :] = y
                return run
            T = (P // 4) * 8 + P % 4
            _strassen(prod, put(T), put(T + 4))

    def taps(ref, t0, t1, r0):
        wins = [ref[t0:t1, HALO + r0 - 2 * w:HALO + r0 - 2 * w + 8, :] for w in range(WB)]
        return _rows(wins).reshape(WB, t1 - t0, 8, 128)

    def logit_b(i, zero, r0):
        ns = CFG['lns']
        acc = []

        def mk(st):
            def run(tok):
                t0, t1 = st * 8 // ns, (st + 1) * 8 // ns
                q = gated(qk_v[t0:t1, HALO + r0:HALO + r0 + 8, :], tok, zero)
                p = q[None] * taps(qk_v, 8 + t0, 8 + t1, r0)
                if acc and CFG['lchain']:
                    a = jnp.sum(lax.concatenate([acc.pop()[:, None], p], 1), axis=1)
                else:
                    a = jnp.sum(p, axis=1)
                    a = acc.pop() + a if acc else a
                if st + 1 < ns:
                    acc.append(a)
                    return
                a = a + pltpu.roll(a, 64, 2)
                a = a + pltpu.roll(a, 32, 2)
                if r0 < 2 * (WB - 1):
                    pos = _iota(a.shape, 1) - 2 * _iota(a.shape, 0) + (i * TB + r0)
                    a = lax.select(pos >= 0, a, jnp.full(a.shape, NEG, F32))
                e = jnp.exp2(a - jnp.max(a, axis=0, keepdims=True))
                e_v[:, r0:r0 + 8, :] = e * _recip(jnp.sum(e, axis=0, keepdims=True))
            return run
        return [mk(st) for st in range(ns)]

    def pv_b(zero, r0):
        x = []

        def mk(st):
            def run(tok):
                r, t0 = r0 + 8 * (st // 2), 4 * (st % 2)
                e = gated(e_v[:, r:r + 8, :], tok, zero)
                x.append(_lanes(jnp.sum(e[:, None] * taps(v_v, t0, t0 + 4, r), axis=0)))
                if st == 3:
                    ob_v[r0 // 2:r0 // 2 + 8, :] = lax.concatenate(_lhs7(*x), 1).astype(BF)
            return run
        return [mk(st) for st in range(4)]

    def out_b(i, r0, nrows, side, done=None):
        ou = _pack(ob_v[r0 // 2:(r0 + nrows) // 2, :])
        r = pl.multiple_of(i * TB + r0, 128)
        st = Stream(side, {}, 0)
        for c in range(4):
            def prod(k):
                w = _unpack(wobp[c, k].reshape(256, 128))
                return st.dot(_dot, ou[:, k * HD:(k + 1) * HD], w)

            def put(y11, y12, y21, y22):
                y = _weave(lax.concatenate([y11, y12], 1), lax.concatenate([y21, y22], 1))
                add_residual(r, nrows, c * 256, (c + 1) * 256, y)
            _strassen(prod, put)
            if done is not None:
                done(c)

    cp_x(0).start()
    for cp in cp_wa(0):
        cp.start()
    z16 = jnp.zeros((16, 128), U32)
    xl_v[TA:TA + 32, 0:128] = jnp.zeros((32, 128), BF)
    wbt[4, 0, 0] = z16.reshape(2, 8, 128)
    wobp[4, 0, 0] = z16.reshape(2, 8, 128)
    k4_v[0, 0:16, :] = z16
    vt_v[S // 128, 0:16, :] = z16
    qt_v[2, 0:16, :] = z16
    tk_v[0] = z16[0:8]
    cp_x(0).wait()
    for cp in cp_wa(1):
        cp.start()
    for run in ln_chunks(0, 0, TA, step=TA):
        run(None)

    def one_pass(p, carry):
        first = p == 0
        zero = p >> 2

        def out_a(blk, zero, st, weights, after):
            part = {}
            n = [0]
            for ph in range(2):
                ou = oa0_v[pl.ds(zero, 7)] if ph == 0 else oa1_v[...]
                for nh in range(2):
                    get = weights(ph, nh)

                    def prod(k):
                        fn, w = get(k)
                        y = st.dot(fn, _lanes(ou[k]), w)
                        n[0] += 1
                        after(n[0])
                        return y

                    def put(half):
                        def run(top, bot):
                            y = _rows([top, bot])
                            if ph == 0:
                                part[nh, half] = y
                            else:
                                c0 = nh * HD + half * 256
                                add_residual(blk, TA, c0, c0 + 256, y + part[nh, half])
                        return run
                    _strassen(prod, put(0), put(1))

        def f_body(c, c_):
            @pl.when(first)
            def _():
                buf = wa_v.at[pl.ds(3 * c, 3)]
                pltpu.make_async_copy(buf, buf, sems.at[5 + c]).wait()
            xl = xl_v[0:TA // 2, :]
            for n, part in enumerate(CFG['forder']):
                w = wa_v[3 * c + part]

                def keep(k, wu):
                    if k not in RAW:
                        wu = _rows([wu[:, j * 128:(j + 1) * 128] for j in range(4)])
                    wap[(part * 4 + c) * 7 + k] = wu
                rs = make_rhs([w[:HD, :128], w[:HD, 128:], w[HD:, :128], w[HD:, 128:]], keep)

                def put(t):
                    def run(top, bot):
                        y = _weave(top, bot)
                        if part == 0:
                            store_t(y * QSCALE, qt_v, 0, t)
                        elif part == 2:
                            store_t(y, vt_v, 0, t)
                        else:
                            kp = _pack(y.astype(BF))
                            k0_v[t] = kp
                            if n < 2:
                                kt_v[t] = kp[80:128]
                                build_k4(kp, t, 48)
                    return run
                _strassen(lambda k: _dot(xl[:, k * HD:(k + 1) * HD], rs[k]),
                          put(2 * c), put(2 * c + 1))
                if n == 0:
                    for k in range(NC1 - 2):
                        @pl.when(jnp.logical_and(first, c == k))
                        def _():
                            for cp in cp_wa(k + 2):
                                cp.start()

            @pl.when(jnp.logical_and(first, c == NC1 - 3))
            def _():
                cp_woa.start()

            @pl.when(jnp.logical_and(first, c == NC1 - 2))
            def _():
                cp_x(1).start()
                for cp in cp_wb(0):
                    cp.start()
            return c_

        def a_first():
            lax.fori_loop(0, NC1, f_body, 0)
            at = Attn(0)
            at.issue(CFG['flook'])
            while at.issued < 2 * H:
                at.issue()
                at.finish()

            @pl.when(first)
            def _():
                cp_woa.wait()
                cp_x(1).wait()
                for cp in cp_wb(0):
                    cp.wait()
                cp_x(2).start()
                for cp in cp_wb(1):
                    cp.start()

            def mk_k4(t):
                def run(tok):
                    k0_v[8, 0:8, :] = pltpu.bitcast(tok[0:8], U32)
                    kp = k0_v[t + zero]
                    kt_v[t] = kp[80:128]
                    build_k4(kp, t, 48)
                return run
            hi = CFG['fhi']
            side = _both(_spread(prep_chunks(zero), 28, 0, hi),
                         _spread(ln_chunks(TA + zero * TA, 0, TA), 28, 0, hi))
            if CFG['forder'][2] == 1:
                side = _both(side, _spread([mk_k4(t) for t in range(8)], 28, 0, hi))
            st = Stream(side, {27: lambda: fence_side(zero) | fence_k(zero)}, 1)

            def weights(ph, nh):
                w = [woa_v[(4 * ph + g) * 128:(4 * ph + g + 1) * 128, nh * HD:(nh + 1) * HD]
                     for g in range(4)]
                w1, w2 = _rows([w[0], w[2]]), _rows([w[1], w[3]])

                def keep(k, wu):
                    woap[(ph * 2 + nh) * 7 + k] = _rows([wu[:, :128], wu[:, 128:]])
                rs = make_rhs([w1[:, :256], w1[:, 256:], w2[:, :256], w2[:, 256:]], keep)
                return lambda k: (_dot, rs[k])
            out_a(0, zero, st, weights, lambda u: at.finish(2 * H if u == 1 else 0))

        if CFG['first']:
            a_first()

        @pl.when(first)
        def _():
            cp_x(2).wait()
            for cp in cp_wb(1):
                cp.wait()
            cp_x(3).start()
            for cp in cp_wb(2):
                cp.start()

        def a_body(i, c_):
            @pl.when(jnp.logical_and(first, i == 2))
            def _():
                cp_x(3).wait()
                for cp in cp_wb(2):
                    cp.wait()
            xu = _pack(xl_v[0:TA // 2, :])
            side = _spread(ln_chunks((((i + 1) & (NA - 1)) + zero) * TA, 0, TA),
                           112, CFG['llo'], CFG['lhi'])
            for u, c in zip(CFG['ppos'], prep_chunks(i)):
                side[u].append(c)
            fences = {u: (lambda: fence_side(zero)) for u in CFG['fpos']}
            for n in range(1, 12):
                fe = (fence_k, fence_v, fence_q)[(n - 1) % 3]
                u = 7 * n + 6
                fences[u] = ((lambda fe=fe: fe(zero) | fence_side(zero)) if u in fences
                             else (lambda fe=fe: fe(zero)))
            st = Stream(side, fences, CFG['lag'])
            at = Attn(i)
            for n in range(12):
                gp, kind = n // 3, n % 3

                def prod(k):
                    if n == 11 and k == 4:
                        at.issue(CFG['look'])
                    w = wap[((1, 2, 0)[kind] * 4 + gp) * 7 + k]
                    lhs = xu[:, k * HD:(k + 1) * HD]
                    if k in RAW:
                        return st.dot(_dot, lhs, _unpack(w))
                    return st.dot(_dot_nt, lhs, _unpack(_lanes(w.reshape(4, 64, 128))))

                def put(t):
                    def run(top, bot):
                        y = _weave(top, bot)
                        if kind == 0:
                            kp = _pack(y.astype(BF))
                            full = _rows([kt_v[t], kp])
                            kt_v[t] = kp[80:128]
                            build_k4(full, t, pl.multiple_of(i * (TA // 2), TA // 2))
                        elif kind == 1:
                            store_t(y, vt_v, i * (TA // 128), t)
                        else:
                            store_t(y * QSCALE, qt_v, 0, t)
                    return run
                _strassen(prod, put(2 * gp), put(2 * gp + 1))
            while at.issued < 2 * H - CFG['tail']:
                at.issue()
                at.finish()

            def weights(ph, nh):
                def get(k):
                    w = _unpack(_lanes(woap[(ph * 2 + nh) * 7 + k].reshape(2, 128, 128)))
                    return (_dot if k in RAW else _dot_nt), w
                return get

            def after(u):
                at.finish()
                at.issue()
            at.issue()
            out_a(pl.multiple_of(i * TA, TA), zero, st, weights, after)
            assert at.done == 2 * H
            return c_
        if CFG['a']:
            lax.fori_loop(1, NA, a_body, 0)

        qk_v[8:16, 0:HALO, :] = jnp.zeros((8, HALO, 128), F32)
        v_v[:, 0:HALO, :] = jnp.zeros((8, HALO, 128), F32)

        def b_body(i, c_):
            def send(k):
                for ii in range(NB if k < 2 else NB - 1):
                    @pl.when(jnp.logical_and(p == 1, i == ii))
                    def _():
                        cp_out(ii, k).start()

            def send_last(c):
                @pl.when(jnp.logical_and(p == 1, i == NB - 1))
                def _():
                    cp_out(NB - 1, 2, c).start()
            ln1 = ln_chunks(i * TB + 256, TA // 2, 256)
            ln2 = ln_chunks((((i + 1) & (NB - 1)) + zero) * TB, 0, TA)
            lg = [logit_b(i, zero, g * 8) for g in range(TB // 8)]
            pv = [pv_b(zero, g * 16) for g in range(TB // 16)]
            n0, n1, n2 = CFG['bn']

            def mix(a, b):
                return _flat(_merge([_flat(a[u:u + 2]) for u in range(0, len(a), 2)], b))
            proj_b(xl_v[0:TA // 2, :], 0, _both(_spread(ln1 + ln2, 84, 0, CFG['bln']),
                                                _spread(_flat(lg[0:n0]), 84, 57, 84)))
            xl1 = xl_v[pl.ds(pl.multiple_of(TA // 2 + zero * 32, 32), TA // 2), :]
            proj_b(xl1, 256, _both(_spread(mix(lg[n0:32], pv[0:16]), 84, 1, 57),
                                   _spread(_flat(lg[32:n1]), 84, 57, 84)))
            out_b(i, 0, 256, _spread(mix(lg[n1:64], pv[16:n2]), 28, 1, 28))
            send(0)
            out_b(i, 256, 128, _spread(_flat(pv[n2:32]), 28, 0, CFG['bhi']))
            send(1)
            qk_v[8:16, 0:HALO, :] = qk_v[8:16, TB:TB + HALO, :]
            v_v[:, 0:HALO, :] = v_v[:, TB:TB + HALO, :]
            out_b(i, 384, 128, [[]] * 28, send_last)
            send(2)
            return c_
        if CFG['b']:
            lax.fori_loop(0, NB, b_body, 0)
        return carry

    lax.fori_loop(0, 2, one_pass, 0)
    for i in range(NB):
        for k in range(len(OUT_PIECES)):
            if (i, k) != (NB - 1, 2):
                cp_out(i, k).wait()
    for c in range(4):
        cp_out(NB - 1, 2, c).wait()


@jax.jit
def pallas_interleave_layers__sliding_block__sliding_local_dilated__prompt_kernel(
    A_x: jax.Array,
    A_wqkv: jax.Array,
    A_wo: jax.Array,
    B_x: jax.Array,
    B_wqkv: jax.Array,
    B_wo: jax.Array,
):
    del B_x
    x = A_x.reshape(S, D)
    any_spec = pl.BlockSpec(memory_space=pl.ANY)
    out = pl.pallas_call(
        _kernel,
        out_shape=jax.ShapeDtypeStruct((S, D), BF),
        in_specs=[any_spec] * 5,
        out_specs=any_spec,
        scratch_shapes=[
            pltpu.VMEM((S + 16, D), BF),
            pltpu.VMEM((3 * NC1, D, G1 * 128), BF),
            pltpu.VMEM((D, D), BF),
            pltpu.VMEM((6, D + 16, 512), BF),
            pltpu.VMEM((5, D, 256), BF),
            pltpu.VMEM((84, 256, 128), U32),
            pltpu.VMEM((28, 256, 128), U32),
            pltpu.VMEM((5, 7, 48, 2, 8, 128), U32),
            pltpu.VMEM((5, 7, 16, 2, 8, 128), U32),
            pltpu.VMEM((TA + 32, 7 * HD), BF),
            pltpu.VMEM((9, TA // 2, 128), U32),
            pltpu.VMEM((8, 48, 128), U32),
            pltpu.VMEM((H, S // 2, 128), U32),
            pltpu.VMEM((3, D // 2, 128), U32),
            pltpu.VMEM((S // 128 + 1, D // 2, 128), U32),
            pltpu.VMEM((7, 2, 64, 128), U32),
            pltpu.VMEM((7, 2, 64, 128), U32),
            pltpu.VMEM((16, HALO + TB, 128), F32),
            pltpu.VMEM((8, HALO + TB, 128), F32),
            pltpu.VMEM((WB, TB, 128), F32),
            pltpu.VMEM((TB // 2, 7 * HD), BF),
            pltpu.VMEM((4, 8, 128), U32),
            pltpu.SemaphoreType.DMA((5 + NC1,)),
        ],
        compiler_params=pltpu.CompilerParams(vmem_limit_bytes=112 * 1024 * 1024),
        name="interleave_attn",
    )(x, A_wqkv, A_wo, B_wqkv, B_wo)
    return out.reshape(1, S, D)
```

```python
import math

import jax
import jax.numpy as jnp
from jax import lax
import jax.experimental.pallas as pl
import jax.experimental.pallas.tpu as pltpu

BF = jnp.bfloat16
F32 = jnp.float32
U32 = jnp.uint32

S = 2048
D = 1024
H = 32
DH = 32
TA = 256
NA = S // TA
TB = 512
NB = S // TB
HALO = 16
WB = 8
NEG = -1e30
EPS = 1e-5
HD = D // 2
QSCALE = (DH ** -0.5) * math.log2(math.e)
NC1 = 4
G1 = 8 // NC1
OUT_PIECES = ((0, 256), (256, 128), (384, 128))

CFG = dict(first=1, a=1, b=1, look=3, tail=4, cuts=(5, 10, 14), lsum=2,
           lag=4, lrng=(2, 72), prng=(1, 73), orng=(92, 104), pnd=2,
           fpos=(13, 20, 27, 34, 41, 48, 55, 62, 69, 76, 83, 111),
           flook=5, fhi=22, fnr=32, frng=((0, 4), (4, 9), (9, 14)), forder=(2, 0, 1),
           bn=(16, 60, 27), bln=50, bhi=18, lns=2, lchain=1)


def _dot(a, b):
    return lax.dot_general(a, b, (((1,), (0,)), ((), ())), preferred_element_type=F32)


def _dot_nt(a, b):
    return lax.dot_general(a, b, (((1,), (1,)), ((), ())), preferred_element_type=F32)


def _pack(x_bf16):
    return pltpu.bitcast(x_bf16, U32)


def _unpack(x_u32):
    return pltpu.bitcast(x_u32, BF)


def _iota(shape, dim):
    return lax.broadcasted_iota(jnp.int32, shape, dim)


def _rows(xs):
    return lax.concatenate(xs, 0)


def _lanes(x3):
    n, r, _ = x3.shape
    x2 = x3.reshape(n * r, 128)
    return lax.concatenate([x2[t * r:(t + 1) * r] for t in range(n)], 1)


def _layernorm(x_bf16):
    x = x_bf16.astype(F32)
    m = jnp.sum(x, axis=1, keepdims=True) * (1.0 / D)
    xc = x - m
    v = jnp.sum(xc * xc, axis=1, keepdims=True) * (1.0 / D)
    return xc * lax.rsqrt(v + EPS)


def _lhs7(x11, x12, x21, x22):
    return [x11 + x22, x21 + x22, x11, x22, x11 + x12, x21 - x11, x12 - x22]


def _rhs7(w11, w12, w21, w22):
    return [w11 + w22, w11, w12 - w22, w21 - w11, w22, w11 + w12, w21 + w22]


RAW = (1, 4)
QUAD = (1, 7, 8, 4)


def _strassen(prod, left, right=None):
    m1 = prod(1)
    m3 = prod(3)
    y21 = m1 + m3
    m0 = prod(0)
    y11, y22 = m3 + m0, m0 - m1
    y11 = y11 + prod(6)
    m4 = prod(4)
    y11 = y11 - m4
    if right is not None:
        left(y11, y21)
    m2 = prod(2)
    y12 = m2 + m4
    y22 = (y22 + m2) + prod(5)
    if right is not None:
        right(y12, y22)
    else:
        left(y11, y12, y21, y22)


def _weave(top, bot):
    n, c = top.shape
    both = lax.concatenate([top.reshape(n // 8, 1, 8, c), bot.reshape(n // 8, 1, 8, c)], 1)
    return both.reshape(2 * n, c)


def _recip(l):
    r = pl.reciprocal(l, approx=True)
    return r * (2.0 - l * r)


def _swap16(xu):
    for bit in range(4):
        x5 = xu.reshape(8 >> bit, 2, 2 << bit, 8, 128)
        x, y = x5[:, 0:1], x5[:, 1:2]
        if bit == 0:
            x, y = ((x & U32(0xFFFF)) | (y << 16), (x >> 16) | (y & U32(0xFFFF0000)))
        else:
            dist = 1 << (bit - 1)
            lo = (_iota(x.shape, 3) & dist) == 0
            x, y = (lax.select(lo, x, pltpu.roll(y, dist, 3)),
                    lax.select(lo, pltpu.roll(x, 8 - dist, 3), y))
        xu = lax.concatenate([x, y], 1)
    return xu.reshape(16, 2, 8, 128)


def _spread(chunks, nslots, lo=0, hi=None):
    hi = nslots if hi is None else hi
    out = [[] for _ in range(nslots)]
    for u, c in enumerate(chunks):
        out[lo + u * (hi - lo) // len(chunks)].append(c)
    return out


def _merge(a, b):
    out = []
    for u in range(max(len(a), len(b))):
        out += a[u:u + 1] + b[u:u + 1]
    return out


def _flat(lists):
    return sum(lists, [])


def _both(*lists):
    return [sum(parts, []) for parts in zip(*lists)]


def _kernel(x_hbm, wa_hbm, woa_hbm, wb_hbm, wob_hbm, out_hbm,
            x_v, wa_v, woa_v, wb_v, wob_v, wq_p, wk_p, wv_p, woap, wbt, wobp, xl_v,
            k0_v, kt_v, k4_v, qt_v, vt_v, oa0_v, oa1_v, qk_v, v_v, e_v, ob_v, tk_v,
            sems):
    wap = (wq_p, wk_p, wv_p)
    def cp_x(i):
        n = TA if i < 3 else S - 3 * TA
        return pltpu.make_async_copy(x_hbm.at[pl.ds(i * TA, n), :],
                                     x_v.at[pl.ds(i * TA, n), :], sems.at[i])

    def cp_wa(c):
        w = G1 * 128
        return [pltpu.make_async_copy(wa_hbm.at[:, pl.ds(part * D + c * w, w)],
                                      wa_v.at[3 * c + part], sems.at[5 + c])
                for part in range(3)]

    cp_woa = pltpu.make_async_copy(woa_hbm, woa_v, sems.at[1])

    def cp_wb(st):
        qkv = [[], [(c, r0, 128) for c in range(6) for r0 in (0, 512)],
               [(c, r0, 384) for c in range(6) for r0 in (128, 640)]][st]
        out = [(0, 512 * st, 512)] if st < 2 else [(c, 0, D) for c in range(1, 4)]
        sem = sems.at[st + 1]
        return ([pltpu.make_async_copy(wb_hbm.at[pl.ds(r0, n), pl.ds(c * 512, 512)],
                                       wb_v.at[c, pl.ds(r0, n), :], sem) for c, r0, n in qkv]
                + [pltpu.make_async_copy(wob_hbm.at[pl.ds(r0, n), pl.ds(c * 256, 256)],
                                         wob_v.at[c, pl.ds(r0, n), :], sem) for c, r0, n in out])

    def cp_out(i, k, c=None):
        rows = pl.ds(i * TB + OUT_PIECES[k][0], OUT_PIECES[k][1])
        cols = pl.ds(0, D) if c is None else pl.ds(c * (D // 4), D // 4)
        return pltpu.make_async_copy(x_v.at[rows, cols], out_hbm.at[rows, cols], sems.at[4])

    def release(y, chunks):
        n = len(chunks)
        nt = y.shape[1] // 128
        for u, run in enumerate(chunks):
            pos = (u * y.shape[0] * nt // n) // 16 * 16
            t, rr = pos // y.shape[0], pos % y.shape[0]
            run(y[rr:rr + 16, t * 128:(t + 1) * 128])

    def gated(x, tok, zero):
        tk_v[1] = pltpu.bitcast(tok[0:8], U32)
        return pltpu.bitcast(pltpu.bitcast(x, U32) | tk_v[pl.ds(zero, 1)], F32)

    def fence_side(zero):
        zx = _pack(xl_v[pl.ds(pl.multiple_of(TA + zero * 32, 32), 32), 0:128])
        return zx | (wbt[4, 0, 0] | wobp[4, 0, 0]).reshape(16, 128)

    def fence_k(zero):
        return k4_v[zero, 0:16, :]

    def fence_q(zero):
        return qt_v[2 + zero, 0:16, :]

    def fence_v(zero):
        return vt_v[S // 128 + zero, 0:16, :]

    def with_fence(xu, fen):
        r, c = xu.shape
        last = lax.concatenate([xu[r - 16:, :c - 128], xu[r - 16:, c - 128:] | fen], 1)
        return _rows([xu[:r - 16], last])

    def ln_chunks(row0, dst, nrows, step=16):
        def mk(c):
            def run(tok):
                if tok is not None:
                    x_v[S:S + 16, 0:128] = tok.astype(BF)
                r = pl.multiple_of(row0 + c * step, step)
                xn = _layernorm(x_v[pl.ds(r, step), :]).reshape(step // 16, 2, 8, D)
                top, bot = xn[:, 0].reshape(step // 2, D), xn[:, 1].reshape(step // 2, D)
                ls = _lhs7(top[:, :HD], top[:, HD:], bot[:, :HD], bot[:, HD:])
                o = dst + c * (step // 2)
                xl_v[o:o + step // 2, :] = lax.concatenate(ls, 1).astype(BF)
            return run
        return [mk(c) for c in range(nrows // step)]

    def sum_chunks(dst, blk, d0, hh):
        nd = CFG['pnd']

        def mk(d):
            def run(tok):
                dst[4, 1, 0, 0] = pltpu.bitcast(tok[0:8], U32)
                ds = pl.ds(d0 + d, nd)
                wide = [_unpack(dst[blk, q, ds, hh].reshape(nd * 8, 128)).astype(F32)
                        for q in QUAD]
                for k, r in enumerate(_rhs7(*wide)):
                    if k not in RAW:
                        dst[blk, k, ds, hh] = _pack(r.astype(BF)).reshape(nd, 8, 128)
            return run
        return [mk(d) for d in range(0, 16, nd)]

    def prep_qkv(u):
        blk = lax.div(u, 6)
        c = u - 6 * blk
        d0, hh = (c >> 1) * 16, c & 1

        def mk(half):
            def run(tok):
                wb_v[0, D:D + 16, 0:128] = tok.astype(BF)
                rows = pl.ds(pl.multiple_of(blk * 128 + half * HD, 128), 128)
                v = _swap16(_pack(wb_v[c, rows, :].T))
                for dh in range(2):
                    wbt[blk, QUAD[2 * half + dh], pl.ds(d0, 16), hh] = v[:, dh]
            return run
        return [mk(0), mk(1)] + sum_chunks(wbt, blk, d0, hh)

    def prep_out(j):
        blk, hh = j >> 1, j & 1

        def mk(half):
            def run(tok):
                wob_v[4, 0:16, 0:128] = tok.astype(BF)
                rows = pl.ds(pl.multiple_of(hh * HD, HD), HD)
                v = _swap16(_pack(wob_v[blk, rows, half * 128:(half + 1) * 128]))
                for dh in range(2):
                    wobp[blk, QUAD[2 * dh + half], :, hh] = v[:, dh]
            return run
        return [mk(0), mk(1)] + sum_chunks(wobp, blk, 0, hh)

    class Stream:
        def __init__(self, side, fences, lag):
            self.side, self.fences, self.lag = side, fences, lag
            self.u, self.ys = 0, []

        def dot(self, fn, lhs_u, w):
            if self.u in self.fences:
                lhs_u = with_fence(lhs_u, self.fences[self.u]())
            y = fn(_unpack(lhs_u), w)
            self.ys.append(y)
            if self.u >= self.lag:
                release(self.ys[self.u - self.lag], self.side[self.u - self.lag])
            self.u += 1
            return y

    def make_rhs(quads):
        rs = _rhs7(*[w.astype(F32) for w in quads])
        return [_pack(quads[3 * (k == 4)] if k in RAW else r.astype(BF))
                for k, r in enumerate(rs)]

    def build_k4(full, t, row0):
        n = full.shape[0] - 48
        rolled = [full] + [pltpu.roll(full, 32 * r, 1) for r in range(1, 4)]
        grp_id = _iota((n, 128), 1) >> 5
        is_g = [grp_id == g for g in range(4)]
        for a in range(4):
            val = rolled[(0 - a) % 4][0:n]
            for g in range(1, 4):
                val = lax.select(is_g[g], rolled[(g - a) % 4][16 * g:16 * g + n], val)
            k4_v[4 * t + a, pl.ds(row0, n), :] = val

    def store_t(y, dst, slot0, t):
        yt = _pack(y.astype(BF).T)
        rows = pl.ds(t * 64 if isinstance(t, int) else pl.multiple_of(t * 64, 64), 64)
        for b in range(TA // 128):
            dst[slot0 + b, rows, :] = yt[:, b * 128:(b + 1) * 128]

    class Attn:
        def __init__(self, blk):
            self.blk = blk
            self.first = isinstance(blk, int)
            self.items = [(qb, 4 * t + a) for t in range(8) for qb in range(2) for a in range(4)]
            self.issued, self.done, self.queue, self.outs, self.tiles = 0, 0, [], [], []
            row, lane = _iota((128, 128), 0), _iota((128, 128), 1)
            self.tri = lane >= row
            if self.first:
                self.neg = jnp.full((128, 128), NEG, F32)
                self.zq = jnp.zeros((16, 128), U32)
            else:
                self.zero = jnp.zeros((128, 128), F32)
                self.slot = (lane >> 5) == (row >> 5)
                new = (_iota((32, 128), 1) & 31) >= _iota((32, 128), 0)
                self.new = (new[0:16], new[16:32])
                lane2 = _iota((256, 128), 1)
                self.odd, self.hi = (lane2 & 32) != 0, lane2 >= 64
                self.base = [pl.multiple_of((blk * 2 + qb) * 64 - 80, 16) for qb in range(2)]

        def scores_first(self, qb, h):
            qh = qt_v[qb, h * 16:(h + 1) * 16, :]
            wq = _unpack(_rows([qh if jj == h % 4 else self.zq for jj in range(4)]))
            n = (qb + 1) * 32
            kk = _unpack(k0_v[h // 4, 0:2 * n, :])
            s = _rows([_dot(kk[c * n:(c + 1) * n], wq) for c in range(4)])
            diag = lax.select(self.tri, s[qb * 128:], self.neg)
            return diag if qb == 0 else _rows([s[0:128], diag])

        def scores(self, qb, h):
            qf = _unpack(qt_v[qb, h * 16:(h + 1) * 16, :]).astype(F32)
            wq = lax.select(self.slot, _rows([qf] * 4), self.zero).astype(BF)
            w = k4_v[h, pl.ds(self.base[qb], 144), :]
            kk = _unpack(_rows([w[0:8], w[128:136], w[8:16], w[136:144], w[16:128]]))
            cuts = (0,) + CFG['cuts'] + (18,)
            s = _rows([_dot(kk[16 * a:16 * b], wq) for a, b in zip(cuts[:-1], cuts[1:])])
            return _rows([lax.select(self.new[0], s[16:32], s[0:16]),
                          lax.select(self.new[1], s[48:64], s[32:48]), s[64:]])

        def softmax_pv(self, s, qb, h):
            mx = jnp.max(s, axis=0, keepdims=True)
            if self.first:
                p = jnp.exp2(s - mx)
                l = jnp.sum(p, axis=0, keepdims=True)
                v3 = vt_v[0:qb + 1, h * 16:(h + 1) * 16, :]
            else:
                s = lax.select(self.odd, _rows([s[224:], s[:224]]), s)
                s = lax.select(self.hi, _rows([s[192:], s[:192]]), s)
                p = jnp.exp2(s - mx)
                if CFG['lsum'] == 0:
                    l = jnp.sum(p, axis=0, keepdims=True)
                else:
                    p3 = p.reshape(2, 128, 128)
                    if CFG['lsum'] == 1:
                        acc = jnp.sum(p.reshape(2, 16, 8, 128), axis=1)
                    else:
                        acc = p3[:, 120:128]
                        for v in range(14, -1, -1):
                            acc = acc + p3[:, 8 * v:8 * v + 8]
                    l = jnp.sum(acc.reshape(16, 128), axis=0, keepdims=True)
                pm = p[0:128]
                p = _rows([lax.select(self.tri, self.zero, pm), p[128:256],
                           lax.select(self.tri, pm, self.zero)])
                v3 = vt_v[pl.ds(self.blk * 2 + qb - 2, 3), h * 16:(h + 1) * 16, :]
            return _dot(_unpack(_lanes(v3)), p.astype(BF)) * _recip(l)

        def store_o(self, gp):
            x = self.tiles
            ready = {2: (2, 5), 4: (4, 0, 1, 3, 6)}.get(len(x), ())
            if ready:
                ls = _lhs7(x[0], x[2 % len(x)], x[1], x[3 % len(x)])
                for k in ready:
                    (oa0_v, oa1_v)[gp // 2][k, gp % 2] = _pack(ls[k].astype(BF).T)
            if len(x) == 4:
                self.tiles = []

        def issue(self, n=1):
            for _ in range(n):
                if self.issued < len(self.items):
                    fn = self.scores_first if self.first else self.scores
                    self.queue.append(fn(*self.items[self.issued]))
                    self.issued += 1

        def finish(self, n=1):
            for _ in range(n):
                if self.done < self.issued:
                    qb, h = self.items[self.done]
                    self.outs.append(self.softmax_pv(self.queue.pop(0), qb, h))
                    if len(self.outs) == 4:
                        self.tiles.append(_rows(self.outs))
                        self.outs = []
                        self.store_o(h // 8)
                    self.done += 1

    def add_residual(r, nrows, c0, c1, y):
        x_v[pl.ds(r, nrows), c0:c1] = (x_v[pl.ds(r, nrows), c0:c1].astype(F32) + y).astype(BF)

    def proj_b(xl, r0, side):
        rows = slice(HALO + r0, HALO + r0 + TA)
        xu = _pack(xl)
        st = Stream(side, {}, 0)
        for P in range(12):
            def prod(k):
                w = wbt[0:4, k, 4 * P:4 * P + 4].reshape(4, 64, 128)
                return st.dot(_dot_nt, xu[:, k * HD:(k + 1) * HD], _unpack(_lanes(w)))

            def put(T):
                def run(top, bot):
                    y = _weave(top, bot)
                    if T < 8:
                        qk_v[T, rows, :] = y * QSCALE
                    elif T < 16:
                        qk_v[T, rows, :] = y
                    else:
                        v_v[T - 16, rows, :] = y
                return run
            T = (P // 4) * 8 + P % 4
            _strassen(prod, put(T), put(T + 4))

    def taps(ref, t0, t1, r0):
        wins = [ref[t0:t1, HALO + r0 - 2 * w:HALO + r0 - 2 * w + 8, :] for w in range(WB)]
        return _rows(wins).reshape(WB, t1 - t0, 8, 128)

    def logit_b(i, zero, r0):
        ns = CFG['lns']
        acc = []

        def mk(st):
            def run(tok):
                t0, t1 = st * 8 // ns, (st + 1) * 8 // ns
                q = gated(qk_v[t0:t1, HALO + r0:HALO + r0 + 8, :], tok, zero)
                p = q[None] * taps(qk_v, 8 + t0, 8 + t1, r0)
                if acc and CFG['lchain']:
                    a = jnp.sum(lax.concatenate([acc.pop()[:, None], p], 1), axis=1)
                else:
                    a = jnp.sum(p, axis=1)
                    a = acc.pop() + a if acc else a
                if st + 1 < ns:
                    acc.append(a)
                    return
                a = a + pltpu.roll(a, 64, 2)
                a = a + pltpu.roll(a, 32, 2)
                if r0 < 2 * (WB - 1):
                    pos = _iota(a.shape, 1) - 2 * _iota(a.shape, 0) + (i * TB + r0)
                    a = lax.select(pos >= 0, a, jnp.full(a.shape, NEG, F32))
                e = jnp.exp2(a - jnp.max(a, axis=0, keepdims=True))
                e_v[:, r0:r0 + 8, :] = e * _recip(jnp.sum(e, axis=0, keepdims=True))
            return run
        return [mk(st) for st in range(ns)]

    def pv_b(zero, r0):
        x = []

        def mk(st):
            def run(tok):
                r, t0 = r0 + 8 * (st // 2), 4 * (st % 2)
                e = gated(e_v[:, r:r + 8, :], tok, zero)
                x.append(_lanes(jnp.sum(e[:, None] * taps(v_v, t0, t0 + 4, r), axis=0)))
                if st == 3:
                    ob_v[r0 // 2:r0 // 2 + 8, :] = lax.concatenate(_lhs7(*x), 1).astype(BF)
            return run
        return [mk(st) for st in range(4)]

    def out_b(i, r0, nrows, side, done=None):
        ou = _pack(ob_v[r0 // 2:(r0 + nrows) // 2, :])
        r = pl.multiple_of(i * TB + r0, 128)
        st = Stream(side, {}, 0)
        for c in range(4):
            def prod(k):
                w = _unpack(wobp[c, k].reshape(256, 128))
                return st.dot(_dot, ou[:, k * HD:(k + 1) * HD], w)

            def put(y11, y12, y21, y22):
                y = _weave(lax.concatenate([y11, y12], 1), lax.concatenate([y21, y22], 1))
                add_residual(r, nrows, c * 256, (c + 1) * 256, y)
            _strassen(prod, put)
            if done is not None:
                done(c)

    cp_x(0).start()
    for cp in cp_wa(0):
        cp.start()
    z16 = jnp.zeros((16, 128), U32)
    xl_v[TA:TA + 32, 0:128] = jnp.zeros((32, 128), BF)
    wbt[4, 0, 0] = z16.reshape(2, 8, 128)
    wobp[4, 0, 0] = z16.reshape(2, 8, 128)
    k4_v[0, 0:16, :] = z16
    vt_v[S // 128, 0:16, :] = z16
    qt_v[2, 0:16, :] = z16
    tk_v[0] = z16[0:8]
    cp_x(0).wait()
    for cp in cp_wa(1):
        cp.start()
    for run in ln_chunks(0, 0, TA, step=TA):
        run(None)

    def one_pass(p, carry):
        first = p == 0
        zero = p >> 2

        def out_a(blk, zero, st, after):
            part = {}
            n = [0]
            for ph in range(2):
                ou = oa0_v[pl.ds(zero, 7)] if ph == 0 else oa1_v[...]
                for nh in range(2):
                    def prod(k):
                        w = _unpack(_lanes(woap[(ph * 2 + nh) * 7 + k]))
                        y = st.dot(_dot, _lanes(ou[k]), w)
                        n[0] += 1
                        after(n[0])
                        return y

                    def put(half):
                        def run(top, bot):
                            y = _rows([top, bot])
                            if ph == 0:
                                part[nh, half] = y
                            else:
                                c0 = nh * HD + half * 256
                                add_residual(blk, TA, c0, c0 + 256, y + part[nh, half])
                        return run
                    _strassen(prod, put(0), put(1))

        def f_body(c, c_):
            @pl.when(first)
            def _():
                buf = wa_v.at[pl.ds(3 * c, 3)]
                pltpu.make_async_copy(buf, buf, sems.at[5 + c]).wait()
            xl = xl_v[0:TA // 2, :]
            raw = {}
            for part in CFG['forder']:
                for k in RAW:
                    o = int(k == 4)
                    w = wa_v[3 * c + part, o * HD:(o + 1) * HD, o * 128:(o + 1) * 128]
                    raw[part, k] = _dot(xl[:, k * HD:(k + 1) * HD], w)
            nr = CFG['fnr']

            def mk_w(part, r0):
                def run(tok):
                    wa_v[3 * NC1, 0:16, 0:128] = tok.astype(BF)
                    w1 = wa_v[3 * c + part, r0:r0 + nr, :]
                    w2 = wa_v[3 * c + part, HD + r0:HD + r0 + nr, :]
                    rs = make_rhs([w1[:, :128], w1[:, 128:], w2[:, :128], w2[:, 128:]])
                    for k in range(7):
                        wap[part][c * 7 + k, r0 // 2:(r0 + nr) // 2, :] = rs[k]
                return run
            side = _both(*[_spread([mk_w(part, r0) for r0 in range(0, HD, nr)], 21, *rng)
                           for part, rng in zip(CFG['forder'], CFG['frng'])])
            for y in raw.values():
                release(y, side.pop(0))
            for n, part in enumerate(CFG['forder']):
                def prod(k):
                    if k in RAW:
                        return raw[part, k]
                    y = _dot(xl[:, k * HD:(k + 1) * HD], _unpack(wap[part][c * 7 + k + zero]))
                    release(y, side.pop(0))
                    return y

                def put(t):
                    def run(top, bot):
                        y = _weave(top, bot)
                        if part == 0:
                            store_t(y * QSCALE, qt_v, 0, t)
                        elif part == 2:
                            store_t(y, vt_v, 0, t)
                        else:
                            kp = _pack(y.astype(BF))
                            k0_v[t] = kp
                            if n < 2:
                                kt_v[t] = kp[80:128]
                                build_k4(kp, t, 48)
                    return run
                _strassen(prod, put(2 * c), put(2 * c + 1))
                if n == 0:
                    for k in range(NC1 - 2):
                        @pl.when(jnp.logical_and(first, c == k))
                        def _():
                            for cp in cp_wa(k + 2):
                                cp.start()

            @pl.when(jnp.logical_and(first, c == NC1 - 3))
            def _():
                cp_woa.start()

            @pl.when(jnp.logical_and(first, c == NC1 - 2))
            def _():
                cp_x(1).start()
                for cp in cp_wb(0):
                    cp.start()
            return c_

        def a_first():
            lax.fori_loop(0, NC1, f_body, 0)
            at = Attn(0)
            at.issue(CFG['flook'])
            while at.issued < 2 * H:
                at.issue()
                at.finish()

            @pl.when(first)
            def _():
                for cp in [cp_woa, cp_x(1)] + cp_wb(0):
                    cp.wait()
                for cp in [cp_x(2)] + cp_wb(1):
                    cp.start()

                def once(gp, c_):
                    r0 = pl.multiple_of(gp * 256, 256)
                    rows = pl.ds(pl.multiple_of((gp & 1) * 64, 64), 64)
                    for nh in range(2):
                        for nt in range(2):
                            c0 = nh * HD + nt * 128
                            rs = make_rhs([woa_v[pl.ds(r0 + dr, 128), c0 + dc:c0 + dc + 128]
                                           for dr in (0, 128) for dc in (0, 256)])
                            for k in range(7):
                                woap[((gp >> 1) * 2 + nh) * 7 + k, nt, rows, :] = rs[k]
                    return c_
                lax.fori_loop(0, 4, once, 0)

            def mk_k4(t):
                def run(tok):
                    k0_v[8, 0:8, :] = pltpu.bitcast(tok[0:8], U32)
                    kp = k0_v[t + zero]
                    kt_v[t] = kp[80:128]
                    build_k4(kp, t, 48)
                return run
            hi = CFG['fhi']
            side = _both(_spread(prep_out(zero), 28, 0, hi),
                         _spread(ln_chunks(TA + zero * TA, 0, TA), 28, 0, hi))
            if CFG['forder'][2] == 1:
                side = _both(side, _spread([mk_k4(t) for t in range(8)], 28, 0, hi))
            st = Stream(side, {27: lambda: fence_side(zero) | fence_k(zero)}, 1)
            out_a(0, zero, st, lambda u: at.finish(2 * H if u == 1 else 0))

        if CFG['first']:
            a_first()

        @pl.when(first)
        def _():
            cp_x(2).wait()
            for cp in cp_wb(1):
                cp.wait()
            cp_x(3).start()
            for cp in cp_wb(2):
                cp.start()

        def a_body(i, c_):
            @pl.when(jnp.logical_and(first, i == 2))
            def _():
                cp_x(3).wait()
                for cp in cp_wb(2):
                    cp.wait()
            xu = _pack(xl_v[0:TA // 2, :])
            pw = _flat([prep_qkv(jnp.minimum(4 * (i - 1) + n, 23)) for n in range(4)])
            po = prep_out(i)
            side = _both(_spread(ln_chunks((((i + 1) & (NA - 1)) + zero) * TA, 0, TA),
                                 112, *CFG['lrng']),
                         _spread(pw, 112, *CFG['prng']), _spread(po, 112, *CFG['orng']))
            fences = {u: (lambda: fence_side(zero)) for u in CFG['fpos']}
            for n in range(1, 12):
                fe = (fence_k, fence_v, fence_q)[(n - 1) % 3]
                u = 7 * n + 6
                fences[u] = ((lambda fe=fe: fe(zero) | fence_side(zero)) if u in fences
                             else (lambda fe=fe: fe(zero)))
            st = Stream(side, fences, CFG['lag'])
            at = Attn(i)
            for n in range(12):
                gp, kind = n // 3, n % 3

                def prod(k):
                    if n == 11 and k == 4:
                        at.issue(CFG['look'])
                    w = wap[(1, 2, 0)[kind]][gp * 7 + k]
                    return st.dot(_dot, xu[:, k * HD:(k + 1) * HD], _unpack(w))

                def put(t):
                    def run(top, bot):
                        y = _weave(top, bot)
                        if kind == 0:
                            kp = _pack(y.astype(BF))
                            full = _rows([kt_v[t], kp])
                            kt_v[t] = kp[80:128]
                            build_k4(full, t, pl.multiple_of(i * (TA // 2), TA // 2))
                        elif kind == 1:
                            store_t(y, vt_v, i * (TA // 128), t)
                        else:
                            store_t(y * QSCALE, qt_v, 0, t)
                    return run
                _strassen(prod, put(2 * gp), put(2 * gp + 1))
            while at.issued < 2 * H - CFG['tail']:
                at.issue()
                at.finish()

            def after(u):
                at.finish()
                at.issue()
            at.issue()
            out_a(pl.multiple_of(i * TA, TA), zero, st, after)
            assert at.done == 2 * H
            return c_
        if CFG['a']:
            lax.fori_loop(1, NA, a_body, 0)

        qk_v[8:16, 0:HALO, :] = jnp.zeros((8, HALO, 128), F32)
        v_v[:, 0:HALO, :] = jnp.zeros((8, HALO, 128), F32)

        def b_body(i, c_):
            def send(k):
                for ii in range(NB if k < 2 else NB - 1):
                    @pl.when(jnp.logical_and(p == 1, i == ii))
                    def _():
                        cp_out(ii, k).start()

            def send_last(c):
                @pl.when(jnp.logical_and(p == 1, i == NB - 1))
                def _():
                    cp_out(NB - 1, 2, c).start()
            ln1 = ln_chunks(i * TB + 256, TA // 2, 256)
            ln2 = ln_chunks((((i + 1) & (NB - 1)) + zero) * TB, 0, TA)
            lg = [logit_b(i, zero, g * 8) for g in range(TB // 8)]
            pv = [pv_b(zero, g * 16) for g in range(TB // 16)]
            n0, n1, n2 = CFG['bn']

            def mix(a, b):
                return _flat(_merge([_flat(a[u:u + 2]) for u in range(0, len(a), 2)], b))
            proj_b(xl_v[0:TA // 2, :], 0, _both(_spread(ln1 + ln2, 84, 0, CFG['bln']),
                                                _spread(_flat(lg[0:n0]), 84, 57, 84)))
            xl1 = xl_v[pl.ds(pl.multiple_of(TA // 2 + zero * 32, 32), TA // 2), :]
            proj_b(xl1, 256, _both(_spread(mix(lg[n0:32], pv[0:16]), 84, 1, 57),
                                   _spread(_flat(lg[32:n1]), 84, 57, 84)))
            out_b(i, 0, 256, _spread(mix(lg[n1:64], pv[16:n2]), 28, 1, 28))
            send(0)
            out_b(i, 256, 128, _spread(_flat(pv[n2:32]), 28, 0, CFG['bhi']))
            send(1)
            qk_v[8:16, 0:HALO, :] = qk_v[8:16, TB:TB + HALO, :]
            v_v[:, 0:HALO, :] = v_v[:, TB:TB + HALO, :]
            out_b(i, 384, 128, [[]] * 28, send_last)
            send(2)
            return c_
        if CFG['b']:
            lax.fori_loop(0, NB, b_body, 0)
        return carry

    lax.fori_loop(0, 2, one_pass, 0)
    for i in range(NB):
        for k in range(len(OUT_PIECES)):
            if (i, k) != (NB - 1, 2):
                cp_out(i, k).wait()
    for c in range(4):
        cp_out(NB - 1, 2, c).wait()


@jax.jit
def pallas_interleave_layers__sliding_block__sliding_local_dilated__prompt_kernel(
    A_x: jax.Array,
    A_wqkv: jax.Array,
    A_wo: jax.Array,
    B_x: jax.Array,
    B_wqkv: jax.Array,
    B_wo: jax.Array,
):
    del B_x
    x = A_x.reshape(S, D)
    any_spec = pl.BlockSpec(memory_space=pl.ANY)
    out = pl.pallas_call(
        _kernel,
        out_shape=jax.ShapeDtypeStruct((S, D), BF),
        in_specs=[any_spec] * 5,
        out_specs=any_spec,
        scratch_shapes=[
            pltpu.VMEM((S + 16, D), BF),
            pltpu.VMEM((3 * NC1 + 1, D, G1 * 128), BF),
            pltpu.VMEM((D, D), BF),
            pltpu.VMEM((6, D + 16, 512), BF),
            pltpu.VMEM((5, D, 256), BF),
            pltpu.VMEM((28, 256, 128), U32),
            pltpu.VMEM((28, 256, 128), U32),
            pltpu.VMEM((28, 256, 128), U32),
            pltpu.VMEM((28, 2, 128, 128), U32),
            pltpu.VMEM((5, 9, 48, 2, 8, 128), U32),
            pltpu.VMEM((5, 9, 16, 2, 8, 128), U32),
            pltpu.VMEM((TA + 32, 7 * HD), BF),
            pltpu.VMEM((9, TA // 2, 128), U32),
            pltpu.VMEM((8, 48, 128), U32),
            pltpu.VMEM((H, S // 2, 128), U32),
            pltpu.VMEM((3, D // 2, 128), U32),
            pltpu.VMEM((S // 128 + 1, D // 2, 128), U32),
            pltpu.VMEM((7, 2, 64, 128), U32),
            pltpu.VMEM((7, 2, 64, 128), U32),
            pltpu.VMEM((16, HALO + TB, 128), F32),
            pltpu.VMEM((8, HALO + TB, 128), F32),
            pltpu.VMEM((WB, TB, 128), F32),
            pltpu.VMEM((TB // 2, 7 * HD), BF),
            pltpu.VMEM((4, 8, 128), U32),
            pltpu.SemaphoreType.DMA((5 + NC1,)),
        ],
        compiler_params=pltpu.CompilerParams(vmem_limit_bytes=112 * 1024 * 1024),
        name="interleave_attn",
    )(x, A_wqkv, A_wo, B_wqkv, B_wo)
    return out.reshape(1, S, D)
```

```python
import math

import jax
import jax.numpy as jnp
from jax import lax
import jax.experimental.pallas as pl
import jax.experimental.pallas.tpu as pltpu

BF = jnp.bfloat16
F32 = jnp.float32
U32 = jnp.uint32

S = 2048
D = 1024
H = 32
DH = 32
TA = 256
NA = S // TA
TB = 512
NB = S // TB
HALO = 16
WB = 8
NEG = -1e30
EPS = 1e-5
HD = D // 2
QSCALE = (DH ** -0.5) * math.log2(math.e)
NC1 = 4
G1 = 8 // NC1
OUT_PIECES = ((0, 256), (256, 128), (384, 128))

CFG = dict(first=1, a=1, b=1, look=3, tail=2, cuts=(5, 10, 14), lsum=2, kord=(0, 1, 2), hk=0,
           lag=6, lrng=(0, 64), orng=(90, 102), pnd=2,
           urng=((3, 21), (19, 38), (38, 57), (57, 78)),
           fpos=tuple(range(11, 84, 4)) + (111,),
           flook=6, fhi=24, fnr=16, frng=((0, 4), (4, 9), (9, 14)), forder=(2, 0, 1),
           bn=(20, 64, 26), bln=53, bhi=20, lns=2, lchain=1,
           bmix=2, bfx=tuple(range(8, 60, 4)), bfe=tuple(range(69, 168, 7)), blag=6)


def _dot(a, b):
    return lax.dot_general(a, b, (((1,), (0,)), ((), ())), preferred_element_type=F32)


def _dot_nt(a, b):
    return lax.dot_general(a, b, (((1,), (1,)), ((), ())), preferred_element_type=F32)


def _pack(x_bf16):
    return pltpu.bitcast(x_bf16, U32)


def _unpack(x_u32):
    return pltpu.bitcast(x_u32, BF)


def _iota(shape, dim):
    return lax.broadcasted_iota(jnp.int32, shape, dim)


def _rows(xs):
    return lax.concatenate(xs, 0)


def _lanes(x3):
    n, r, _ = x3.shape
    x2 = x3.reshape(n * r, 128)
    return lax.concatenate([x2[t * r:(t + 1) * r] for t in range(n)], 1)


def _layernorm(x_bf16):
    x = x_bf16.astype(F32)
    m = jnp.sum(x, axis=1, keepdims=True) * (1.0 / D)
    xc = x - m
    v = jnp.sum(xc * xc, axis=1, keepdims=True) * (1.0 / D)
    return xc * lax.rsqrt(v + EPS)


def _lhs7(x11, x12, x21, x22):
    return [x11 + x22, x21 + x22, x11, x22, x11 + x12, x21 - x11, x12 - x22]


def _rhs7(w11, w12, w21, w22):
    return [w11 + w22, w11, w12 - w22, w21 - w11, w22, w11 + w12, w21 + w22]


RAW = (1, 4)
QUAD = (1, 7, 8, 4)


def _strassen(prod, left, right=None):
    m1 = prod(1)
    m3 = prod(3)
    y21 = m1 + m3
    m0 = prod(0)
    y11, y22 = m3 + m0, m0 - m1
    y11 = y11 + prod(6)
    m4 = prod(4)
    y11 = y11 - m4
    if right is not None:
        left(y11, y21)
    m2 = prod(2)
    y12 = m2 + m4
    y22 = (y22 + m2) + prod(5)
    if right is not None:
        right(y12, y22)
    else:
        left(y11, y12, y21, y22)


def _weave(top, bot):
    n, c = top.shape
    both = lax.concatenate([top.reshape(n // 8, 1, 8, c), bot.reshape(n // 8, 1, 8, c)], 1)
    return both.reshape(2 * n, c)


def _recip(l):
    r = pl.reciprocal(l, approx=True)
    return r * (2.0 - l * r)


def _swap16(xu):
    for bit in range(4):
        x5 = xu.reshape(8 >> bit, 2, 2 << bit, 8, 128)
        x, y = x5[:, 0:1], x5[:, 1:2]
        if bit == 0:
            x, y = ((x & U32(0xFFFF)) | (y << 16), (x >> 16) | (y & U32(0xFFFF0000)))
        else:
            dist = 1 << (bit - 1)
            lo = (_iota(x.shape, 3) & dist) == 0
            x, y = (lax.select(lo, x, pltpu.roll(y, dist, 3)),
                    lax.select(lo, pltpu.roll(x, 8 - dist, 3), y))
        xu = lax.concatenate([x, y], 1)
    return xu.reshape(16, 2, 8, 128)


def _spread(chunks, nslots, lo=0, hi=None):
    hi = nslots if hi is None else hi
    out = [[] for _ in range(nslots)]
    for u, c in enumerate(chunks):
        out[lo + u * (hi - lo) // len(chunks)].append(c)
    return out


def _merge(a, b):
    out = []
    for u in range(max(len(a), len(b))):
        out += a[u:u + 1] + b[u:u + 1]
    return out


def _flat(lists):
    return sum(lists, [])


def _both(*lists):
    return [sum(parts, []) for parts in zip(*lists)]


def _kernel(x_hbm, wa_hbm, woa_hbm, wb_hbm, wob_hbm, out_hbm,
            x_v, wa_v, woa_v, wb_v, wob_v, wq_p, wk_p, wv_p, woap, wbt, wobp, xl_v,
            k0_v, kt_v, k4_v, qt_v, vt_v, oa0_v, oa1_v, qk_v, v_v, e_v, ob_v, tk_v,
            sems):
    wap = (wq_p, wk_p, wv_p)
    def cp_x(i):
        n = TA if i < 3 else S - 3 * TA
        return pltpu.make_async_copy(x_hbm.at[pl.ds(i * TA, n), :],
                                     x_v.at[pl.ds(i * TA, n), :], sems.at[i])

    def cp_wa(c):
        w = G1 * 128
        return [pltpu.make_async_copy(wa_hbm.at[:, pl.ds(part * D + c * w, w)],
                                      wa_v.at[3 * c + part], sems.at[5 + c])
                for part in range(3)]

    cp_woa = pltpu.make_async_copy(woa_hbm, woa_v, sems.at[1])

    def cp_wb(st):
        qkv = [[], [(c, r0, 128) for c in range(6) for r0 in (0, 512)],
               [(c, r0, 384) for c in range(6) for r0 in (128, 640)]][st]
        out = [(0, 512 * st, 512)] if st < 2 else [(c, 0, D) for c in range(1, 4)]
        sem = sems.at[st + 1]
        return ([pltpu.make_async_copy(wb_hbm.at[pl.ds(r0, n), pl.ds(c * 512, 512)],
                                       wb_v.at[c, pl.ds(r0, n), :], sem) for c, r0, n in qkv]
                + [pltpu.make_async_copy(wob_hbm.at[pl.ds(r0, n), pl.ds(c * 256, 256)],
                                         wob_v.at[c, pl.ds(r0, n), :], sem) for c, r0, n in out])

    def cp_out(i, k, c=None):
        rows = pl.ds(i * TB + OUT_PIECES[k][0], OUT_PIECES[k][1])
        cols = pl.ds(0, D) if c is None else pl.ds(c * (D // 4), D // 4)
        return pltpu.make_async_copy(x_v.at[rows, cols], out_hbm.at[rows, cols], sems.at[4])

    def release(y, chunks):
        n = len(chunks)
        nt = y.shape[1] // 128
        for u, run in enumerate(chunks):
            pos = (u * y.shape[0] * nt // n) // 16 * 16
            t, rr = pos // y.shape[0], pos % y.shape[0]
            run(y[rr:rr + 16, t * 128:(t + 1) * 128])

    def gated(x, tok, zero):
        tk_v[1] = pltpu.bitcast(tok[0:8], U32)
        return pltpu.bitcast(pltpu.bitcast(x, U32) | tk_v[pl.ds(zero, 1)], F32)

    def fence_x(zero):
        return _pack(xl_v[pl.ds(pl.multiple_of(TA + zero * 32, 32), 32), 0:128])

    def fence_e(zero):
        return pltpu.bitcast(e_v[0, pl.ds(pl.multiple_of(TB + zero * 16, 16), 16), :], U32)

    def fence_side(zero):
        return fence_x(zero) | (wbt[4, 0, 0] | wobp[4, 0, 0]).reshape(16, 128)

    def fence_k(zero):
        return k4_v[zero, 0:16, :]

    def fence_q(zero):
        return qt_v[2 + zero, 0:16, :]

    def fence_v(zero):
        return vt_v[S // 128 + zero, 0:16, :]

    def with_fence(xu, fen):
        r, c = xu.shape
        last = lax.concatenate([xu[r - 16:, :c - 128], xu[r - 16:, c - 128:] | fen], 1)
        return _rows([xu[:r - 16], last])

    def ln_chunks(row0, dst, nrows, step=16):
        def mk(c):
            def run(tok):
                if tok is not None:
                    x_v[S:S + 16, 0:128] = tok.astype(BF)
                r = pl.multiple_of(row0 + c * step, step)
                xn = _layernorm(x_v[pl.ds(r, step), :]).reshape(step // 16, 2, 8, D)
                top, bot = xn[:, 0].reshape(step // 2, D), xn[:, 1].reshape(step // 2, D)
                ls = _lhs7(top[:, :HD], top[:, HD:], bot[:, :HD], bot[:, HD:])
                o = dst + c * (step // 2)
                xl_v[o:o + step // 2, :] = lax.concatenate(ls, 1).astype(BF)
            return run
        return [mk(c) for c in range(nrows // step)]

    def sum_chunks(dst, blk, d0, hh):
        nd = CFG['pnd']

        def mk(d):
            def run(tok):
                dst[4, 1, 0, 0] = pltpu.bitcast(tok[0:8], U32)
                ds = pl.ds(d0 + d, nd)
                wide = [_unpack(dst[blk, q, ds, hh].reshape(nd * 8, 128)).astype(F32)
                        for q in QUAD]
                for k, r in enumerate(_rhs7(*wide)):
                    if k not in RAW:
                        dst[blk, k, ds, hh] = _pack(r.astype(BF)).reshape(nd, 8, 128)
            return run
        return [mk(d) for d in range(0, 16, nd)]

    def prep_qkv(u):
        blk = lax.div(u, 6)
        c = u - 6 * blk
        d0, hh = (c >> 1) * 16, c & 1

        def mk(half):
            def run(tok):
                wb_v[0, D:D + 16, 0:128] = tok.astype(BF)
                rows = pl.ds(pl.multiple_of(blk * 128 + half * HD, 128), 128)
                v = _swap16(_pack(wb_v[c, rows, :].T))
                for dh in range(2):
                    wbt[blk, QUAD[2 * half + dh], pl.ds(d0, 16), hh] = v[:, dh]
            return run
        return [mk(0), mk(1)] + sum_chunks(wbt, blk, d0, hh)

    def prep_out(j):
        blk, hh = j >> 1, j & 1

        def mk(half):
            def run(tok):
                wob_v[4, 0:16, 0:128] = tok.astype(BF)
                rows = pl.ds(pl.multiple_of(hh * HD, HD), HD)
                v = _swap16(_pack(wob_v[blk, rows, half * 128:(half + 1) * 128]))
                for dh in range(2):
                    wobp[blk, QUAD[2 * dh + half], :, hh] = v[:, dh]
            return run
        return [mk(0), mk(1)] + sum_chunks(wobp, blk, 0, hh)

    class Stream:
        def __init__(self, side, fences, lag):
            self.side, self.fences, self.lag = side, fences, lag
            self.u, self.ys = 0, []

        def dot(self, fn, lhs_u, w):
            if self.u in self.fences:
                lhs_u = with_fence(lhs_u, self.fences[self.u]())
            y = fn(_unpack(lhs_u), w)
            self.ys.append(y)
            if self.u >= self.lag:
                release(self.ys[self.u - self.lag], self.side[self.u - self.lag])
            self.u += 1
            return y

        def flush(self):
            for u in range(max(self.u - self.lag, 0), self.u):
                release(self.ys[u], self.side[u])

    def make_rhs(quads):
        rs = _rhs7(*[w.astype(F32) for w in quads])
        return [_pack(quads[3 * (k == 4)] if k in RAW else r.astype(BF))
                for k, r in enumerate(rs)]

    def build_k4(full, t, row0):
        n = full.shape[0] - 48
        rolled = [full] + [pltpu.roll(full, 32 * r, 1) for r in range(1, 4)]
        grp_id = _iota((n, 128), 1) >> 5
        is_g = [grp_id == g for g in range(4)]
        for a in range(4):
            val = rolled[(0 - a) % 4][0:n]
            for g in range(1, 4):
                val = lax.select(is_g[g], rolled[(g - a) % 4][16 * g:16 * g + n], val)
            k4_v[4 * t + a, pl.ds(row0, n), :] = val

    def store_t(y, dst, slot0, t):
        yt = _pack(y.astype(BF).T)
        rows = pl.ds(t * 64 if isinstance(t, int) else pl.multiple_of(t * 64, 64), 64)
        for b in range(TA // 128):
            dst[slot0 + b, rows, :] = yt[:, b * 128:(b + 1) * 128]

    class Attn:
        def __init__(self, blk):
            self.blk = blk
            self.first = isinstance(blk, int)
            self.items = [(qb, 4 * t + a) for t in range(8) for qb in range(2) for a in range(4)]
            self.issued, self.done, self.queue, self.outs, self.tiles = 0, 0, [], [], []
            row, lane = _iota((128, 128), 0), _iota((128, 128), 1)
            self.tri = lane >= row
            if self.first:
                self.neg = jnp.full((128, 128), NEG, F32)
                self.zq = jnp.zeros((16, 128), U32)
            else:
                self.zero = jnp.zeros((128, 128), F32)
                self.slot = (lane >> 5) == (row >> 5)
                new = (_iota((32, 128), 1) & 31) >= _iota((32, 128), 0)
                self.new = (new[0:16], new[16:32])
                lane2 = _iota((256, 128), 1)
                self.odd, self.hi = (lane2 & 32) != 0, lane2 >= 64
                self.base = [pl.multiple_of((blk * 2 + qb) * 64 - 80, 16) for qb in range(2)]

        def scores_first(self, qb, h):
            qh = qt_v[qb, h * 16:(h + 1) * 16, :]
            wq = _unpack(_rows([qh if jj == h % 4 else self.zq for jj in range(4)]))
            n = (qb + 1) * 32
            kk = _unpack(k0_v[h // 4, 0:2 * n, :])
            s = _rows([_dot(kk[c * n:(c + 1) * n], wq) for c in range(4)])
            diag = lax.select(self.tri, s[qb * 128:], self.neg)
            return diag if qb == 0 else _rows([s[0:128], diag])

        def scores(self, qb, h):
            qf = _unpack(qt_v[qb, h * 16:(h + 1) * 16, :]).astype(F32)
            wq = lax.select(self.slot, _rows([qf] * 4), self.zero).astype(BF)
            w = k4_v[h, pl.ds(self.base[qb], 144), :]
            kk = _unpack(_rows([w[0:8], w[128:136], w[8:16], w[136:144], w[16:128]]))
            cuts = (0,) + CFG['cuts'] + (18,)
            s = _rows([_dot(kk[16 * a:16 * b], wq) for a, b in zip(cuts[:-1], cuts[1:])])
            return _rows([lax.select(self.new[0], s[16:32], s[0:16]),
                          lax.select(self.new[1], s[48:64], s[32:48]), s[64:]])

        def softmax_pv(self, s, qb, h):
            mx = jnp.max(s, axis=0, keepdims=True)
            if self.first:
                p = jnp.exp2(s - mx)
                l = jnp.sum(p, axis=0, keepdims=True)
                v3 = vt_v[0:qb + 1, h * 16:(h + 1) * 16, :]
            else:
                s = lax.select(self.odd, _rows([s[224:], s[:224]]), s)
                s = lax.select(self.hi, _rows([s[192:], s[:192]]), s)
                p = jnp.exp2(s - mx)
                if CFG['lsum'] == 0:
                    l = jnp.sum(p, axis=0, keepdims=True)
                else:
                    p3 = p.reshape(2, 128, 128)
                    if CFG['lsum'] == 1:
                        acc = jnp.sum(p.reshape(2, 16, 8, 128), axis=1)
                    else:
                        acc = p3[:, 120:128]
                        for v in range(14, -1, -1):
                            acc = acc + p3[:, 8 * v:8 * v + 8]
                    l = jnp.sum(acc.reshape(16, 128), axis=0, keepdims=True)
                pm = p[0:128]
                p = _rows([lax.select(self.tri, self.zero, pm), p[128:256],
                           lax.select(self.tri, pm, self.zero)])
                v3 = vt_v[pl.ds(self.blk * 2 + qb - 2, 3), h * 16:(h + 1) * 16, :]
            return _dot(_unpack(_lanes(v3)), p.astype(BF)) * _recip(l)

        def store_o(self, gp):
            x = self.tiles
            ready = {2: (2, 5), 4: (4, 0, 1, 3, 6)}.get(len(x), ())
            if ready:
                ls = _lhs7(x[0], x[2 % len(x)], x[1], x[3 % len(x)])
                for k in ready:
                    (oa0_v, oa1_v)[gp // 2][k, gp % 2] = _pack(ls[k].astype(BF).T)
            if len(x) == 4:
                self.tiles = []

        def issue(self, n=1):
            for _ in range(n):
                if self.issued < len(self.items):
                    fn = self.scores_first if self.first else self.scores
                    self.queue.append(fn(*self.items[self.issued]))
                    self.issued += 1

        def finish(self, n=1):
            for _ in range(n):
                if self.done < self.issued:
                    qb, h = self.items[self.done]
                    self.outs.append(self.softmax_pv(self.queue.pop(0), qb, h))
                    if len(self.outs) == 4:
                        self.tiles.append(_rows(self.outs))
                        self.outs = []
                        self.store_o(h // 8)
                    self.done += 1

    def add_residual(r, nrows, c0, c1, y):
        x_v[pl.ds(r, nrows), c0:c1] = (x_v[pl.ds(r, nrows), c0:c1].astype(F32) + y).astype(BF)

    def proj_b(xl, r0, side, fences, lag):
        rows = slice(HALO + r0, HALO + r0 + TA)
        xu = _pack(xl)
        st = Stream(side, fences, lag)
        for P in range(12):
            def prod(k):
                w = wbt[0:4, k, 4 * P:4 * P + 4].reshape(4, 64, 128)
                return st.dot(_dot_nt, xu[:, k * HD:(k + 1) * HD], _unpack(_lanes(w)))

            def put(T):
                def run(top, bot):
                    y = _weave(top, bot)
                    if T < 8:
                        qk_v[T, rows, :] = y * QSCALE
                    elif T < 16:
                        qk_v[T, rows, :] = y
                    else:
                        v_v[T - 16, rows, :] = y
                return run
            T = (P // 4) * 8 + P % 4
            _strassen(prod, put(T), put(T + 4))
        st.flush()

    def taps(ref, t0, t1, r0):
        wins = [ref[t0:t1, HALO + r0 - 2 * w:HALO + r0 - 2 * w + 8, :] for w in range(WB)]
        return _rows(wins).reshape(WB, t1 - t0, 8, 128)

    def logit_b(i, zero, r0):
        ns = CFG['lns']
        acc = []

        def mk(st):
            def run(tok):
                t0, t1 = st * 8 // ns, (st + 1) * 8 // ns
                q = gated(qk_v[t0:t1, HALO + r0:HALO + r0 + 8, :], tok, zero)
                p = q[None] * taps(qk_v, 8 + t0, 8 + t1, r0)
                if acc and CFG['lchain']:
                    a = jnp.sum(lax.concatenate([acc.pop()[:, None], p], 1), axis=1)
                else:
                    a = jnp.sum(p, axis=1)
                    a = acc.pop() + a if acc else a
                if st + 1 < ns:
                    acc.append(a)
                    return
                a = a + pltpu.roll(a, 64, 2)
                a = a + pltpu.roll(a, 32, 2)
                if r0 < 2 * (WB - 1):
                    pos = _iota(a.shape, 1) - 2 * _iota(a.shape, 0) + (i * TB + r0)
                    a = lax.select(pos >= 0, a, jnp.full(a.shape, NEG, F32))
                e = jnp.exp2(a - jnp.max(a, axis=0, keepdims=True))
                e_v[:, r0:r0 + 8, :] = e * _recip(jnp.sum(e, axis=0, keepdims=True))
            return run
        return [mk(st) for st in range(ns)]

    def pv_b(zero, r0):
        x = []

        def mk(st):
            def run(tok):
                r, t0 = r0 + 8 * (st // 2), 4 * (st % 2)
                e = gated(e_v[:, r:r + 8, :], tok, zero)
                x.append(_lanes(jnp.sum(e[:, None] * taps(v_v, t0, t0 + 4, r), axis=0)))
                if st == 3:
                    ob_v[r0 // 2:r0 // 2 + 8, :] = lax.concatenate(_lhs7(*x), 1).astype(BF)
            return run
        return [mk(st) for st in range(4)]

    def out_b(i, r0, nrows, side, done=None):
        ou = _pack(ob_v[r0 // 2:(r0 + nrows) // 2, :])
        r = pl.multiple_of(i * TB + r0, 128)
        st = Stream(side, {}, 0)
        for c in range(4):
            def prod(k):
                w = _unpack(wobp[c, k].reshape(256, 128))
                return st.dot(_dot, ou[:, k * HD:(k + 1) * HD], w)

            def put(y11, y12, y21, y22):
                y = _weave(lax.concatenate([y11, y12], 1), lax.concatenate([y21, y22], 1))
                add_residual(r, nrows, c * 256, (c + 1) * 256, y)
            _strassen(prod, put)
            if done is not None:
                done(c)

    cp_x(0).start()
    for cp in cp_wa(0):
        cp.start()
    z16 = jnp.zeros((16, 128), U32)
    xl_v[TA:TA + 32, 0:128] = jnp.zeros((32, 128), BF)
    wbt[4, 0, 0] = z16.reshape(2, 8, 128)
    wobp[4, 0, 0] = z16.reshape(2, 8, 128)
    k4_v[0, 0:16, :] = z16
    vt_v[S // 128, 0:16, :] = z16
    qt_v[2, 0:16, :] = z16
    tk_v[0] = z16[0:8]
    e_v[0, TB:TB + 16, :] = jnp.zeros((16, 128), F32)
    cp_x(0).wait()
    for cp in cp_wa(1):
        cp.start()
    for run in ln_chunks(0, 0, TA, step=TA):
        run(None)

    def one_pass(p, carry):
        first = p == 0
        zero = p >> 2

        def out_a(blk, zero, st, after):
            part = {}
            n = [0]
            for ph in range(2):
                ou = oa0_v[pl.ds(zero, 7)] if ph == 0 else oa1_v[...]
                for nh in range(2):
                    def prod(k):
                        w = _unpack(_lanes(woap[(ph * 2 + nh) * 7 + k]))
                        y = st.dot(_dot, _lanes(ou[k]), w)
                        n[0] += 1
                        after(n[0])
                        return y

                    def put(half):
                        def run(top, bot):
                            y = _rows([top, bot])
                            if ph == 0:
                                part[nh, half] = y
                            else:
                                c0 = nh * HD + half * 256
                                add_residual(blk, TA, c0, c0 + 256, y + part[nh, half])
                        return run
                    _strassen(prod, put(0), put(1))

        def f_body(c, c_):
            @pl.when(first)
            def _():
                buf = wa_v.at[pl.ds(3 * c, 3)]
                pltpu.make_async_copy(buf, buf, sems.at[5 + c]).wait()
            xl = xl_v[0:TA // 2, :]
            raw = {}
            for part in CFG['forder']:
                for k in RAW:
                    o = int(k == 4)
                    w = wa_v[3 * c + part, o * HD:(o + 1) * HD, o * 128:(o + 1) * 128]
                    raw[part, k] = _dot(xl[:, k * HD:(k + 1) * HD], w)
            nr = CFG['fnr']

            def mk_w(part, r0):
                def run(tok):
                    wa_v[3 * NC1, 0:16, 0:128] = tok.astype(BF)
                    w1 = wa_v[3 * c + part, r0:r0 + nr, :]
                    w2 = wa_v[3 * c + part, HD + r0:HD + r0 + nr, :]
                    rs = make_rhs([w1[:, :128], w1[:, 128:], w2[:, :128], w2[:, 128:]])
                    for k in range(7):
                        wap[part][c * 7 + k, r0 // 2:(r0 + nr) // 2, :] = rs[k]
                return run
            side = _both(*[_spread([mk_w(part, r0) for r0 in range(0, HD, nr)], 21, *rng)
                           for part, rng in zip(CFG['forder'], CFG['frng'])])
            for y in raw.values():
                release(y, side.pop(0))
            for n, part in enumerate(CFG['forder']):
                def prod(k):
                    if k in RAW:
                        return raw[part, k]
                    y = _dot(xl[:, k * HD:(k + 1) * HD], _unpack(wap[part][c * 7 + k + zero]))
                    release(y, side.pop(0))
                    return y

                def put(t):
                    def run(top, bot):
                        y = _weave(top, bot)
                        if part == 0:
                            store_t(y * QSCALE, qt_v, 0, t)
                        elif part == 2:
                            store_t(y, vt_v, 0, t)
                        else:
                            kp = _pack(y.astype(BF))
                            k0_v[t] = kp
                            if n < 2:
                                kt_v[t] = kp[80:128]
                                build_k4(kp, t, 48)
                    return run
                _strassen(prod, put(2 * c), put(2 * c + 1))
                if n == 0:
                    for k in range(NC1 - 2):
                        @pl.when(jnp.logical_and(first, c == k))
                        def _():
                            for cp in cp_wa(k + 2):
                                cp.start()

            @pl.when(jnp.logical_and(first, c == NC1 - 3))
            def _():
                cp_woa.start()

            @pl.when(jnp.logical_and(first, c == NC1 - 2))
            def _():
                cp_x(1).start()
                for cp in cp_wb(0):
                    cp.start()
            return c_

        def a_first():
            lax.fori_loop(0, NC1, f_body, 0)
            at = Attn(0)
            at.issue(CFG['flook'])
            while at.issued < 2 * H:
                at.issue()
                at.finish()

            @pl.when(first)
            def _():
                for cp in [cp_woa, cp_x(1)] + cp_wb(0):
                    cp.wait()
                for cp in [cp_x(2)] + cp_wb(1):
                    cp.start()

                def once(gp, c_):
                    r0 = pl.multiple_of(gp * 256, 256)
                    rows = pl.ds(pl.multiple_of((gp & 1) * 64, 64), 64)
                    for nh in range(2):
                        for nt in range(2):
                            c0 = nh * HD + nt * 128
                            rs = make_rhs([woa_v[pl.ds(r0 + dr, 128), c0 + dc:c0 + dc + 128]
                                           for dr in (0, 128) for dc in (0, 256)])
                            for k in range(7):
                                woap[((gp >> 1) * 2 + nh) * 7 + k, nt, rows, :] = rs[k]
                    return c_
                lax.fori_loop(0, 4, once, 0)

            def mk_k4(t):
                def run(tok):
                    k0_v[8, 0:8, :] = pltpu.bitcast(tok[0:8], U32)
                    kp = k0_v[t + zero]
                    kt_v[t] = kp[80:128]
                    build_k4(kp, t, 48)
                return run
            hi = CFG['fhi']
            side = _both(_spread(prep_out(zero), 28, 0, hi),
                         _spread(ln_chunks(TA + zero * TA, 0, TA), 28, 0, hi))
            if CFG['forder'][2] == 1:
                side = _both(side, _spread([mk_k4(t) for t in range(8)], 28, 0, hi))
            st = Stream(side, {27: lambda: fence_side(zero) | fence_k(zero)}, 1)
            out_a(0, zero, st, lambda u: at.finish(2 * H if u == 1 else 0))

        if CFG['first']:
            a_first()

        @pl.when(first)
        def _():
            cp_x(2).wait()
            for cp in cp_wb(1):
                cp.wait()
            cp_x(3).start()
            for cp in cp_wb(2):
                cp.start()

        def a_body(i, c_):
            @pl.when(jnp.logical_and(first, i == 2))
            def _():
                cp_x(3).wait()
                for cp in cp_wb(2):
                    cp.wait()
            xu = _pack(xl_v[0:TA // 2, :])
            pw = [_spread(prep_qkv(jnp.minimum(4 * (i - 1) + n, 23)), 112, *CFG['urng'][n])
                  for n in range(4)]
            po = prep_out(i)
            side = _both(_spread(ln_chunks((((i + 1) & (NA - 1)) + zero) * TA, 0, TA),
                                 112, *CFG['lrng']),
                         _spread(po, 112, *CFG['orng']), *pw)
            fences = {u: (lambda: fence_side(zero)) for u in CFG['fpos']}
            for n in range(1, 12):
                fe = (fence_k, fence_v, fence_q)[CFG['kord'][(n - 1) % 3]]
                u = 7 * n + 6
                fences[u] = ((lambda fe=fe: fe(zero) | fence_side(zero)) if u in fences
                             else (lambda fe=fe: fe(zero)))
            st = Stream(side, fences, CFG['lag'])
            at = Attn(i)
            for n in range(12):
                gp, kind = n // 3, CFG['kord'][n % 3]

                def prod(k):
                    if n == 11 and k == CFG['hk']:
                        at.issue(CFG['look'])
                    w = wap[(1, 2, 0)[kind]][gp * 7 + k]
                    return st.dot(_dot, xu[:, k * HD:(k + 1) * HD], _unpack(w))

                def put(t):
                    def run(top, bot):
                        y = _weave(top, bot)
                        if kind == 0:
                            kp = _pack(y.astype(BF))
                            full = _rows([kt_v[t], kp])
                            kt_v[t] = kp[80:128]
                            build_k4(full, t, pl.multiple_of(i * (TA // 2), TA // 2))
                        elif kind == 1:
                            store_t(y, vt_v, i * (TA // 128), t)
                        else:
                            store_t(y * QSCALE, qt_v, 0, t)
                    return run
                _strassen(prod, put(2 * gp), put(2 * gp + 1))
            while at.issued < 2 * H - CFG['tail']:
                at.issue()
                at.finish()

            def after(u):
                at.finish()
                at.issue()
            at.issue()
            out_a(pl.multiple_of(i * TA, TA), zero, st, after)
            assert at.done == 2 * H
            return c_
        if CFG['a']:
            lax.fori_loop(1, NA, a_body, 0)

        qk_v[8:16, 0:HALO, :] = jnp.zeros((8, HALO, 128), F32)
        v_v[:, 0:HALO, :] = jnp.zeros((8, HALO, 128), F32)

        def b_body(i, c_):
            def send(k):
                for ii in range(NB if k < 2 else NB - 1):
                    @pl.when(jnp.logical_and(p == 1, i == ii))
                    def _():
                        cp_out(ii, k).start()

            def send_last(c):
                @pl.when(jnp.logical_and(p == 1, i == NB - 1))
                def _():
                    cp_out(NB - 1, 2, c).start()
            ln1 = ln_chunks(i * TB + 256, TA // 2, 256)
            ln2 = ln_chunks((((i + 1) & (NB - 1)) + zero) * TB, 0, TA)
            lg = [logit_b(i, zero, g * 8) for g in range(TB // 8)]
            pv = [pv_b(zero, g * 16) for g in range(TB // 16)]
            n0, n1, n2 = CFG['bn']

            def mix(a, b):
                if CFG['bmix'] == 0:
                    return _flat(_merge([_flat(a[u:u + 2]) for u in range(0, len(a), 2)], b))
                if CFG['bmix'] == 1:
                    return _flat(_merge(a, _flat([[c[0:2], c[2:4]] for c in b])))
                return _merge(_flat(a), _flat(b))
            f0 = {u: (lambda: fence_x(zero)) for u in CFG['bfx']}
            f0.update({u: (lambda: fence_e(zero)) for u in CFG['bfe'] if u < 84})
            f1 = {u - 84: (lambda: fence_e(zero)) for u in CFG['bfe'] if u >= 84}
            proj_b(xl_v[0:TA // 2, :], 0, _both(_spread(ln1 + ln2, 84, 0, CFG['bln']),
                                                _spread(_flat(lg[0:n0]), 84, 57, 84)),
                   f0, CFG['blag'])
            xl1 = xl_v[pl.ds(pl.multiple_of(TA // 2 + zero * 32, 32), TA // 2), :]
            proj_b(xl1, 256, _both(_spread(mix(lg[n0:32], pv[0:16]), 84, 1, 57),
                                   _spread(_flat(lg[32:n1]), 84, 57, 84)),
                   f1, CFG['blag'])
            out_b(i, 0, 256, _spread(mix(lg[n1:64], pv[16:n2]), 28, 1, 28))
            send(0)
            out_b(i, 256, 128, _spread(_flat(pv[n2:32]), 28, 0, CFG['bhi']))
            send(1)
            qk_v[8:16, 0:HALO, :] = qk_v[8:16, TB:TB + HALO, :]
            v_v[:, 0:HALO, :] = v_v[:, TB:TB + HALO, :]
            out_b(i, 384, 128, [[]] * 28, send_last)
            send(2)
            return c_
        if CFG['b']:
            lax.fori_loop(0, NB, b_body, 0)
        return carry

    lax.fori_loop(0, 2, one_pass, 0)
    for i in range(NB):
        for k in range(len(OUT_PIECES)):
            if (i, k) != (NB - 1, 2):
                cp_out(i, k).wait()
    for c in range(4):
        cp_out(NB - 1, 2, c).wait()


@jax.jit
def pallas_interleave_layers__sliding_block__sliding_local_dilated__prompt_kernel(
    A_x: jax.Array,
    A_wqkv: jax.Array,
    A_wo: jax.Array,
    B_x: jax.Array,
    B_wqkv: jax.Array,
    B_wo: jax.Array,
):
    del B_x
    x = A_x.reshape(S, D)
    any_spec = pl.BlockSpec(memory_space=pl.ANY)
    out = pl.pallas_call(
        _kernel,
        out_shape=jax.ShapeDtypeStruct((S, D), BF),
        in_specs=[any_spec] * 5,
        out_specs=any_spec,
        scratch_shapes=[
            pltpu.VMEM((S + 16, D), BF),
            pltpu.VMEM((3 * NC1 + 1, D, G1 * 128), BF),
            pltpu.VMEM((D, D), BF),
            pltpu.VMEM((6, D + 16, 512), BF),
            pltpu.VMEM((5, D, 256), BF),
            pltpu.VMEM((28, 256, 128), U32),
            pltpu.VMEM((28, 256, 128), U32),
            pltpu.VMEM((28, 256, 128), U32),
            pltpu.VMEM((28, 2, 128, 128), U32),
            pltpu.VMEM((5, 9, 48, 2, 8, 128), U32),
            pltpu.VMEM((5, 9, 16, 2, 8, 128), U32),
            pltpu.VMEM((TA + 32, 7 * HD), BF),
            pltpu.VMEM((9, TA // 2, 128), U32),
            pltpu.VMEM((8, 48, 128), U32),
            pltpu.VMEM((H, S // 2, 128), U32),
            pltpu.VMEM((3, D // 2, 128), U32),
            pltpu.VMEM((S // 128 + 1, D // 2, 128), U32),
            pltpu.VMEM((7, 2, 64, 128), U32),
            pltpu.VMEM((7, 2, 64, 128), U32),
            pltpu.VMEM((16, HALO + TB, 128), F32),
            pltpu.VMEM((8, HALO + TB, 128), F32),
            pltpu.VMEM((WB, TB + 16, 128), F32),
            pltpu.VMEM((TB // 2, 7 * HD), BF),
            pltpu.VMEM((4, 8, 128), U32),
            pltpu.SemaphoreType.DMA((5 + NC1,)),
        ],
        compiler_params=pltpu.CompilerParams(vmem_limit_bytes=112 * 1024 * 1024),
        name="interleave_attn",
    )(x, A_wqkv, A_wo, B_wqkv, B_wo)
    return out.reshape(1, S, D)
```

```python
import math

import jax
import jax.numpy as jnp
from jax import lax
import jax.experimental.pallas as pl
import jax.experimental.pallas.tpu as pltpu

BF = jnp.bfloat16
F32 = jnp.float32
U32 = jnp.uint32

S = 2048
D = 1024
H = 32
DH = 32
TA = 256
NA = S // TA
TB = 512
NB = S // TB
HALO = 16
WB = 8
NEG = -1e30
EPS = 1e-5
HD = D // 2
QSCALE = (DH ** -0.5) * math.log2(math.e)
NC1 = 4
G1 = 8 // NC1
FORDER = (2, 0, 1)
OUT_PIECES = ((0, 256), (256, 128), (384, 128))

CFG = dict(first=1, a=1, b=1, look=3, tail=2, cuts=(5, 10, 14), lsum=2, kord=(0, 1, 2), hk=0,
           lag=6, lrng=(0, 64), orng=(90, 102), pnd=2,
           urng=((3, 21), (19, 38), (38, 57), (57, 78)),
           fpos=tuple(range(11, 84, 4)) + (111,),
           flook=6, fhi=24, fnr=32, frng=((0, 4), (4, 9), (9, 14)),
           bn=(20, 64, 26), bln=53, bhi=20, lns=2, lchain=1,
           bmix=2, bfx=tuple(range(8, 60, 4)), bfe=tuple(range(69, 168, 7)), blag=6)


def _dot(a, b):
    return lax.dot_general(a, b, (((1,), (0,)), ((), ())), preferred_element_type=F32)


def _dot_nt(a, b):
    return lax.dot_general(a, b, (((1,), (1,)), ((), ())), preferred_element_type=F32)


def _pack(x_bf16):
    return pltpu.bitcast(x_bf16, U32)


def _unpack(x_u32):
    return pltpu.bitcast(x_u32, BF)


def _iota(shape, dim):
    return lax.broadcasted_iota(jnp.int32, shape, dim)


def _rows(xs):
    return lax.concatenate(xs, 0)


def _lanes(x3):
    n, r, _ = x3.shape
    x2 = x3.reshape(n * r, 128)
    return lax.concatenate([x2[t * r:(t + 1) * r] for t in range(n)], 1)


def _layernorm(x_bf16):
    x = x_bf16.astype(F32)
    m = jnp.sum(x, axis=1, keepdims=True) * (1.0 / D)
    xc = x - m
    v = jnp.sum(xc * xc, axis=1, keepdims=True) * (1.0 / D)
    return xc * lax.rsqrt(v + EPS)


def _lhs7(x11, x12, x21, x22):
    return [x11 + x22, x21 + x22, x11, x22, x11 + x12, x21 - x11, x12 - x22]


def _rhs7(w11, w12, w21, w22):
    return [w11 + w22, w11, w12 - w22, w21 - w11, w22, w11 + w12, w21 + w22]


RAW = (1, 4)
QUAD = (1, 7, 8, 4)


def _strassen(prod, left, right=None):
    m1 = prod(1)
    m3 = prod(3)
    y21 = m1 + m3
    m0 = prod(0)
    y11, y22 = m3 + m0, m0 - m1
    y11 = y11 + prod(6)
    m4 = prod(4)
    y11 = y11 - m4
    if right is not None:
        left(y11, y21)
    m2 = prod(2)
    y12 = m2 + m4
    y22 = (y22 + m2) + prod(5)
    if right is not None:
        right(y12, y22)
    else:
        left(y11, y12, y21, y22)


def _weave(top, bot):
    n, c = top.shape
    both = lax.concatenate([top.reshape(n // 8, 1, 8, c), bot.reshape(n // 8, 1, 8, c)], 1)
    return both.reshape(2 * n, c)


def _recip(l):
    r = pl.reciprocal(l, approx=True)
    return r * (2.0 - l * r)


def _swap16(xu):
    for bit in range(4):
        x5 = xu.reshape(8 >> bit, 2, 2 << bit, 8, 128)
        x, y = x5[:, 0:1], x5[:, 1:2]
        if bit == 0:
            x, y = ((x & U32(0xFFFF)) | (y << 16), (x >> 16) | (y & U32(0xFFFF0000)))
        else:
            dist = 1 << (bit - 1)
            lo = (_iota(x.shape, 3) & dist) == 0
            x, y = (lax.select(lo, x, pltpu.roll(y, dist, 3)),
                    lax.select(lo, pltpu.roll(x, 8 - dist, 3), y))
        xu = lax.concatenate([x, y], 1)
    return xu.reshape(16, 2, 8, 128)


def _spread(chunks, nslots, lo=0, hi=None):
    hi = nslots if hi is None else hi
    out = [[] for _ in range(nslots)]
    for u, c in enumerate(chunks):
        out[lo + u * (hi - lo) // len(chunks)].append(c)
    return out


def _merge(a, b):
    out = []
    for u in range(max(len(a), len(b))):
        out += a[u:u + 1] + b[u:u + 1]
    return out


def _flat(lists):
    return sum(lists, [])


def _both(*lists):
    return [sum(parts, []) for parts in zip(*lists)]


def _kernel(x_hbm, wa_hbm, woa_hbm, wb_hbm, wob_hbm, out_hbm,
            x_v, wa_v, woa_v, wb_v, wob_v, wq_p, wk_p, wv_p, woap, wbt, wobp, xl_v,
            k0_v, kt_v, k4_v, qt_v, vt_v, oa0_v, oa1_v, qk_v, v_v, e_v, ob_v, tk_v,
            sems):
    wap = (wq_p, wk_p, wv_p)
    def cp_x(i):
        n = TA if i < 3 else S - 3 * TA
        return pltpu.make_async_copy(x_hbm.at[pl.ds(i * TA, n), :],
                                     x_v.at[pl.ds(i * TA, n), :], sems.at[i])

    def cp_wa(c):
        w = G1 * 128
        return [pltpu.make_async_copy(wa_hbm.at[:, pl.ds(part * D + c * w, w)],
                                      wa_v.at[3 * c + part], sems.at[5 + c])
                for part in range(3)]

    cp_woa = pltpu.make_async_copy(woa_hbm, woa_v, sems.at[1])

    def cp_wb(st):
        qkv = [[], [(c, r0, 128) for c in range(6) for r0 in (0, 512)],
               [(c, r0, 384) for c in range(6) for r0 in (128, 640)]][st]
        out = [(0, 512 * st, 512)] if st < 2 else [(c, 0, D) for c in range(1, 4)]
        sem = sems.at[st + 1]
        return ([pltpu.make_async_copy(wb_hbm.at[pl.ds(r0, n), pl.ds(c * 512, 512)],
                                       wb_v.at[c, pl.ds(r0, n), :], sem) for c, r0, n in qkv]
                + [pltpu.make_async_copy(wob_hbm.at[pl.ds(r0, n), pl.ds(c * 256, 256)],
                                         wob_v.at[c, pl.ds(r0, n), :], sem) for c, r0, n in out])

    def cp_out(i, k, c=None):
        rows = pl.ds(i * TB + OUT_PIECES[k][0], OUT_PIECES[k][1])
        cols = pl.ds(0, D) if c is None else pl.ds(c * (D // 4), D // 4)
        return pltpu.make_async_copy(x_v.at[rows, cols], out_hbm.at[rows, cols], sems.at[4])

    def release(y, chunks):
        n = len(chunks)
        nt = y.shape[1] // 128
        for u, run in enumerate(chunks):
            pos = (u * y.shape[0] * nt // n) // 16 * 16
            t, rr = pos // y.shape[0], pos % y.shape[0]
            run(y[rr:rr + 16, t * 128:(t + 1) * 128])

    def gated(x, tok, zero):
        tk_v[1] = pltpu.bitcast(tok[0:8], U32)
        return pltpu.bitcast(pltpu.bitcast(x, U32) | tk_v[pl.ds(zero, 1)], F32)

    def fence_x(zero):
        return _pack(xl_v[pl.ds(pl.multiple_of(TA + zero * 32, 32), 32), 0:128])

    def fence_e(zero):
        return pltpu.bitcast(e_v[0, pl.ds(pl.multiple_of(TB + zero * 16, 16), 16), :], U32)

    def fence_side(zero):
        return fence_x(zero) | (wbt[4, 0, 0] | wobp[4, 0, 0]).reshape(16, 128)

    def fence_k(zero):
        return k4_v[zero, 0:16, :]

    def fence_q(zero):
        return qt_v[2 + zero, 0:16, :]

    def fence_v(zero):
        return vt_v[S // 128 + zero, 0:16, :]

    def with_fence(xu, fen):
        r, c = xu.shape
        last = lax.concatenate([xu[r - 16:, :c - 128], xu[r - 16:, c - 128:] | fen], 1)
        return _rows([xu[:r - 16], last])

    def ln_chunks(row0, dst, nrows, step=16):
        def mk(c):
            def run(tok):
                if tok is not None:
                    x_v[S:S + 16, 0:128] = tok.astype(BF)
                r = pl.multiple_of(row0 + c * step, step)
                xn = _layernorm(x_v[pl.ds(r, step), :]).reshape(step // 16, 2, 8, D)
                top, bot = xn[:, 0].reshape(step // 2, D), xn[:, 1].reshape(step // 2, D)
                ls = _lhs7(top[:, :HD], top[:, HD:], bot[:, :HD], bot[:, HD:])
                o = dst + c * (step // 2)
                xl_v[o:o + step // 2, :] = lax.concatenate(ls, 1).astype(BF)
            return run
        return [mk(c) for c in range(nrows // step)]

    def sum_chunks(dst, blk, d0, hh):
        nd = CFG['pnd']

        def mk(d):
            def run(tok):
                dst[4, 1, 0, 0] = pltpu.bitcast(tok[0:8], U32)
                ds = pl.ds(d0 + d, nd)
                wide = [_unpack(dst[blk, q, ds, hh].reshape(nd * 8, 128)).astype(F32)
                        for q in QUAD]
                for k, r in enumerate(_rhs7(*wide)):
                    if k not in RAW:
                        dst[blk, k, ds, hh] = _pack(r.astype(BF)).reshape(nd, 8, 128)
            return run
        return [mk(d) for d in range(0, 16, nd)]

    def prep_qkv(u):
        blk = lax.div(u, 6)
        c = u - 6 * blk
        d0, hh = (c >> 1) * 16, c & 1

        def mk(half):
            def run(tok):
                wb_v[0, D:D + 16, 0:128] = tok.astype(BF)
                rows = pl.ds(pl.multiple_of(blk * 128 + half * HD, 128), 128)
                v = _swap16(_pack(wb_v[c, rows, :].T))
                for dh in range(2):
                    wbt[blk, QUAD[2 * half + dh], pl.ds(d0, 16), hh] = v[:, dh]
            return run
        return [mk(0), mk(1)] + sum_chunks(wbt, blk, d0, hh)

    def prep_out(j):
        blk, hh = j >> 1, j & 1

        def mk(half):
            def run(tok):
                wob_v[4, 0:16, 0:128] = tok.astype(BF)
                rows = pl.ds(pl.multiple_of(hh * HD, HD), HD)
                v = _swap16(_pack(wob_v[blk, rows, half * 128:(half + 1) * 128]))
                for dh in range(2):
                    wobp[blk, QUAD[2 * dh + half], :, hh] = v[:, dh]
            return run
        return [mk(0), mk(1)] + sum_chunks(wobp, blk, 0, hh)

    class Stream:
        def __init__(self, side, fences, lag):
            self.side, self.fences, self.lag = side, fences, lag
            self.u, self.ys = 0, []

        def dot(self, fn, lhs_u, w):
            if self.u in self.fences:
                lhs_u = with_fence(lhs_u, self.fences[self.u]())
            y = fn(_unpack(lhs_u), w)
            self.ys.append(y)
            if self.u >= self.lag:
                release(self.ys[self.u - self.lag], self.side[self.u - self.lag])
            self.u += 1
            return y

        def flush(self):
            for u in range(max(self.u - self.lag, 0), self.u):
                release(self.ys[u], self.side[u])

    def make_rhs(quads):
        rs = _rhs7(*[w.astype(F32) for w in quads])
        return [_pack(quads[3 * (k == 4)] if k in RAW else r.astype(BF))
                for k, r in enumerate(rs)]

    def build_k4(full, t, row0):
        n = full.shape[0] - 48
        rolled = [full] + [pltpu.roll(full, 32 * r, 1) for r in range(1, 4)]
        grp_id = _iota((n, 128), 1) >> 5
        is_g = [grp_id == g for g in range(4)]
        for a in range(4):
            val = rolled[(0 - a) % 4][0:n]
            for g in range(1, 4):
                val = lax.select(is_g[g], rolled[(g - a) % 4][16 * g:16 * g + n], val)
            k4_v[4 * t + a, pl.ds(row0, n), :] = val

    def store_t(y, dst, slot0, t):
        yt = _pack(y.astype(BF).T)
        rows = pl.ds(t * 64 if isinstance(t, int) else pl.multiple_of(t * 64, 64), 64)
        for b in range(TA // 128):
            dst[slot0 + b, rows, :] = yt[:, b * 128:(b + 1) * 128]

    class Attn:
        def __init__(self, blk):
            self.blk = blk
            self.first = isinstance(blk, int)
            self.items = [(qb, 4 * t + a) for t in range(8) for qb in range(2) for a in range(4)]
            self.issued, self.done, self.queue, self.outs, self.tiles = 0, 0, [], [], []
            row, lane = _iota((128, 128), 0), _iota((128, 128), 1)
            self.tri = lane >= row
            if self.first:
                self.neg = jnp.full((128, 128), NEG, F32)
                self.zq = jnp.zeros((16, 128), U32)
            else:
                self.zero = jnp.zeros((128, 128), F32)
                self.slot = (lane >> 5) == (row >> 5)
                new = (_iota((32, 128), 1) & 31) >= _iota((32, 128), 0)
                self.new = (new[0:16], new[16:32])
                lane2 = _iota((256, 128), 1)
                self.odd, self.hi = (lane2 & 32) != 0, lane2 >= 64
                self.base = [pl.multiple_of((blk * 2 + qb) * 64 - 80, 16) for qb in range(2)]

        def scores_first(self, qb, h):
            qh = qt_v[qb, h * 16:(h + 1) * 16, :]
            wq = _unpack(_rows([qh if jj == h % 4 else self.zq for jj in range(4)]))
            n = (qb + 1) * 32
            kk = _unpack(k0_v[h // 4, 0:2 * n, :])
            s = _rows([_dot(kk[c * n:(c + 1) * n], wq) for c in range(4)])
            diag = lax.select(self.tri, s[qb * 128:], self.neg)
            return diag if qb == 0 else _rows([s[0:128], diag])

        def scores(self, qb, h):
            qf = _unpack(qt_v[qb, h * 16:(h + 1) * 16, :]).astype(F32)
            wq = lax.select(self.slot, _rows([qf] * 4), self.zero).astype(BF)
            w = k4_v[h, pl.ds(self.base[qb], 144), :]
            kk = _unpack(_rows([w[0:8], w[128:136], w[8:16], w[136:144], w[16:128]]))
            cuts = (0,) + CFG['cuts'] + (18,)
            s = _rows([_dot(kk[16 * a:16 * b], wq) for a, b in zip(cuts[:-1], cuts[1:])])
            return _rows([lax.select(self.new[0], s[16:32], s[0:16]),
                          lax.select(self.new[1], s[48:64], s[32:48]), s[64:]])

        def softmax_pv(self, s, qb, h):
            mx = jnp.max(s, axis=0, keepdims=True)
            if self.first:
                p = jnp.exp2(s - mx)
                l = jnp.sum(p, axis=0, keepdims=True)
                v3 = vt_v[0:qb + 1, h * 16:(h + 1) * 16, :]
            else:
                s = lax.select(self.odd, _rows([s[224:], s[:224]]), s)
                s = lax.select(self.hi, _rows([s[192:], s[:192]]), s)
                p = jnp.exp2(s - mx)
                if CFG['lsum'] == 0:
                    l = jnp.sum(p, axis=0, keepdims=True)
                else:
                    p3 = p.reshape(2, 128, 128)
                    if CFG['lsum'] == 1:
                        acc = jnp.sum(p.reshape(2, 16, 8, 128), axis=1)
                    else:
                        acc = p3[:, 120:128]
                        for v in range(14, -1, -1):
                            acc = acc + p3[:, 8 * v:8 * v + 8]
                    l = jnp.sum(acc.reshape(16, 128), axis=0, keepdims=True)
                pm = p[0:128]
                p = _rows([lax.select(self.tri, self.zero, pm), p[128:256],
                           lax.select(self.tri, pm, self.zero)])
                v3 = vt_v[pl.ds(self.blk * 2 + qb - 2, 3), h * 16:(h + 1) * 16, :]
            return _dot(_unpack(_lanes(v3)), p.astype(BF)) * _recip(l)

        def store_o(self, gp):
            x = self.tiles
            ready = {2: (2, 5), 4: (4, 0, 1, 3, 6)}.get(len(x), ())
            if ready:
                ls = _lhs7(x[0], x[2 % len(x)], x[1], x[3 % len(x)])
                for k in ready:
                    (oa0_v, oa1_v)[gp // 2][k, gp % 2] = _pack(ls[k].astype(BF).T)
            if len(x) == 4:
                self.tiles = []

        def issue(self, n=1):
            for _ in range(n):
                if self.issued < len(self.items):
                    fn = self.scores_first if self.first else self.scores
                    self.queue.append(fn(*self.items[self.issued]))
                    self.issued += 1

        def finish(self, n=1):
            for _ in range(n):
                if self.done < self.issued:
                    qb, h = self.items[self.done]
                    self.outs.append(self.softmax_pv(self.queue.pop(0), qb, h))
                    if len(self.outs) == 4:
                        self.tiles.append(_rows(self.outs))
                        self.outs = []
                        self.store_o(h // 8)
                    self.done += 1

    def add_residual(r, nrows, c0, c1, y):
        x_v[pl.ds(r, nrows), c0:c1] = (x_v[pl.ds(r, nrows), c0:c1].astype(F32) + y).astype(BF)

    def proj_b(xl, r0, side, fences, lag):
        rows = slice(HALO + r0, HALO + r0 + TA)
        xu = _pack(xl)
        st = Stream(side, fences, lag)
        for P in range(12):
            def prod(k):
                w = wbt[0:4, k, 4 * P:4 * P + 4].reshape(4, 64, 128)
                return st.dot(_dot_nt, xu[:, k * HD:(k + 1) * HD], _unpack(_lanes(w)))

            def put(T):
                def run(top, bot):
                    y = _weave(top, bot)
                    if T < 8:
                        qk_v[T, rows, :] = y * QSCALE
                    elif T < 16:
                        qk_v[T, rows, :] = y
                    else:
                        v_v[T - 16, rows, :] = y
                return run
            T = (P // 4) * 8 + P % 4
            _strassen(prod, put(T), put(T + 4))
        st.flush()

    def taps(ref, t0, t1, r0):
        wins = [ref[t0:t1, HALO + r0 - 2 * w:HALO + r0 - 2 * w + 8, :] for w in range(WB)]
        return _rows(wins).reshape(WB, t1 - t0, 8, 128)

    def logit_b(i, zero, r0):
        ns = CFG['lns']
        acc = []

        def mk(st):
            def run(tok):
                t0, t1 = st * 8 // ns, (st + 1) * 8 // ns
                q = gated(qk_v[t0:t1, HALO + r0:HALO + r0 + 8, :], tok, zero)
                p = q[None] * taps(qk_v, 8 + t0, 8 + t1, r0)
                if acc and CFG['lchain']:
                    a = jnp.sum(lax.concatenate([acc.pop()[:, None], p], 1), axis=1)
                else:
                    a = jnp.sum(p, axis=1)
                    a = acc.pop() + a if acc else a
                if st + 1 < ns:
                    acc.append(a)
                    return
                a = a + pltpu.roll(a, 64, 2)
                a = a + pltpu.roll(a, 32, 2)
                if r0 < 2 * (WB - 1):
                    pos = _iota(a.shape, 1) - 2 * _iota(a.shape, 0) + (i * TB + r0)
                    a = lax.select(pos >= 0, a, jnp.full(a.shape, NEG, F32))
                e = jnp.exp2(a - jnp.max(a, axis=0, keepdims=True))
                e_v[:, r0:r0 + 8, :] = e * _recip(jnp.sum(e, axis=0, keepdims=True))
            return run
        return [mk(st) for st in range(ns)]

    def pv_b(zero, r0):
        x = []

        def mk(st):
            def run(tok):
                r, t0 = r0 + 8 * (st // 2), 4 * (st % 2)
                e = gated(e_v[:, r:r + 8, :], tok, zero)
                x.append(_lanes(jnp.sum(e[:, None] * taps(v_v, t0, t0 + 4, r), axis=0)))
                if st == 3:
                    ob_v[r0 // 2:r0 // 2 + 8, :] = lax.concatenate(_lhs7(*x), 1).astype(BF)
            return run
        return [mk(st) for st in range(4)]

    def out_b(i, r0, nrows, side, done=None):
        ou = _pack(ob_v[r0 // 2:(r0 + nrows) // 2, :])
        r = pl.multiple_of(i * TB + r0, 128)
        st = Stream(side, {}, 0)
        for c in range(4):
            def prod(k):
                w = _unpack(wobp[c, k].reshape(256, 128))
                return st.dot(_dot, ou[:, k * HD:(k + 1) * HD], w)

            def put(y11, y12, y21, y22):
                y = _weave(lax.concatenate([y11, y12], 1), lax.concatenate([y21, y22], 1))
                add_residual(r, nrows, c * 256, (c + 1) * 256, y)
            _strassen(prod, put)
            if done is not None:
                done(c)

    cp_x(0).start()
    for cp in cp_wa(0):
        cp.start()
    z16 = jnp.zeros((16, 128), U32)
    xl_v[TA:TA + 32, 0:128] = jnp.zeros((32, 128), BF)
    wbt[4, 0, 0] = z16.reshape(2, 8, 128)
    wobp[4, 0, 0] = z16.reshape(2, 8, 128)
    k4_v[0, 0:16, :] = z16
    vt_v[S // 128, 0:16, :] = z16
    qt_v[2, 0:16, :] = z16
    tk_v[0] = z16[0:8]
    e_v[0, TB:TB + 16, :] = jnp.zeros((16, 128), F32)
    cp_x(0).wait()
    for cp in cp_wa(1):
        cp.start()
    for run in ln_chunks(0, 0, TA, step=TA):
        run(None)

    def one_pass(p, carry):
        first = p == 0
        zero = p >> 2

        def out_a(blk, zero, st, after):
            part = {}
            n = [0]
            for ph in range(2):
                ou = oa0_v[pl.ds(zero, 7)] if ph == 0 else oa1_v[...]
                for nh in range(2):
                    def prod(k):
                        w = _unpack(_lanes(woap[(ph * 2 + nh) * 7 + k]))
                        y = st.dot(_dot, _lanes(ou[k]), w)
                        n[0] += 1
                        after(n[0])
                        return y

                    def put(half):
                        def run(top, bot):
                            y = _rows([top, bot])
                            if ph == 0:
                                part[nh, half] = y
                            else:
                                c0 = nh * HD + half * 256
                                add_residual(blk, TA, c0, c0 + 256, y + part[nh, half])
                        return run
                    _strassen(prod, put(0), put(1))

        def put_first(part, t):
            def run(top, bot):
                y = _weave(top, bot)
                if part == 0:
                    store_t(y * QSCALE, qt_v, 0, t)
                elif part == 2:
                    store_t(y, vt_v, 0, t)
                else:
                    k0_v[t] = _pack(y.astype(BF))
            return run

        def f_body(c, c_):
            buf = wa_v.at[pl.ds(3 * c, 3)]
            pltpu.make_async_copy(buf, buf, sems.at[5 + c]).wait()
            xl = xl_v[0:TA // 2, :]
            raw = {}
            for part in FORDER:
                for k in RAW:
                    o = int(k == 4)
                    w = wa_v[3 * c + part, o * HD:(o + 1) * HD, o * 128:(o + 1) * 128]
                    raw[part, k] = _dot(xl[:, k * HD:(k + 1) * HD], w)
            nr = CFG['fnr']

            def mk_w(part, r0):
                def run(tok):
                    wa_v[3 * NC1, 0:16, 0:128] = tok.astype(BF)
                    w1 = wa_v[3 * c + part, r0:r0 + nr, :]
                    w2 = wa_v[3 * c + part, HD + r0:HD + r0 + nr, :]
                    rs = make_rhs([w1[:, :128], w1[:, 128:], w2[:, :128], w2[:, 128:]])
                    for k in range(7):
                        wap[part][c * 7 + k, r0 // 2:(r0 + nr) // 2, :] = rs[k]
                return run
            side = _both(*[_spread([mk_w(part, r0) for r0 in range(0, HD, nr)], 21, *rng)
                           for part, rng in zip(FORDER, CFG['frng'])])
            for y in raw.values():
                release(y, side.pop(0))
            for n, part in enumerate(FORDER):
                def prod(k):
                    if k in RAW:
                        return raw[part, k]
                    y = _dot(xl[:, k * HD:(k + 1) * HD], _unpack(wap[part][c * 7 + k + zero]))
                    release(y, side.pop(0))
                    return y
                _strassen(prod, put_first(part, 2 * c), put_first(part, 2 * c + 1))
                if n == 0:
                    for k in range(NC1 - 2):
                        @pl.when(c == k)
                        def _():
                            for cp in cp_wa(k + 2):
                                cp.start()

            @pl.when(c == NC1 - 3)
            def _():
                cp_woa.start()

            @pl.when(c == NC1 - 2)
            def _():
                for cp in [cp_x(1)] + cp_wb(0):
                    cp.start()
            return c_

        def g_body(c, c_):
            xl = xl_v[0:TA // 2, :]
            for part in FORDER:
                _strassen(lambda k: _dot(xl[:, k * HD:(k + 1) * HD], _unpack(wap[part][c * 7 + k])),
                          put_first(part, 2 * c), put_first(part, 2 * c + 1))
            return c_

        def a_first():
            @pl.when(first)
            def _():
                lax.fori_loop(0, NC1, f_body, 0)

            @pl.when(jnp.logical_not(first))
            def _():
                lax.fori_loop(0, NC1, g_body, 0)
            at = Attn(0)
            at.issue(CFG['flook'])
            while at.issued < 2 * H:
                at.issue()
                at.finish()

            @pl.when(first)
            def _():
                for cp in [cp_woa, cp_x(1)] + cp_wb(0):
                    cp.wait()
                for cp in [cp_x(2)] + cp_wb(1):
                    cp.start()

                def once(gp, c_):
                    r0 = pl.multiple_of(gp * 256, 256)
                    rows = pl.ds(pl.multiple_of((gp & 1) * 64, 64), 64)
                    for nh in range(2):
                        for nt in range(2):
                            c0 = nh * HD + nt * 128
                            rs = make_rhs([woa_v[pl.ds(r0 + dr, 128), c0 + dc:c0 + dc + 128]
                                           for dr in (0, 128) for dc in (0, 256)])
                            for k in range(7):
                                woap[((gp >> 1) * 2 + nh) * 7 + k, nt, rows, :] = rs[k]
                    return c_
                lax.fori_loop(0, 4, once, 0)

            def mk_k4(t):
                def run(tok):
                    k0_v[8, 0:8, :] = pltpu.bitcast(tok[0:8], U32)
                    kp = k0_v[t + zero]
                    kt_v[t] = kp[80:128]
                    build_k4(kp, t, 48)
                return run
            hi = CFG['fhi']
            side = _both(_spread(prep_out(zero), 28, 0, hi),
                         _spread(ln_chunks(TA + zero * TA, 0, TA), 28, 0, hi))
            side = _both(side, _spread([mk_k4(t) for t in range(8)], 28, 0, hi))
            st = Stream(side, {27: lambda: fence_side(zero) | fence_k(zero)}, 1)
            out_a(0, zero, st, lambda u: at.finish(2 * H if u == 1 else 0))

        if CFG['first']:
            a_first()

        @pl.when(first)
        def _():
            cp_x(2).wait()
            for cp in cp_wb(1):
                cp.wait()
            cp_x(3).start()
            for cp in cp_wb(2):
                cp.start()

        def a_body(i, c_):
            @pl.when(jnp.logical_and(first, i == 2))
            def _():
                cp_x(3).wait()
                for cp in cp_wb(2):
                    cp.wait()
            xu = _pack(xl_v[0:TA // 2, :])
            pw = [_spread(prep_qkv(jnp.minimum(4 * (i - 1) + n, 23)), 112, *CFG['urng'][n])
                  for n in range(4)]
            po = prep_out(i)
            side = _both(_spread(ln_chunks((((i + 1) & (NA - 1)) + zero) * TA, 0, TA),
                                 112, *CFG['lrng']),
                         _spread(po, 112, *CFG['orng']), *pw)
            fences = {u: (lambda: fence_side(zero)) for u in CFG['fpos']}
            for n in range(1, 12):
                fe = (fence_k, fence_v, fence_q)[CFG['kord'][(n - 1) % 3]]
                u = 7 * n + 6
                fences[u] = ((lambda fe=fe: fe(zero) | fence_side(zero)) if u in fences
                             else (lambda fe=fe: fe(zero)))
            st = Stream(side, fences, CFG['lag'])
            at = Attn(i)
            for n in range(12):
                gp, kind = n // 3, CFG['kord'][n % 3]

                def prod(k):
                    if n == 11 and k == CFG['hk']:
                        at.issue(CFG['look'])
                    w = wap[(1, 2, 0)[kind]][gp * 7 + k]
                    return st.dot(_dot, xu[:, k * HD:(k + 1) * HD], _unpack(w))

                def put(t):
                    def run(top, bot):
                        y = _weave(top, bot)
                        if kind == 0:
                            kp = _pack(y.astype(BF))
                            full = _rows([kt_v[t], kp])
                            kt_v[t] = kp[80:128]
                            build_k4(full, t, pl.multiple_of(i * (TA // 2), TA // 2))
                        elif kind == 1:
                            store_t(y, vt_v, i * (TA // 128), t)
                        else:
                            store_t(y * QSCALE, qt_v, 0, t)
                    return run
                _strassen(prod, put(2 * gp), put(2 * gp + 1))
            while at.issued < 2 * H - CFG['tail']:
                at.issue()
                at.finish()

            def after(u):
                at.finish()
                at.issue()
            at.issue()
            out_a(pl.multiple_of(i * TA, TA), zero, st, after)
            assert at.done == 2 * H
            return c_
        if CFG['a']:
            lax.fori_loop(1, NA, a_body, 0)

        qk_v[8:16, 0:HALO, :] = jnp.zeros((8, HALO, 128), F32)
        v_v[:, 0:HALO, :] = jnp.zeros((8, HALO, 128), F32)

        def b_body(i, c_):
            def send(k):
                for ii in range(NB if k < 2 else NB - 1):
                    @pl.when(jnp.logical_and(p == 1, i == ii))
                    def _():
                        cp_out(ii, k).start()

            def send_last(c):
                @pl.when(jnp.logical_and(p == 1, i == NB - 1))
                def _():
                    cp_out(NB - 1, 2, c).start()
            ln1 = ln_chunks(i * TB + 256, TA // 2, 256)
            ln2 = ln_chunks((((i + 1) & (NB - 1)) + zero) * TB, 0, TA)
            lg = [logit_b(i, zero, g * 8) for g in range(TB // 8)]
            pv = [pv_b(zero, g * 16) for g in range(TB // 16)]
            n0, n1, n2 = CFG['bn']

            def mix(a, b):
                if CFG['bmix'] == 0:
                    return _flat(_merge([_flat(a[u:u + 2]) for u in range(0, len(a), 2)], b))
                if CFG['bmix'] == 1:
                    return _flat(_merge(a, _flat([[c[0:2], c[2:4]] for c in b])))
                return _merge(_flat(a), _flat(b))
            f0 = {u: (lambda: fence_x(zero)) for u in CFG['bfx']}
            f0.update({u: (lambda: fence_e(zero)) for u in CFG['bfe'] if u < 84})
            f1 = {u - 84: (lambda: fence_e(zero)) for u in CFG['bfe'] if u >= 84}
            proj_b(xl_v[0:TA // 2, :], 0, _both(_spread(ln1 + ln2, 84, 0, CFG['bln']),
                                                _spread(_flat(lg[0:n0]), 84, 57, 84)),
                   f0, CFG['blag'])
            xl1 = xl_v[pl.ds(pl.multiple_of(TA // 2 + zero * 32, 32), TA // 2), :]
            proj_b(xl1, 256, _both(_spread(mix(lg[n0:32], pv[0:16]), 84, 1, 57),
                                   _spread(_flat(lg[32:n1]), 84, 57, 84)),
                   f1, CFG['blag'])
            out_b(i, 0, 256, _spread(mix(lg[n1:64], pv[16:n2]), 28, 1, 28))
            send(0)
            out_b(i, 256, 128, _spread(_flat(pv[n2:32]), 28, 0, CFG['bhi']))
            send(1)
            qk_v[8:16, 0:HALO, :] = qk_v[8:16, TB:TB + HALO, :]
            v_v[:, 0:HALO, :] = v_v[:, TB:TB + HALO, :]
            out_b(i, 384, 128, [[]] * 28, send_last)
            send(2)
            return c_
        if CFG['b']:
            lax.fori_loop(0, NB, b_body, 0)
        return carry

    lax.fori_loop(0, 2, one_pass, 0)
    for i in range(NB):
        for k in range(len(OUT_PIECES)):
            if (i, k) != (NB - 1, 2):
                cp_out(i, k).wait()
    for c in range(4):
        cp_out(NB - 1, 2, c).wait()


@jax.jit
def pallas_interleave_layers__sliding_block__sliding_local_dilated__prompt_kernel(
    A_x: jax.Array,
    A_wqkv: jax.Array,
    A_wo: jax.Array,
    B_x: jax.Array,
    B_wqkv: jax.Array,
    B_wo: jax.Array,
):
    del B_x
    x = A_x.reshape(S, D)
    any_spec = pl.BlockSpec(memory_space=pl.ANY)
    out = pl.pallas_call(
        _kernel,
        out_shape=jax.ShapeDtypeStruct((S, D), BF),
        in_specs=[any_spec] * 5,
        out_specs=any_spec,
        scratch_shapes=[
            pltpu.VMEM((S + 16, D), BF),
            pltpu.VMEM((3 * NC1 + 1, D, G1 * 128), BF),
            pltpu.VMEM((D, D), BF),
            pltpu.VMEM((6, D + 16, 512), BF),
            pltpu.VMEM((5, D, 256), BF),
            pltpu.VMEM((28, 256, 128), U32),
            pltpu.VMEM((28, 256, 128), U32),
            pltpu.VMEM((28, 256, 128), U32),
            pltpu.VMEM((28, 2, 128, 128), U32),
            pltpu.VMEM((5, 9, 48, 2, 8, 128), U32),
            pltpu.VMEM((5, 9, 16, 2, 8, 128), U32),
            pltpu.VMEM((TA + 32, 7 * HD), BF),
            pltpu.VMEM((9, TA // 2, 128), U32),
            pltpu.VMEM((8, 48, 128), U32),
            pltpu.VMEM((H, S // 2, 128), U32),
            pltpu.VMEM((3, D // 2, 128), U32),
            pltpu.VMEM((S // 128 + 1, D // 2, 128), U32),
            pltpu.VMEM((7, 2, 64, 128), U32),
            pltpu.VMEM((7, 2, 64, 128), U32),
            pltpu.VMEM((16, HALO + TB, 128), F32),
            pltpu.VMEM((8, HALO + TB, 128), F32),
            pltpu.VMEM((WB, TB + 16, 128), F32),
            pltpu.VMEM((TB // 2, 7 * HD), BF),
            pltpu.VMEM((4, 8, 128), U32),
            pltpu.SemaphoreType.DMA((5 + NC1,)),
        ],
        compiler_params=pltpu.CompilerParams(vmem_limit_bytes=112 * 1024 * 1024),
        name="interleave_attn",
    )(x, A_wqkv, A_wo, B_wqkv, B_wo)
    return out.reshape(1, S, D)
```

```python
import math

import jax
import jax.numpy as jnp
from jax import lax
import jax.experimental.pallas as pl
import jax.experimental.pallas.tpu as pltpu

BF = jnp.bfloat16
F32 = jnp.float32
U32 = jnp.uint32

S = 2048
D = 1024
H = 32
DH = 32
TA = 256
NA = S // TA
TB = 512
NB = S // TB
HALO = 16
WB = 8
NEG = -1e30
EPS = 1e-5
HD = D // 2
QSCALE = (DH ** -0.5) * math.log2(math.e)
NC1 = 4
G1 = 8 // NC1
FORDER = (2, 0, 1)
OUT_PIECES = ((0, 256), (256, 128), (384, 128))

CFG = dict(
    first=1, a=1, b=1,
    look=3, tail=2, hk=0, cuts=(5, 10, 14), kord=(0, 1, 2),
    lag=6, lrng=(0, 64), orng=(90, 102), pnd=2,
    urng=((3, 21), (19, 38), (38, 57), (57, 78)),
    fpos=tuple(range(11, 84, 4)) + (111,),
    flook=6, fhi=24, fnr=32, frng=((0, 4), (4, 9), (9, 14)),
    bn=(20, 64, 26), bln=53, bhi=20, lns=2, blag=6,
    bfx=tuple(range(8, 60, 4)), bfe=tuple(range(69, 168, 7)))


def _dot(a, b):
    return lax.dot_general(a, b, (((1,), (0,)), ((), ())), preferred_element_type=F32)


def _dot_nt(a, b):
    return lax.dot_general(a, b, (((1,), (1,)), ((), ())), preferred_element_type=F32)


def _pack(x_bf16):
    return pltpu.bitcast(x_bf16, U32)


def _unpack(x_u32):
    return pltpu.bitcast(x_u32, BF)


def _iota(shape, dim):
    return lax.broadcasted_iota(jnp.int32, shape, dim)


def _rows(xs):
    return lax.concatenate(xs, 0)


def _lanes(x3):
    n, r, _ = x3.shape
    x2 = x3.reshape(n * r, 128)
    return lax.concatenate([x2[t * r:(t + 1) * r] for t in range(n)], 1)


def _layernorm(x_bf16):
    x = x_bf16.astype(F32)
    m = jnp.sum(x, axis=1, keepdims=True) * (1.0 / D)
    xc = x - m
    v = jnp.sum(xc * xc, axis=1, keepdims=True) * (1.0 / D)
    return xc * lax.rsqrt(v + EPS)


def _lhs7(x11, x12, x21, x22):
    return [x11 + x22, x21 + x22, x11, x22, x11 + x12, x21 - x11, x12 - x22]


def _rhs7(w11, w12, w21, w22):
    return [w11 + w22, w11, w12 - w22, w21 - w11, w22, w11 + w12, w21 + w22]


RAW = (1, 4)
QUAD = (1, 7, 8, 4)


def _strassen(prod, left, right=None):
    m1 = prod(1)
    m3 = prod(3)
    y21 = m1 + m3
    m0 = prod(0)
    y11, y22 = m3 + m0, m0 - m1
    y11 = y11 + prod(6)
    m4 = prod(4)
    y11 = y11 - m4
    if right is not None:
        left(y11, y21)
    m2 = prod(2)
    y12 = m2 + m4
    y22 = (y22 + m2) + prod(5)
    if right is not None:
        right(y12, y22)
    else:
        left(y11, y12, y21, y22)


def _weave(top, bot):
    n, c = top.shape
    both = lax.concatenate([top.reshape(n // 8, 1, 8, c), bot.reshape(n // 8, 1, 8, c)], 1)
    return both.reshape(2 * n, c)


def _recip(l):
    r = pl.reciprocal(l, approx=True)
    return r * (2.0 - l * r)


def _swap16(xu):
    for bit in range(4):
        x5 = xu.reshape(8 >> bit, 2, 2 << bit, 8, 128)
        x, y = x5[:, 0:1], x5[:, 1:2]
        if bit == 0:
            x, y = ((x & U32(0xFFFF)) | (y << 16), (x >> 16) | (y & U32(0xFFFF0000)))
        else:
            dist = 1 << (bit - 1)
            lo = (_iota(x.shape, 3) & dist) == 0
            x, y = (lax.select(lo, x, pltpu.roll(y, dist, 3)),
                    lax.select(lo, pltpu.roll(x, 8 - dist, 3), y))
        xu = lax.concatenate([x, y], 1)
    return xu.reshape(16, 2, 8, 128)


def _spread(chunks, nslots, lo=0, hi=None):
    hi = nslots if hi is None else hi
    out = [[] for _ in range(nslots)]
    for u, c in enumerate(chunks):
        out[lo + u * (hi - lo) // len(chunks)].append(c)
    return out


def _merge(a, b):
    out = []
    for u in range(max(len(a), len(b))):
        out += a[u:u + 1] + b[u:u + 1]
    return out


def _flat(lists):
    return sum(lists, [])


def _both(*lists):
    return [sum(parts, []) for parts in zip(*lists)]


def _kernel(x_hbm, wa_hbm, woa_hbm, wb_hbm, wob_hbm, out_hbm,
            x_v, wa_v, woa_v, wb_v, wob_v, wq_p, wk_p, wv_p, woap, wbt, wobp, xl_v,
            k0_v, kt_v, k4_v, qt_v, vt_v, oa0_v, oa1_v, qk_v, v_v, e_v, ob_v, tk_v,
            sems):
    wap = (wq_p, wk_p, wv_p)
    def cp_x(i):
        n = TA if i < 3 else S - 3 * TA
        return pltpu.make_async_copy(x_hbm.at[pl.ds(i * TA, n), :],
                                     x_v.at[pl.ds(i * TA, n), :], sems.at[i])

    def cp_wa(c):
        w = G1 * 128
        return [pltpu.make_async_copy(wa_hbm.at[:, pl.ds(part * D + c * w, w)],
                                      wa_v.at[3 * c + part], sems.at[5 + c])
                for part in range(3)]

    cp_woa = pltpu.make_async_copy(woa_hbm, woa_v, sems.at[1])

    def cp_wb(st):
        qkv = [[], [(c, r0, 128) for c in range(6) for r0 in (0, 512)],
               [(c, r0, 384) for c in range(6) for r0 in (128, 640)]][st]
        out = [(0, 512 * st, 512)] if st < 2 else [(c, 0, D) for c in range(1, 4)]
        sem = sems.at[st + 1]
        return ([pltpu.make_async_copy(wb_hbm.at[pl.ds(r0, n), pl.ds(c * 512, 512)],
                                       wb_v.at[c, pl.ds(r0, n), :], sem) for c, r0, n in qkv]
                + [pltpu.make_async_copy(wob_hbm.at[pl.ds(r0, n), pl.ds(c * 256, 256)],
                                         wob_v.at[c, pl.ds(r0, n), :], sem) for c, r0, n in out])

    def cp_out(i, k, c=None):
        rows = pl.ds(i * TB + OUT_PIECES[k][0], OUT_PIECES[k][1])
        cols = pl.ds(0, D) if c is None else pl.ds(c * (D // 4), D // 4)
        return pltpu.make_async_copy(x_v.at[rows, cols], out_hbm.at[rows, cols], sems.at[4])

    def release(y, chunks):
        n = len(chunks)
        nt = y.shape[1] // 128
        for u, run in enumerate(chunks):
            pos = (u * y.shape[0] * nt // n) // 16 * 16
            t, rr = pos // y.shape[0], pos % y.shape[0]
            run(y[rr:rr + 16, t * 128:(t + 1) * 128])

    def gated(x, tok, zero):
        tk_v[1] = pltpu.bitcast(tok[0:8], U32)
        return pltpu.bitcast(pltpu.bitcast(x, U32) | tk_v[pl.ds(zero, 1)], F32)

    def fence_x(zero):
        return _pack(xl_v[pl.ds(pl.multiple_of(TA + zero * 32, 32), 32), 0:128])

    def fence_e(zero):
        return pltpu.bitcast(e_v[0, pl.ds(pl.multiple_of(TB + zero * 16, 16), 16), :], U32)

    def fence_side(zero):
        return fence_x(zero) | (wbt[4, 0, 0] | wobp[4, 0, 0]).reshape(16, 128)

    def fence_k(zero):
        return k4_v[zero, 0:16, :]

    def fence_q(zero):
        return qt_v[2 + zero, 0:16, :]

    def fence_v(zero):
        return vt_v[S // 128 + zero, 0:16, :]

    def with_fence(xu, fen):
        r, c = xu.shape
        last = lax.concatenate([xu[r - 16:, :c - 128], xu[r - 16:, c - 128:] | fen], 1)
        return _rows([xu[:r - 16], last])

    def ln_chunks(row0, dst, nrows, step=16):
        def mk(c):
            def run(tok):
                if tok is not None:
                    x_v[S:S + 16, 0:128] = tok.astype(BF)
                r = pl.multiple_of(row0 + c * step, step)
                xn = _layernorm(x_v[pl.ds(r, step), :]).reshape(step // 16, 2, 8, D)
                top, bot = xn[:, 0].reshape(step // 2, D), xn[:, 1].reshape(step // 2, D)
                ls = _lhs7(top[:, :HD], top[:, HD:], bot[:, :HD], bot[:, HD:])
                o = dst + c * (step // 2)
                xl_v[o:o + step // 2, :] = lax.concatenate(ls, 1).astype(BF)
            return run
        return [mk(c) for c in range(nrows // step)]

    def sum_chunks(dst, blk, d0, hh):
        nd = CFG['pnd']

        def mk(d):
            def run(tok):
                dst[4, 1, 0, 0] = pltpu.bitcast(tok[0:8], U32)
                ds = pl.ds(d0 + d, nd)
                wide = [_unpack(dst[blk, q, ds, hh].reshape(nd * 8, 128)).astype(F32)
                        for q in QUAD]
                for k, r in enumerate(_rhs7(*wide)):
                    if k not in RAW:
                        dst[blk, k, ds, hh] = _pack(r.astype(BF)).reshape(nd, 8, 128)
            return run
        return [mk(d) for d in range(0, 16, nd)]

    def prep_qkv(u):
        blk = lax.div(u, 6)
        c = u - 6 * blk
        d0, hh = (c >> 1) * 16, c & 1

        def mk(half):
            def run(tok):
                wb_v[0, D:D + 16, 0:128] = tok.astype(BF)
                rows = pl.ds(pl.multiple_of(blk * 128 + half * HD, 128), 128)
                v = _swap16(_pack(wb_v[c, rows, :].T))
                for dh in range(2):
                    wbt[blk, QUAD[2 * half + dh], pl.ds(d0, 16), hh] = v[:, dh]
            return run
        return [mk(0), mk(1)] + sum_chunks(wbt, blk, d0, hh)

    def prep_out(j):
        blk, hh = j >> 1, j & 1

        def mk(half):
            def run(tok):
                wob_v[4, 0:16, 0:128] = tok.astype(BF)
                rows = pl.ds(pl.multiple_of(hh * HD, HD), HD)
                v = _swap16(_pack(wob_v[blk, rows, half * 128:(half + 1) * 128]))
                for dh in range(2):
                    wobp[blk, QUAD[2 * dh + half], :, hh] = v[:, dh]
            return run
        return [mk(0), mk(1)] + sum_chunks(wobp, blk, 0, hh)

    class Stream:
        def __init__(self, side, fences, lag):
            self.side, self.fences, self.lag = side, fences, lag
            self.u, self.ys = 0, []

        def dot(self, fn, lhs_u, w):
            if self.u in self.fences:
                lhs_u = with_fence(lhs_u, self.fences[self.u]())
            y = fn(_unpack(lhs_u), w)
            self.ys.append(y)
            if self.u >= self.lag:
                release(self.ys[self.u - self.lag], self.side[self.u - self.lag])
            self.u += 1
            return y

        def flush(self):
            for u in range(max(self.u - self.lag, 0), self.u):
                release(self.ys[u], self.side[u])

    def make_rhs(quads):
        rs = _rhs7(*[w.astype(F32) for w in quads])
        return [_pack(quads[3 * (k == 4)] if k in RAW else r.astype(BF))
                for k, r in enumerate(rs)]

    def build_k4(full, t, row0):
        n = full.shape[0] - 48
        rolled = [full] + [pltpu.roll(full, 32 * r, 1) for r in range(1, 4)]
        grp_id = _iota((n, 128), 1) >> 5
        is_g = [grp_id == g for g in range(4)]
        for a in range(4):
            val = rolled[(0 - a) % 4][0:n]
            for g in range(1, 4):
                val = lax.select(is_g[g], rolled[(g - a) % 4][16 * g:16 * g + n], val)
            k4_v[4 * t + a, pl.ds(row0, n), :] = val

    def store_t(y, dst, slot0, t):
        yt = _pack(y.astype(BF).T)
        rows = pl.ds(t * 64 if isinstance(t, int) else pl.multiple_of(t * 64, 64), 64)
        for b in range(TA // 128):
            dst[slot0 + b, rows, :] = yt[:, b * 128:(b + 1) * 128]

    class Attn:
        def __init__(self, blk):
            self.blk = blk
            self.first = isinstance(blk, int)
            self.items = [(qb, 4 * t + a) for t in range(8) for qb in range(2) for a in range(4)]
            self.issued, self.done, self.queue, self.outs, self.tiles = 0, 0, [], [], []
            row, lane = _iota((128, 128), 0), _iota((128, 128), 1)
            self.tri = lane >= row
            if self.first:
                self.neg = jnp.full((128, 128), NEG, F32)
                self.zq = jnp.zeros((16, 128), U32)
            else:
                self.zero = jnp.zeros((128, 128), F32)
                self.slot = (lane >> 5) == (row >> 5)
                new = (_iota((32, 128), 1) & 31) >= _iota((32, 128), 0)
                self.new = (new[0:16], new[16:32])
                lane2 = _iota((256, 128), 1)
                self.odd, self.hi = (lane2 & 32) != 0, lane2 >= 64
                self.base = [pl.multiple_of((blk * 2 + qb) * 64 - 80, 16) for qb in range(2)]

        def scores_first(self, qb, h):
            qh = qt_v[qb, h * 16:(h + 1) * 16, :]
            wq = _unpack(_rows([qh if jj == h % 4 else self.zq for jj in range(4)]))
            n = (qb + 1) * 32
            kk = _unpack(k0_v[h // 4, 0:2 * n, :])
            s = _rows([_dot(kk[c * n:(c + 1) * n], wq) for c in range(4)])
            diag = lax.select(self.tri, s[qb * 128:], self.neg)
            return diag if qb == 0 else _rows([s[0:128], diag])

        def scores(self, qb, h):
            qf = _unpack(qt_v[qb, h * 16:(h + 1) * 16, :]).astype(F32)
            wq = lax.select(self.slot, _rows([qf] * 4), self.zero).astype(BF)
            w = k4_v[h, pl.ds(self.base[qb], 144), :]
            kk = _unpack(_rows([w[0:8], w[128:136], w[8:16], w[136:144], w[16:128]]))
            cuts = (0,) + CFG['cuts'] + (18,)
            s = _rows([_dot(kk[16 * a:16 * b], wq) for a, b in zip(cuts[:-1], cuts[1:])])
            return _rows([lax.select(self.new[0], s[16:32], s[0:16]),
                          lax.select(self.new[1], s[48:64], s[32:48]), s[64:]])

        def softmax_pv(self, s, qb, h):
            mx = jnp.max(s, axis=0, keepdims=True)
            if self.first:
                p = jnp.exp2(s - mx)
                l = jnp.sum(p, axis=0, keepdims=True)
                v3 = vt_v[0:qb + 1, h * 16:(h + 1) * 16, :]
            else:
                s = lax.select(self.odd, _rows([s[224:], s[:224]]), s)
                s = lax.select(self.hi, _rows([s[192:], s[:192]]), s)
                p = jnp.exp2(s - mx)
                p3 = p.reshape(2, 128, 128)
                acc = p3[:, 120:128]
                for v in range(14, -1, -1):
                    acc = acc + p3[:, 8 * v:8 * v + 8]
                l = jnp.sum(acc.reshape(16, 128), axis=0, keepdims=True)
                pm = p[0:128]
                p = _rows([lax.select(self.tri, self.zero, pm), p[128:256],
                           lax.select(self.tri, pm, self.zero)])
                v3 = vt_v[pl.ds(self.blk * 2 + qb - 2, 3), h * 16:(h + 1) * 16, :]
            return _dot(_unpack(_lanes(v3)), p.astype(BF)) * _recip(l)

        def store_o(self, gp):
            x = self.tiles
            ready = {2: (2, 5), 4: (4, 0, 1, 3, 6)}.get(len(x), ())
            if ready:
                ls = _lhs7(x[0], x[2 % len(x)], x[1], x[3 % len(x)])
                for k in ready:
                    (oa0_v, oa1_v)[gp // 2][k, gp % 2] = _pack(ls[k].astype(BF).T)
            if len(x) == 4:
                self.tiles = []

        def issue(self, n=1):
            for _ in range(n):
                if self.issued < len(self.items):
                    fn = self.scores_first if self.first else self.scores
                    self.queue.append(fn(*self.items[self.issued]))
                    self.issued += 1

        def finish(self, n=1):
            for _ in range(n):
                if self.done < self.issued:
                    qb, h = self.items[self.done]
                    self.outs.append(self.softmax_pv(self.queue.pop(0), qb, h))
                    if len(self.outs) == 4:
                        self.tiles.append(_rows(self.outs))
                        self.outs = []
                        self.store_o(h // 8)
                    self.done += 1

    def add_residual(r, nrows, c0, c1, y):
        x_v[pl.ds(r, nrows), c0:c1] = (x_v[pl.ds(r, nrows), c0:c1].astype(F32) + y).astype(BF)

    def proj_b(xl, r0, side, fences, lag):
        rows = slice(HALO + r0, HALO + r0 + TA)
        xu = _pack(xl)
        st = Stream(side, fences, lag)
        for P in range(12):
            def prod(k):
                w = wbt[0:4, k, 4 * P:4 * P + 4].reshape(4, 64, 128)
                return st.dot(_dot_nt, xu[:, k * HD:(k + 1) * HD], _unpack(_lanes(w)))

            def put(T):
                def run(top, bot):
                    y = _weave(top, bot)
                    if T < 8:
                        qk_v[T, rows, :] = y * QSCALE
                    elif T < 16:
                        qk_v[T, rows, :] = y
                    else:
                        v_v[T - 16, rows, :] = y
                return run
            T = (P // 4) * 8 + P % 4
            _strassen(prod, put(T), put(T + 4))
        st.flush()

    def taps(ref, t0, t1, r0):
        wins = [ref[t0:t1, HALO + r0 - 2 * w:HALO + r0 - 2 * w + 8, :] for w in range(WB)]
        return _rows(wins).reshape(WB, t1 - t0, 8, 128)

    def logit_b(i, zero, r0):
        ns = CFG['lns']
        acc = []

        def mk(st):
            def run(tok):
                t0, t1 = st * 8 // ns, (st + 1) * 8 // ns
                q = gated(qk_v[t0:t1, HALO + r0:HALO + r0 + 8, :], tok, zero)
                p = q[None] * taps(qk_v, 8 + t0, 8 + t1, r0)
                if acc:
                    p = lax.concatenate([acc.pop()[:, None], p], 1)
                a = jnp.sum(p, axis=1)
                if st + 1 < ns:
                    acc.append(a)
                    return
                a = a + pltpu.roll(a, 64, 2)
                a = a + pltpu.roll(a, 32, 2)
                if r0 < 2 * (WB - 1):
                    pos = _iota(a.shape, 1) - 2 * _iota(a.shape, 0) + (i * TB + r0)
                    a = lax.select(pos >= 0, a, jnp.full(a.shape, NEG, F32))
                e = jnp.exp2(a - jnp.max(a, axis=0, keepdims=True))
                e_v[:, r0:r0 + 8, :] = e * _recip(jnp.sum(e, axis=0, keepdims=True))
            return run
        return [mk(st) for st in range(ns)]

    def pv_b(zero, r0):
        x = []

        def mk(st):
            def run(tok):
                r, t0 = r0 + 8 * (st // 2), 4 * (st % 2)
                e = gated(e_v[:, r:r + 8, :], tok, zero)
                x.append(_lanes(jnp.sum(e[:, None] * taps(v_v, t0, t0 + 4, r), axis=0)))
                if st == 3:
                    ob_v[r0 // 2:r0 // 2 + 8, :] = lax.concatenate(_lhs7(*x), 1).astype(BF)
            return run
        return [mk(st) for st in range(4)]

    def out_b(i, r0, nrows, side, done=None):
        ou = _pack(ob_v[r0 // 2:(r0 + nrows) // 2, :])
        r = pl.multiple_of(i * TB + r0, 128)
        st = Stream(side, {}, 0)
        for c in range(4):
            def prod(k):
                w = _unpack(wobp[c, k].reshape(256, 128))
                return st.dot(_dot, ou[:, k * HD:(k + 1) * HD], w)

            def put(y11, y12, y21, y22):
                y = _weave(lax.concatenate([y11, y12], 1), lax.concatenate([y21, y22], 1))
                add_residual(r, nrows, c * 256, (c + 1) * 256, y)
            _strassen(prod, put)
            if done is not None:
                done(c)

    cp_x(0).start()
    for cp in cp_wa(0):
        cp.start()
    z16 = jnp.zeros((16, 128), U32)
    xl_v[TA:TA + 32, 0:128] = jnp.zeros((32, 128), BF)
    wbt[4, 0, 0] = z16.reshape(2, 8, 128)
    wobp[4, 0, 0] = z16.reshape(2, 8, 128)
    k4_v[0, 0:16, :] = z16
    vt_v[S // 128, 0:16, :] = z16
    qt_v[2, 0:16, :] = z16
    tk_v[0] = z16[0:8]
    e_v[0, TB:TB + 16, :] = jnp.zeros((16, 128), F32)
    cp_x(0).wait()
    for cp in cp_wa(1):
        cp.start()
    for run in ln_chunks(0, 0, TA, step=TA):
        run(None)

    def one_pass(p, carry):
        first = p == 0
        zero = p >> 2

        def out_a(blk, zero, st, after):
            part = {}
            n = [0]
            for ph in range(2):
                ou = oa0_v[pl.ds(zero, 7)] if ph == 0 else oa1_v[...]
                for nh in range(2):
                    def prod(k):
                        w = _unpack(_lanes(woap[(ph * 2 + nh) * 7 + k]))
                        y = st.dot(_dot, _lanes(ou[k]), w)
                        n[0] += 1
                        after(n[0])
                        return y

                    def put(half):
                        def run(top, bot):
                            y = _rows([top, bot])
                            if ph == 0:
                                part[nh, half] = y
                            else:
                                c0 = nh * HD + half * 256
                                add_residual(blk, TA, c0, c0 + 256, y + part[nh, half])
                        return run
                    _strassen(prod, put(0), put(1))

        def put_first(part, t):
            def run(top, bot):
                y = _weave(top, bot)
                if part == 0:
                    store_t(y * QSCALE, qt_v, 0, t)
                elif part == 2:
                    store_t(y, vt_v, 0, t)
                else:
                    k0_v[t] = _pack(y.astype(BF))
            return run

        def f_body(c, c_):
            buf = wa_v.at[pl.ds(3 * c, 3)]
            pltpu.make_async_copy(buf, buf, sems.at[5 + c]).wait()
            xl = xl_v[0:TA // 2, :]
            raw = {}
            for part in FORDER:
                for k in RAW:
                    o = int(k == 4)
                    w = wa_v[3 * c + part, o * HD:(o + 1) * HD, o * 128:(o + 1) * 128]
                    raw[part, k] = _dot(xl[:, k * HD:(k + 1) * HD], w)
            nr = CFG['fnr']

            def mk_w(part, r0):
                def run(tok):
                    wa_v[3 * NC1, 0:16, 0:128] = tok.astype(BF)
                    w1 = wa_v[3 * c + part, r0:r0 + nr, :]
                    w2 = wa_v[3 * c + part, HD + r0:HD + r0 + nr, :]
                    rs = make_rhs([w1[:, :128], w1[:, 128:], w2[:, :128], w2[:, 128:]])
                    for k in range(7):
                        wap[part][c * 7 + k, r0 // 2:(r0 + nr) // 2, :] = rs[k]
                return run
            side = _both(*[_spread([mk_w(part, r0) for r0 in range(0, HD, nr)], 21, *rng)
                           for part, rng in zip(FORDER, CFG['frng'])])
            for y in raw.values():
                release(y, side.pop(0))
            for n, part in enumerate(FORDER):
                def prod(k):
                    if k in RAW:
                        return raw[part, k]
                    y = _dot(xl[:, k * HD:(k + 1) * HD], _unpack(wap[part][c * 7 + k + zero]))
                    release(y, side.pop(0))
                    return y
                _strassen(prod, put_first(part, 2 * c), put_first(part, 2 * c + 1))
                if n == 0:
                    for k in range(NC1 - 2):
                        @pl.when(c == k)
                        def _():
                            for cp in cp_wa(k + 2):
                                cp.start()

            @pl.when(c == NC1 - 3)
            def _():
                cp_woa.start()

            @pl.when(c == NC1 - 2)
            def _():
                for cp in [cp_x(1)] + cp_wb(0):
                    cp.start()
            return c_

        def g_body(c, c_):
            xl = xl_v[0:TA // 2, :]
            for part in FORDER:
                _strassen(lambda k: _dot(xl[:, k * HD:(k + 1) * HD], _unpack(wap[part][c * 7 + k])),
                          put_first(part, 2 * c), put_first(part, 2 * c + 1))
            return c_

        def a_first():
            @pl.when(first)
            def _():
                lax.fori_loop(0, NC1, f_body, 0)

            @pl.when(jnp.logical_not(first))
            def _():
                lax.fori_loop(0, NC1, g_body, 0)
            at = Attn(0)
            at.issue(CFG['flook'])
            while at.issued < 2 * H:
                at.issue()
                at.finish()

            @pl.when(first)
            def _():
                for cp in [cp_woa, cp_x(1)] + cp_wb(0):
                    cp.wait()
                for cp in [cp_x(2)] + cp_wb(1):
                    cp.start()

                def once(gp, c_):
                    r0 = pl.multiple_of(gp * 256, 256)
                    rows = pl.ds(pl.multiple_of((gp & 1) * 64, 64), 64)
                    for nh in range(2):
                        for nt in range(2):
                            c0 = nh * HD + nt * 128
                            rs = make_rhs([woa_v[pl.ds(r0 + dr, 128), c0 + dc:c0 + dc + 128]
                                           for dr in (0, 128) for dc in (0, 256)])
                            for k in range(7):
                                woap[((gp >> 1) * 2 + nh) * 7 + k, nt, rows, :] = rs[k]
                    return c_
                lax.fori_loop(0, 4, once, 0)

            def mk_k4(t):
                def run(tok):
                    k0_v[8, 0:8, :] = pltpu.bitcast(tok[0:8], U32)
                    kp = k0_v[t + zero]
                    kt_v[t] = kp[80:128]
                    build_k4(kp, t, 48)
                return run
            hi = CFG['fhi']
            side = _both(_spread(prep_out(zero), 28, 0, hi),
                         _spread(ln_chunks(TA + zero * TA, 0, TA), 28, 0, hi))
            side = _both(side, _spread([mk_k4(t) for t in range(8)], 28, 0, hi))
            st = Stream(side, {27: lambda: fence_side(zero) | fence_k(zero)}, 1)
            out_a(0, zero, st, lambda u: at.finish(2 * H if u == 1 else 0))

        if CFG['first']:
            a_first()

        @pl.when(first)
        def _():
            cp_x(2).wait()
            for cp in cp_wb(1):
                cp.wait()
            cp_x(3).start()
            for cp in cp_wb(2):
                cp.start()

        def a_body(i, c_):
            @pl.when(jnp.logical_and(first, i == 2))
            def _():
                cp_x(3).wait()
                for cp in cp_wb(2):
                    cp.wait()
            xu = _pack(xl_v[0:TA // 2, :])
            pw = [_spread(prep_qkv(jnp.minimum(4 * (i - 1) + n, 23)), 112, *CFG['urng'][n])
                  for n in range(4)]
            po = prep_out(i)
            side = _both(_spread(ln_chunks((((i + 1) & (NA - 1)) + zero) * TA, 0, TA),
                                 112, *CFG['lrng']),
                         _spread(po, 112, *CFG['orng']), *pw)
            fences = {u: (lambda: fence_side(zero)) for u in CFG['fpos']}
            for n in range(1, 12):
                fe = (fence_k, fence_v, fence_q)[CFG['kord'][(n - 1) % 3]]
                u = 7 * n + 6
                fences[u] = ((lambda fe=fe: fe(zero) | fence_side(zero)) if u in fences
                             else (lambda fe=fe: fe(zero)))
            st = Stream(side, fences, CFG['lag'])
            at = Attn(i)
            for n in range(12):
                gp, kind = n // 3, CFG['kord'][n % 3]

                def prod(k):
                    if n == 11 and k == CFG['hk']:
                        at.issue(CFG['look'])
                    w = wap[(1, 2, 0)[kind]][gp * 7 + k]
                    return st.dot(_dot, xu[:, k * HD:(k + 1) * HD], _unpack(w))

                def put(t):
                    def run(top, bot):
                        y = _weave(top, bot)
                        if kind == 0:
                            kp = _pack(y.astype(BF))
                            full = _rows([kt_v[t], kp])
                            kt_v[t] = kp[80:128]
                            build_k4(full, t, pl.multiple_of(i * (TA // 2), TA // 2))
                        elif kind == 1:
                            store_t(y, vt_v, i * (TA // 128), t)
                        else:
                            store_t(y * QSCALE, qt_v, 0, t)
                    return run
                _strassen(prod, put(2 * gp), put(2 * gp + 1))
            while at.issued < 2 * H - CFG['tail']:
                at.issue()
                at.finish()

            def after(u):
                at.finish()
                at.issue()
            at.issue()
            out_a(pl.multiple_of(i * TA, TA), zero, st, after)
            assert at.done == 2 * H
            return c_
        if CFG['a']:
            lax.fori_loop(1, NA, a_body, 0)

        qk_v[8:16, 0:HALO, :] = jnp.zeros((8, HALO, 128), F32)
        v_v[:, 0:HALO, :] = jnp.zeros((8, HALO, 128), F32)

        def b_body(i, c_):
            def send(k):
                for ii in range(NB if k < 2 else NB - 1):
                    @pl.when(jnp.logical_and(p == 1, i == ii))
                    def _():
                        cp_out(ii, k).start()

            def send_last(c):
                @pl.when(jnp.logical_and(p == 1, i == NB - 1))
                def _():
                    cp_out(NB - 1, 2, c).start()
            ln1 = ln_chunks(i * TB + 256, TA // 2, 256)
            ln2 = ln_chunks((((i + 1) & (NB - 1)) + zero) * TB, 0, TA)
            lg = [logit_b(i, zero, g * 8) for g in range(TB // 8)]
            pv = [pv_b(zero, g * 16) for g in range(TB // 16)]
            n0, n1, n2 = CFG['bn']

            def mix(a, b):
                return _merge(_flat(a), _flat(b))
            f0 = {u: (lambda: fence_x(zero)) for u in CFG['bfx']}
            f0.update({u: (lambda: fence_e(zero)) for u in CFG['bfe'] if u < 84})
            f1 = {u - 84: (lambda: fence_e(zero)) for u in CFG['bfe'] if u >= 84}
            proj_b(xl_v[0:TA // 2, :], 0, _both(_spread(ln1 + ln2, 84, 0, CFG['bln']),
                                                _spread(_flat(lg[0:n0]), 84, 57, 84)),
                   f0, CFG['blag'])
            xl1 = xl_v[pl.ds(pl.multiple_of(TA // 2 + zero * 32, 32), TA // 2), :]
            proj_b(xl1, 256, _both(_spread(mix(lg[n0:32], pv[0:16]), 84, 1, 57),
                                   _spread(_flat(lg[32:n1]), 84, 57, 84)),
                   f1, CFG['blag'])
            out_b(i, 0, 256, _spread(mix(lg[n1:64], pv[16:n2]), 28, 1, 28))
            send(0)
            out_b(i, 256, 128, _spread(_flat(pv[n2:32]), 28, 0, CFG['bhi']))
            send(1)
            qk_v[8:16, 0:HALO, :] = qk_v[8:16, TB:TB + HALO, :]
            v_v[:, 0:HALO, :] = v_v[:, TB:TB + HALO, :]
            out_b(i, 384, 128, [[]] * 28, send_last)
            send(2)
            return c_
        if CFG['b']:
            lax.fori_loop(0, NB, b_body, 0)
        return carry

    lax.fori_loop(0, 2, one_pass, 0)
    for i in range(NB):
        for k in range(len(OUT_PIECES)):
            if (i, k) != (NB - 1, 2):
                cp_out(i, k).wait()
    for c in range(4):
        cp_out(NB - 1, 2, c).wait()


@jax.jit
def pallas_interleave_layers__sliding_block__sliding_local_dilated__prompt_kernel(
    A_x: jax.Array,
    A_wqkv: jax.Array,
    A_wo: jax.Array,
    B_x: jax.Array,
    B_wqkv: jax.Array,
    B_wo: jax.Array,
):
    del B_x
    x = A_x.reshape(S, D)
    any_spec = pl.BlockSpec(memory_space=pl.ANY)
    out = pl.pallas_call(
        _kernel,
        out_shape=jax.ShapeDtypeStruct((S, D), BF),
        in_specs=[any_spec] * 5,
        out_specs=any_spec,
        scratch_shapes=[
            pltpu.VMEM((S + 16, D), BF),
            pltpu.VMEM((3 * NC1 + 1, D, G1 * 128), BF),
            pltpu.VMEM((D, D), BF),
            pltpu.VMEM((6, D + 16, 512), BF),
            pltpu.VMEM((5, D, 256), BF),
            pltpu.VMEM((28, 256, 128), U32),
            pltpu.VMEM((28, 256, 128), U32),
            pltpu.VMEM((28, 256, 128), U32),
            pltpu.VMEM((28, 2, 128, 128), U32),
            pltpu.VMEM((5, 9, 48, 2, 8, 128), U32),
            pltpu.VMEM((5, 9, 16, 2, 8, 128), U32),
            pltpu.VMEM((TA + 32, 7 * HD), BF),
            pltpu.VMEM((9, TA // 2, 128), U32),
            pltpu.VMEM((8, 48, 128), U32),
            pltpu.VMEM((H, S // 2, 128), U32),
            pltpu.VMEM((3, D // 2, 128), U32),
            pltpu.VMEM((S // 128 + 1, D // 2, 128), U32),
            pltpu.VMEM((7, 2, 64, 128), U32),
            pltpu.VMEM((7, 2, 64, 128), U32),
            pltpu.VMEM((16, HALO + TB, 128), F32),
            pltpu.VMEM((8, HALO + TB, 128), F32),
            pltpu.VMEM((WB, TB + 16, 128), F32),
            pltpu.VMEM((TB // 2, 7 * HD), BF),
            pltpu.VMEM((4, 8, 128), U32),
            pltpu.SemaphoreType.DMA((5 + NC1,)),
        ],
        compiler_params=pltpu.CompilerParams(vmem_limit_bytes=112 * 1024 * 1024),
        name="interleave_attn",
    )(x, A_wqkv, A_wo, B_wqkv, B_wo)
    return out.reshape(1, S, D)
```

```python
import math

import jax
import jax.numpy as jnp
from jax import lax
import jax.experimental.pallas as pl
import jax.experimental.pallas.tpu as pltpu

BF = jnp.bfloat16
F32 = jnp.float32
U32 = jnp.uint32

S = 2048
D = 1024
H = 32
DH = 32
TA = 256
NA = S // TA
TB = 512
NB = S // TB
HALO = 16
WB = 8
NEG = -1e30
EPS = 1e-5
HD = D // 2
QSCALE = (DH ** -0.5) * math.log2(math.e)
NC1 = 4
G1 = 8 // NC1
FORDER = (2, 0, 1)
OUT_PIECES = ((0, 256), (256, 128), (384, 128))

CFG = dict(
    first=1, a=1, b=1,
    look=3, tail=2, hk=0, cuts=(5, 10, 14), kord=(0, 1, 2),
    lag=6, lrng=(0, 64), orng=(90, 102), pnd=2,
    urng=((3, 21), (19, 38), (38, 57), (57, 78)),
    fpos=tuple(range(11, 84, 4)) + (111,),
    flook=5, fhi=26, fnr=32, frng=((0, 4), (4, 9), (9, 14)),
    bn=(20, 64, 26), bln=53, bhi=20, lns=2, blag=6,
    bfx=tuple(range(8, 60, 4)), bfe=tuple(range(69, 168, 7)))


def _dot(a, b):
    return lax.dot_general(a, b, (((1,), (0,)), ((), ())), preferred_element_type=F32)


def _dot_nt(a, b):
    return lax.dot_general(a, b, (((1,), (1,)), ((), ())), preferred_element_type=F32)


def _pack(x_bf16):
    return pltpu.bitcast(x_bf16, U32)


def _unpack(x_u32):
    return pltpu.bitcast(x_u32, BF)


def _iota(shape, dim):
    return lax.broadcasted_iota(jnp.int32, shape, dim)


def _rows(xs):
    return lax.concatenate(xs, 0)


def _lanes(x3):
    n, r, _ = x3.shape
    x2 = x3.reshape(n * r, 128)
    return lax.concatenate([x2[t * r:(t + 1) * r] for t in range(n)], 1)


def _layernorm(x_bf16):
    x = x_bf16.astype(F32)
    m = jnp.sum(x, axis=1, keepdims=True) * (1.0 / D)
    xc = x - m
    v = jnp.sum(xc * xc, axis=1, keepdims=True) * (1.0 / D)
    return xc * lax.rsqrt(v + EPS)


def _lhs7(x11, x12, x21, x22):
    return [x11 + x22, x21 + x22, x11, x22, x11 + x12, x21 - x11, x12 - x22]


def _rhs7(w11, w12, w21, w22):
    return [w11 + w22, w11, w12 - w22, w21 - w11, w22, w11 + w12, w21 + w22]


RAW = (1, 4)
QUAD = (1, 7, 8, 4)


def _strassen(prod, left, right=None):
    m1 = prod(1)
    m3 = prod(3)
    y21 = m1 + m3
    m0 = prod(0)
    y11, y22 = m3 + m0, m0 - m1
    y11 = y11 + prod(6)
    m4 = prod(4)
    y11 = y11 - m4
    if right is not None:
        left(y11, y21)
    m2 = prod(2)
    y12 = m2 + m4
    y22 = (y22 + m2) + prod(5)
    if right is not None:
        right(y12, y22)
    else:
        left(y11, y12, y21, y22)


def _weave(top, bot):
    n, c = top.shape
    both = lax.concatenate([top.reshape(n // 8, 1, 8, c), bot.reshape(n // 8, 1, 8, c)], 1)
    return both.reshape(2 * n, c)


def _recip(l):
    r = pl.reciprocal(l, approx=True)
    return r * (2.0 - l * r)


def _swap16(xu):
    for bit in range(4):
        x5 = xu.reshape(8 >> bit, 2, 2 << bit, 8, 128)
        x, y = x5[:, 0:1], x5[:, 1:2]
        if bit == 0:
            x, y = ((x & U32(0xFFFF)) | (y << 16), (x >> 16) | (y & U32(0xFFFF0000)))
        else:
            dist = 1 << (bit - 1)
            lo = (_iota(x.shape, 3) & dist) == 0
            x, y = (lax.select(lo, x, pltpu.roll(y, dist, 3)),
                    lax.select(lo, pltpu.roll(x, 8 - dist, 3), y))
        xu = lax.concatenate([x, y], 1)
    return xu.reshape(16, 2, 8, 128)


def _spread(chunks, nslots, lo=0, hi=None):
    hi = nslots if hi is None else hi
    out = [[] for _ in range(nslots)]
    for u, c in enumerate(chunks):
        out[lo + u * (hi - lo) // len(chunks)].append(c)
    return out


def _merge(a, b):
    out = []
    for u in range(max(len(a), len(b))):
        out += a[u:u + 1] + b[u:u + 1]
    return out


def _flat(lists):
    return sum(lists, [])


def _both(*lists):
    return [sum(parts, []) for parts in zip(*lists)]


def _kernel(x_hbm, wa_hbm, woa_hbm, wb_hbm, wob_hbm, out_hbm,
            x_v, wa_v, woa_v, wb_v, wob_v, wq_p, wk_p, wv_p, woap, wbt, wobp, xl_v,
            k0_v, kt_v, k4_v, qt_v, vt_v, oa0_v, oa1_v, qk_v, v_v, e_v, ob_v, tk_v,
            sems):
    wap = (wq_p, wk_p, wv_p)
    def cp_x(i):
        n = TA if i < 3 else S - 3 * TA
        return pltpu.make_async_copy(x_hbm.at[pl.ds(i * TA, n), :],
                                     x_v.at[pl.ds(i * TA, n), :], sems.at[i])

    def cp_wa(c):
        w = G1 * 128
        return [pltpu.make_async_copy(wa_hbm.at[:, pl.ds(part * D + c * w, w)],
                                      wa_v.at[3 * c + part], sems.at[5 + c])
                for part in range(3)]

    cp_woa = pltpu.make_async_copy(woa_hbm, woa_v, sems.at[1])

    def cp_wb(st):
        qkv = [[], [(c, r0, 128) for c in range(6) for r0 in (0, 512)],
               [(c, r0, 384) for c in range(6) for r0 in (128, 640)]][st]
        out = [(0, 512 * st, 512)] if st < 2 else [(c, 0, D) for c in range(1, 4)]
        sem = sems.at[st + 1]
        return ([pltpu.make_async_copy(wb_hbm.at[pl.ds(r0, n), pl.ds(c * 512, 512)],
                                       wb_v.at[c, pl.ds(r0, n), :], sem) for c, r0, n in qkv]
                + [pltpu.make_async_copy(wob_hbm.at[pl.ds(r0, n), pl.ds(c * 256, 256)],
                                         wob_v.at[c, pl.ds(r0, n), :], sem) for c, r0, n in out])

    def cp_out(i, k, c=None):
        rows = pl.ds(i * TB + OUT_PIECES[k][0], OUT_PIECES[k][1])
        cols = pl.ds(0, D) if c is None else pl.ds(c * (D // 4), D // 4)
        return pltpu.make_async_copy(x_v.at[rows, cols], out_hbm.at[rows, cols], sems.at[4])

    def release(y, chunks):
        n = len(chunks)
        nt = y.shape[1] // 128
        for u, run in enumerate(chunks):
            pos = (u * y.shape[0] * nt // n) // 16 * 16
            t, rr = pos // y.shape[0], pos % y.shape[0]
            run(y[rr:rr + 16, t * 128:(t + 1) * 128])

    def gated(x, tok, zero):
        tk_v[1] = pltpu.bitcast(tok[0:8], U32)
        return pltpu.bitcast(pltpu.bitcast(x, U32) | tk_v[pl.ds(zero, 1)], F32)

    def fence_x(zero):
        return _pack(xl_v[pl.ds(pl.multiple_of(TA + zero * 32, 32), 32), 0:128])

    def fence_e(zero):
        return pltpu.bitcast(e_v[0, pl.ds(pl.multiple_of(TB + zero * 16, 16), 16), :], U32)

    def fence_side(zero):
        return fence_x(zero) | (wbt[4, 0, 0] | wobp[4, 0, 0]).reshape(16, 128)

    def fence_k(zero):
        return k4_v[zero, 0:16, :]

    def fence_q(zero):
        return qt_v[2 + zero, 0:16, :]

    def fence_v(zero):
        return vt_v[S // 128 + zero, 0:16, :]

    def with_fence(xu, fen):
        r, c = xu.shape
        last = lax.concatenate([xu[r - 16:, :c - 128], xu[r - 16:, c - 128:] | fen], 1)
        return _rows([xu[:r - 16], last])

    def ln_chunks(row0, dst, nrows, step=16):
        def mk(c):
            def run(tok):
                if tok is not None:
                    x_v[S:S + 16, 0:128] = tok.astype(BF)
                r = pl.multiple_of(row0 + c * step, step)
                xn = _layernorm(x_v[pl.ds(r, step), :]).reshape(step // 16, 2, 8, D)
                top, bot = xn[:, 0].reshape(step // 2, D), xn[:, 1].reshape(step // 2, D)
                ls = _lhs7(top[:, :HD], top[:, HD:], bot[:, :HD], bot[:, HD:])
                o = dst + c * (step // 2)
                xl_v[o:o + step // 2, :] = lax.concatenate(ls, 1).astype(BF)
            return run
        return [mk(c) for c in range(nrows // step)]

    def sum_chunks(dst, blk, d0, hh):
        nd = CFG['pnd']

        def mk(d):
            def run(tok):
                dst[4, 1, 0, 0] = pltpu.bitcast(tok[0:8], U32)
                ds = pl.ds(d0 + d, nd)
                wide = [_unpack(dst[blk, q, ds, hh].reshape(nd * 8, 128)).astype(F32)
                        for q in QUAD]
                for k, r in enumerate(_rhs7(*wide)):
                    if k not in RAW:
                        dst[blk, k, ds, hh] = _pack(r.astype(BF)).reshape(nd, 8, 128)
            return run
        return [mk(d) for d in range(0, 16, nd)]

    def prep_qkv(u):
        blk = lax.div(u, 6)
        c = u - 6 * blk
        d0, hh = (c >> 1) * 16, c & 1

        def mk(half):
            def run(tok):
                wb_v[0, D:D + 16, 0:128] = tok.astype(BF)
                rows = pl.ds(pl.multiple_of(blk * 128 + half * HD, 128), 128)
                v = _swap16(_pack(wb_v[c, rows, :].T))
                for dh in range(2):
                    wbt[blk, QUAD[2 * half + dh], pl.ds(d0, 16), hh] = v[:, dh]
            return run
        return [mk(0), mk(1)] + sum_chunks(wbt, blk, d0, hh)

    def prep_out(j):
        blk, hh = j >> 1, j & 1

        def mk(half):
            def run(tok):
                wob_v[4, 0:16, 0:128] = tok.astype(BF)
                rows = pl.ds(pl.multiple_of(hh * HD, HD), HD)
                v = _swap16(_pack(wob_v[blk, rows, half * 128:(half + 1) * 128]))
                for dh in range(2):
                    wobp[blk, QUAD[2 * dh + half], :, hh] = v[:, dh]
            return run
        return [mk(0), mk(1)] + sum_chunks(wobp, blk, 0, hh)

    class Stream:
        def __init__(self, side, fences, lag):
            self.side, self.fences, self.lag = side, fences, lag
            self.u, self.ys = 0, []

        def dot(self, fn, lhs_u, w):
            if self.u in self.fences:
                lhs_u = with_fence(lhs_u, self.fences[self.u]())
            y = fn(_unpack(lhs_u), w)
            self.ys.append(y)
            if self.u >= self.lag:
                release(self.ys[self.u - self.lag], self.side[self.u - self.lag])
            self.u += 1
            return y

        def flush(self):
            for u in range(max(self.u - self.lag, 0), self.u):
                release(self.ys[u], self.side[u])

    def make_rhs(quads):
        rs = _rhs7(*[w.astype(F32) for w in quads])
        return [_pack(quads[3 * (k == 4)] if k in RAW else r.astype(BF))
                for k, r in enumerate(rs)]

    def build_k4(full, t, row0):
        n = full.shape[0] - 48
        rolled = [full] + [pltpu.roll(full, 32 * r, 1) for r in range(1, 4)]
        grp_id = _iota((n, 128), 1) >> 5
        is_g = [grp_id == g for g in range(4)]
        for a in range(4):
            val = rolled[(0 - a) % 4][0:n]
            for g in range(1, 4):
                val = lax.select(is_g[g], rolled[(g - a) % 4][16 * g:16 * g + n], val)
            k4_v[4 * t + a, pl.ds(row0, n), :] = val

    def store_t(y, dst, slot0, t):
        yt = _pack(y.astype(BF).T)
        rows = pl.ds(t * 64 if isinstance(t, int) else pl.multiple_of(t * 64, 64), 64)
        for b in range(TA // 128):
            dst[slot0 + b, rows, :] = yt[:, b * 128:(b + 1) * 128]

    class Attn:
        def __init__(self, blk):
            self.blk = blk
            self.first = isinstance(blk, int)
            self.items = [(qb, 4 * t + a) for t in range(8) for qb in range(2) for a in range(4)]
            self.issued, self.done, self.queue, self.outs, self.tiles = 0, 0, [], [], []
            row, lane = _iota((128, 128), 0), _iota((128, 128), 1)
            self.tri = lane >= row
            if self.first:
                self.neg = jnp.full((128, 128), NEG, F32)
                self.zq = jnp.zeros((16, 128), U32)
            else:
                self.zero = jnp.zeros((128, 128), F32)
                self.slot = (lane >> 5) == (row >> 5)
                new = (_iota((32, 128), 1) & 31) >= _iota((32, 128), 0)
                self.new = (new[0:16], new[16:32])
                lane2 = _iota((256, 128), 1)
                self.odd, self.hi = (lane2 & 32) != 0, lane2 >= 64
                self.base = [pl.multiple_of((blk * 2 + qb) * 64 - 80, 16) for qb in range(2)]

        def scores_first(self, qb, h):
            qh = qt_v[qb, h * 16:(h + 1) * 16, :]
            wq = _unpack(_rows([qh if jj == h % 4 else self.zq for jj in range(4)]))
            n = (qb + 1) * 32
            kk = _unpack(k0_v[h // 4, 0:2 * n, :])
            s = _rows([_dot(kk[c * n:(c + 1) * n], wq) for c in range(4)])
            diag = lax.select(self.tri, s[qb * 128:], self.neg)
            return diag if qb == 0 else _rows([s[0:128], diag])

        def scores(self, qb, h):
            qf = _unpack(qt_v[qb, h * 16:(h + 1) * 16, :]).astype(F32)
            wq = lax.select(self.slot, _rows([qf] * 4), self.zero).astype(BF)
            w = k4_v[h, pl.ds(self.base[qb], 144), :]
            kk = _unpack(_rows([w[0:8], w[128:136], w[8:16], w[136:144], w[16:128]]))
            cuts = (0,) + CFG['cuts'] + (18,)
            s = _rows([_dot(kk[16 * a:16 * b], wq) for a, b in zip(cuts[:-1], cuts[1:])])
            return _rows([lax.select(self.new[0], s[16:32], s[0:16]),
                          lax.select(self.new[1], s[48:64], s[32:48]), s[64:]])

        def softmax_pv(self, s, qb, h):
            mx = jnp.max(s, axis=0, keepdims=True)
            if self.first:
                p = jnp.exp2(s - mx)
                l = jnp.sum(p, axis=0, keepdims=True)
                v3 = vt_v[0:qb + 1, h * 16:(h + 1) * 16, :]
            else:
                s = lax.select(self.odd, _rows([s[224:], s[:224]]), s)
                s = lax.select(self.hi, _rows([s[192:], s[:192]]), s)
                p = jnp.exp2(s - mx)
                p3 = p.reshape(2, 128, 128)
                acc = p3[:, 120:128]
                for v in range(14, -1, -1):
                    acc = acc + p3[:, 8 * v:8 * v + 8]
                l = jnp.sum(acc.reshape(16, 128), axis=0, keepdims=True)
                pm = p[0:128]
                p = _rows([lax.select(self.tri, self.zero, pm), p[128:256],
                           lax.select(self.tri, pm, self.zero)])
                v3 = vt_v[pl.ds(self.blk * 2 + qb - 2, 3), h * 16:(h + 1) * 16, :]
            return _dot(_unpack(_lanes(v3)), p.astype(BF)) * _recip(l)

        def store_o(self, gp):
            x = self.tiles
            ready = {2: (2, 5), 4: (4, 0, 1, 3, 6)}.get(len(x), ())
            if ready:
                ls = _lhs7(x[0], x[2 % len(x)], x[1], x[3 % len(x)])
                for k in ready:
                    (oa0_v, oa1_v)[gp // 2][k, gp % 2] = _pack(ls[k].astype(BF).T)
            if len(x) == 4:
                self.tiles = []

        def issue(self, n=1):
            for _ in range(n):
                if self.issued < len(self.items):
                    fn = self.scores_first if self.first else self.scores
                    self.queue.append(fn(*self.items[self.issued]))
                    self.issued += 1

        def finish(self, n=1):
            for _ in range(n):
                if self.done < self.issued:
                    qb, h = self.items[self.done]
                    self.outs.append(self.softmax_pv(self.queue.pop(0), qb, h))
                    if len(self.outs) == 4:
                        self.tiles.append(_rows(self.outs))
                        self.outs = []
                        self.store_o(h // 8)
                    self.done += 1

    def add_residual(r, nrows, c0, c1, y):
        x_v[pl.ds(r, nrows), c0:c1] = (x_v[pl.ds(r, nrows), c0:c1].astype(F32) + y).astype(BF)

    def proj_b(xl, r0, side, fences, lag):
        rows = slice(HALO + r0, HALO + r0 + TA)
        xu = _pack(xl)
        st = Stream(side, fences, lag)
        for P in range(12):
            def prod(k):
                w = wbt[0:4, k, 4 * P:4 * P + 4].reshape(4, 64, 128)
                return st.dot(_dot_nt, xu[:, k * HD:(k + 1) * HD], _unpack(_lanes(w)))

            def put(T):
                def run(top, bot):
                    y = _weave(top, bot)
                    if T < 8:
                        qk_v[T, rows, :] = y * QSCALE
                    elif T < 16:
                        qk_v[T, rows, :] = y
                    else:
                        v_v[T - 16, rows, :] = y
                return run
            T = (P // 4) * 8 + P % 4
            _strassen(prod, put(T), put(T + 4))
        st.flush()

    def taps(ref, t0, t1, r0):
        wins = [ref[t0:t1, HALO + r0 - 2 * w:HALO + r0 - 2 * w + 8, :] for w in range(WB)]
        return _rows(wins).reshape(WB, t1 - t0, 8, 128)

    def logit_b(i, zero, r0):
        ns = CFG['lns']
        acc = []

        def mk(st):
            def run(tok):
                t0, t1 = st * 8 // ns, (st + 1) * 8 // ns
                q = gated(qk_v[t0:t1, HALO + r0:HALO + r0 + 8, :], tok, zero)
                p = q[None] * taps(qk_v, 8 + t0, 8 + t1, r0)
                if acc:
                    p = lax.concatenate([acc.pop()[:, None], p], 1)
                a = jnp.sum(p, axis=1)
                if st + 1 < ns:
                    acc.append(a)
                    return
                a = a + pltpu.roll(a, 64, 2)
                a = a + pltpu.roll(a, 32, 2)
                if r0 < 2 * (WB - 1):
                    pos = _iota(a.shape, 1) - 2 * _iota(a.shape, 0) + (i * TB + r0)
                    a = lax.select(pos >= 0, a, jnp.full(a.shape, NEG, F32))
                e = jnp.exp2(a - jnp.max(a, axis=0, keepdims=True))
                e_v[:, r0:r0 + 8, :] = e * _recip(jnp.sum(e, axis=0, keepdims=True))
            return run
        return [mk(st) for st in range(ns)]

    def pv_b(zero, r0):
        x = []

        def mk(st):
            def run(tok):
                r, t0 = r0 + 8 * (st // 2), 4 * (st % 2)
                e = gated(e_v[:, r:r + 8, :], tok, zero)
                x.append(_lanes(jnp.sum(e[:, None] * taps(v_v, t0, t0 + 4, r), axis=0)))
                if st == 3:
                    ob_v[r0 // 2:r0 // 2 + 8, :] = lax.concatenate(_lhs7(*x), 1).astype(BF)
            return run
        return [mk(st) for st in range(4)]

    def out_b(i, r0, nrows, side, done=None):
        ou = _pack(ob_v[r0 // 2:(r0 + nrows) // 2, :])
        r = pl.multiple_of(i * TB + r0, 128)
        st = Stream(side, {}, 0)
        for c in range(4):
            def prod(k):
                w = _unpack(wobp[c, k].reshape(256, 128))
                return st.dot(_dot, ou[:, k * HD:(k + 1) * HD], w)

            def put(y11, y12, y21, y22):
                y = _weave(lax.concatenate([y11, y12], 1), lax.concatenate([y21, y22], 1))
                add_residual(r, nrows, c * 256, (c + 1) * 256, y)
            _strassen(prod, put)
            if done is not None:
                done(c)

    cp_x(0).start()
    for cp in cp_wa(0):
        cp.start()
    z16 = jnp.zeros((16, 128), U32)
    xl_v[TA:TA + 32, 0:128] = jnp.zeros((32, 128), BF)
    wbt[4, 0, 0] = z16.reshape(2, 8, 128)
    wobp[4, 0, 0] = z16.reshape(2, 8, 128)
    k4_v[0, 0:16, :] = z16
    vt_v[S // 128, 0:16, :] = z16
    qt_v[2, 0:16, :] = z16
    tk_v[0] = z16[0:8]
    e_v[0, TB:TB + 16, :] = jnp.zeros((16, 128), F32)
    cp_x(0).wait()
    for cp in cp_wa(1):
        cp.start()
    for run in ln_chunks(0, 0, TA, step=TA):
        run(None)

    def one_pass(p, carry):
        first = p == 0
        zero = p >> 2

        def out_a(blk, zero, st, after):
            part = {}
            n = [0]
            for ph in range(2):
                ou = oa0_v[pl.ds(zero, 7)] if ph == 0 else oa1_v[...]
                for nh in range(2):
                    def prod(k):
                        w = woap[(ph * 2 + nh) * 7 + k]
                        y = st.dot(_dot, _lanes(ou[k]), w)
                        n[0] += 1
                        after(n[0])
                        return y

                    def put(half):
                        def run(top, bot):
                            y = _rows([top, bot])
                            if ph == 0:
                                part[nh, half] = y
                            else:
                                c0 = nh * HD + half * 256
                                add_residual(blk, TA, c0, c0 + 256, y + part[nh, half])
                        return run
                    _strassen(prod, put(0), put(1))
            st.flush()

        def put_first(part, t):
            def run(top, bot):
                y = _weave(top, bot)
                if part == 0:
                    store_t(y * QSCALE, qt_v, 0, t)
                elif part == 2:
                    store_t(y, vt_v, 0, t)
                else:
                    k0_v[t] = _pack(y.astype(BF))
            return run

        def f_body(c, c_):
            buf = wa_v.at[pl.ds(3 * c, 3)]
            pltpu.make_async_copy(buf, buf, sems.at[5 + c]).wait()
            xl = xl_v[0:TA // 2, :]
            raw = {}
            for part in FORDER:
                for k in RAW:
                    o = int(k == 4)
                    w = wa_v[3 * c + part, o * HD:(o + 1) * HD, o * 128:(o + 1) * 128]
                    raw[part, k] = _dot(xl[:, k * HD:(k + 1) * HD], w)
            nr = CFG['fnr']

            def mk_w(part, r0):
                def run(tok):
                    wa_v[3 * NC1, 0:16, 0:128] = tok.astype(BF)
                    w1 = wa_v[3 * c + part, r0:r0 + nr, :]
                    w2 = wa_v[3 * c + part, HD + r0:HD + r0 + nr, :]
                    rs = make_rhs([w1[:, :128], w1[:, 128:], w2[:, :128], w2[:, 128:]])
                    for k in range(7):
                        wap[part][c * 7 + k, r0 // 2:(r0 + nr) // 2, :] = rs[k]
                return run
            side = _both(*[_spread([mk_w(part, r0) for r0 in range(0, HD, nr)], 21, *rng)
                           for part, rng in zip(FORDER, CFG['frng'])])
            for y in raw.values():
                release(y, side.pop(0))
            for n, part in enumerate(FORDER):
                def prod(k):
                    if k in RAW:
                        return raw[part, k]
                    y = _dot(xl[:, k * HD:(k + 1) * HD], _unpack(wap[part][c * 7 + k + zero]))
                    release(y, side.pop(0))
                    return y
                _strassen(prod, put_first(part, 2 * c), put_first(part, 2 * c + 1))
                if n == 0:
                    for k in range(NC1 - 2):
                        @pl.when(c == k)
                        def _():
                            for cp in cp_wa(k + 2):
                                cp.start()

            @pl.when(c == NC1 - 3)
            def _():
                cp_woa.start()

            @pl.when(c == NC1 - 2)
            def _():
                for cp in [cp_x(1)] + cp_wb(0):
                    cp.start()
            return c_

        def g_body(c, c_):
            xl = xl_v[0:TA // 2, :]
            for part in FORDER:
                _strassen(lambda k: _dot(xl[:, k * HD:(k + 1) * HD], _unpack(wap[part][c * 7 + k])),
                          put_first(part, 2 * c), put_first(part, 2 * c + 1))
            return c_

        def a_first():
            @pl.when(first)
            def _():
                lax.fori_loop(0, NC1, f_body, 0)

            @pl.when(jnp.logical_not(first))
            def _():
                lax.fori_loop(0, NC1, g_body, 0)
            at = Attn(0)
            at.issue(CFG['flook'])
            while at.issued < 2 * H:
                at.issue()
                at.finish()

            @pl.when(first)
            def _():
                for cp in [cp_woa, cp_x(1)] + cp_wb(0):
                    cp.wait()
                for cp in [cp_x(2)] + cp_wb(1):
                    cp.start()

                def once(gp, c_):
                    r0 = pl.multiple_of(gp * 256, 256)
                    for nh in range(2):
                        for rr in range(0, 128, 32):
                            rows = pl.ds(pl.multiple_of((gp & 1) * 128 + rr, 32), 32)
                            quads = [woa_v[pl.ds(r0 + dr + rr, 32), nh * HD + dc:nh * HD + dc + 256]
                                     for dr in (0, 128) for dc in (0, 256)]
                            rs = _rhs7(*[w.astype(F32) for w in quads])
                            for k in range(7):
                                val = quads[3 * (k == 4)] if k in RAW else rs[k].astype(BF)
                                woap[((gp >> 1) * 2 + nh) * 7 + k, rows, :] = val
                    return c_
                lax.fori_loop(0, 4, once, 0)

            def mk_k4(t):
                def run(tok):
                    k0_v[8, 0:8, :] = pltpu.bitcast(tok[0:8], U32)
                    kp = k0_v[t + zero]
                    kt_v[t] = kp[80:128]
                    build_k4(kp, t, 48)
                return run
            hi = CFG['fhi']
            side = _both(_spread(prep_out(zero), 28, 0, hi),
                         _spread(ln_chunks(TA + zero * TA, 0, TA), 28, 0, hi))
            side = _both(side, _spread([mk_k4(t) for t in range(8)], 28, 0, hi))
            st = Stream(side, {27: lambda: fence_side(zero) | fence_k(zero)}, 1)
            out_a(0, zero, st, lambda u: at.finish(2 * H if u == 1 else 0))

        if CFG['first']:
            a_first()

        @pl.when(first)
        def _():
            cp_x(2).wait()
            for cp in cp_wb(1):
                cp.wait()
            cp_x(3).start()
            for cp in cp_wb(2):
                cp.start()

        def a_body(i, c_):
            @pl.when(jnp.logical_and(first, i == 2))
            def _():
                cp_x(3).wait()
                for cp in cp_wb(2):
                    cp.wait()
            xu = _pack(xl_v[0:TA // 2, :])
            pw = [_spread(prep_qkv(jnp.minimum(4 * (i - 1) + n, 23)), 112, *CFG['urng'][n])
                  for n in range(4)]
            po = prep_out(i)
            side = _both(_spread(ln_chunks((((i + 1) & (NA - 1)) + zero) * TA, 0, TA),
                                 112, *CFG['lrng']),
                         _spread(po, 112, *CFG['orng']), *pw)
            fences = {u: (lambda: fence_side(zero)) for u in CFG['fpos']}
            for n in range(1, 12):
                fe = (fence_k, fence_v, fence_q)[CFG['kord'][(n - 1) % 3]]
                u = 7 * n + 6
                fences[u] = ((lambda fe=fe: fe(zero) | fence_side(zero)) if u in fences
                             else (lambda fe=fe: fe(zero)))
            st = Stream(side, fences, CFG['lag'])
            at = Attn(i)
            for n in range(12):
                gp, kind = n // 3, CFG['kord'][n % 3]

                def prod(k):
                    if n == 11 and k == CFG['hk']:
                        at.issue(CFG['look'])
                    w = wap[(1, 2, 0)[kind]][gp * 7 + k]
                    return st.dot(_dot, xu[:, k * HD:(k + 1) * HD], _unpack(w))

                def put(t):
                    def run(top, bot):
                        y = _weave(top, bot)
                        if kind == 0:
                            kp = _pack(y.astype(BF))
                            full = _rows([kt_v[t], kp])
                            kt_v[t] = kp[80:128]
                            build_k4(full, t, pl.multiple_of(i * (TA // 2), TA // 2))
                        elif kind == 1:
                            store_t(y, vt_v, i * (TA // 128), t)
                        else:
                            store_t(y * QSCALE, qt_v, 0, t)
                    return run
                _strassen(prod, put(2 * gp), put(2 * gp + 1))
            while at.issued < 2 * H - CFG['tail']:
                at.issue()
                at.finish()

            def after(u):
                at.finish()
                at.issue()
            at.issue()
            out_a(pl.multiple_of(i * TA, TA), zero, st, after)
            assert at.done == 2 * H
            return c_
        if CFG['a']:
            lax.fori_loop(1, NA, a_body, 0)

        qk_v[8:16, 0:HALO, :] = jnp.zeros((8, HALO, 128), F32)
        v_v[:, 0:HALO, :] = jnp.zeros((8, HALO, 128), F32)

        def b_body(i, c_):
            def send(k):
                for ii in range(NB if k < 2 else NB - 1):
                    @pl.when(jnp.logical_and(p == 1, i == ii))
                    def _():
                        cp_out(ii, k).start()

            def send_last(c):
                @pl.when(jnp.logical_and(p == 1, i == NB - 1))
                def _():
                    cp_out(NB - 1, 2, c).start()
            ln1 = ln_chunks(i * TB + 256, TA // 2, 256)
            ln2 = ln_chunks((((i + 1) & (NB - 1)) + zero) * TB, 0, TA)
            lg = [logit_b(i, zero, g * 8) for g in range(TB // 8)]
            pv = [pv_b(zero, g * 16) for g in range(TB // 16)]
            n0, n1, n2 = CFG['bn']

            def mix(a, b):
                return _merge(_flat(a), _flat(b))
            f0 = {u: (lambda: fence_x(zero)) for u in CFG['bfx']}
            f0.update({u: (lambda: fence_e(zero)) for u in CFG['bfe'] if u < 84})
            f1 = {u - 84: (lambda: fence_e(zero)) for u in CFG['bfe'] if u >= 84}
            proj_b(xl_v[0:TA // 2, :], 0, _both(_spread(ln1 + ln2, 84, 0, CFG['bln']),
                                                _spread(_flat(lg[0:n0]), 84, 57, 84)),
                   f0, CFG['blag'])
            xl1 = xl_v[pl.ds(pl.multiple_of(TA // 2 + zero * 32, 32), TA // 2), :]
            proj_b(xl1, 256, _both(_spread(mix(lg[n0:32], pv[0:16]), 84, 1, 57),
                                   _spread(_flat(lg[32:n1]), 84, 57, 84)),
                   f1, CFG['blag'])
            out_b(i, 0, 256, _spread(mix(lg[n1:64], pv[16:n2]), 28, 1, 28))
            send(0)
            out_b(i, 256, 128, _spread(_flat(pv[n2:32]), 28, 0, CFG['bhi']))
            send(1)
            qk_v[8:16, 0:HALO, :] = qk_v[8:16, TB:TB + HALO, :]
            v_v[:, 0:HALO, :] = v_v[:, TB:TB + HALO, :]
            out_b(i, 384, 128, [[]] * 28, send_last)
            send(2)
            return c_
        if CFG['b']:
            lax.fori_loop(0, NB, b_body, 0)
        return carry

    lax.fori_loop(0, 2, one_pass, 0)
    for i in range(NB):
        for k in range(len(OUT_PIECES)):
            if (i, k) != (NB - 1, 2):
                cp_out(i, k).wait()
    for c in range(4):
        cp_out(NB - 1, 2, c).wait()


@jax.jit
def pallas_interleave_layers__sliding_block__sliding_local_dilated__prompt_kernel(
    A_x: jax.Array,
    A_wqkv: jax.Array,
    A_wo: jax.Array,
    B_x: jax.Array,
    B_wqkv: jax.Array,
    B_wo: jax.Array,
):
    del B_x
    x = A_x.reshape(S, D)
    any_spec = pl.BlockSpec(memory_space=pl.ANY)
    out = pl.pallas_call(
        _kernel,
        out_shape=jax.ShapeDtypeStruct((S, D), BF),
        in_specs=[any_spec] * 5,
        out_specs=any_spec,
        scratch_shapes=[
            pltpu.VMEM((S + 16, D), BF),
            pltpu.VMEM((3 * NC1 + 1, D, G1 * 128), BF),
            pltpu.VMEM((D, D), BF),
            pltpu.VMEM((6, D + 16, 512), BF),
            pltpu.VMEM((5, D, 256), BF),
            pltpu.VMEM((28, 256, 128), U32),
            pltpu.VMEM((28, 256, 128), U32),
            pltpu.VMEM((28, 256, 128), U32),
            pltpu.VMEM((28, 256, 256), BF),
            pltpu.VMEM((5, 9, 48, 2, 8, 128), U32),
            pltpu.VMEM((5, 9, 16, 2, 8, 128), U32),
            pltpu.VMEM((TA + 32, 7 * HD), BF),
            pltpu.VMEM((9, TA // 2, 128), U32),
            pltpu.VMEM((8, 48, 128), U32),
            pltpu.VMEM((H, S // 2, 128), U32),
            pltpu.VMEM((3, D // 2, 128), U32),
            pltpu.VMEM((S // 128 + 1, D // 2, 128), U32),
            pltpu.VMEM((7, 2, 64, 128), U32),
            pltpu.VMEM((7, 2, 64, 128), U32),
            pltpu.VMEM((16, HALO + TB, 128), F32),
            pltpu.VMEM((8, HALO + TB, 128), F32),
            pltpu.VMEM((WB, TB + 16, 128), F32),
            pltpu.VMEM((TB // 2, 7 * HD), BF),
            pltpu.VMEM((4, 8, 128), U32),
            pltpu.SemaphoreType.DMA((5 + NC1,)),
        ],
        compiler_params=pltpu.CompilerParams(vmem_limit_bytes=112 * 1024 * 1024),
        name="interleave_attn",
    )(x, A_wqkv, A_wo, B_wqkv, B_wo)
    return out.reshape(1, S, D)
```

```python
import math

import jax
import jax.numpy as jnp
from jax import lax
import jax.experimental.pallas as pl
import jax.experimental.pallas.tpu as pltpu

BF = jnp.bfloat16
F32 = jnp.float32
U32 = jnp.uint32

S = 2048
D = 1024
H = 32
DH = 32
TA = 256
NA = S // TA
TB = 512
NB = S // TB
HALO = 16
WB = 8
NEG = -1e30
EPS = 1e-5
HD = D // 2
QSCALE = (DH ** -0.5) * math.log2(math.e)
NC1 = 4
G1 = 8 // NC1
FORDER = (2, 0, 1)
OUT_PIECES = ((0, 256), (256, 128), (384, 128))

CFG = dict(
    first=1, a=1, b=1,
    look=3, tail=2, hk=0, cuts=(5, 10, 14), kord=(0, 1, 2),
    lag=6, lrng=(0, 64), orng=(90, 102), pnd=2,
    urng=((3, 21), (19, 38), (38, 57), (57, 78)),
    fpos=tuple(range(11, 84, 4)) + (111,),
    flook=5, fhi=26, fnr=32, frng=((0, 4), (4, 9), (9, 14)),
    bn=(20, 64, 26), bln=53, bhi=20, lns=2, blag=6,
    bfx=tuple(range(8, 60, 4)), bfe=tuple(range(69, 168, 7)))


def _dot(a, b):
    return lax.dot_general(a, b, (((1,), (0,)), ((), ())), preferred_element_type=F32)


def _dot_nt(a, b):
    return lax.dot_general(a, b, (((1,), (1,)), ((), ())), preferred_element_type=F32)


def _pack(x_bf16):
    return pltpu.bitcast(x_bf16, U32)


def _unpack(x_u32):
    return pltpu.bitcast(x_u32, BF)


def _iota(shape, dim):
    return lax.broadcasted_iota(jnp.int32, shape, dim)


def _rows(xs):
    return lax.concatenate(xs, 0)


def _lanes(x3):
    n, r, _ = x3.shape
    x2 = x3.reshape(n * r, 128)
    return lax.concatenate([x2[t * r:(t + 1) * r] for t in range(n)], 1)


def _layernorm(x_bf16):
    x = x_bf16.astype(F32)
    m = jnp.sum(x, axis=1, keepdims=True) * (1.0 / D)
    xc = x - m
    v = jnp.sum(xc * xc, axis=1, keepdims=True) * (1.0 / D)
    return xc * lax.rsqrt(v + EPS)


def _lhs7(x11, x12, x21, x22):
    return [x11 + x22, x21 + x22, x11, x22, x11 + x12, x21 - x11, x12 - x22]


def _rhs7(w11, w12, w21, w22):
    return [w11 + w22, w11, w12 - w22, w21 - w11, w22, w11 + w12, w21 + w22]


RAW = (1, 4)
QUAD = (1, 7, 8, 4)


def _strassen(prod, left, right=None):
    m1 = prod(1)
    m3 = prod(3)
    y21 = m1 + m3
    m0 = prod(0)
    y11, y22 = m3 + m0, m0 - m1
    y11 = y11 + prod(6)
    m4 = prod(4)
    y11 = y11 - m4
    if right is not None:
        left(y11, y21)
    m2 = prod(2)
    y12 = m2 + m4
    y22 = (y22 + m2) + prod(5)
    if right is not None:
        right(y12, y22)
    else:
        left(y11, y12, y21, y22)


def _weave(top, bot):
    n, c = top.shape
    both = lax.concatenate([top.reshape(n // 8, 1, 8, c), bot.reshape(n // 8, 1, 8, c)], 1)
    return both.reshape(2 * n, c)


def _recip(l):
    r = pl.reciprocal(l, approx=True)
    return r * (2.0 - l * r)


def _swap16(xu):
    for bit in range(4):
        x5 = xu.reshape(8 >> bit, 2, 2 << bit, 8, 128)
        x, y = x5[:, 0:1], x5[:, 1:2]
        if bit == 0:
            x, y = ((x & U32(0xFFFF)) | (y << 16), (x >> 16) | (y & U32(0xFFFF0000)))
        else:
            dist = 1 << (bit - 1)
            lo = (_iota(x.shape, 3) & dist) == 0
            x, y = (lax.select(lo, x, pltpu.roll(y, dist, 3)),
                    lax.select(lo, pltpu.roll(x, 8 - dist, 3), y))
        xu = lax.concatenate([x, y], 1)
    return xu.reshape(16, 2, 8, 128)


def _spread(chunks, nslots, lo=0, hi=None):
    hi = nslots if hi is None else hi
    out = [[] for _ in range(nslots)]
    for u, c in enumerate(chunks):
        out[lo + u * (hi - lo) // len(chunks)].append(c)
    return out


def _merge(a, b):
    out = []
    for u in range(max(len(a), len(b))):
        out += a[u:u + 1] + b[u:u + 1]
    return out


def _flat(lists):
    return sum(lists, [])


def _both(*lists):
    return [sum(parts, []) for parts in zip(*lists)]


def _kernel(x_hbm, wa_hbm, woa_hbm, wb_hbm, wob_hbm, out_hbm,
            x_v, wa_v, woa_v, wb_v, wob_v, wq_p, wk_p, wv_p, woap, wbt, wobp, xl_v,
            k0_v, kt_v, k4_v, qt_v, vt_v, oa0_v, oa1_v, qk_v, v_v, e_v, ob_v, tk_v,
            sems):
    wap = (wq_p, wk_p, wv_p)
    def cp_x(i):
        n = TA if i < 3 else S - 3 * TA
        return pltpu.make_async_copy(x_hbm.at[pl.ds(i * TA, n), :],
                                     x_v.at[pl.ds(i * TA, n), :], sems.at[i])

    def cp_wa(c):
        w = G1 * 128
        return [pltpu.make_async_copy(wa_hbm.at[:, pl.ds(part * D + c * w, w)],
                                      wa_v.at[3 * c + part], sems.at[5 + c])
                for part in range(3)]

    cp_woa = pltpu.make_async_copy(woa_hbm, woa_v, sems.at[1])

    def cp_wb(st):
        qkv = [[], [(c, r0, 128) for c in range(6) for r0 in (0, 512)],
               [(c, r0, 384) for c in range(6) for r0 in (128, 640)]][st]
        out = [(0, 512 * st, 512)] if st < 2 else [(c, 0, D) for c in range(1, 4)]
        sem = sems.at[st + 1]
        return ([pltpu.make_async_copy(wb_hbm.at[pl.ds(r0, n), pl.ds(c * 512, 512)],
                                       wb_v.at[c, pl.ds(r0, n), :], sem) for c, r0, n in qkv]
                + [pltpu.make_async_copy(wob_hbm.at[pl.ds(r0, n), pl.ds(c * 256, 256)],
                                         wob_v.at[c, pl.ds(r0, n), :], sem) for c, r0, n in out])

    def cp_out(i, k, c=None):
        rows = pl.ds(i * TB + OUT_PIECES[k][0], OUT_PIECES[k][1])
        cols = pl.ds(0, D) if c is None else pl.ds(c * (D // 4), D // 4)
        return pltpu.make_async_copy(x_v.at[rows, cols], out_hbm.at[rows, cols], sems.at[4])

    def release(y, chunks):
        n = len(chunks)
        nt = y.shape[1] // 128
        for u, run in enumerate(chunks):
            pos = (u * y.shape[0] * nt // n) // 16 * 16
            t, rr = pos // y.shape[0], pos % y.shape[0]
            run(y[rr:rr + 16, t * 128:(t + 1) * 128])

    def gated(x, tok, zero):
        tk_v[1] = pltpu.bitcast(tok[0:8], U32)
        return pltpu.bitcast(pltpu.bitcast(x, U32) | tk_v[pl.ds(zero, 1)], F32)

    def fence_x(zero):
        return _pack(xl_v[pl.ds(pl.multiple_of(TA + zero * 32, 32), 32), 0:128])

    def fence_e(zero):
        return pltpu.bitcast(e_v[0, pl.ds(pl.multiple_of(TB + zero * 16, 16), 16), :], U32)

    def fence_side(zero):
        return fence_x(zero) | (wbt[4, 0, 0] | wobp[4, 0, 0, 0:2]).reshape(16, 128)

    def fence_k(zero):
        return k4_v[zero, 0:16, :]

    def fence_q(zero):
        return qt_v[2 + zero, 0:16, :]

    def fence_v(zero):
        return vt_v[S // 128 + zero, 0:16, :]

    def with_fence(xu, fen):
        r, c = xu.shape
        last = lax.concatenate([xu[r - 16:, :c - 128], xu[r - 16:, c - 128:] | fen], 1)
        return _rows([xu[:r - 16], last])

    def ln_chunks(row0, dst, nrows, step=16):
        def mk(c):
            def run(tok):
                if tok is not None:
                    x_v[S:S + 16, 0:128] = tok.astype(BF)
                r = pl.multiple_of(row0 + c * step, step)
                xn = _layernorm(x_v[pl.ds(r, step), :]).reshape(step // 16, 2, 8, D)
                top, bot = xn[:, 0].reshape(step // 2, D), xn[:, 1].reshape(step // 2, D)
                ls = _lhs7(top[:, :HD], top[:, HD:], bot[:, :HD], bot[:, HD:])
                o = dst + c * (step // 2)
                xl_v[o:o + step // 2, :] = lax.concatenate(ls, 1).astype(BF)
            return run
        return [mk(c) for c in range(nrows // step)]

    def sum_chunks(dst, at):
        nd = CFG['pnd']

        def mk(d):
            def run(tok):
                dst[4, 1, 0, 0] = pltpu.bitcast(tok[0:8], U32)
                wide = [_unpack(dst[at(q, d, nd)].reshape(nd * 8, 128)).astype(F32)
                        for q in QUAD]
                for k, r in enumerate(_rhs7(*wide)):
                    if k not in RAW:
                        dst[at(k, d, nd)] = _pack(r.astype(BF)).reshape(nd, 8, 128)
            return run
        return [mk(d) for d in range(0, 16, nd)]

    def prep_qkv(u, hh):
        blk = lax.div(u, 3)
        part = u - 3 * blk

        def at(q, d, n):
            return blk, q, pl.ds(part * 16 + d, n), hh

        def mk(half):
            def run(tok):
                wb_v[0, D:D + 16, 0:128] = tok.astype(BF)
                rows = pl.ds(pl.multiple_of(blk * 128 + half * HD, 128), 128)
                v = _swap16(_pack(wb_v[2 * part + hh, rows, :].T))
                for dh in range(2):
                    wbt[at(QUAD[2 * half + dh], 0, 16)] = v[:, dh]
            return run
        return [mk(0), mk(1)] + sum_chunks(wbt, at)

    def prep_out(j):
        blk, hh = j >> 1, j & 1

        def at(q, d, n):
            return blk, q, hh, pl.ds(d, n)

        def mk(half):
            def run(tok):
                wob_v[4, 0:16, 0:128] = tok.astype(BF)
                rows = pl.ds(pl.multiple_of(hh * HD, HD), HD)
                v = _swap16(_pack(wob_v[blk, rows, half * 128:(half + 1) * 128]))
                for dh in range(2):
                    wobp[at(QUAD[2 * dh + half], 0, 16)] = v[:, dh]
            return run
        return [mk(0), mk(1)] + sum_chunks(wobp, at)

    class Stream:
        def __init__(self, side, fences, lag):
            self.side, self.fences, self.lag = side, fences, lag
            self.u, self.ys = 0, []

        def dot(self, fn, lhs_u, w):
            if self.u in self.fences:
                lhs_u = with_fence(lhs_u, self.fences[self.u]())
            y = fn(_unpack(lhs_u), w)
            self.ys.append(y)
            if self.u >= self.lag:
                release(self.ys[self.u - self.lag], self.side[self.u - self.lag])
            self.u += 1
            return y

        def flush(self):
            for u in range(max(self.u - self.lag, 0), self.u):
                release(self.ys[u], self.side[u])

    def make_rhs(quads):
        rs = _rhs7(*[w.astype(F32) for w in quads])
        return [_pack(quads[3 * (k == 4)] if k in RAW else r.astype(BF))
                for k, r in enumerate(rs)]

    def build_k4(full, t, row0):
        n = full.shape[0] - 48
        rolled = [full] + [pltpu.roll(full, 32 * r, 1) for r in range(1, 4)]
        grp_id = _iota((n, 128), 1) >> 5
        is_g = [grp_id == g for g in range(4)]
        for a in range(4):
            val = rolled[(0 - a) % 4][0:n]
            for g in range(1, 4):
                val = lax.select(is_g[g], rolled[(g - a) % 4][16 * g:16 * g + n], val)
            k4_v[4 * t + a, pl.ds(row0, n), :] = val

    def store_t(y, dst, slot0, t):
        yt = _pack(y.astype(BF).T)
        rows = pl.ds(t * 64 if isinstance(t, int) else pl.multiple_of(t * 64, 64), 64)
        for b in range(TA // 128):
            dst[slot0 + b, rows, :] = yt[:, b * 128:(b + 1) * 128]

    class Attn:
        def __init__(self, blk):
            self.blk = blk
            self.first = isinstance(blk, int)
            self.items = [(qb, 4 * t + a) for t in range(8) for qb in range(2) for a in range(4)]
            self.issued, self.done, self.queue, self.outs, self.tiles = 0, 0, [], [], []
            row, lane = _iota((128, 128), 0), _iota((128, 128), 1)
            self.tri = lane >= row
            if self.first:
                self.neg = jnp.full((128, 128), NEG, F32)
                self.zq = jnp.zeros((16, 128), U32)
            else:
                self.zero = jnp.zeros((128, 128), F32)
                self.slot = (lane >> 5) == (row >> 5)
                new = (_iota((32, 128), 1) & 31) >= _iota((32, 128), 0)
                self.new = (new[0:16], new[16:32])
                lane2 = _iota((256, 128), 1)
                self.odd, self.hi = (lane2 & 32) != 0, lane2 >= 64
                self.base = [pl.multiple_of((blk * 2 + qb) * 64 - 80, 16) for qb in range(2)]

        def scores_first(self, qb, h):
            qh = qt_v[qb, h * 16:(h + 1) * 16, :]
            wq = _unpack(_rows([qh if jj == h % 4 else self.zq for jj in range(4)]))
            n = (qb + 1) * 32
            kk = _unpack(k0_v[h // 4, 0:2 * n, :])
            s = _rows([_dot(kk[c * n:(c + 1) * n], wq) for c in range(4)])
            diag = lax.select(self.tri, s[qb * 128:], self.neg)
            return diag if qb == 0 else _rows([s[0:128], diag])

        def scores(self, qb, h):
            qf = _unpack(qt_v[qb, h * 16:(h + 1) * 16, :]).astype(F32)
            wq = lax.select(self.slot, _rows([qf] * 4), self.zero).astype(BF)
            w = k4_v[h, pl.ds(self.base[qb], 144), :]
            kk = _unpack(_rows([w[0:8], w[128:136], w[8:16], w[136:144], w[16:128]]))
            cuts = (0,) + CFG['cuts'] + (18,)
            s = _rows([_dot(kk[16 * a:16 * b], wq) for a, b in zip(cuts[:-1], cuts[1:])])
            return _rows([lax.select(self.new[0], s[16:32], s[0:16]),
                          lax.select(self.new[1], s[48:64], s[32:48]), s[64:]])

        def softmax_pv(self, s, qb, h):
            mx = jnp.max(s, axis=0, keepdims=True)
            if self.first:
                p = jnp.exp2(s - mx)
                l = jnp.sum(p, axis=0, keepdims=True)
                v3 = vt_v[0:qb + 1, h * 16:(h + 1) * 16, :]
            else:
                s = lax.select(self.odd, _rows([s[224:], s[:224]]), s)
                s = lax.select(self.hi, _rows([s[192:], s[:192]]), s)
                p = jnp.exp2(s - mx)
                p3 = p.reshape(2, 128, 128)
                acc = p3[:, 120:128]
                for v in range(14, -1, -1):
                    acc = acc + p3[:, 8 * v:8 * v + 8]
                l = jnp.sum(acc.reshape(16, 128), axis=0, keepdims=True)
                pm = p[0:128]
                p = _rows([lax.select(self.tri, self.zero, pm), p[128:256],
                           lax.select(self.tri, pm, self.zero)])
                v3 = vt_v[pl.ds(self.blk * 2 + qb - 2, 3), h * 16:(h + 1) * 16, :]
            return _dot(_unpack(_lanes(v3)), p.astype(BF)) * _recip(l)

        def store_o(self, gp):
            x = self.tiles
            ready = {2: (2, 5), 4: (4, 0, 1, 3, 6)}.get(len(x), ())
            if ready:
                ls = _lhs7(x[0], x[2 % len(x)], x[1], x[3 % len(x)])
                for k in ready:
                    (oa0_v, oa1_v)[gp // 2][k, gp % 2] = _pack(ls[k].astype(BF).T)
            if len(x) == 4:
                self.tiles = []

        def issue(self, n=1):
            for _ in range(n):
                if self.issued < len(self.items):
                    fn = self.scores_first if self.first else self.scores
                    self.queue.append(fn(*self.items[self.issued]))
                    self.issued += 1

        def finish(self, n=1):
            for _ in range(n):
                if self.done < self.issued:
                    qb, h = self.items[self.done]
                    self.outs.append(self.softmax_pv(self.queue.pop(0), qb, h))
                    if len(self.outs) == 4:
                        self.tiles.append(_rows(self.outs))
                        self.outs = []
                        self.store_o(h // 8)
                    self.done += 1

    def add_residual(r, nrows, c0, c1, y):
        x_v[pl.ds(r, nrows), c0:c1] = (x_v[pl.ds(r, nrows), c0:c1].astype(F32) + y).astype(BF)

    def proj_b(xl, r0, side, fences, lag):
        rows = slice(HALO + r0, HALO + r0 + TA)
        xu = _pack(xl)
        st = Stream(side, fences, lag)
        for P in range(12):
            def prod(k):
                w = wbt[0:4, k, 4 * P:4 * P + 4].reshape(4, 64, 128)
                return st.dot(_dot_nt, xu[:, k * HD:(k + 1) * HD], _unpack(_lanes(w)))

            def put(T):
                def run(top, bot):
                    y = _weave(top, bot)
                    if T < 8:
                        qk_v[T, rows, :] = y * QSCALE
                    elif T < 16:
                        qk_v[T, rows, :] = y
                    else:
                        v_v[T - 16, rows, :] = y
                return run
            T = (P // 4) * 8 + P % 4
            _strassen(prod, put(T), put(T + 4))
        st.flush()

    def taps(ref, t0, t1, r0):
        wins = [ref[t0:t1, HALO + r0 - 2 * w:HALO + r0 - 2 * w + 8, :] for w in range(WB)]
        return _rows(wins).reshape(WB, t1 - t0, 8, 128)

    def logit_b(i, zero, r0):
        ns = CFG['lns']
        acc = []

        def mk(st):
            def run(tok):
                t0, t1 = st * 8 // ns, (st + 1) * 8 // ns
                q = gated(qk_v[t0:t1, HALO + r0:HALO + r0 + 8, :], tok, zero)
                p = q[None] * taps(qk_v, 8 + t0, 8 + t1, r0)
                if acc:
                    p = lax.concatenate([acc.pop()[:, None], p], 1)
                a = jnp.sum(p, axis=1)
                if st + 1 < ns:
                    acc.append(a)
                    return
                a = a + pltpu.roll(a, 64, 2)
                a = a + pltpu.roll(a, 32, 2)
                if r0 < 2 * (WB - 1):
                    pos = _iota(a.shape, 1) - 2 * _iota(a.shape, 0) + (i * TB + r0)
                    a = lax.select(pos >= 0, a, jnp.full(a.shape, NEG, F32))
                e = jnp.exp2(a - jnp.max(a, axis=0, keepdims=True))
                e_v[:, r0:r0 + 8, :] = e * _recip(jnp.sum(e, axis=0, keepdims=True))
            return run
        return [mk(st) for st in range(ns)]

    def pv_b(zero, r0):
        x = []

        def mk(st):
            def run(tok):
                r, t0 = r0 + 8 * (st // 2), 4 * (st % 2)
                e = gated(e_v[:, r:r + 8, :], tok, zero)
                x.append(_lanes(jnp.sum(e[:, None] * taps(v_v, t0, t0 + 4, r), axis=0)))
                if st == 3:
                    ob_v[r0 // 2:r0 // 2 + 8, :] = lax.concatenate(_lhs7(*x), 1).astype(BF)
            return run
        return [mk(st) for st in range(4)]

    def out_b(i, r0, nrows, side, done=None):
        ou = _pack(ob_v[r0 // 2:(r0 + nrows) // 2, :])
        r = pl.multiple_of(i * TB + r0, 128)
        st = Stream(side, {}, 0)
        for c in range(4):
            def prod(k):
                w2 = wobp[c, k].reshape(256, 128)
                w = _unpack(_weave(w2[0:128], w2[128:256]))
                return st.dot(_dot, ou[:, k * HD:(k + 1) * HD], w)

            def put(y11, y12, y21, y22):
                y = _weave(lax.concatenate([y11, y12], 1), lax.concatenate([y21, y22], 1))
                add_residual(r, nrows, c * 256, (c + 1) * 256, y)
            _strassen(prod, put)
            if done is not None:
                done(c)

    cp_x(0).start()
    for cp in cp_wa(0):
        cp.start()
    z16 = jnp.zeros((16, 128), U32)
    xl_v[TA:TA + 32, 0:128] = jnp.zeros((32, 128), BF)
    wbt[4, 0, 0] = z16.reshape(2, 8, 128)
    wobp[4, 0, 0, 0:2] = z16.reshape(2, 8, 128)
    k4_v[0, 0:16, :] = z16
    vt_v[S // 128, 0:16, :] = z16
    qt_v[2, 0:16, :] = z16
    tk_v[0] = z16[0:8]
    e_v[0, TB:TB + 16, :] = jnp.zeros((16, 128), F32)
    cp_x(0).wait()
    for cp in cp_wa(1):
        cp.start()
    for run in ln_chunks(0, 0, TA, step=TA):
        run(None)

    def one_pass(p, carry):
        first = p == 0
        zero = p >> 2

        def out_a(blk, zero, st, after):
            part = {}
            n = [0]
            for ph in range(2):
                ou = oa0_v[pl.ds(zero, 7)] if ph == 0 else oa1_v[...]
                for nh in range(2):
                    def prod(k):
                        w = woap[(ph * 2 + nh) * 7 + k]
                        y = st.dot(_dot, _lanes(ou[k]), w)
                        n[0] += 1
                        after(n[0])
                        return y

                    def put(half):
                        def run(top, bot):
                            y = _rows([top, bot])
                            if ph == 0:
                                part[nh, half] = y
                            else:
                                c0 = nh * HD + half * 256
                                add_residual(blk, TA, c0, c0 + 256, y + part[nh, half])
                        return run
                    _strassen(prod, put(0), put(1))
            st.flush()

        def put_first(part, t):
            def run(top, bot):
                y = _weave(top, bot)
                if part == 0:
                    store_t(y * QSCALE, qt_v, 0, t)
                elif part == 2:
                    store_t(y, vt_v, 0, t)
                else:
                    k0_v[t] = _pack(y.astype(BF))
            return run

        def f_body(c, c_):
            buf = wa_v.at[pl.ds(3 * c, 3)]
            pltpu.make_async_copy(buf, buf, sems.at[5 + c]).wait()
            xl = xl_v[0:TA // 2, :]
            raw = {}
            for part in FORDER:
                for k in RAW:
                    o = int(k == 4)
                    w = wa_v[3 * c + part, o * HD:(o + 1) * HD, o * 128:(o + 1) * 128]
                    raw[part, k] = _dot(xl[:, k * HD:(k + 1) * HD], w)
            nr = CFG['fnr']

            def mk_w(part, r0):
                def run(tok):
                    wa_v[3 * NC1, 0:16, 0:128] = tok.astype(BF)
                    w1 = wa_v[3 * c + part, r0:r0 + nr, :]
                    w2 = wa_v[3 * c + part, HD + r0:HD + r0 + nr, :]
                    rs = make_rhs([w1[:, :128], w1[:, 128:], w2[:, :128], w2[:, 128:]])
                    for k in range(7):
                        wap[part][c * 7 + k, r0 // 2:(r0 + nr) // 2, :] = rs[k]
                return run
            side = _both(*[_spread([mk_w(part, r0) for r0 in range(0, HD, nr)], 21, *rng)
                           for part, rng in zip(FORDER, CFG['frng'])])
            for y in raw.values():
                release(y, side.pop(0))
            for n, part in enumerate(FORDER):
                def prod(k):
                    if k in RAW:
                        return raw[part, k]
                    y = _dot(xl[:, k * HD:(k + 1) * HD], _unpack(wap[part][c * 7 + k + zero]))
                    release(y, side.pop(0))
                    return y
                _strassen(prod, put_first(part, 2 * c), put_first(part, 2 * c + 1))
                if n == 0:
                    for k in range(NC1 - 2):
                        @pl.when(c == k)
                        def _():
                            for cp in cp_wa(k + 2):
                                cp.start()

            @pl.when(c == NC1 - 3)
            def _():
                cp_woa.start()

            @pl.when(c == NC1 - 2)
            def _():
                for cp in [cp_x(1)] + cp_wb(0):
                    cp.start()
            return c_

        def g_body(c, c_):
            xl = xl_v[0:TA // 2, :]
            for part in FORDER:
                _strassen(lambda k: _dot(xl[:, k * HD:(k + 1) * HD], _unpack(wap[part][c * 7 + k])),
                          put_first(part, 2 * c), put_first(part, 2 * c + 1))
            return c_

        def a_first():
            @pl.when(first)
            def _():
                lax.fori_loop(0, NC1, f_body, 0)

            @pl.when(jnp.logical_not(first))
            def _():
                lax.fori_loop(0, NC1, g_body, 0)
            at = Attn(0)
            at.issue(CFG['flook'])
            while at.issued < 2 * H:
                at.issue()
                at.finish()

            @pl.when(first)
            def _():
                for cp in [cp_woa, cp_x(1)] + cp_wb(0):
                    cp.wait()
                for cp in [cp_x(2)] + cp_wb(1):
                    cp.start()

                def once(gp, c_):
                    r0 = pl.multiple_of(gp * 256, 256)
                    for nh in range(2):
                        for rr in range(0, 128, 32):
                            rows = pl.ds(pl.multiple_of((gp & 1) * 128 + rr, 32), 32)
                            quads = [woa_v[pl.ds(r0 + dr + rr, 32), nh * HD + dc:nh * HD + dc + 256]
                                     for dr in (0, 128) for dc in (0, 256)]
                            rs = _rhs7(*[w.astype(F32) for w in quads])
                            for k in range(7):
                                val = quads[3 * (k == 4)] if k in RAW else rs[k].astype(BF)
                                woap[((gp >> 1) * 2 + nh) * 7 + k, rows, :] = val
                    return c_
                lax.fori_loop(0, 4, once, 0)

            def mk_k4(t):
                def run(tok):
                    k0_v[8, 0:8, :] = pltpu.bitcast(tok[0:8], U32)
                    kp = k0_v[t + zero]
                    kt_v[t] = kp[80:128]
                    build_k4(kp, t, 48)
                return run
            hi = CFG['fhi']
            side = _both(_spread(prep_out(zero), 28, 0, hi),
                         _spread(ln_chunks(TA + zero * TA, 0, TA), 28, 0, hi))
            side = _both(side, _spread([mk_k4(t) for t in range(8)], 28, 0, hi))
            st = Stream(side, {27: lambda: fence_side(zero) | fence_k(zero)}, 1)
            out_a(0, zero, st, lambda u: at.finish(2 * H if u == 1 else 0))

        if CFG['first']:
            a_first()

        @pl.when(first)
        def _():
            cp_x(2).wait()
            for cp in cp_wb(1):
                cp.wait()
            cp_x(3).start()
            for cp in cp_wb(2):
                cp.start()

        def a_body(i, c_):
            @pl.when(jnp.logical_and(first, i == 2))
            def _():
                cp_x(3).wait()
                for cp in cp_wb(2):
                    cp.wait()
            xu = _pack(xl_v[0:TA // 2, :])
            pw = [_spread(prep_qkv(jnp.minimum(2 * (i - 1) + n // 2, 11), n % 2), 112, *CFG['urng'][n])
                  for n in range(4)]
            po = prep_out(i)
            side = _both(_spread(ln_chunks((((i + 1) & (NA - 1)) + zero) * TA, 0, TA),
                                 112, *CFG['lrng']),
                         _spread(po, 112, *CFG['orng']), *pw)
            fences = {u: (lambda: fence_side(zero)) for u in CFG['fpos']}
            for n in range(1, 12):
                fe = (fence_k, fence_v, fence_q)[CFG['kord'][(n - 1) % 3]]
                u = 7 * n + 6
                fences[u] = ((lambda fe=fe: fe(zero) | fence_side(zero)) if u in fences
                             else (lambda fe=fe: fe(zero)))
            st = Stream(side, fences, CFG['lag'])
            at = Attn(i)
            for n in range(12):
                gp, kind = n // 3, CFG['kord'][n % 3]

                def prod(k):
                    if n == 11 and k == CFG['hk']:
                        at.issue(CFG['look'])
                    w = wap[(1, 2, 0)[kind]][gp * 7 + k]
                    return st.dot(_dot, xu[:, k * HD:(k + 1) * HD], _unpack(w))

                def put(t):
                    def run(top, bot):
                        y = _weave(top, bot)
                        if kind == 0:
                            kp = _pack(y.astype(BF))
                            full = _rows([kt_v[t], kp])
                            kt_v[t] = kp[80:128]
                            build_k4(full, t, pl.multiple_of(i * (TA // 2), TA // 2))
                        elif kind == 1:
                            store_t(y, vt_v, i * (TA // 128), t)
                        else:
                            store_t(y * QSCALE, qt_v, 0, t)
                    return run
                _strassen(prod, put(2 * gp), put(2 * gp + 1))
            while at.issued < 2 * H - CFG['tail']:
                at.issue()
                at.finish()

            def after(u):
                at.finish()
                at.issue()
            at.issue()
            out_a(pl.multiple_of(i * TA, TA), zero, st, after)
            assert at.done == 2 * H
            return c_
        if CFG['a']:
            lax.fori_loop(1, NA, a_body, 0)

        qk_v[8:16, 0:HALO, :] = jnp.zeros((8, HALO, 128), F32)
        v_v[:, 0:HALO, :] = jnp.zeros((8, HALO, 128), F32)

        def b_body(i, c_):
            def send(k):
                for ii in range(NB if k < 2 else NB - 1):
                    @pl.when(jnp.logical_and(p == 1, i == ii))
                    def _():
                        cp_out(ii, k).start()

            def send_last(c):
                @pl.when(jnp.logical_and(p == 1, i == NB - 1))
                def _():
                    cp_out(NB - 1, 2, c).start()
            ln1 = ln_chunks(i * TB + 256, TA // 2, 256)
            ln2 = ln_chunks((((i + 1) & (NB - 1)) + zero) * TB, 0, TA)
            lg = [logit_b(i, zero, g * 8) for g in range(TB // 8)]
            pv = [pv_b(zero, g * 16) for g in range(TB // 16)]
            n0, n1, n2 = CFG['bn']

            def mix(a, b):
                return _merge(_flat(a), _flat(b))
            f0 = {u: (lambda: fence_x(zero)) for u in CFG['bfx']}
            f0.update({u: (lambda: fence_e(zero)) for u in CFG['bfe'] if u < 84})
            f1 = {u - 84: (lambda: fence_e(zero)) for u in CFG['bfe'] if u >= 84}
            proj_b(xl_v[0:TA // 2, :], 0, _both(_spread(ln1 + ln2, 84, 0, CFG['bln']),
                                                _spread(_flat(lg[0:n0]), 84, 57, 84)),
                   f0, CFG['blag'])
            xl1 = xl_v[pl.ds(pl.multiple_of(TA // 2 + zero * 32, 32), TA // 2), :]
            proj_b(xl1, 256, _both(_spread(mix(lg[n0:32], pv[0:16]), 84, 1, 57),
                                   _spread(_flat(lg[32:n1]), 84, 57, 84)),
                   f1, CFG['blag'])
            out_b(i, 0, 256, _spread(mix(lg[n1:64], pv[16:n2]), 28, 1, 28))
            send(0)
            out_b(i, 256, 128, _spread(_flat(pv[n2:32]), 28, 0, CFG['bhi']))
            send(1)
            qk_v[8:16, 0:HALO, :] = qk_v[8:16, TB:TB + HALO, :]
            v_v[:, 0:HALO, :] = v_v[:, TB:TB + HALO, :]
            out_b(i, 384, 128, [[]] * 28, send_last)
            send(2)
            return c_
        if CFG['b']:
            lax.fori_loop(0, NB, b_body, 0)
        return carry

    lax.fori_loop(0, 2, one_pass, 0)
    for i in range(NB):
        for k in range(len(OUT_PIECES)):
            if (i, k) != (NB - 1, 2):
                cp_out(i, k).wait()
    for c in range(4):
        cp_out(NB - 1, 2, c).wait()


@jax.jit
def pallas_interleave_layers__sliding_block__sliding_local_dilated__prompt_kernel(
    A_x: jax.Array,
    A_wqkv: jax.Array,
    A_wo: jax.Array,
    B_x: jax.Array,
    B_wqkv: jax.Array,
    B_wo: jax.Array,
):
    del B_x
    x = A_x.reshape(S, D)
    any_spec = pl.BlockSpec(memory_space=pl.ANY)
    out = pl.pallas_call(
        _kernel,
        out_shape=jax.ShapeDtypeStruct((S, D), BF),
        in_specs=[any_spec] * 5,
        out_specs=any_spec,
        scratch_shapes=[
            pltpu.VMEM((S + 16, D), BF),
            pltpu.VMEM((3 * NC1 + 1, D, G1 * 128), BF),
            pltpu.VMEM((D, D), BF),
            pltpu.VMEM((6, D + 16, 512), BF),
            pltpu.VMEM((5, D, 256), BF),
            pltpu.VMEM((28, 256, 128), U32),
            pltpu.VMEM((28, 256, 128), U32),
            pltpu.VMEM((28, 256, 128), U32),
            pltpu.VMEM((28, 256, 256), BF),
            pltpu.VMEM((5, 9, 48, 2, 8, 128), U32),
            pltpu.VMEM((5, 9, 2, 16, 8, 128), U32),
            pltpu.VMEM((TA + 32, 7 * HD), BF),
            pltpu.VMEM((9, TA // 2, 128), U32),
            pltpu.VMEM((8, 48, 128), U32),
            pltpu.VMEM((H, S // 2, 128), U32),
            pltpu.VMEM((3, D // 2, 128), U32),
            pltpu.VMEM((S // 128 + 1, D // 2, 128), U32),
            pltpu.VMEM((7, 2, 64, 128), U32),
            pltpu.VMEM((7, 2, 64, 128), U32),
            pltpu.VMEM((16, HALO + TB, 128), F32),
            pltpu.VMEM((8, HALO + TB, 128), F32),
            pltpu.VMEM((WB, TB + 16, 128), F32),
            pltpu.VMEM((TB // 2, 7 * HD), BF),
            pltpu.VMEM((4, 8, 128), U32),
            pltpu.SemaphoreType.DMA((5 + NC1,)),
        ],
        compiler_params=pltpu.CompilerParams(vmem_limit_bytes=112 * 1024 * 1024),
        name="interleave_attn",
    )(x, A_wqkv, A_wo, B_wqkv, B_wo)
    return out.reshape(1, S, D)
```

```python
import math

import jax
import jax.numpy as jnp
from jax import lax
import jax.experimental.pallas as pl
import jax.experimental.pallas.tpu as pltpu

BF = jnp.bfloat16
F32 = jnp.float32
U32 = jnp.uint32

S = 2048
D = 1024
H = 32
DH = 32
TA = 256
NA = S // TA
TB = 512
NB = S // TB
HALO = 16
WB = 8
NEG = -1e30
EPS = 1e-5
HD = D // 2
QSCALE = (DH ** -0.5) * math.log2(math.e)
NC1 = 4
G1 = 8 // NC1
FORDER = (2, 0, 1)
OUT_PIECES = ((0, 256), (256, 128), (384, 128))

CFG = dict(
    first=1, a=1, b=1,
    look=3, tail=2, hk=6, cuts=(5, 10, 14), kord=(0, 1, 2),
    lag=6, lrng=(3, 58), orng=(88, 97), pnd=2, qnd=2,
    urng=((2, 18), (16, 29), (30, 39), (39, 55)), s3n=19, s3a=(55, 77), s3b=(91, 105), tok1=1,
    fpos=tuple(range(11, 84, 4)) + (111,),
    flook=5, fhi=26, fnr=32, frng=((0, 4), (4, 9), (9, 14)),
    bn=(26, 60, 25), bhi=19, lns=2, blag=12, narrow=1, bmix=1,
    bl1=(13, 67), bsp=(67, 108), bl2=(174, 226), be0=150, bw1=(151, 245),
    bks=((0, 1, 2, 3), (4, 5, 6)),
    bfx=tuple(range(29, 125, 6)) + tuple(range(180, 262, 6)), bfe=tuple(range(116, 294, 4)))


def _dot(a, b):
    return lax.dot_general(a, b, (((1,), (0,)), ((), ())), preferred_element_type=F32)


def _pack(x_bf16):
    return pltpu.bitcast(x_bf16, U32)


def _unpack(x_u32):
    return pltpu.bitcast(x_u32, BF)


def _iota(shape, dim):
    return lax.broadcasted_iota(jnp.int32, shape, dim)


def _rows(xs):
    return lax.concatenate(xs, 0)


def _lanes(x3):
    n, r, _ = x3.shape
    x2 = x3.reshape(n * r, 128)
    return lax.concatenate([x2[t * r:(t + 1) * r] for t in range(n)], 1)


def _layernorm(x_bf16):
    x = x_bf16.astype(F32)
    m = jnp.sum(x, axis=1, keepdims=True) * (1.0 / D)
    xc = x - m
    v = jnp.sum(xc * xc, axis=1, keepdims=True) * (1.0 / D)
    return xc * lax.rsqrt(v + EPS)


def _lhs7(x11, x12, x21, x22):
    return [x11 + x22, x21 + x22, x11, x22, x11 + x12, x21 - x11, x12 - x22]


def _rhs7(w11, w12, w21, w22):
    return [w11 + w22, w11, w12 - w22, w21 - w11, w22, w11 + w12, w21 + w22]


RAW = (1, 4)
USES = ((0, 3), (0,), (1, 3), (2, 0), (3,), (0, 1), (2, 3))
SUMS = (0, 1, 4, 5, 6)
QUAD = (1, 7, 8, 4)


def _strassen(prod, left, right=None):
    m1 = prod(1)
    m3 = prod(3)
    y21 = m1 + m3
    m0 = prod(0)
    y11, y22 = m3 + m0, m0 - m1
    y11 = y11 + prod(6)
    m4 = prod(4)
    y11 = y11 - m4
    if right is not None:
        left(y11, y21)
    m2 = prod(2)
    y12 = m2 + m4
    y22 = (y22 + m2) + prod(5)
    if right is not None:
        right(y12, y22)
    else:
        left(y11, y12, y21, y22)


def _weave(top, bot):
    n, c = top.shape
    both = lax.concatenate([top.reshape(n // 8, 1, 8, c), bot.reshape(n // 8, 1, 8, c)], 1)
    return both.reshape(2 * n, c)


def _recip(l):
    r = pl.reciprocal(l, approx=True)
    return r * (2.0 - l * r)


def _swap16(xu):
    for bit in range(4):
        x5 = xu.reshape(8 >> bit, 2, 2 << bit, 8, 128)
        x, y = x5[:, 0:1], x5[:, 1:2]
        if bit == 0:
            x, y = ((x & U32(0xFFFF)) | (y << 16), (x >> 16) | (y & U32(0xFFFF0000)))
        else:
            dist = 1 << (bit - 1)
            lo = (_iota(x.shape, 3) & dist) == 0
            x, y = (lax.select(lo, x, pltpu.roll(y, dist, 3)),
                    lax.select(lo, pltpu.roll(x, 8 - dist, 3), y))
        xu = lax.concatenate([x, y], 1)
    return xu.reshape(16, 2, 8, 128)


def _spread(chunks, nslots, lo=0, hi=None):
    hi = nslots if hi is None else hi
    out = [[] for _ in range(nslots)]
    for u, c in enumerate(chunks):
        out[lo + u * (hi - lo) // len(chunks)].append(c)
    return out


def _merge(a, b):
    out = []
    for u in range(max(len(a), len(b))):
        out += a[u:u + 1] + b[u:u + 1]
    return out


def _flat(lists):
    return sum(lists, [])


def _both(*lists):
    return [sum(parts, []) for parts in zip(*lists)]


def _kernel(x_hbm, wa_hbm, woa_hbm, wb_hbm, wob_hbm, out_hbm,
            x_v, wa_v, woa_v, wb_v, wob_v, wq_p, wk_p, wv_p, woap, wbt, wbf, wb2, wobp, xl_v, xm_v, x2_v,
            k0_v, kt_v, k4_v, qt_v, vt_v, oa0_v, oa1_v, qk_v, v_v, e_v, ob_v, tk_v,
            sems):
    wap = (wq_p, wk_p, wv_p)
    def cp_x(i):
        n = TA if i < 3 else S - 3 * TA
        return pltpu.make_async_copy(x_hbm.at[pl.ds(i * TA, n), :],
                                     x_v.at[pl.ds(i * TA, n), :], sems.at[i])

    def cp_wa(c):
        w = G1 * 128
        return [pltpu.make_async_copy(wa_hbm.at[:, pl.ds(part * D + c * w, w)],
                                      wa_v.at[3 * c + part], sems.at[5 + c])
                for part in range(3)]

    cp_woa = pltpu.make_async_copy(woa_hbm, woa_v, sems.at[1])

    def cp_wb(st):
        qkv = [[], [(c, r0, 128) for c in range(2) for r0 in range(0, D, 256)],
               [(c, r0, 128) for c in range(2) for r0 in range(128, D, 256)]
               + [(c, 0, D) for c in range(2, 6)]][st]
        out = [(0, 512 * st, 512)] if st < 2 else [(c, 0, D) for c in range(1, 4)]
        sem = sems.at[st + 1]
        return ([pltpu.make_async_copy(wb_hbm.at[pl.ds(r0, n), pl.ds(c * 512, 512)],
                                       wb_v.at[c, pl.ds(r0, n), :], sem) for c, r0, n in qkv]
                + [pltpu.make_async_copy(wob_hbm.at[pl.ds(r0, n), pl.ds(c * 256, 256)],
                                         wob_v.at[c, pl.ds(r0, n), :], sem) for c, r0, n in out])

    def cp_out(i, k, c=None):
        rows = pl.ds(i * TB + OUT_PIECES[k][0], OUT_PIECES[k][1])
        cols = pl.ds(0, D) if c is None else pl.ds(c * (D // 4), D // 4)
        return pltpu.make_async_copy(x_v.at[rows, cols], out_hbm.at[rows, cols], sems.at[4])

    def release(y, chunks):
        n = len(chunks)
        nt = y.shape[1] // 128
        for u, run in enumerate(chunks):
            pos = (u * y.shape[0] * nt // n) // 16 * 16
            t, rr = pos // y.shape[0], pos % y.shape[0]
            run(y[rr:rr + 16, t * 128:(t + 1) * 128])

    def gated(x, tok, zero):
        tk_v[1] = pltpu.bitcast(tok[0:8], U32)
        return pltpu.bitcast(pltpu.bitcast(x, U32) | tk_v[pl.ds(zero, 1)], F32)

    def fence_x(zero, ref=xl_v):
        return _pack(ref[pl.ds(pl.multiple_of(TA // 2 + zero * 32, 32), 32), 0:128])

    def fence_e(zero):
        return pltpu.bitcast(e_v[0, pl.ds(pl.multiple_of(TB + zero * 16, 16), 16), :], U32)

    def fence_side(zero):
        return (fence_x(zero) | wb2[147, 0, 0:16, :] | pltpu.bitcast(wbf[2, 0, 0, 0], U32)
                | (wbt[2, 0, 0] | wobp[4, 0, 0, 0:2]).reshape(16, 128))

    def fence_k(zero):
        return k4_v[zero, 0:16, :]

    def fence_q(zero):
        return qt_v[2 + zero, 0:16, :]

    def fence_v(zero):
        return vt_v[S // 128 + zero, 0:16, :]

    def with_fence(xu, fen):
        r, c = xu.shape
        last = lax.concatenate([xu[r - 16:, :c - 128], xu[r - 16:, c - 128:] | fen], 1)
        return _rows([xu[:r - 16], last])

    def ln_chunks(row0, dst, nrows, step=16):
        def mk(c):
            def run(tok):
                if tok is not None:
                    x_v[S:S + 16, 0:128] = tok.astype(BF)
                r = pl.multiple_of(row0 + c * step, step)
                xn = _layernorm(x_v[pl.ds(r, step), :]).reshape(step // 16, 2, 8, D)
                top, bot = xn[:, 0].reshape(step // 2, D), xn[:, 1].reshape(step // 2, D)
                ls = _lhs7(top[:, :HD], top[:, HD:], bot[:, :HD], bot[:, HD:])
                o = c * (step // 2)
                dst[o:o + step // 2, :] = lax.concatenate(ls, 1).astype(BF)
            return run
        return [mk(c) for c in range(nrows // step)]

    def sum_chunks(dst, at, nd, wide_dst=None):
        def mk(d):
            def run(tok):
                dst[dst.shape[0] - 1, 1, 0, 0] = pltpu.bitcast(tok[0:8], U32)
                wide = [_unpack(dst[at(q, d, nd)].reshape(nd * 8, 128)).astype(F32)
                        for q in QUAD]
                for k, r in enumerate(_rhs7(*wide)):
                    if k in RAW:
                        continue
                    if wide_dst is None:
                        dst[at(k, d, nd)] = _pack(r.astype(BF)).reshape(nd, 8, 128)
                    else:
                        wide_dst[at(k, d, nd)] = r.reshape(nd, 16, 128)
            return run
        return [mk(d) for d in range(0, 16, nd)]

    def prep_qkv(g, zero):
        part, par = g >> 1, g & 1
        units = []
        for b in range(2):
            for hh in range(2):
                def at(q, d, n, b=b, hh=hh):
                    return b + zero, q, pl.ds(d, n), hh

                def mk(half, b=b, hh=hh, at=at):
                    def run(tok):
                        wb_v[0, D:D + 16, 0:128] = tok.astype(BF)
                        rows = pl.ds(pl.multiple_of((par + 2 * b) * 128 + half * HD, 128), 128)
                        v = _swap16(_pack(wb_v[2 * part + hh, rows, :].T))
                        for dh in range(2):
                            wbt[at(QUAD[2 * half + dh], 0, 16)] = v[:, dh]
                    return run
                units.append([mk(0), mk(1)] + sum_chunks(wbt, at, CFG['qnd'], wbf))

        def mk2(k1, k2):
            def run(tok):
                idx = [(u // 2 + zero, k1, pl.ds(8 * (u % 2), 8)) for u in USES[k2]]
                if k1 in RAW:
                    wbt[2, 1, 0, 0] = pltpu.bitcast(tok[0:8], U32)
                    q = [_unpack(wbt[ix].reshape(128, 128)) for ix in idx]
                else:
                    wbf[2, 1, 0, 0] = tok
                    q = [wbf[ix].reshape(256, 128) for ix in idx]
                if len(q) == 2:
                    a, b = q[0].astype(F32), q[1].astype(F32)
                    q = [a - b if k2 in (2, 3) else a + b]
                q = [q[0].astype(BF)]
                wt = _pack(q[0].T)
                rows = pl.ds(pl.multiple_of(par * 64, 64), 64)
                for j in range(2):
                    wb2[part * 49 + k1 * 7 + k2, j, rows, :] = wt[:, j * 128:(j + 1) * 128]
            return run
        return units, [mk2(k1, k2) for k1 in range(7) for k2 in range(7)]

    def prep_out(j):
        blk, hh = j >> 1, j & 1

        def at(q, d, n):
            return blk, q, hh, pl.ds(d, n)

        def mk(half):
            def run(tok):
                wob_v[4, 0:16, 0:128] = tok.astype(BF)
                rows = pl.ds(pl.multiple_of(hh * HD, HD), HD)
                v = _swap16(_pack(wob_v[blk, rows, half * 128:(half + 1) * 128]))
                for dh in range(2):
                    wobp[at(QUAD[2 * dh + half], 0, 16)] = v[:, dh]
            return run
        return [mk(0), mk(1)] + sum_chunks(wobp, at, CFG['pnd'])

    class Stream:
        def __init__(self, side, fences, lag):
            self.side, self.fences, self.lag = side, fences, lag
            self.u, self.ys = 0, []

        def dot(self, lhs, w):
            fen = self.fences[self.u]() if self.u in self.fences else None
            if lhs.dtype == U32:
                lhs = _unpack(lhs if fen is None else with_fence(lhs, fen))
            else:
                if fen is not None:
                    top = w[0:16, 0:128] | fen
                    if w.shape[1] > 128:
                        top = lax.concatenate([top, w[0:16, 128:]], 1)
                    w = _rows([top, w[16:]])
                w = _unpack(w)
            y = _dot(lhs, w)
            self.ys.append(y[:, 0:128] if CFG['tok1'] else y)
            if self.u >= self.lag:
                release(self.ys[self.u - self.lag], self.side[self.u - self.lag])
            self.u += 1
            return y

        def flush(self):
            for u in range(max(self.u - self.lag, 0), self.u):
                release(self.ys[u], self.side[u])

    def make_rhs(quads):
        rs = _rhs7(*[w.astype(F32) for w in quads])
        return [_pack(quads[3 * (k == 4)] if k in RAW else r.astype(BF))
                for k, r in enumerate(rs)]

    def build_k4(full, t, row0):
        n = full.shape[0] - 48
        rolled = [full] + [pltpu.roll(full, 32 * r, 1) for r in range(1, 4)]
        grp_id = _iota((n, 128), 1) >> 5
        is_g = [grp_id == g for g in range(4)]
        for a in range(4):
            val = rolled[(0 - a) % 4][0:n]
            for g in range(1, 4):
                val = lax.select(is_g[g], rolled[(g - a) % 4][16 * g:16 * g + n], val)
            k4_v[4 * t + a, pl.ds(row0, n), :] = val

    def store_t(y, dst, slot0, t):
        yt = _pack(y.astype(BF).T)
        rows = pl.ds(t * 64 if isinstance(t, int) else pl.multiple_of(t * 64, 64), 64)
        for b in range(TA // 128):
            dst[slot0 + b, rows, :] = yt[:, b * 128:(b + 1) * 128]

    class Attn:
        def __init__(self, blk):
            self.blk = blk
            self.first = isinstance(blk, int)
            self.items = [(qb, 4 * t + a) for t in range(8) for qb in range(2) for a in range(4)]
            self.issued, self.done, self.queue, self.outs, self.tiles = 0, 0, [], [], []
            row, lane = _iota((128, 128), 0), _iota((128, 128), 1)
            self.tri = lane >= row
            if self.first:
                self.neg = jnp.full((128, 128), NEG, F32)
                self.zq = jnp.zeros((16, 128), U32)
            else:
                self.zero = jnp.zeros((128, 128), F32)
                self.slot = (lane >> 5) == (row >> 5)
                new = (_iota((32, 128), 1) & 31) >= _iota((32, 128), 0)
                self.new = (new[0:16], new[16:32])
                lane2 = _iota((256, 128), 1)
                self.odd, self.hi = (lane2 & 32) != 0, lane2 >= 64
                self.base = [pl.multiple_of((blk * 2 + qb) * 64 - 80, 16) for qb in range(2)]

        def scores_first(self, qb, h):
            qh = qt_v[qb, h * 16:(h + 1) * 16, :]
            wq = _unpack(_rows([qh if jj == h % 4 else self.zq for jj in range(4)]))
            n = (qb + 1) * 32
            kk = _unpack(k0_v[h // 4, 0:2 * n, :])
            s = _rows([_dot(kk[c * n:(c + 1) * n], wq) for c in range(4)])
            diag = lax.select(self.tri, s[qb * 128:], self.neg)
            return diag if qb == 0 else _rows([s[0:128], diag])

        def scores(self, qb, h):
            qf = _unpack(qt_v[qb, h * 16:(h + 1) * 16, :]).astype(F32)
            wq = lax.select(self.slot, _rows([qf] * 4), self.zero).astype(BF)
            w = k4_v[h, pl.ds(self.base[qb], 144), :]
            kk = _unpack(_rows([w[0:8], w[128:136], w[8:16], w[136:144], w[16:128]]))
            cuts = (0,) + CFG['cuts'] + (18,)
            s = _rows([_dot(kk[16 * a:16 * b], wq) for a, b in zip(cuts[:-1], cuts[1:])])
            return _rows([lax.select(self.new[0], s[16:32], s[0:16]),
                          lax.select(self.new[1], s[48:64], s[32:48]), s[64:]])

        def softmax_pv(self, s, qb, h):
            mx = jnp.max(s, axis=0, keepdims=True)
            if self.first:
                p = jnp.exp2(s - mx)
                l = jnp.sum(p, axis=0, keepdims=True)
                v3 = vt_v[0:qb + 1, h * 16:(h + 1) * 16, :]
            else:
                s = lax.select(self.odd, _rows([s[224:], s[:224]]), s)
                s = lax.select(self.hi, _rows([s[192:], s[:192]]), s)
                p = jnp.exp2(s - mx)
                p3 = p.reshape(2, 128, 128)
                acc = p3[:, 120:128]
                for v in range(14, -1, -1):
                    acc = acc + p3[:, 8 * v:8 * v + 8]
                l = jnp.sum(acc.reshape(16, 128), axis=0, keepdims=True)
                pm = p[0:128]
                p = _rows([lax.select(self.tri, self.zero, pm), p[128:256],
                           lax.select(self.tri, pm, self.zero)])
                v3 = vt_v[pl.ds(self.blk * 2 + qb - 2, 3), h * 16:(h + 1) * 16, :]
            return _dot(_unpack(_lanes(v3)), p.astype(BF)) * _recip(l)

        def store_o(self, gp):
            x = self.tiles
            ready = {2: (2, 5), 4: (4, 0, 1, 3, 6)}.get(len(x), ())
            if ready:
                ls = _lhs7(x[0], x[2 % len(x)], x[1], x[3 % len(x)])
                for k in ready:
                    (oa0_v, oa1_v)[gp // 2][k, gp % 2] = _pack(ls[k].astype(BF).T)
            if len(x) == 4:
                self.tiles = []

        def issue(self, n=1):
            for _ in range(n):
                if self.issued < len(self.items):
                    fn = self.scores_first if self.first else self.scores
                    self.queue.append(fn(*self.items[self.issued]))
                    self.issued += 1

        def finish(self, n=1):
            for _ in range(n):
                if self.done < self.issued:
                    qb, h = self.items[self.done]
                    self.outs.append(self.softmax_pv(self.queue.pop(0), qb, h))
                    if len(self.outs) == 4:
                        self.tiles.append(_rows(self.outs))
                        self.outs = []
                        self.store_o(h // 8)
                    self.done += 1

    def add_residual(r, nrows, c0, c1, y):
        x_v[pl.ds(r, nrows), c0:c1] = (x_v[pl.ds(r, nrows), c0:c1].astype(F32) + y).astype(BF)

    def split7(top, bot):
        q = [top[:, :256], top[:, 256:], bot[:, :256], bot[:, 256:]]
        return q, _lhs7(*[v.astype(F32) for v in q])

    def split_now():
        ls = {}
        for k1 in range(7):
            x = xl_v[0:TA // 2, k1 * HD:(k1 + 1) * HD]
            q, sums = split7(x[0:64], x[64:128])
            for k2 in range(7):
                ls[k1, k2] = q[3 * (k2 == 3)] if k2 in (2, 3) else sums[k2].astype(BF)
        return ls

    def split_chunks(zero):
        def mk(r, ks):
            def run(tok):
                xm_v[TA // 2:TA // 2 + 16, 128:256] = tok.astype(BF)
                cols = slice(ks[0] * HD, (ks[-1] + 1) * HD)
                half = [xm_v[pl.ds(pl.multiple_of(o + zero * 32, 8), 8), cols] for o in (r, r + 64)]
                out = []
                for n in range(len(ks)):
                    sums = split7(*[h[:, n * HD:(n + 1) * HD] for h in half])[1]
                    out += [sums[k2] for k2 in SUMS]
                x2_v[r:r + 8, ks[0] * 1280:(ks[-1] + 1) * 1280] = lax.concatenate(out, 1).astype(BF)
            return run
        return [mk(r, ks) for r in range(0, 64, 8) for ks in CFG['bks']]

    def split_load(zero):
        r = pl.ds(pl.multiple_of(zero * 32, 32), 64)
        ls = {}
        for k1 in range(7):
            ls[k1, 2] = xm_v[0:64, k1 * HD:k1 * HD + 256]
            ls[k1, 3] = xm_v[64:128, k1 * HD + 256:(k1 + 1) * HD]
            for n, k2 in enumerate(SUMS):
                ls[k1, k2] = x2_v[r, (k1 * 5 + n) * 256:(k1 * 5 + n + 1) * 256]
        return ls

    def proj_b(ls, r0, st):
        rows = slice(HALO + r0, HALO + r0 + TA)
        cnt = [0]
        for part in range(3):
            for js in ([(0,), (1,)] if CFG['narrow'] else [(0, 1)]):
                def inner(k1, k2):
                    w = _lanes(wb2[part * 49 + k1 * 7 + k2, js[0]:js[-1] + 1])
                    cnt[0] += 1
                    if CFG['narrow'] and cnt[0] % 2:
                        return _dot(ls[k1, k2], _unpack(w))
                    return st.dot(ls[k1, k2], w)

                def outer(k1):
                    res = []
                    _strassen(lambda k2: inner(k1, k2),
                              lambda a, b, c, d: res.append(
                                  _rows([lax.concatenate([a, b], 1), lax.concatenate([c, d], 1)])))
                    return res[0]

                def put(half):
                    def run(top, bot):
                        y = _weave(top, bot)
                        if part == 0:
                            y = y * QSCALE
                        tiles = [2 * h2 + j for h2 in range(2) for j in js]
                        for n, t in enumerate(tiles):
                            dst, T = (qk_v, part * 8) if part < 2 else (v_v, 0)
                            dst[T + half * 4 + t, rows, :] = y[:, n * 128:(n + 1) * 128]
                    return run
                _strassen(outer, put(0), put(1))

    def taps(ref, t0, t1, r0):
        wins = [ref[t0:t1, HALO + r0 - 2 * w:HALO + r0 - 2 * w + 8, :] for w in range(WB)]
        return _rows(wins).reshape(WB, t1 - t0, 8, 128)

    def logit_b(i, zero, r0):
        ns = CFG['lns']
        acc = []

        def mk(st):
            def run(tok):
                t0, t1 = st * 8 // ns, (st + 1) * 8 // ns
                q = gated(qk_v[t0:t1, HALO + r0:HALO + r0 + 8, :], tok, zero)
                p = q[None] * taps(qk_v, 8 + t0, 8 + t1, r0)
                if acc:
                    p = lax.concatenate([acc.pop()[:, None], p], 1)
                a = jnp.sum(p, axis=1)
                if st + 1 < ns:
                    acc.append(a)
                    return
                a = a + pltpu.roll(a, 64, 2)
                a = a + pltpu.roll(a, 32, 2)
                if r0 < 2 * (WB - 1):
                    pos = _iota(a.shape, 1) - 2 * _iota(a.shape, 0) + (i * TB + r0)
                    a = lax.select(pos >= 0, a, jnp.full(a.shape, NEG, F32))
                e = jnp.exp2(a - jnp.max(a, axis=0, keepdims=True))
                e_v[:, r0:r0 + 8, :] = e * _recip(jnp.sum(e, axis=0, keepdims=True))
            return run
        return [mk(st) for st in range(ns)]

    def pv_b(zero, r0):
        x = []

        def mk(st):
            def run(tok):
                r, t0 = r0 + 8 * (st // 2), 4 * (st % 2)
                e = gated(e_v[:, r:r + 8, :], tok, zero)
                x.append(_lanes(jnp.sum(e[:, None] * taps(v_v, t0, t0 + 4, r), axis=0)))
                if st == 3:
                    ob_v[r0 // 2:r0 // 2 + 8, :] = lax.concatenate(_lhs7(*x), 1).astype(BF)
            return run
        return [mk(st) for st in range(4)]

    def out_b(i, r0, nrows, side, done=None):
        ou = _pack(ob_v[r0 // 2:(r0 + nrows) // 2, :])
        r = pl.multiple_of(i * TB + r0, 128)
        st = Stream(side, {}, 0)
        for c in range(4):
            def prod(k):
                w2 = wobp[c, k].reshape(256, 128)
                w = _unpack(_weave(w2[0:128], w2[128:256]))
                return st.dot(ou[:, k * HD:(k + 1) * HD], w)

            def put(y11, y12, y21, y22):
                y = _weave(lax.concatenate([y11, y12], 1), lax.concatenate([y21, y22], 1))
                add_residual(r, nrows, c * 256, (c + 1) * 256, y)
            _strassen(prod, put)
            if done is not None:
                done(c)

    cp_x(0).start()
    for cp in cp_wa(0):
        cp.start()
    z16 = jnp.zeros((16, 128), U32)
    xl_v[TA // 2:TA // 2 + 32, 0:128] = jnp.zeros((32, 128), BF)
    xm_v[TA // 2:TA // 2 + 32, 0:128] = jnp.zeros((32, 128), BF)
    x2_v[64:96, 0:128] = jnp.zeros((32, 128), BF)
    wbt[2, 0, 0] = z16.reshape(2, 8, 128)
    wb2[147, 0, 0:16, :] = z16
    wbf[2, 0, 0, 0] = jnp.zeros((16, 128), F32)
    wobp[4, 0, 0, 0:2] = z16.reshape(2, 8, 128)
    k4_v[0, 0:16, :] = z16
    vt_v[S // 128, 0:16, :] = z16
    qt_v[2, 0:16, :] = z16
    tk_v[0] = z16[0:8]
    e_v[0, TB:TB + 16, :] = jnp.zeros((16, 128), F32)
    cp_x(0).wait()
    for cp in cp_wa(1):
        cp.start()
    for run in ln_chunks(0, xl_v, TA, step=TA):
        run(None)

    def one_pass(p, carry):
        first = p == 0
        zero = p >> 2

        def out_a(blk, zero, st, after):
            part = {}
            n = [0]
            for ph in range(2):
                ou = oa0_v[pl.ds(zero, 7)] if ph == 0 else oa1_v[...]
                for nh in range(2):
                    def prod(k):
                        w = woap[(ph * 2 + nh) * 7 + k]
                        y = st.dot(_lanes(ou[k]), w)
                        n[0] += 1
                        after(n[0])
                        return y

                    def put(half):
                        def run(top, bot):
                            y = _rows([top, bot])
                            if ph == 0:
                                part[nh, half] = y
                            else:
                                c0 = nh * HD + half * 256
                                add_residual(blk, TA, c0, c0 + 256, y + part[nh, half])
                        return run
                    _strassen(prod, put(0), put(1))
            st.flush()

        def put_first(part, t):
            def run(top, bot):
                y = _weave(top, bot)
                if part == 0:
                    store_t(y * QSCALE, qt_v, 0, t)
                elif part == 2:
                    store_t(y, vt_v, 0, t)
                else:
                    k0_v[t] = _pack(y.astype(BF))
            return run

        def f_body(c, c_):
            buf = wa_v.at[pl.ds(3 * c, 3)]
            pltpu.make_async_copy(buf, buf, sems.at[5 + c]).wait()
            xl = xl_v[0:TA // 2, :]
            raw = {}
            for part in FORDER:
                for k in RAW:
                    o = int(k == 4)
                    w = wa_v[3 * c + part, o * HD:(o + 1) * HD, o * 128:(o + 1) * 128]
                    raw[part, k] = _dot(xl[:, k * HD:(k + 1) * HD], w)
            nr = CFG['fnr']

            def mk_w(part, r0):
                def run(tok):
                    wa_v[3 * NC1, 0:16, 0:128] = tok.astype(BF)
                    w1 = wa_v[3 * c + part, r0:r0 + nr, :]
                    w2 = wa_v[3 * c + part, HD + r0:HD + r0 + nr, :]
                    rs = make_rhs([w1[:, :128], w1[:, 128:], w2[:, :128], w2[:, 128:]])
                    for k in range(7):
                        wap[part][c * 7 + k, r0 // 2:(r0 + nr) // 2, :] = rs[k]
                return run
            side = _both(*[_spread([mk_w(part, r0) for r0 in range(0, HD, nr)], 21, *rng)
                           for part, rng in zip(FORDER, CFG['frng'])])
            for y in raw.values():
                release(y, side.pop(0))
            for n, part in enumerate(FORDER):
                def prod(k):
                    if k in RAW:
                        return raw[part, k]
                    y = _dot(xl[:, k * HD:(k + 1) * HD], _unpack(wap[part][c * 7 + k + zero]))
                    release(y, side.pop(0))
                    return y
                _strassen(prod, put_first(part, 2 * c), put_first(part, 2 * c + 1))
                if n == 0:
                    for k in range(NC1 - 2):
                        @pl.when(c == k)
                        def _():
                            for cp in cp_wa(k + 2):
                                cp.start()

            @pl.when(c == NC1 - 3)
            def _():
                cp_woa.start()

            @pl.when(c == NC1 - 2)
            def _():
                for cp in [cp_x(1)] + cp_wb(0):
                    cp.start()
            return c_

        def g_body(c, c_):
            xl = xl_v[0:TA // 2, :]
            for part in FORDER:
                _strassen(lambda k: _dot(xl[:, k * HD:(k + 1) * HD], _unpack(wap[part][c * 7 + k])),
                          put_first(part, 2 * c), put_first(part, 2 * c + 1))
            return c_

        def a_first():
            @pl.when(first)
            def _():
                lax.fori_loop(0, NC1, f_body, 0)

            @pl.when(jnp.logical_not(first))
            def _():
                lax.fori_loop(0, NC1, g_body, 0)
            at = Attn(0)
            at.issue(CFG['flook'])
            while at.issued < 2 * H:
                at.issue()
                at.finish()

            @pl.when(first)
            def _():
                for cp in [cp_woa, cp_x(1)] + cp_wb(0):
                    cp.wait()
                for cp in [cp_x(2)] + cp_wb(1):
                    cp.start()

                def once(gp, c_):
                    r0 = pl.multiple_of(gp * 256, 256)
                    for nh in range(2):
                        for rr in range(0, 128, 32):
                            rows = pl.ds(pl.multiple_of((gp & 1) * 128 + rr, 32), 32)
                            quads = [woa_v[pl.ds(r0 + dr + rr, 32), nh * HD + dc:nh * HD + dc + 256]
                                     for dr in (0, 128) for dc in (0, 256)]
                            rs = _rhs7(*[w.astype(F32) for w in quads])
                            for k in range(7):
                                val = quads[3 * (k == 4)] if k in RAW else rs[k].astype(BF)
                                woap[((gp >> 1) * 2 + nh) * 7 + k, rows, :] = val
                    return c_
                lax.fori_loop(0, 4, once, 0)

            def mk_k4(t):
                def run(tok):
                    k0_v[8, 0:8, :] = pltpu.bitcast(tok[0:8], U32)
                    kp = k0_v[t + zero]
                    kt_v[t] = kp[80:128]
                    build_k4(kp, t, 48)
                return run
            hi = CFG['fhi']
            side = _both(_spread(prep_out(zero), 28, 0, hi),
                         _spread(ln_chunks(TA + zero * TA, xl_v, TA), 28, 0, hi))
            side = _both(side, _spread([mk_k4(t) for t in range(8)], 28, 0, hi))
            st = Stream(side, {27: lambda: fence_side(zero) | fence_k(zero)}, 1)
            out_a(0, zero, st, lambda u: at.finish(2 * H if u == 1 else 0))

        if CFG['first']:
            a_first()

        @pl.when(first)
        def _():
            cp_x(2).wait()
            for cp in cp_wb(1):
                cp.wait()
            cp_x(3).start()
            for cp in cp_wb(2):
                cp.start()

        def a_body(i, c_):
            @pl.when(jnp.logical_and(first, i == 2))
            def _():
                cp_x(3).wait()
                for cp in cp_wb(2):
                    cp.wait()
            xu = _pack(xl_v[0:TA // 2, :])
            units, lvl2 = prep_qkv(jnp.minimum(i - 1, 5), zero)
            pw = [_spread(un, 112, *rng) for un, rng in zip(units, CFG['urng'])]
            ns = CFG['s3n']
            pw += [_spread(lvl2[:ns], 112, *CFG['s3a']), _spread(lvl2[ns:], 112, *CFG['s3b'])]
            po = prep_out(i)
            side = _both(_spread(ln_chunks((((i + 1) & (NA - 1)) + zero) * TA, xl_v, TA),
                                 112, *CFG['lrng']),
                         _spread(po, 112, *CFG['orng']), *pw)
            fences = {u: (lambda: fence_side(zero)) for u in CFG['fpos']}
            for n in range(1, 12):
                fe = (fence_k, fence_v, fence_q)[CFG['kord'][(n - 1) % 3]]
                u = 7 * n + 6
                fences[u] = ((lambda fe=fe: fe(zero) | fence_side(zero)) if u in fences
                             else (lambda fe=fe: fe(zero)))
            st = Stream(side, fences, CFG['lag'])
            at = Attn(i)
            for n in range(12):
                gp, kind = n // 3, CFG['kord'][n % 3]

                def prod(k):
                    if n == 11 and k == CFG['hk']:
                        at.issue(CFG['look'])
                    w = wap[(1, 2, 0)[kind]][gp * 7 + k]
                    return st.dot(xu[:, k * HD:(k + 1) * HD], _unpack(w))

                def put(t):
                    def run(top, bot):
                        y = _weave(top, bot)
                        if kind == 0:
                            kp = _pack(y.astype(BF))
                            full = _rows([kt_v[t], kp])
                            kt_v[t] = kp[80:128]
                            build_k4(full, t, pl.multiple_of(i * (TA // 2), TA // 2))
                        elif kind == 1:
                            store_t(y, vt_v, i * (TA // 128), t)
                        else:
                            store_t(y * QSCALE, qt_v, 0, t)
                    return run
                _strassen(prod, put(2 * gp), put(2 * gp + 1))
            while at.issued < 2 * H - CFG['tail']:
                at.issue()
                at.finish()

            def after(u):
                at.finish()
                at.issue()
            at.issue()
            out_a(pl.multiple_of(i * TA, TA), zero, st, after)
            assert at.done == 2 * H
            return c_
        if CFG['a']:
            lax.fori_loop(1, NA, a_body, 0)

        qk_v[8:16, 0:HALO, :] = jnp.zeros((8, HALO, 128), F32)
        v_v[:, 0:HALO, :] = jnp.zeros((8, HALO, 128), F32)

        def b_body(i, c_):
            def send(k):
                for ii in range(NB if k < 2 else NB - 1):
                    @pl.when(jnp.logical_and(p == 1, i == ii))
                    def _():
                        cp_out(ii, k).start()

            def send_last(c):
                @pl.when(jnp.logical_and(p == 1, i == NB - 1))
                def _():
                    cp_out(NB - 1, 2, c).start()
            ln1 = ln_chunks(i * TB + 256, xm_v, 256)
            ln2 = ln_chunks((((i + 1) & (NB - 1)) + zero) * TB, xl_v, TA)
            lg = [logit_b(i, zero, g * 8) for g in range(TB // 8)]
            pv = [pv_b(zero, g * 16) for g in range(TB // 16)]
            n0, n1, n2 = CFG['bn']

            def mix(a, b):
                return _merge(_flat(a), _flat(b)) if CFG['bmix'] else _flat(a) + _flat(b)
            def fx():
                z2 = _pack(x2_v[pl.ds(pl.multiple_of(64 + zero * 32, 32), 32), 0:128])
                return fence_x(zero) | fence_x(zero, xm_v) | z2
            fences = {u: fx for u in CFG['bfx']}
            for u in CFG['bfe']:
                fences[u] = (lambda: fx() | fence_e(zero)) if u in fences else (lambda: fence_e(zero))
            side = _both(_spread(ln1, 294, *CFG['bl1']), _spread(ln2, 294, *CFG['bl2']),
                         _spread(split_chunks(zero), 294, *CFG['bsp']),
                         _spread(_flat(lg[0:n0]), 294, 100, CFG['be0']),
                         _spread(mix(lg[n0:32], pv[0:16]), 294, *CFG['bw1']),
                         _spread(_flat(lg[32:n1]), 294, 247, 294))
            st = Stream(side, fences, CFG['blag'])
            proj_b(split_now(), 0, st)
            proj_b(split_load(zero), 256, st)
            st.flush()
            out_b(i, 0, 256, _spread(mix(lg[n1:64], pv[16:n2]), 28, 1, 28))
            send(0)
            out_b(i, 256, 128, _spread(_flat(pv[n2:32]), 28, 0, CFG['bhi']))
            send(1)
            qk_v[8:16, 0:HALO, :] = qk_v[8:16, TB:TB + HALO, :]
            v_v[:, 0:HALO, :] = v_v[:, TB:TB + HALO, :]
            out_b(i, 384, 128, [[]] * 28, send_last)
            send(2)
            return c_
        if CFG['b']:
            lax.fori_loop(0, NB, b_body, 0)
        return carry

    lax.fori_loop(0, 2, one_pass, 0)
    for i in range(NB):
        for k in range(len(OUT_PIECES)):
            if (i, k) != (NB - 1, 2):
                cp_out(i, k).wait()
    for c in range(4):
        cp_out(NB - 1, 2, c).wait()


@jax.jit
def pallas_interleave_layers__sliding_block__sliding_local_dilated__prompt_kernel(
    A_x: jax.Array,
    A_wqkv: jax.Array,
    A_wo: jax.Array,
    B_x: jax.Array,
    B_wqkv: jax.Array,
    B_wo: jax.Array,
):
    del B_x
    x = A_x.reshape(S, D)
    any_spec = pl.BlockSpec(memory_space=pl.ANY)
    out = pl.pallas_call(
        _kernel,
        out_shape=jax.ShapeDtypeStruct((S, D), BF),
        in_specs=[any_spec] * 5,
        out_specs=any_spec,
        scratch_shapes=[
            pltpu.VMEM((S + 16, D), BF),
            pltpu.VMEM((3 * NC1 + 1, D, G1 * 128), BF),
            pltpu.VMEM((D, D), BF),
            pltpu.VMEM((6, D + 16, 512), BF),
            pltpu.VMEM((5, D, 256), BF),
            pltpu.VMEM((28, 256, 128), U32),
            pltpu.VMEM((28, 256, 128), U32),
            pltpu.VMEM((28, 256, 128), U32),
            pltpu.VMEM((28, 256, 256), BF),
            pltpu.VMEM((3, 9, 16, 2, 8, 128), U32),
            pltpu.VMEM((3, 7, 16, 2, 16, 128), F32),
            pltpu.VMEM((148, 2, 128, 128), U32),
            pltpu.VMEM((5, 9, 2, 16, 8, 128), U32),
            pltpu.VMEM((TA // 2 + 32, 7 * HD), BF),
            pltpu.VMEM((TA // 2 + 32, 7 * HD), BF),
            pltpu.VMEM((96, 35 * 256), BF),
            pltpu.VMEM((9, TA // 2, 128), U32),
            pltpu.VMEM((8, 48, 128), U32),
            pltpu.VMEM((H, S // 2, 128), U32),
            pltpu.VMEM((3, D // 2, 128), U32),
            pltpu.VMEM((S // 128 + 1, D // 2, 128), U32),
            pltpu.VMEM((7, 2, 64, 128), U32),
            pltpu.VMEM((7, 2, 64, 128), U32),
            pltpu.VMEM((16, HALO + TB, 128), F32),
            pltpu.VMEM((8, HALO + TB, 128), F32),
            pltpu.VMEM((WB, TB + 16, 128), F32),
            pltpu.VMEM((TB // 2, 7 * HD), BF),
            pltpu.VMEM((4, 8, 128), U32),
            pltpu.SemaphoreType.DMA((5 + NC1,)),
        ],
        compiler_params=pltpu.CompilerParams(vmem_limit_bytes=112 * 1024 * 1024),
        name="interleave_attn",
    )(x, A_wqkv, A_wo, B_wqkv, B_wo)
    return out.reshape(1, S, D)
```

```python
import math

import jax
import jax.numpy as jnp
from jax import lax
import jax.experimental.pallas as pl
import jax.experimental.pallas.tpu as pltpu

BF = jnp.bfloat16
F32 = jnp.float32
U32 = jnp.uint32

S = 2048
D = 1024
H = 32
DH = 32
TA = 256
NA = S // TA
TB = 512
NB = S // TB
HALO = 16
WB = 8
NEG = -1e30
EPS = 1e-5
HD = D // 2
QSCALE = (DH ** -0.5) * math.log2(math.e)
NC1 = 4
G1 = 8 // NC1
FORDER = (2, 0, 1)
OUT_PIECES = ((0, 256), (256, 128), (384, 128))

CFG = dict(
    first=1, a=1, b=1,
    look=3, tail=2, hk=6, cuts=(5, 10, 14), kord=(0, 1, 2),
    lag=6, lrng=(0, 54), orng=(88, 97), pnd=2, qnd=2,
    urng=((2, 18), (18, 27), (30, 39), (39, 55)), s3n=19, s3a=(55, 78), s3b=(90, 105),
    fpos=tuple(range(8, 84, 3)) + (99, 105, 111),
    flook=5, fhi=26, fnr=32, frng=((0, 4), (4, 9), (9, 14)),
    bn=(26, 60, 25), bhi=19, lns=2, blag=12, bmix=1,
    bl1=(5, 66), bsp=(67, 108), bl2=(184, 236), bna=7, bl2a=(60, 98),
    bof=(6, 12), bolag=5, be0=150, bw1=(159, 253),
    bks=((0, 1, 2, 3), (4, 5, 6)),
    bfx=tuple(range(27, 125, 4)) + tuple(range(178, 262, 4)), bfe=tuple(range(116, 294, 4)))


def _dot(a, b):
    return lax.dot_general(a, b, (((1,), (0,)), ((), ())), preferred_element_type=F32)


def _pack(x_bf16):
    return pltpu.bitcast(x_bf16, U32)


def _unpack(x_u32):
    return pltpu.bitcast(x_u32, BF)


def _iota(shape, dim):
    return lax.broadcasted_iota(jnp.int32, shape, dim)


def _rows(xs):
    return lax.concatenate(xs, 0)


def _lanes(x3):
    n, r, _ = x3.shape
    x2 = x3.reshape(n * r, 128)
    return lax.concatenate([x2[t * r:(t + 1) * r] for t in range(n)], 1)


def _layernorm(x_bf16):
    x = x_bf16.astype(F32)
    m = jnp.sum(x, axis=1, keepdims=True) * (1.0 / D)
    xc = x - m
    v = jnp.sum(xc * xc, axis=1, keepdims=True) * (1.0 / D)
    return xc * lax.rsqrt(v + EPS)


def _lhs7(x11, x12, x21, x22):
    return [x11 + x22, x21 + x22, x11, x22, x11 + x12, x21 - x11, x12 - x22]


def _rhs7(w11, w12, w21, w22):
    return [w11 + w22, w11, w12 - w22, w21 - w11, w22, w11 + w12, w21 + w22]


RAW = (1, 4)
USES = ((0, 3), (0,), (1, 3), (2, 0), (3,), (0, 1), (2, 3))
SUMS = (0, 1, 4, 5, 6)
QUAD = (1, 7, 8, 4)


def _strassen(prod, left, right=None):
    m1 = prod(1)
    m3 = prod(3)
    y21 = m1 + m3
    m0 = prod(0)
    y11, y22 = m3 + m0, m0 - m1
    y11 = y11 + prod(6)
    m4 = prod(4)
    y11 = y11 - m4
    if right is not None:
        left(y11, y21)
    m2 = prod(2)
    y12 = m2 + m4
    y22 = (y22 + m2) + prod(5)
    if right is not None:
        right(y12, y22)
    else:
        left(y11, y12, y21, y22)


def _weave(top, bot):
    n, c = top.shape
    both = lax.concatenate([top.reshape(n // 8, 1, 8, c), bot.reshape(n // 8, 1, 8, c)], 1)
    return both.reshape(2 * n, c)


def _recip(l):
    r = pl.reciprocal(l, approx=True)
    return r * (2.0 - l * r)


def _swap16(xu):
    for bit in range(4):
        x5 = xu.reshape(8 >> bit, 2, 2 << bit, 8, 128)
        x, y = x5[:, 0:1], x5[:, 1:2]
        if bit == 0:
            x, y = ((x & U32(0xFFFF)) | (y << 16), (x >> 16) | (y & U32(0xFFFF0000)))
        else:
            dist = 1 << (bit - 1)
            lo = (_iota(x.shape, 3) & dist) == 0
            x, y = (lax.select(lo, x, pltpu.roll(y, dist, 3)),
                    lax.select(lo, pltpu.roll(x, 8 - dist, 3), y))
        xu = lax.concatenate([x, y], 1)
    return xu.reshape(16, 2, 8, 128)


def _spread(chunks, nslots, lo=0, hi=None):
    hi = nslots if hi is None else hi
    out = [[] for _ in range(nslots)]
    for u, c in enumerate(chunks):
        out[lo + u * (hi - lo) // len(chunks)].append(c)
    return out


def _merge(a, b):
    out = []
    for u in range(max(len(a), len(b))):
        out += a[u:u + 1] + b[u:u + 1]
    return out


def _flat(lists):
    return sum(lists, [])


def _both(*lists):
    return [sum(parts, []) for parts in zip(*lists)]


def _kernel(x_hbm, wa_hbm, woa_hbm, wb_hbm, wob_hbm, out_hbm,
            x_v, wa_v, woa_v, wb_v, wob_v, wq_p, wk_p, wv_p, woap, wbt, wbf, wb2, wobp, xl_v, xm_v, x2_v,
            k0_v, kt_v, k4_v, qt_v, vt_v, oa0_v, oa1_v, qk_v, v_v, e_v, ob_v, tk_v,
            sems):
    wap = (wq_p, wk_p, wv_p)
    def cp_x(i):
        n = TA if i < 3 else S - 3 * TA
        return pltpu.make_async_copy(x_hbm.at[pl.ds(i * TA, n), :],
                                     x_v.at[pl.ds(i * TA, n), :], sems.at[i])

    def cp_wa(c):
        w = G1 * 128
        return [pltpu.make_async_copy(wa_hbm.at[:, pl.ds(part * D + c * w, w)],
                                      wa_v.at[3 * c + part], sems.at[5 + c])
                for part in range(3)]

    cp_woa = pltpu.make_async_copy(woa_hbm, woa_v, sems.at[1])

    def cp_wb(st):
        qkv = [[], [(c, r0, 128) for c in range(2) for r0 in range(0, D, 256)],
               [(c, r0, 128) for c in range(2) for r0 in range(128, D, 256)]
               + [(c, 0, D) for c in range(2, 6)]][st]
        out = [(0, 512 * st, 512)] if st < 2 else [(c, 0, D) for c in range(1, 4)]
        sem = sems.at[st + 1]
        return ([pltpu.make_async_copy(wb_hbm.at[pl.ds(r0, n), pl.ds(c * 512, 512)],
                                       wb_v.at[c, pl.ds(r0, n), :], sem) for c, r0, n in qkv]
                + [pltpu.make_async_copy(wob_hbm.at[pl.ds(r0, n), pl.ds(c * 256, 256)],
                                         wob_v.at[c, pl.ds(r0, n), :], sem) for c, r0, n in out])

    def cp_out(i, k, c=None):
        rows = pl.ds(i * TB + OUT_PIECES[k][0], OUT_PIECES[k][1])
        cols = pl.ds(0, D) if c is None else pl.ds(c * (D // 4), D // 4)
        return pltpu.make_async_copy(x_v.at[rows, cols], out_hbm.at[rows, cols], sems.at[4])

    def release(y, chunks):
        n = len(chunks)
        nt = y.shape[1] // 128
        for u, run in enumerate(chunks):
            pos = (u * y.shape[0] * nt // n) // 16 * 16
            t, rr = pos // y.shape[0], pos % y.shape[0]
            run(y[rr:rr + 16, t * 128:(t + 1) * 128])

    def gated(x, tok, zero):
        tk_v[1] = pltpu.bitcast(tok[0:8], U32)
        return pltpu.bitcast(pltpu.bitcast(x, U32) | tk_v[pl.ds(zero, 1)], F32)

    def fence_x(zero, ref=xl_v):
        return _pack(ref[pl.ds(pl.multiple_of(TA // 2 + zero * 32, 32), 32), 0:128])

    def fence_e(zero):
        return pltpu.bitcast(e_v[0, pl.ds(pl.multiple_of(TB + zero * 16, 16), 16), :], U32)

    def fence_side(zero):
        return (fence_x(zero) | wb2[147, 0, 0:16, :] | pltpu.bitcast(wbf[2, 0, 0, 0], U32)
                | (wbt[2, 0, 0] | wobp[4, 0, 0, 0:2]).reshape(16, 128))

    def fence_k(zero):
        return k4_v[zero, 0:16, :]

    def fence_q(zero):
        return qt_v[2 + zero, 0:16, :]

    def fence_v(zero):
        return vt_v[S // 128 + zero, 0:16, :]

    def with_fence(xu, fen):
        r, c = xu.shape
        last = lax.concatenate([xu[r - 16:, :c - 128], xu[r - 16:, c - 128:] | fen], 1)
        return _rows([xu[:r - 16], last])

    def ln_chunks(row0, dst, nrows, step=16):
        def mk(c):
            def run(tok):
                if tok is not None:
                    x_v[S:S + 16, 0:128] = tok.astype(BF)
                r = pl.multiple_of(row0 + c * step, step)
                xn = _layernorm(x_v[pl.ds(r, step), :]).reshape(step // 16, 2, 8, D)
                top, bot = xn[:, 0].reshape(step // 2, D), xn[:, 1].reshape(step // 2, D)
                ls = _lhs7(top[:, :HD], top[:, HD:], bot[:, :HD], bot[:, HD:])
                o = c * (step // 2)
                dst[o:o + step // 2, :] = lax.concatenate(ls, 1).astype(BF)
            return run
        return [mk(c) for c in range(nrows // step)]

    def sum_chunks(dst, at, nd, wide_dst=None):
        def mk(d):
            def run(tok):
                dst[dst.shape[0] - 1, 1, 0, 0] = pltpu.bitcast(tok[0:8], U32)
                wide = [_unpack(dst[at(q, d, nd)].reshape(nd * 8, 128)).astype(F32)
                        for q in QUAD]
                for k, r in enumerate(_rhs7(*wide)):
                    if k in RAW:
                        continue
                    if wide_dst is None:
                        dst[at(k, d, nd)] = _pack(r.astype(BF)).reshape(nd, 8, 128)
                    else:
                        wide_dst[at(k, d, nd)] = r.reshape(nd, 16, 128)
            return run
        return [mk(d) for d in range(0, 16, nd)]

    def prep_qkv(g, zero):
        part, par = g >> 1, g & 1
        units = []
        for b in range(2):
            for hh in range(2):
                def at(q, d, n, b=b, hh=hh):
                    return b + zero, q, pl.ds(d, n), hh

                def mk(half, b=b, hh=hh, at=at):
                    def run(tok):
                        wb_v[0, D:D + 16, 0:128] = tok.astype(BF)
                        rows = pl.ds(pl.multiple_of((par + 2 * b) * 128 + half * HD, 128), 128)
                        v = _swap16(_pack(wb_v[2 * part + hh, rows, :].T))
                        for dh in range(2):
                            wbt[at(QUAD[2 * half + dh], 0, 16)] = v[:, dh]
                    return run
                units.append([mk(0), mk(1)] + sum_chunks(wbt, at, CFG['qnd'], wbf))

        def mk2(k1, k2):
            def run(tok):
                idx = [(u // 2 + zero, k1, pl.ds(8 * (u % 2), 8)) for u in USES[k2]]
                if k1 in RAW:
                    wbt[2, 1, 0, 0] = pltpu.bitcast(tok[0:8], U32)
                    q = [_unpack(wbt[ix].reshape(128, 128)) for ix in idx]
                else:
                    wbf[2, 1, 0, 0] = tok
                    q = [wbf[ix].reshape(256, 128) for ix in idx]
                if len(q) == 2:
                    a, b = q[0].astype(F32), q[1].astype(F32)
                    q = [a - b if k2 in (2, 3) else a + b]
                q = [q[0].astype(BF)]
                wt = _pack(q[0].T)
                rows = pl.ds(pl.multiple_of(par * 64, 64), 64)
                for j in range(2):
                    wb2[part * 49 + k1 * 7 + k2, j, rows, :] = wt[:, j * 128:(j + 1) * 128]
            return run
        return units, [mk2(k1, k2) for k1 in range(7) for k2 in range(7)]

    def prep_out(j):
        blk, hh = j >> 1, j & 1

        def at(q, d, n):
            return blk, q, hh, pl.ds(d, n)

        def mk(half):
            def run(tok):
                wob_v[4, 0:16, 0:128] = tok.astype(BF)
                rows = pl.ds(pl.multiple_of(hh * HD, HD), HD)
                v = _swap16(_pack(wob_v[blk, rows, half * 128:(half + 1) * 128]))
                for dh in range(2):
                    wobp[at(QUAD[2 * dh + half], 0, 16)] = v[:, dh]
            return run
        return [mk(0), mk(1)] + sum_chunks(wobp, at, CFG['pnd'])

    class Stream:
        def __init__(self, side, fences, lag):
            self.side, self.fences, self.lag = side, fences, lag
            self.u, self.ys = 0, []

        def dot(self, lhs, w):
            fen = self.fences[self.u]() if self.u in self.fences else None
            if lhs.dtype == U32:
                lhs = _unpack(lhs if fen is None else with_fence(lhs, fen))
            else:
                if fen is not None:
                    w = _rows([w[0:16] | fen, w[16:]])
                w = _unpack(w)
            y = _dot(lhs, w)
            self.ys.append(y[:, 0:128])
            if self.u >= self.lag:
                release(self.ys[self.u - self.lag], self.side[self.u - self.lag])
            self.u += 1
            return y

        def flush(self):
            for u in range(max(self.u - self.lag, 0), self.u):
                release(self.ys[u], self.side[u])

    def make_rhs(quads):
        rs = _rhs7(*[w.astype(F32) for w in quads])
        return [_pack(quads[3 * (k == 4)] if k in RAW else r.astype(BF))
                for k, r in enumerate(rs)]

    def build_k4(full, t, row0):
        n = full.shape[0] - 48
        rolled = [full] + [pltpu.roll(full, 32 * r, 1) for r in range(1, 4)]
        grp_id = _iota((n, 128), 1) >> 5
        is_g = [grp_id == g for g in range(4)]
        for a in range(4):
            val = rolled[(0 - a) % 4][0:n]
            for g in range(1, 4):
                val = lax.select(is_g[g], rolled[(g - a) % 4][16 * g:16 * g + n], val)
            k4_v[4 * t + a, pl.ds(row0, n), :] = val

    def store_t(y, dst, slot0, t):
        yt = _pack(y.astype(BF).T)
        rows = pl.ds(t * 64 if isinstance(t, int) else pl.multiple_of(t * 64, 64), 64)
        for b in range(TA // 128):
            dst[slot0 + b, rows, :] = yt[:, b * 128:(b + 1) * 128]

    class Attn:
        def __init__(self, blk):
            self.blk = blk
            self.first = isinstance(blk, int)
            self.items = [(qb, 4 * t + a) for t in range(8) for qb in range(2) for a in range(4)]
            self.issued, self.done, self.queue, self.outs, self.tiles = 0, 0, [], [], []
            row, lane = _iota((128, 128), 0), _iota((128, 128), 1)
            self.tri = lane >= row
            if self.first:
                self.neg = jnp.full((128, 128), NEG, F32)
                self.zq = jnp.zeros((16, 128), U32)
            else:
                self.zero = jnp.zeros((128, 128), F32)
                self.slot = (lane >> 5) == (row >> 5)
                new = (_iota((32, 128), 1) & 31) >= _iota((32, 128), 0)
                self.new = (new[0:16], new[16:32])
                lane2 = _iota((256, 128), 1)
                self.odd, self.hi = (lane2 & 32) != 0, lane2 >= 64
                self.base = [pl.multiple_of((blk * 2 + qb) * 64 - 80, 16) for qb in range(2)]

        def scores_first(self, qb, h):
            qh = qt_v[qb, h * 16:(h + 1) * 16, :]
            wq = _unpack(_rows([qh if jj == h % 4 else self.zq for jj in range(4)]))
            n = (qb + 1) * 32
            kk = _unpack(k0_v[h // 4, 0:2 * n, :])
            s = _rows([_dot(kk[c * n:(c + 1) * n], wq) for c in range(4)])
            diag = lax.select(self.tri, s[qb * 128:], self.neg)
            return diag if qb == 0 else _rows([s[0:128], diag])

        def scores(self, qb, h):
            qf = _unpack(qt_v[qb, h * 16:(h + 1) * 16, :]).astype(F32)
            wq = lax.select(self.slot, _rows([qf] * 4), self.zero).astype(BF)
            w = k4_v[h, pl.ds(self.base[qb], 144), :]
            kk = _unpack(_rows([w[0:8], w[128:136], w[8:16], w[136:144], w[16:128]]))
            cuts = (0,) + CFG['cuts'] + (18,)
            s = _rows([_dot(kk[16 * a:16 * b], wq) for a, b in zip(cuts[:-1], cuts[1:])])
            return _rows([lax.select(self.new[0], s[16:32], s[0:16]),
                          lax.select(self.new[1], s[48:64], s[32:48]), s[64:]])

        def softmax_pv(self, s, qb, h):
            mx = jnp.max(s, axis=0, keepdims=True)
            if self.first:
                p = jnp.exp2(s - mx)
                l = jnp.sum(p, axis=0, keepdims=True)
                v3 = vt_v[0:qb + 1, h * 16:(h + 1) * 16, :]
            else:
                s = lax.select(self.odd, _rows([s[224:], s[:224]]), s)
                s = lax.select(self.hi, _rows([s[192:], s[:192]]), s)
                p = jnp.exp2(s - mx)
                p3 = p.reshape(2, 128, 128)
                acc = p3[:, 120:128]
                for v in range(14, -1, -1):
                    acc = acc + p3[:, 8 * v:8 * v + 8]
                l = jnp.sum(acc.reshape(16, 128), axis=0, keepdims=True)
                pm = p[0:128]
                p = _rows([lax.select(self.tri, self.zero, pm), p[128:256],
                           lax.select(self.tri, pm, self.zero)])
                v3 = vt_v[pl.ds(self.blk * 2 + qb - 2, 3), h * 16:(h + 1) * 16, :]
            return _dot(_unpack(_lanes(v3)), p.astype(BF)) * _recip(l)

        def store_o(self, gp):
            x = self.tiles
            ready = {2: (2, 5), 4: (4, 0, 1, 3, 6)}.get(len(x), ())
            if ready:
                ls = _lhs7(x[0], x[2 % len(x)], x[1], x[3 % len(x)])
                for k in ready:
                    (oa0_v, oa1_v)[gp // 2][k, gp % 2] = _pack(ls[k].astype(BF).T)
            if len(x) == 4:
                self.tiles = []

        def issue(self, n=1):
            for _ in range(n):
                if self.issued < len(self.items):
                    fn = self.scores_first if self.first else self.scores
                    self.queue.append(fn(*self.items[self.issued]))
                    self.issued += 1

        def finish(self, n=1):
            for _ in range(n):
                if self.done < self.issued:
                    qb, h = self.items[self.done]
                    self.outs.append(self.softmax_pv(self.queue.pop(0), qb, h))
                    if len(self.outs) == 4:
                        self.tiles.append(_rows(self.outs))
                        self.outs = []
                        self.store_o(h // 8)
                    self.done += 1

    def add_residual(r, nrows, c0, c1, y):
        x_v[pl.ds(r, nrows), c0:c1] = (x_v[pl.ds(r, nrows), c0:c1].astype(F32) + y).astype(BF)

    def split7(top, bot):
        q = [top[:, :256], top[:, 256:], bot[:, :256], bot[:, 256:]]
        return q, _lhs7(*[v.astype(F32) for v in q])

    def split_now():
        ls = {}
        for k1 in range(7):
            x = xl_v[0:TA // 2, k1 * HD:(k1 + 1) * HD]
            q, sums = split7(x[0:64], x[64:128])
            for k2 in range(7):
                ls[k1, k2] = q[3 * (k2 == 3)] if k2 in (2, 3) else sums[k2].astype(BF)
        return ls

    def split_chunks(zero):
        def mk(r, ks):
            def run(tok):
                xm_v[TA // 2:TA // 2 + 16, 128:256] = tok.astype(BF)
                cols = slice(ks[0] * HD, (ks[-1] + 1) * HD)
                half = [xm_v[pl.ds(pl.multiple_of(o + zero * 32, 8), 8), cols] for o in (r, r + 64)]
                out = []
                for n in range(len(ks)):
                    sums = split7(*[h[:, n * HD:(n + 1) * HD] for h in half])[1]
                    out += [sums[k2] for k2 in SUMS]
                x2_v[r:r + 8, ks[0] * 1280:(ks[-1] + 1) * 1280] = lax.concatenate(out, 1).astype(BF)
            return run
        return [mk(r, ks) for r in range(0, 64, 8) for ks in CFG['bks']]

    def split_load(zero):
        r = pl.ds(pl.multiple_of(zero * 32, 32), 64)
        ls = {}
        for k1 in range(7):
            ls[k1, 2] = xm_v[0:64, k1 * HD:k1 * HD + 256]
            ls[k1, 3] = xm_v[64:128, k1 * HD + 256:(k1 + 1) * HD]
            for n, k2 in enumerate(SUMS):
                ls[k1, k2] = x2_v[r, (k1 * 5 + n) * 256:(k1 * 5 + n + 1) * 256]
        return ls

    def proj_b(ls, r0, st):
        rows = slice(HALO + r0, HALO + r0 + TA)
        cnt = [0]
        for part in range(3):
            for j in range(2):
                def inner(k1, k2):
                    w = wb2[part * 49 + k1 * 7 + k2, j]
                    cnt[0] += 1
                    return _dot(ls[k1, k2], _unpack(w)) if cnt[0] % 2 else st.dot(ls[k1, k2], w)

                def outer(k1):
                    res = []
                    _strassen(lambda k2: inner(k1, k2),
                              lambda a, b, c, d: res.append(
                                  _rows([lax.concatenate([a, b], 1), lax.concatenate([c, d], 1)])))
                    return res[0]

                def put(half):
                    def run(top, bot):
                        y = _weave(top, bot)
                        if part == 0:
                            y = y * QSCALE
                        dst, T = (qk_v, part * 8) if part < 2 else (v_v, 0)
                        for n in range(2):
                            dst[T + half * 4 + 2 * n + j, rows, :] = y[:, n * 128:(n + 1) * 128]
                    return run
                _strassen(outer, put(0), put(1))

    def taps(ref, t0, t1, r0):
        wins = [ref[t0:t1, HALO + r0 - 2 * w:HALO + r0 - 2 * w + 8, :] for w in range(WB)]
        return _rows(wins).reshape(WB, t1 - t0, 8, 128)

    def logit_b(i, zero, r0):
        ns = CFG['lns']
        acc = []

        def mk(st):
            def run(tok):
                t0, t1 = st * 8 // ns, (st + 1) * 8 // ns
                q = gated(qk_v[t0:t1, HALO + r0:HALO + r0 + 8, :], tok, zero)
                p = q[None] * taps(qk_v, 8 + t0, 8 + t1, r0)
                if acc:
                    p = lax.concatenate([acc.pop()[:, None], p], 1)
                a = jnp.sum(p, axis=1)
                if st + 1 < ns:
                    acc.append(a)
                    return
                a = a + pltpu.roll(a, 64, 2)
                a = a + pltpu.roll(a, 32, 2)
                if r0 < 2 * (WB - 1):
                    pos = _iota(a.shape, 1) - 2 * _iota(a.shape, 0) + (i * TB + r0)
                    a = lax.select(pos >= 0, a, jnp.full(a.shape, NEG, F32))
                e = jnp.exp2(a - jnp.max(a, axis=0, keepdims=True))
                e_v[:, r0:r0 + 8, :] = e * _recip(jnp.sum(e, axis=0, keepdims=True))
            return run
        return [mk(st) for st in range(ns)]

    def pv_b(zero, r0):
        x = []

        def mk(st):
            def run(tok):
                r, t0 = r0 + 8 * (st // 2), 4 * (st % 2)
                e = gated(e_v[:, r:r + 8, :], tok, zero)
                x.append(_lanes(jnp.sum(e[:, None] * taps(v_v, t0, t0 + 4, r), axis=0)))
                if st == 3:
                    ob_v[r0 // 2:r0 // 2 + 8, :] = lax.concatenate(_lhs7(*x), 1).astype(BF)
            return run
        return [mk(st) for st in range(4)]

    def out_b(i, r0, nrows, side, done=None, fences={}, lag=0):
        ou = _pack(ob_v[r0 // 2:(r0 + nrows) // 2, :])
        r = pl.multiple_of(i * TB + r0, 128)
        st = Stream(side, fences, lag)
        for c in range(4):
            def prod(k):
                w2 = wobp[c, k].reshape(256, 128)
                w = _unpack(_weave(w2[0:128], w2[128:256]))
                return st.dot(ou[:, k * HD:(k + 1) * HD], w)

            def put(y11, y12, y21, y22):
                y = _weave(lax.concatenate([y11, y12], 1), lax.concatenate([y21, y22], 1))
                add_residual(r, nrows, c * 256, (c + 1) * 256, y)
            _strassen(prod, put)
            if done is not None:
                done(c)
        st.flush()

    cp_x(0).start()
    for cp in cp_wa(0):
        cp.start()
    z16 = jnp.zeros((16, 128), U32)
    xl_v[TA // 2:TA // 2 + 32, 0:128] = jnp.zeros((32, 128), BF)
    xm_v[TA // 2:TA // 2 + 32, 0:128] = jnp.zeros((32, 128), BF)
    x2_v[64:96, 0:128] = jnp.zeros((32, 128), BF)
    wbt[2, 0, 0] = z16.reshape(2, 8, 128)
    wb2[147, 0, 0:16, :] = z16
    wbf[2, 0, 0, 0] = jnp.zeros((16, 128), F32)
    wobp[4, 0, 0, 0:2] = z16.reshape(2, 8, 128)
    k4_v[0, 0:16, :] = z16
    vt_v[S // 128, 0:16, :] = z16
    qt_v[2, 0:16, :] = z16
    tk_v[0] = z16[0:8]
    e_v[0, TB:TB + 16, :] = jnp.zeros((16, 128), F32)
    cp_x(0).wait()
    for cp in cp_wa(1):
        cp.start()
    for run in ln_chunks(0, xl_v, TA, step=TA):
        run(None)

    def one_pass(p, carry):
        first = p == 0
        zero = p >> 2

        def out_a(blk, zero, st, after):
            part = {}
            n = [0]
            for ph in range(2):
                ou = oa0_v[pl.ds(zero, 7)] if ph == 0 else oa1_v[...]
                for nh in range(2):
                    def prod(k):
                        w = woap[(ph * 2 + nh) * 7 + k]
                        y = st.dot(_lanes(ou[k]), w)
                        n[0] += 1
                        after(n[0])
                        return y

                    def put(half):
                        def run(top, bot):
                            y = _rows([top, bot])
                            if ph == 0:
                                part[nh, half] = y
                            else:
                                c0 = nh * HD + half * 256
                                add_residual(blk, TA, c0, c0 + 256, y + part[nh, half])
                        return run
                    _strassen(prod, put(0), put(1))
            st.flush()

        def put_first(part, t):
            def run(top, bot):
                y = _weave(top, bot)
                if part == 0:
                    store_t(y * QSCALE, qt_v, 0, t)
                elif part == 2:
                    store_t(y, vt_v, 0, t)
                else:
                    k0_v[t] = _pack(y.astype(BF))
            return run

        def f_body(c, c_):
            buf = wa_v.at[pl.ds(3 * c, 3)]
            pltpu.make_async_copy(buf, buf, sems.at[5 + c]).wait()
            xl = xl_v[0:TA // 2, :]
            raw = {}
            for part in FORDER:
                for k in RAW:
                    o = int(k == 4)
                    w = wa_v[3 * c + part, o * HD:(o + 1) * HD, o * 128:(o + 1) * 128]
                    raw[part, k] = _dot(xl[:, k * HD:(k + 1) * HD], w)
            nr = CFG['fnr']

            def mk_w(part, r0):
                def run(tok):
                    wa_v[3 * NC1, 0:16, 0:128] = tok.astype(BF)
                    w1 = wa_v[3 * c + part, r0:r0 + nr, :]
                    w2 = wa_v[3 * c + part, HD + r0:HD + r0 + nr, :]
                    rs = make_rhs([w1[:, :128], w1[:, 128:], w2[:, :128], w2[:, 128:]])
                    for k in range(7):
                        wap[part][c * 7 + k, r0 // 2:(r0 + nr) // 2, :] = rs[k]
                return run
            side = _both(*[_spread([mk_w(part, r0) for r0 in range(0, HD, nr)], 21, *rng)
                           for part, rng in zip(FORDER, CFG['frng'])])
            for y in raw.values():
                release(y, side.pop(0))
            for n, part in enumerate(FORDER):
                def prod(k):
                    if k in RAW:
                        return raw[part, k]
                    y = _dot(xl[:, k * HD:(k + 1) * HD], _unpack(wap[part][c * 7 + k + zero]))
                    release(y, side.pop(0))
                    return y
                _strassen(prod, put_first(part, 2 * c), put_first(part, 2 * c + 1))
                if n == 0:
                    for k in range(NC1 - 2):
                        @pl.when(c == k)
                        def _():
                            for cp in cp_wa(k + 2):
                                cp.start()

            @pl.when(c == NC1 - 3)
            def _():
                cp_woa.start()

            @pl.when(c == NC1 - 2)
            def _():
                for cp in [cp_x(1)] + cp_wb(0):
                    cp.start()
            return c_

        def g_body(c, c_):
            xl = xl_v[0:TA // 2, :]
            for part in FORDER:
                _strassen(lambda k: _dot(xl[:, k * HD:(k + 1) * HD], _unpack(wap[part][c * 7 + k])),
                          put_first(part, 2 * c), put_first(part, 2 * c + 1))
            return c_

        def a_first():
            @pl.when(first)
            def _():
                lax.fori_loop(0, NC1, f_body, 0)

            @pl.when(jnp.logical_not(first))
            def _():
                lax.fori_loop(0, NC1, g_body, 0)
            at = Attn(0)
            at.issue(CFG['flook'])
            while at.issued < 2 * H:
                at.issue()
                at.finish()

            @pl.when(first)
            def _():
                for cp in [cp_woa, cp_x(1)] + cp_wb(0):
                    cp.wait()
                for cp in [cp_x(2)] + cp_wb(1):
                    cp.start()

                def once(gp, c_):
                    r0 = pl.multiple_of(gp * 256, 256)
                    for nh in range(2):
                        for rr in range(0, 128, 32):
                            rows = pl.ds(pl.multiple_of((gp & 1) * 128 + rr, 32), 32)
                            quads = [woa_v[pl.ds(r0 + dr + rr, 32), nh * HD + dc:nh * HD + dc + 256]
                                     for dr in (0, 128) for dc in (0, 256)]
                            rs = _rhs7(*[w.astype(F32) for w in quads])
                            for k in range(7):
                                val = quads[3 * (k == 4)] if k in RAW else rs[k].astype(BF)
                                woap[((gp >> 1) * 2 + nh) * 7 + k, rows, :] = val
                    return c_
                lax.fori_loop(0, 4, once, 0)

            def mk_k4(t):
                def run(tok):
                    k0_v[8, 0:8, :] = pltpu.bitcast(tok[0:8], U32)
                    kp = k0_v[t + zero]
                    kt_v[t] = kp[80:128]
                    build_k4(kp, t, 48)
                return run
            hi = CFG['fhi']
            side = _both(_spread(prep_out(zero), 28, 0, hi),
                         _spread(ln_chunks(TA + zero * TA, xl_v, TA), 28, 0, hi))
            side = _both(side, _spread([mk_k4(t) for t in range(8)], 28, 0, hi))
            st = Stream(side, {27: lambda: fence_side(zero) | fence_k(zero)}, 1)
            out_a(0, zero, st, lambda u: at.finish(2 * H if u == 1 else 0))

        if CFG['first']:
            a_first()

        @pl.when(first)
        def _():
            cp_x(2).wait()
            for cp in cp_wb(1):
                cp.wait()
            cp_x(3).start()
            for cp in cp_wb(2):
                cp.start()

        def a_body(i, c_):
            @pl.when(jnp.logical_and(first, i == 2))
            def _():
                cp_x(3).wait()
                for cp in cp_wb(2):
                    cp.wait()
            xu = _pack(xl_v[0:TA // 2, :])
            units, lvl2 = prep_qkv(jnp.minimum(i - 1, 5), zero)
            pw = [_spread(un, 112, *rng) for un, rng in zip(units, CFG['urng'])]
            ns = CFG['s3n']
            pw += [_spread(lvl2[:ns], 112, *CFG['s3a']), _spread(lvl2[ns:], 112, *CFG['s3b'])]
            po = prep_out(i)
            side = _both(_spread(ln_chunks((((i + 1) & (NA - 1)) + zero) * TA, xl_v, TA),
                                 112, *CFG['lrng']),
                         _spread(po, 112, *CFG['orng']), *pw)
            fences = {u: (lambda: fence_side(zero)) for u in CFG['fpos']}
            for n in range(1, 12):
                fe = (fence_k, fence_v, fence_q)[CFG['kord'][(n - 1) % 3]]
                u = 7 * n + 6
                fences[u] = ((lambda fe=fe: fe(zero) | fence_side(zero)) if u in fences
                             else (lambda fe=fe: fe(zero)))
            st = Stream(side, fences, CFG['lag'])
            at = Attn(i)
            for n in range(12):
                gp, kind = n // 3, CFG['kord'][n % 3]

                def prod(k):
                    if n == 11 and k == CFG['hk']:
                        at.issue(CFG['look'])
                    w = wap[(1, 2, 0)[kind]][gp * 7 + k]
                    return st.dot(xu[:, k * HD:(k + 1) * HD], _unpack(w))

                def put(t):
                    def run(top, bot):
                        y = _weave(top, bot)
                        if kind == 0:
                            kp = _pack(y.astype(BF))
                            full = _rows([kt_v[t], kp])
                            kt_v[t] = kp[80:128]
                            build_k4(full, t, pl.multiple_of(i * (TA // 2), TA // 2))
                        elif kind == 1:
                            store_t(y, vt_v, i * (TA // 128), t)
                        else:
                            store_t(y * QSCALE, qt_v, 0, t)
                    return run
                _strassen(prod, put(2 * gp), put(2 * gp + 1))
            while at.issued < 2 * H - CFG['tail']:
                at.issue()
                at.finish()

            def after(u):
                at.finish()
                at.issue()
            at.issue()
            out_a(pl.multiple_of(i * TA, TA), zero, st, after)
            assert at.done == 2 * H
            return c_
        if CFG['a']:
            lax.fori_loop(1, NA, a_body, 0)

        qk_v[8:16, 0:HALO, :] = jnp.zeros((8, HALO, 128), F32)
        v_v[:, 0:HALO, :] = jnp.zeros((8, HALO, 128), F32)

        def b_body(i, c_):
            def send(k):
                for ii in range(NB if k < 2 else NB - 1):
                    @pl.when(jnp.logical_and(p == 1, i == ii))
                    def _():
                        cp_out(ii, k).start()

            def send_last(c):
                @pl.when(jnp.logical_and(p == 1, i == NB - 1))
                def _():
                    cp_out(NB - 1, 2, c).start()
            ln1 = ln_chunks(i * TB + 256, xm_v, 256)
            ln2 = ln_chunks((((i + 1) & (NB - 1)) + zero) * TB, xl_v, TA)
            lg = [logit_b(i, zero, g * 8) for g in range(TB // 8)]
            pv = [pv_b(zero, g * 16) for g in range(TB // 16)]
            n0, n1, n2 = CFG['bn']

            def mix(a, b):
                return _merge(_flat(a), _flat(b)) if CFG['bmix'] else _flat(a) + _flat(b)
            def fx():
                z2 = _pack(x2_v[pl.ds(pl.multiple_of(64 + zero * 32, 32), 32), 0:128])
                return fence_x(zero) | fence_x(zero, xm_v) | z2
            fences = {u: fx for u in CFG['bfx']}
            for u in CFG['bfe']:
                fences[u] = (lambda: fx() | fence_e(zero)) if u in fences else (lambda: fence_e(zero))
            side = _both(_spread(ln1, 294, *CFG['bl1']), _spread(ln2[CFG['bna']:], 294, *CFG['bl2']),
                         _spread(ln2[:CFG['bna']], 294, *CFG['bl2a']),
                         _spread(split_chunks(zero), 294, *CFG['bsp']),
                         _spread(_flat(lg[0:n0]), 294, 100, CFG['be0']),
                         _spread(mix(lg[n0:32], pv[0:16]), 294, *CFG['bw1']),
                         _spread(_flat(lg[32:n1]), 294, 247, 294))
            st = Stream(side, fences, CFG['blag'])
            proj_b(split_now(), 0, st)
            proj_b(split_load(zero), 256, st)
            st.flush()
            out_b(i, 0, 256, _spread(mix(lg[n1:64], pv[16:n2]), 28, 1, 28), None,
                  {u: (lambda: fence_e(zero)) for u in CFG['bof']}, CFG['bolag'])
            send(0)
            out_b(i, 256, 128, _spread(_flat(pv[n2:32]), 28, 0, CFG['bhi']))
            send(1)
            qk_v[8:16, 0:HALO, :] = qk_v[8:16, TB:TB + HALO, :]
            v_v[:, 0:HALO, :] = v_v[:, TB:TB + HALO, :]
            out_b(i, 384, 128, [[]] * 28, send_last)
            send(2)
            return c_
        if CFG['b']:
            lax.fori_loop(0, NB, b_body, 0)
        return carry

    lax.fori_loop(0, 2, one_pass, 0)
    for i in range(NB):
        for k in range(len(OUT_PIECES)):
            if (i, k) != (NB - 1, 2):
                cp_out(i, k).wait()
    for c in range(4):
        cp_out(NB - 1, 2, c).wait()


@jax.jit
def pallas_interleave_layers__sliding_block__sliding_local_dilated__prompt_kernel(
    A_x: jax.Array,
    A_wqkv: jax.Array,
    A_wo: jax.Array,
    B_x: jax.Array,
    B_wqkv: jax.Array,
    B_wo: jax.Array,
):
    del B_x
    x = A_x.reshape(S, D)
    any_spec = pl.BlockSpec(memory_space=pl.ANY)
    out = pl.pallas_call(
        _kernel,
        out_shape=jax.ShapeDtypeStruct((S, D), BF),
        in_specs=[any_spec] * 5,
        out_specs=any_spec,
        scratch_shapes=[
            pltpu.VMEM((S + 16, D), BF),
            pltpu.VMEM((3 * NC1 + 1, D, G1 * 128), BF),
            pltpu.VMEM((D, D), BF),
            pltpu.VMEM((6, D + 16, 512), BF),
            pltpu.VMEM((5, D, 256), BF),
            pltpu.VMEM((28, 256, 128), U32),
            pltpu.VMEM((28, 256, 128), U32),
            pltpu.VMEM((28, 256, 128), U32),
            pltpu.VMEM((28, 256, 256), BF),
            pltpu.VMEM((3, 9, 16, 2, 8, 128), U32),
            pltpu.VMEM((3, 7, 16, 2, 16, 128), F32),
            pltpu.VMEM((148, 2, 128, 128), U32),
            pltpu.VMEM((5, 9, 2, 16, 8, 128), U32),
            pltpu.VMEM((TA // 2 + 32, 7 * HD), BF),
            pltpu.VMEM((TA // 2 + 32, 7 * HD), BF),
            pltpu.VMEM((96, 35 * 256), BF),
            pltpu.VMEM((9, TA // 2, 128), U32),
            pltpu.VMEM((8, 48, 128), U32),
            pltpu.VMEM((H, S // 2, 128), U32),
            pltpu.VMEM((3, D // 2, 128), U32),
            pltpu.VMEM((S // 128 + 1, D // 2, 128), U32),
            pltpu.VMEM((7, 2, 64, 128), U32),
            pltpu.VMEM((7, 2, 64, 128), U32),
            pltpu.VMEM((16, HALO + TB, 128), F32),
            pltpu.VMEM((8, HALO + TB, 128), F32),
            pltpu.VMEM((WB, TB + 16, 128), F32),
            pltpu.VMEM((TB // 2, 7 * HD), BF),
            pltpu.VMEM((4, 8, 128), U32),
            pltpu.SemaphoreType.DMA((5 + NC1,)),
        ],
        compiler_params=pltpu.CompilerParams(vmem_limit_bytes=120 * 1024 * 1024),
        name="interleave_attn",
    )(x, A_wqkv, A_wo, B_wqkv, B_wo)
    return out.reshape(1, S, D)
```
